```python
import jax
import jax.numpy as jnp

def _softmax(x, axis=-1):
    return jax.nn.softmax(x, axis=axis)

def _gelu(x):
    return jax.nn.gelu(x, approximate=True)

def _silu(x):
    return jax.nn.silu(x)

def _sigmoid(x):
    return jax.nn.sigmoid(x)

def _layernorm(x, axis=-1, eps=1e-05):
    m = jnp.mean(x, axis=axis, keepdims=True)
    v = jnp.var(x, axis=axis, keepdims=True)
    return (x - m) / jnp.sqrt(v + eps)

def _scatter_add(tgt, idx, src, axis=0):
    return tgt.at[idx].add(src)

def _segment_sum(src, seg, n):
    return jax.ops.segment_sum(src, seg, n)

class _Rng:

    def __init__(self, key):
        self._k = key

    def _next(self):
        self._k, sub = jax.random.split(self._k)
        return sub

    def normal(self, shape):
        return jax.random.normal(self._next(), shape, dtype=jnp.bfloat16)

    def randint(self, lo, hi, shape):
        return jax.random.randint(self._next(), shape, lo, hi, dtype=jnp.int32)

    def uniform(self, shape, lo=0.0, hi=1.0):
        return jax.random.uniform(self._next(), shape, jnp.bfloat16, lo, hi)

    def permutation(self, n):
        return jax.random.permutation(self._next(), n)
kernel_name = 'adaLN_cond__gqa_block_cached__moe_arch_mod__prompt'

def setup_inputs():
    _rng = _Rng(jax.random.key(int.from_bytes(__import__("os").urandom(4), "little")))
    _w = lambda a: (lambda t: t.astype(jnp.bfloat16) if jnp.issubdtype(t.dtype, jnp.floating) else t)(jnp.asarray(a))

    def _A_setup():
        B, Sq, D = (1, 2048, 576)
        Hq, Hkv, Sk, Dh = (32, 16, 2048, 128)
        assert Hq % Hkv == 0, (Hq, Hkv)
        return {'x': _w((lambda *s: _rng.normal(s) * 0.05)(B, Sq, D)), 'k_cache': _w((lambda *s: _rng.normal(s) * 0.05)(B, Hkv, Sk, Dh)), 'v_cache': _w((lambda *s: _rng.normal(s) * 0.05)(B, Hkv, Sk, Dh)), 'wq': _w((lambda *s: _rng.normal(s) * 0.05)(D, Hq * Dh) * D ** (-0.5)), 'wo': _w((lambda *s: _rng.normal(s) * 0.05)(Hq * Dh, D) * (Hq * Dh) ** (-0.5))}
    _A_in = _A_setup()

    def _B_setup():
        B, S, D, F, C = (1, 2048, 576, 4608, 8)
        return {'x': _w((lambda *s: _rng.normal(s) * 0.05)(B, S, D)), 'w_r': _w((lambda *s: _rng.normal(s) * 0.05)(D)), 'w_gate': _w((lambda *s: _rng.normal(s) * 0.05)(D, F)), 'w_up': _w((lambda *s: _rng.normal(s) * 0.05)(D, F)), 'w_down': _w((lambda *s: _rng.normal(s) * 0.05)(F, D))}
    _B_in = _B_setup()
    return {'A_x': _A_in['x'], 'A_k_cache': _A_in['k_cache'], 'A_v_cache': _A_in['v_cache'], 'A_wq': _A_in['wq'], 'A_wo': _A_in['wo'], 'B_x': _B_in['x'], 'B_w_r': _B_in['w_r'], 'B_w_gate': _B_in['w_gate'], 'B_w_up': _B_in['w_up'], 'B_w_down': _B_in['w_down'], 'c': _w((lambda *s: _rng.normal(s) * 0.05)(1, 576)), 'w_mod': _w((lambda *s: _rng.normal(s) * 0.05)(576, 6 * 576) * 576 ** (-0.5))}

def reference(A_x, A_k_cache, A_v_cache, A_wq, A_wo, B_x, B_w_r, B_w_gate, B_w_up, B_w_down, c, w_mod):

    def _A_ref(x, k_cache, v_cache, wq, wo):
        B, Sq, D = x.shape
        Hq, Dh = (32, 128)
        Hkv = k_cache.shape[1]
        rep = Hq // Hkv
        q = (lambda x, *d: x.transpose(*d))((x @ wq).reshape(B, Sq, Hq, Dh), 0, 2, 1, 3)
        k = jnp.repeat(k_cache, rep, axis=1)
        v = jnp.repeat(v_cache, rep, axis=1)
        scores = jnp.einsum('bhqd,bhkd->bhqk', q, k) * Dh ** (-0.5)
        p = _softmax(scores, axis=-1)
        o = jnp.einsum('bhqk,bhkd->bhqd', p, v)
        return (lambda x, *d: x.transpose(*d))(o, 0, 2, 1, 3).reshape(B, Sq, Hq * Dh) @ wo

    def _B_ref(x, w_r, w_gate, w_up, w_down):
        B, S, D = x.shape
        C = 8
        r = x @ w_r
        idx = jnp.argsort(-r, axis=-1)[:, :C]
        idx_e = jnp.repeat(idx.reshape(B, C, 1), D, axis=2)
        x_sel = jnp.take_along_axis(x, idx_e, axis=1)
        g = _silu(x_sel @ w_gate)
        u = x_sel @ w_up
        y = g * u @ w_down
        r_sel = _sigmoid(jnp.take_along_axis(r, idx, axis=1))
        y = y * r_sel.reshape(B, C, 1)
        b_off = (jnp.arange(B) * S).reshape(B, 1)
        flat_idx = (idx + b_off).reshape(B * C)
        zero = (x * 0.0).reshape(B * S, D)
        upd = _scatter_add(zero, flat_idx, y.reshape(B * C, D), axis=0)
        return x + upd.reshape(B, S, D)
    x = A_x
    mod = (_silu(c) @ w_mod).reshape(c.shape[0], 6, 1, -1)
    sa, ca, ga, sb, cb, gb = (mod[:, 0].copy(), mod[:, 1].copy(), mod[:, 2].copy(), mod[:, 3].copy(), mod[:, 4].copy(), mod[:, 5].copy())
    h = _layernorm(x, axis=-1) * (1 + ca) + sa
    x = x + ga * _A_ref(h, A_k_cache, A_v_cache, A_wq, A_wo)
    h = _layernorm(x, axis=-1) * (1 + cb) + sb
    x = x + gb * _B_ref(h, B_w_r, B_w_gate, B_w_up, B_w_down)
    return x
```

```python
import functools
import math
import os

import jax
import jax.numpy as jnp
from jax import lax
import jax.experimental.pallas as pl
import jax.experimental.pallas.tpu as pltpu

F32 = jnp.float32
BF16 = jnp.bfloat16

HQ = 32
DH = 128
TOPC = 8
EPS = 1e-05

TQ = int(os.environ.get("KP_TQ", "512"))


def _rb(x):
    return x.astype(BF16).astype(F32)


def _sigmoid(x):
    return 1.0 / (1.0 + jnp.exp(-x))


def _ln_mod(x, scale1p, shift):
    d = x.shape[-1]
    mu = jnp.sum(x, axis=-1, keepdims=True) * (1.0 / d)
    xc = x - mu
    var = jnp.sum(xc * xc, axis=-1, keepdims=True) * (1.0 / d)
    den = _rb(jnp.sqrt(_rb(_rb(var) + EPS)))
    ln = _rb(_rb(x - _rb(mu)) / den)
    return _rb(_rb(ln * scale1p) + shift)


def _kernel(x_ref, k_ref, v_ref, wq_ref, wo_ref, wr_ref, wg_hbm, wu_hbm, wd_hbm,
            c_ref, wmod_ref, o_ref,
            h_scr, acc_scr, mod_scr, r_scr, wg_v, wu_v, wd_v, sems,
            *, n_heads, n_q, rep):
    hh = pl.program_id(0)
    qi = pl.program_id(1)
    seq, d = x_ref.shape
    rows = pl.ds(pl.multiple_of(qi * TQ, TQ), TQ)

    def mlp_copies():
        return (pltpu.make_async_copy(wg_hbm, wg_v, sems.at[0]),
                pltpu.make_async_copy(wu_hbm, wu_v, sems.at[1]),
                pltpu.make_async_copy(wd_hbm, wd_v, sems.at[2]))

    @pl.when(jnp.logical_and(hh == 0, qi == 0))
    def _():
        for cp in mlp_copies():
            cp.start()
        cc = c_ref[...].astype(F32)
        sc = (cc * _rb(_sigmoid(cc))).astype(BF16)
        sc = jnp.broadcast_to(sc, (8, d))
        mod = _rb(jnp.dot(sc, wmod_ref[...], preferred_element_type=F32))
        for j in range(6):
            piece = mod[0:1, j * d:(j + 1) * d]
            if j in (1, 4):
                piece = _rb(1.0 + piece)
            mod_scr[j:j + 1, :] = piece

    @pl.when(hh == 0)
    def _():
        x = x_ref[rows, :].astype(F32)
        h_scr[rows, :] = _ln_mod(x, mod_scr[1:2, :], mod_scr[0:1, :]).astype(BF16)

    qscale = (DH ** -0.5) * math.log2(math.e)
    q = jnp.dot(h_scr[rows, :], wq_ref[...], preferred_element_type=F32) * qscale
    q = q.astype(BF16)
    k = k_ref[0]
    v = v_ref[0]
    outs = []
    for j in range(rep):
        s = lax.dot_general(q[:, j * DH:(j + 1) * DH], k, (((1,), (1,)), ((), ())),
                            preferred_element_type=F32)
        m = jnp.max(s, axis=-1, keepdims=True)
        p = jnp.exp2(s - m)
        l = jnp.sum(p, axis=-1, keepdims=True)
        o = jnp.dot(p.astype(BF16), v, preferred_element_type=F32)
        outs.append((o * (1.0 / l)).astype(BF16))
    o2 = jnp.concatenate(outs, axis=1)
    contrib = jnp.dot(o2, wo_ref[...], preferred_element_type=F32)

    @pl.when(hh == 0)
    def _():
        acc_scr[rows, :] = contrib

    @pl.when(hh > 0)
    def _():
        acc_scr[rows, :] += contrib

    @pl.when(hh == n_heads - 1)
    def _():
        x = x_ref[rows, :].astype(F32)
        x1 = _rb(x + _rb(mod_scr[2:3, :] * _rb(acc_scr[rows, :])))
        acc_scr[rows, :] = x1
        h2 = _ln_mod(x1, mod_scr[4:5, :], mod_scr[3:4, :])
        o_ref[rows, :] = (x1 + _rb(mod_scr[5:6, :] * h2)).astype(BF16)
        wr = jnp.broadcast_to(wr_ref[...], (8, d))
        r = lax.dot_general(wr, h2.astype(BF16), (((1,), (1,)), ((), ())),
                            preferred_element_type=F32)
        r_scr[pl.ds(qi, 1), :] = _rb(r[0:1, :])

    @pl.when(jnp.logical_and(hh == n_heads - 1, qi == n_q - 1))
    def _():
        r = r_scr[...]
        pos = (lax.broadcasted_iota(jnp.int32, r.shape, 0) * TQ
               + lax.broadcasted_iota(jnp.int32, r.shape, 1))
        sub8 = lax.broadcasted_iota(jnp.int32, (TOPC, 1), 0)
        idxs = []
        x1_sel = jnp.zeros((TOPC, d), F32)
        r_sel = jnp.zeros((TOPC, 1), F32)
        live = jnp.ones(r.shape, jnp.int32)
        for t in range(TOPC):
            cand = jnp.where(live > 0, r, -jnp.inf)
            mx = jnp.max(cand)
            hit = jnp.logical_and(live > 0, cand == mx)
            idx = jnp.min(jnp.where(hit, pos, seq))
            idx = jnp.minimum(idx, seq - 1)
            live = jnp.where(pos == idx, 0, live)
            idxs.append(idx)
            row = acc_scr[pl.ds(idx, 1), :]
            x1_sel = jnp.where(sub8 == t, row, x1_sel)
            r_sel = jnp.where(sub8 == t, mx, r_sel)
        h2_sel = _ln_mod(x1_sel, mod_scr[4:5, :], mod_scr[3:4, :])
        xs = h2_sel.astype(BF16)
        cg, cu, cd = mlp_copies()
        cg.wait()
        g = _rb(jnp.dot(xs, wg_v[...], preferred_element_type=F32))
        g = _rb(g * _rb(_sigmoid(g)))
        cu.wait()
        u = _rb(jnp.dot(xs, wu_v[...], preferred_element_type=F32))
        cd.wait()
        y = _rb(jnp.dot((g * u).astype(BF16), wd_v[...], preferred_element_type=F32))
        y = _rb(y * _rb(_sigmoid(r_sel)))
        new = x1_sel + _rb(mod_scr[5:6, :] * _rb(h2_sel + y))
        sub16 = lax.broadcasted_iota(jnp.int32, (16, 1), 0)
        for t in range(TOPC):
            base = pl.multiple_of((idxs[t] // 16) * 16, 16)
            blk = o_ref[pl.ds(base, 16), :].astype(F32)
            blk = jnp.where(sub16 == idxs[t] - base, new[t:t + 1, :], blk)
            o_ref[pl.ds(base, 16), :] = blk.astype(BF16)


@jax.jit
def pallas_adaLN_cond__gqa_block_cached__moe_arch_mod__prompt_kernel(
    A_x: jax.Array,
    A_k_cache: jax.Array,
    A_v_cache: jax.Array,
    A_wq: jax.Array,
    A_wo: jax.Array,
    B_x: jax.Array,
    B_w_r: jax.Array,
    B_w_gate: jax.Array,
    B_w_up: jax.Array,
    B_w_down: jax.Array,
    c: jax.Array,
    w_mod: jax.Array,
):
    b, seq, d = A_x.shape
    _, hkv, sk, dh = A_k_cache.shape
    assert b == 1 and dh == DH
    rep = HQ // hkv
    f = B_w_gate.shape[1]
    n_q = seq // TQ

    x2 = A_x.reshape(seq, d)
    k3 = A_k_cache.reshape(hkv, sk, dh)
    v3 = A_v_cache.reshape(hkv, sk, dh)
    wr2 = B_w_r.reshape(1, d)

    const2 = lambda h, q: (0, 0)
    out = pl.pallas_call(
        functools.partial(_kernel, n_heads=hkv, n_q=n_q, rep=rep),
        grid=(hkv, n_q),
        in_specs=[
            pl.BlockSpec((seq, d), const2),
            pl.BlockSpec((1, sk, dh), lambda h, q: (h, 0, 0)),
            pl.BlockSpec((1, sk, dh), lambda h, q: (h, 0, 0)),
            pl.BlockSpec((d, rep * dh), lambda h, q: (0, h)),
            pl.BlockSpec((rep * dh, d), lambda h, q: (h, 0)),
            pl.BlockSpec((1, d), const2),
            pl.BlockSpec(memory_space=pl.ANY),
            pl.BlockSpec(memory_space=pl.ANY),
            pl.BlockSpec(memory_space=pl.ANY),
            pl.BlockSpec((1, d), const2),
            pl.BlockSpec((d, 6 * d), const2),
        ],
        out_specs=pl.BlockSpec((seq, d), const2),
        out_shape=jax.ShapeDtypeStruct((seq, d), BF16),
        scratch_shapes=[
            pltpu.VMEM((seq, d), BF16),
            pltpu.VMEM((seq, d), F32),
            pltpu.VMEM((8, d), F32),
            pltpu.VMEM((n_q, TQ), F32),
            pltpu.VMEM((d, f), BF16),
            pltpu.VMEM((d, f), BF16),
            pltpu.VMEM((f, d), BF16),
            pltpu.SemaphoreType.DMA((3,)),
        ],
        compiler_params=pltpu.CompilerParams(
            dimension_semantics=("arbitrary", "arbitrary"),
            vmem_limit_bytes=100 * 1024 * 1024,
        ),
    )(x2, k3, v3, A_wq, A_wo, wr2, B_w_gate, B_w_up, B_w_down, c, w_mod)
    return out.reshape(b, seq, d)
```

```python
import functools
import math
import os

import jax
import jax.numpy as jnp
from jax import lax
import jax.experimental.pallas as pl
import jax.experimental.pallas.tpu as pltpu

F32 = jnp.float32
BF16 = jnp.bfloat16

HQ = 32
DH = 128
TOPC = 8
EPS = 1e-05
LANES = 128

TQ = int(os.environ.get("KP_TQ", "512"))

_NT = (((1,), (1,)), ((), ()))


def _rb(x):
    return x.astype(BF16).astype(F32)


def _sigmoid(x):
    return 1.0 / (1.0 + jnp.exp(-x))


def _lanes(col, width):
    reps = width // LANES
    return col if reps == 1 else jnp.concatenate([col] * reps, axis=1)


def _kernel(xt_ref, k_ref, v_ref, wq_ref, wot_ref, wr_ref, wg_hbm, wu_hbm, wdt_hbm,
            c_ref, wmod_ref, o_ref,
            h_scr, acc_scr, st_scr, m_scr, vt_scr, mod_scr, col_scr, r_scr, h2_scr, x1_scr,
            wg_v, wu_v, wdt_v, sems,
            *, n_heads, n_q):
    t = pl.program_id(0)
    n_units = n_heads * n_q
    d, seq = xt_ref.shape
    cur = jnp.minimum(t, n_units - 1)
    qi = cur // n_heads
    hh = cur % n_heads
    prev = jnp.maximum(t - 1, 0)
    qp = prev // n_heads
    hp = prev % n_heads
    qscale = (DH ** -0.5) * math.log2(math.e)

    def mlp_copies():
        return (pltpu.make_async_copy(wg_hbm, wg_v, sems.at[0]),
                pltpu.make_async_copy(wu_hbm, wu_v, sems.at[1]),
                pltpu.make_async_copy(wdt_hbm, wdt_v, sems.at[2]))

    def cols(blk):
        return pl.ds(pl.multiple_of(blk * TQ, TQ), TQ)

    @pl.when(t == 0)
    def _():
        for cp in mlp_copies():
            cp.start()
        cc = c_ref[...].astype(F32)
        sc = (cc * _rb(_sigmoid(cc))).astype(BF16)
        sc = jnp.broadcast_to(sc, (8, d))
        mod = _rb(jnp.dot(sc, wmod_ref[...], preferred_element_type=F32))
        for j in range(6):
            piece = mod[0:1, j * d:(j + 1) * d]
            if j in (1, 4):
                piece = _rb(1.0 + piece)
            mod_scr[j:j + 1, :] = piece
            if j >= 2:
                col_scr[j - 2] = jnp.broadcast_to(piece, (LANES, d)).T

    @pl.when(jnp.logical_and(t < n_units, hh == 0))
    def _():
        x = xt_ref[:, cols(qi)].astype(F32)
        mu = jnp.sum(x, axis=0, keepdims=True) * (1.0 / d)
        xc = x - mu
        var = jnp.sum(xc * xc, axis=0, keepdims=True) * (1.0 / d)
        ln = (xc * lax.rsqrt(var + EPS)).T
        h_scr[...] = (ln * mod_scr[1:2, :] + mod_scr[0:1, :]).astype(BF16)

    def qproj():
        q = jnp.dot(h_scr[...], wq_ref[...], preferred_element_type=F32) * qscale
        return q.astype(BF16)

    nb = TQ // LANES

    def qk(q, j):
        st = lax.dot_general(k_ref[0], q[:, j * DH:(j + 1) * DH], _NT,
                             preferred_element_type=F32)
        for i in range(nb):
            blk = st[:, i * LANES:(i + 1) * LANES]
            st_scr[j * nb + i] = blk
            m_scr[j * nb + i] = jnp.max(blk, axis=0, keepdims=True)

    def pv(j):
        sk = st_scr.shape[1]
        nt = sk // LANES
        ps, ls, pairs = [], [], []
        for i in range(nb):
            p = jnp.exp2(st_scr[j * nb + i] - m_scr[j * nb + i])
            accs = [None] * 4
            for tile in range(nt):
                for r0 in range(tile * LANES + LANES - 16, tile * LANES - 16, -16):
                    pair = p[r0:r0 + 8] + p[r0 + 8:r0 + 16]
                    pairs.append(pair)
                    a = accs[tile % 4]
                    accs[tile % 4] = pair if a is None else a + pair
            ls.append(jnp.sum((accs[0] + accs[1]) + (accs[2] + accs[3]), axis=0, keepdims=True))
            ps.append(p.astype(BF16))
        zero = jnp.full((8, LANES), t >> 20, jnp.int32).astype(jnp.uint32)
        tie0 = int(os.environ.get("KP_TIE0", "2"))
        ntie = int(os.environ.get("KP_NTIE", "3"))
        outs = []
        for i in range(nb):
            vu = pltpu.bitcast(vt_scr[...], jnp.uint32)
            tiles = []
            for c in range(nt):
                g = i * nt + c + 4
                rows = []
                for r in range(8):
                    x = vu[8 * r:8 * r + 8, c * LANES:(c + 1) * LANES]
                    if g < nb * nt and tie0 <= r < tie0 + ntie:
                        src = pairs[g * 8 + (r - tie0)]
                        x = x | (lax.bitcast_convert_type(src, jnp.uint32) & zero)
                    rows.append(x)
                tiles.append(jnp.concatenate(rows, axis=0))
            lhs = pltpu.bitcast(jnp.concatenate(tiles, axis=1), BF16)
            o = jnp.dot(lhs, ps[i], preferred_element_type=F32)
            outs.append((o * (1.0 / ls[i])).astype(BF16))
        return jnp.concatenate(outs, axis=1)

    def outproj(oa, ob):
        o2 = jnp.concatenate([oa, ob], axis=0)
        contrib = jnp.dot(wot_ref[...], o2, preferred_element_type=F32)
        old = jnp.where(hp > 0, acc_scr[...], 0.0)
        acc_scr[...] = old + contrib

    @pl.when(t == 0)
    def _():
        q = qproj()
        qk(q, 0)
        qk(q, 1)
        vt_scr[...] = v_ref[0].T

    @pl.when(jnp.logical_and(t > 0, t < n_units))
    def _():
        q = qproj()
        oa = pv(0)
        qk(q, 0)
        ob = pv(1)
        outproj(oa, ob)
        qk(q, 1)
        vt_scr[...] = v_ref[0].T

    @pl.when(t == n_units)
    def _():
        outproj(pv(0), pv(1))

    @pl.when(jnp.logical_and(t > 0, hp == n_heads - 1))
    def _():
        x = xt_ref[:, cols(qp)].astype(F32)
        x1 = _rb(x + _rb(_lanes(col_scr[0], TQ) * _rb(acc_scr[...])))
        mu = jnp.sum(x1, axis=0, keepdims=True) * (1.0 / d)
        xc = x1 - mu
        var = jnp.sum(xc * xc, axis=0, keepdims=True) * (1.0 / d)
        den = _rb(jnp.sqrt(_rb(_rb(var) + EPS)))
        ln = _rb(_rb(x1 - _rb(mu)) / den)
        h2 = (_rb(ln * _lanes(col_scr[2], TQ)) + _lanes(col_scr[1], TQ)).astype(BF16)
        o_ref[:, cols(qp)] = (x1 + _rb(_lanes(col_scr[3], TQ) * h2.astype(F32))).astype(BF16)
        h2_scr[:, cols(qp)] = h2
        x1_scr[:, cols(qp)] = x1.astype(BF16)
        wr = jnp.broadcast_to(wr_ref[...].reshape(1, d), (8, d))
        r = jnp.dot(wr, h2, preferred_element_type=F32)
        r_scr[pl.ds(qp, 1), :] = _rb(r[0:1, :])

    @pl.when(t == n_units)
    def _():
        r = r_scr[...]
        pos = (lax.broadcasted_iota(jnp.int32, r.shape, 0) * TQ
               + lax.broadcasted_iota(jnp.int32, r.shape, 1))
        sub8 = lax.broadcasted_iota(jnp.int32, (TOPC, 1), 0)
        lane = lax.broadcasted_iota(jnp.int32, (TOPC, LANES), 1)
        idxs = []
        idx_col = jnp.zeros((TOPC, 1), jnp.int32)
        r_sel = jnp.zeros((TOPC, 1), F32)
        live = jnp.ones(r.shape, jnp.int32)
        for i in range(TOPC):
            cand = jnp.where(live > 0, r, -jnp.inf)
            mx = jnp.max(cand)
            hit = jnp.logical_and(live > 0, cand == mx)
            idx = jnp.min(jnp.where(hit, pos, seq))
            idx = jnp.minimum(idx, seq - 1)
            live = jnp.where(pos == idx, 0, live)
            idxs.append(idx)
            idx_col = jnp.where(sub8 == i, idx, idx_col)
            r_sel = jnp.where(sub8 == i, mx, r_sel)
        bases = [pl.multiple_of((ix // LANES) * LANES, LANES) for ix in idxs]
        xs = jnp.zeros((TOPC, d), F32)
        for i in range(TOPC):
            pick = jnp.logical_and(sub8 == i, lane + bases[i] == idx_col)
            pick = jnp.where(pick, 1.0, 0.0).astype(BF16)
            xs = xs + lax.dot_general(pick, h2_scr[:, pl.ds(bases[i], LANES)], _NT,
                                      preferred_element_type=F32)
        xs = xs.astype(BF16)
        cg, cu, cd = mlp_copies()
        cg.wait()
        g = _rb(jnp.dot(xs, wg_v[...], preferred_element_type=F32))
        g = _rb(g * _rb(_sigmoid(g)))
        cu.wait()
        u = _rb(jnp.dot(xs, wu_v[...], preferred_element_type=F32))
        cd.wait()
        y = _rb(lax.dot_general((g * u).astype(BF16), wdt_v[...], _NT,
                                preferred_element_type=F32))
        y = _rb(y * _rb(_sigmoid(r_sel)))
        ypad = jnp.concatenate([y, jnp.zeros((LANES - TOPC, d), F32)], axis=0)
        yt = ypad.T.astype(BF16)
        row = lax.broadcasted_iota(jnp.int32, (LANES, 1), 0)
        lane2 = lax.broadcasted_iota(jnp.int32, (LANES, LANES), 1)
        idx_big = jnp.full((LANES, 1), -1, jnp.int32)
        for i in range(TOPC):
            idx_big = jnp.where(row == i, idxs[i], idx_big)
        for i in range(TOPC):
            place = jnp.where(lane2 + bases[i] == idx_big, 1.0, 0.0).astype(BF16)
            upd = jnp.dot(yt, place, preferred_element_type=F32)
            sl = pl.ds(bases[i], LANES)
            hm = _rb(h2_scr[:, sl].astype(F32) + upd)
            o_ref[:, sl] = (x1_scr[:, sl].astype(F32) + _rb(col_scr[3] * hm)).astype(BF16)


@jax.jit
def pallas_adaLN_cond__gqa_block_cached__moe_arch_mod__prompt_kernel(
    A_x: jax.Array,
    A_k_cache: jax.Array,
    A_v_cache: jax.Array,
    A_wq: jax.Array,
    A_wo: jax.Array,
    B_x: jax.Array,
    B_w_r: jax.Array,
    B_w_gate: jax.Array,
    B_w_up: jax.Array,
    B_w_down: jax.Array,
    c: jax.Array,
    w_mod: jax.Array,
):
    b, seq, d = A_x.shape
    _, hkv, sk, dh = A_k_cache.shape
    assert b == 1 and dh == DH and HQ == 2 * hkv
    f = B_w_gate.shape[1]
    n_q = seq // TQ
    n_units = hkv * n_q

    xt = A_x.reshape(seq, d).T
    wot = A_wo.T
    wdt = B_w_down.T
    k3 = A_k_cache.reshape(hkv, sk, dh)
    v3 = A_v_cache.reshape(hkv, sk, dh)

    cur_h = lambda t: jnp.minimum(t, n_units - 1) % hkv
    prev_h = lambda t: jnp.maximum(t - 1, 0) % hkv
    const2 = lambda t: (0, 0)
    hbm = pl.BlockSpec(memory_space=pl.ANY)
    out_t = pl.pallas_call(
        functools.partial(_kernel, n_heads=hkv, n_q=n_q),
        grid=(n_units + 1,),
        in_specs=[
            pl.BlockSpec((d, seq), const2),
            pl.BlockSpec((1, sk, dh), lambda t: (cur_h(t), 0, 0)),
            pl.BlockSpec((1, sk, dh), lambda t: (cur_h(t), 0, 0)),
            pl.BlockSpec((d, 2 * dh), lambda t: (0, cur_h(t))),
            pl.BlockSpec((d, 2 * dh), lambda t: (0, prev_h(t))),
            pl.BlockSpec((d,), lambda t: (0,)),
            hbm, hbm, hbm,
            pl.BlockSpec((1, d), const2),
            pl.BlockSpec((d, 6 * d), const2),
        ],
        out_specs=pl.BlockSpec((d, seq), const2),
        out_shape=jax.ShapeDtypeStruct((d, seq), BF16),
        scratch_shapes=[
            pltpu.VMEM((TQ, d), BF16),
            pltpu.VMEM((d, TQ), F32),
            pltpu.VMEM((2 * TQ // LANES, sk, LANES), F32),
            pltpu.VMEM((2 * TQ // LANES, 1, LANES), F32),
            pltpu.VMEM((dh, sk), BF16),
            pltpu.VMEM((8, d), F32),
            pltpu.VMEM((4, d, LANES), F32),
            pltpu.VMEM((n_q, TQ), F32),
            pltpu.VMEM((d, seq), BF16),
            pltpu.VMEM((d, seq), BF16),
            pltpu.VMEM((d, f), BF16),
            pltpu.VMEM((d, f), BF16),
            pltpu.VMEM((d, f), BF16),
            pltpu.SemaphoreType.DMA((3,)),
        ],
        compiler_params=pltpu.CompilerParams(
            dimension_semantics=("arbitrary",),
            vmem_limit_bytes=100 * 1024 * 1024,
        ),
    )(xt, k3, v3, A_wq, wot, B_w_r, B_w_gate, B_w_up, wdt, c, w_mod)
    return out_t.T.reshape(b, seq, d)
```

```python
import functools
import math
import os

import jax
import jax.numpy as jnp
from jax import lax
import jax.experimental.pallas as pl
import jax.experimental.pallas.tpu as pltpu

F32 = jnp.float32
BF16 = jnp.bfloat16
I32 = jnp.int32
U32 = jnp.uint32

HQ = 32
DH = 128
TOPC = 8
EPS = 1e-05
LANES = 128

TQ = int(os.environ.get("KP_TQ", "512"))
UNROLL = int(os.environ.get("KP_U", "1"))
TIE0 = int(os.environ.get("KP_TIE0", "2"))
NTIE = int(os.environ.get("KP_NTIE", "3"))
HEAD_SLOTS = 8

_NT = (((1,), (1,)), ((), ()))


def _rb(x):
    return x.astype(BF16).astype(F32)


def _sigmoid(x):
    return 1.0 / (1.0 + jnp.exp(-x))


def _lanes(col, width):
    reps = width // LANES
    return col if reps == 1 else jnp.concatenate([col] * reps, axis=1)


def _kernel(xt_hbm, k_hbm, v_hbm, wq_hbm, wot_hbm, wr_ref, wg_hbm, wu_hbm, wdt_hbm,
            c_ref, wmod_hbm, o_hbm,
            xt_v, k_v, v_v, wq_v, wot_v, wmod_v, wg_v, wu_v, wdt_v, ot_v,
            h_scr, acc_scr, st_scr, m_scr, vt_scr, mod_scr, col_scr, key_scr, h2_scr, x1_scr,
            head_sems, misc_sems, mlp_sems, out_sems, fix_sems,
            *, n_heads, n_q):
    n_units = n_heads * n_q
    n_steady = (n_units - 1) // UNROLL
    d, seq = xt_v.shape
    sk = k_v.shape[1]
    nb = TQ // LANES
    nt = sk // LANES
    hbits = n_heads.bit_length() - 1
    qscale = (DH ** -0.5) * math.log2(math.e)

    def head_of(u):
        return u & (n_heads - 1)

    def blk_of(u):
        return u >> hbits

    def cols(blk, width=TQ):
        if isinstance(blk, int):
            return pl.ds(blk * width, width)
        return pl.ds(pl.multiple_of(blk * width, width), width)

    def head_copies(h):
        c2 = cols(h, 2 * DH)
        sl = h & (HEAD_SLOTS - 1)
        return (pltpu.make_async_copy(wq_hbm.at[:, c2], wq_v.at[h], head_sems.at[0, sl]),
                pltpu.make_async_copy(k_hbm.at[h], k_v.at[h], head_sems.at[1, sl]),
                pltpu.make_async_copy(v_hbm.at[h], v_v.at[h], head_sems.at[2, sl]),
                pltpu.make_async_copy(wot_hbm.at[:, c2], wot_v.at[h], head_sems.at[3, sl]))

    def misc_copy(i):
        if i == 0:
            return pltpu.make_async_copy(xt_hbm.at[:, 0:TQ], xt_v.at[:, 0:TQ], misc_sems.at[0])
        if i == 1:
            return pltpu.make_async_copy(wmod_hbm.at[:, 0:2 * d], wmod_v.at[:, 0:2 * d],
                                         misc_sems.at[1])
        if i == 2:
            return pltpu.make_async_copy(xt_hbm.at[:, TQ:seq], xt_v.at[:, TQ:seq], misc_sems.at[2])
        return pltpu.make_async_copy(wmod_hbm.at[:, 2 * d:6 * d], wmod_v.at[:, 2 * d:6 * d],
                                     misc_sems.at[3])

    def mlp_copies():
        return (pltpu.make_async_copy(wg_hbm, wg_v, mlp_sems.at[0]),
                pltpu.make_async_copy(wu_hbm, wu_v, mlp_sems.at[1]),
                pltpu.make_async_copy(wdt_hbm, wdt_v, mlp_sems.at[2]))

    def out_copy(blk):
        return pltpu.make_async_copy(ot_v.at[:, cols(blk)], o_hbm.at[:, cols(blk)],
                                     out_sems.at[blk])

    def silu_c():
        cc = c_ref[...].astype(F32)
        return jnp.broadcast_to((cc * _rb(_sigmoid(cc))).astype(BF16), (8, d))

    def ln1(blk):
        x = xt_v[:, cols(blk)].astype(F32)
        mu = jnp.sum(x, axis=0, keepdims=True) * (1.0 / d)
        xc = x - mu
        var = jnp.sum(xc * xc, axis=0, keepdims=True) * (1.0 / d)
        ln = (xc * lax.rsqrt(var + EPS)).astype(BF16).T
        h_scr[blk & 1] = (ln.astype(F32) * mod_scr[1:2, :] + mod_scr[0:1, :]).astype(BF16)

    def qproj(u):
        q = jnp.dot(h_scr[blk_of(u) & 1], wq_v[head_of(u)], preferred_element_type=F32)
        return (q * qscale).astype(BF16)

    def qk(u, q, j):
        st = lax.dot_general(k_v[head_of(u)], q[:, j * DH:(j + 1) * DH], _NT,
                             preferred_element_type=F32)
        for i in range(nb):
            blk = st[:, i * LANES:(i + 1) * LANES]
            st_scr[j * nb + i] = blk
            m_scr[j * nb + i] = jnp.max(blk, axis=0, keepdims=True)

    def pv(j, zero):
        ps, ls, pairs = [], [], []
        for i in range(nb):
            p = jnp.exp2(st_scr[j * nb + i] - m_scr[j * nb + i])
            accs = [None] * 4
            for tile in range(nt):
                for r0 in range(tile * LANES + LANES - 16, tile * LANES - 16, -16):
                    pair = p[r0:r0 + 8] + p[r0 + 8:r0 + 16]
                    pairs.append(pair)
                    a = accs[tile % 4]
                    accs[tile % 4] = pair if a is None else a + pair
            ls.append(jnp.sum((accs[0] + accs[1]) + (accs[2] + accs[3]), axis=0, keepdims=True))
            ps.append(p.astype(BF16))
        outs = []
        for i in range(nb):
            vu = pltpu.bitcast(vt_scr[...], U32)
            tiles = []
            for c in range(nt):
                g = i * nt + c + 4
                rows = []
                for r in range(8):
                    x = vu[8 * r:8 * r + 8, c * LANES:(c + 1) * LANES]
                    if g < nb * nt and TIE0 <= r < TIE0 + NTIE:
                        src = pairs[g * 8 + (r - TIE0)]
                        x = x | (lax.bitcast_convert_type(src, U32) & zero)
                    rows.append(x)
                tiles.append(jnp.concatenate(rows, axis=0))
            lhs = pltpu.bitcast(jnp.concatenate(tiles, axis=1), BF16)
            o = jnp.dot(lhs, ps[i], preferred_element_type=F32)
            outs.append((o * (1.0 / ls[i])).astype(BF16))
        return jnp.concatenate(outs, axis=1)

    def outproj(u, oa, ob):
        o2 = jnp.concatenate([oa, ob], axis=0)
        contrib = jnp.dot(wot_v[head_of(u)], o2, preferred_element_type=F32)
        slot = blk_of(u) & 1
        old = jnp.where(head_of(u) > 0, acc_scr[slot], 0.0)
        acc_scr[slot] = old + contrib

    def finalize(blk):
        x = xt_v[:, cols(blk)].astype(F32)
        x1b = (x + _lanes(col_scr[0], TQ) * acc_scr[blk & 1]).astype(BF16)
        x1 = x1b.astype(F32)
        mu = jnp.sum(x1, axis=0, keepdims=True) * (1.0 / d)
        xc = x1 - mu
        var = jnp.sum(xc * xc, axis=0, keepdims=True) * (1.0 / d)
        inv = 1.0 / _rb(jnp.sqrt(_rb(_rb(var) + EPS)))
        ln = (x1 - _rb(mu)) * inv
        h2 = (ln * _lanes(col_scr[2], TQ) + _lanes(col_scr[1], TQ)).astype(BF16)
        ot_v[:, cols(blk)] = (x1 + _lanes(col_scr[3], TQ) * h2.astype(F32)).astype(BF16)
        h2_scr[:, cols(blk)] = h2
        x1_scr[:, cols(blk)] = x1b
        wr = jnp.broadcast_to(wr_ref[...].reshape(1, d), (8, d))
        r = _rb(jnp.dot(wr, h2, preferred_element_type=F32)[0:1, :]) + 0.0
        bits = lax.bitcast_convert_type(r, I32) >> 16
        order = jnp.where(bits < 0, -1 - bits, bits + 32768)
        pos = blk * TQ + lax.broadcasted_iota(I32, (1, TQ), 1)
        key = (order << 11) + (seq - 1 - pos) + 0x20000000
        key_scr[pl.ds(blk, 1), :] = lax.bitcast_convert_type(key, F32)
        out_copy(blk).start()

    misc_copy(0).start()
    misc_copy(1).start()
    for cp in head_copies(0):
        cp.start()
    misc_copy(1).wait()
    mod = _rb(jnp.dot(silu_c(), wmod_v[:, 0:2 * d], preferred_element_type=F32))
    mod_scr[0:1, :] = mod[0:1, 0:d]
    mod_scr[1:2, :] = _rb(1.0 + mod[0:1, d:2 * d])
    misc_copy(0).wait()
    for h in range(1, UNROLL + 1):
        for cp in head_copies(h):
            cp.start()
    ln1(0)
    for cp in head_copies(0):
        cp.wait()
    q = qproj(0)
    qk(0, q, 0)
    qk(0, q, 1)
    vt_scr[...] = v_v[0].T

    load_iters = (n_heads - 1 + UNROLL - 1) // UNROLL

    def steady(s, carry):
        first = s * UNROLL + 1
        last = first + UNROLL - 1
        new_blk = blk_of(last) > blk_of(first - 1)
        fin_blk = blk_of(first - 1) > blk_of(jnp.maximum(first - 1 - UNROLL, 0))

        @pl.when(jnp.logical_or(s <= load_iters, jnp.logical_or(new_blk, fin_blk)))
        def _():
            for j in range(UNROLL):
                @pl.when(first + j < n_heads)
                def _():
                    for cp in head_copies(first + j):
                        cp.wait()
            for j in range(UNROLL):
                @pl.when(last + 1 + j < n_heads)
                def _():
                    for cp in head_copies(last + 1 + j):
                        cp.start()

            @pl.when(s == 0)
            def _():
                misc_copy(2).start()
                misc_copy(3).start()

            @pl.when(s == load_iters - 1)
            def _():
                for cp in mlp_copies():
                    cp.start()
                misc_copy(2).wait()
                misc_copy(3).wait()
                mod = _rb(jnp.dot(silu_c(), wmod_v[:, 2 * d:6 * d], preferred_element_type=F32))
                for j in range(4):
                    piece = mod[0:1, j * d:(j + 1) * d]
                    if j == 2:
                        piece = _rb(1.0 + piece)
                    col_scr[j] = jnp.broadcast_to(piece, (LANES, d)).T

            @pl.when(new_blk)
            def _():
                ln1(blk_of(last))

            @pl.when(fin_blk)
            def _():
                finalize(blk_of(first - 1) - 1)

        zero = jnp.full((8, LANES), s >> 20, I32).astype(U32)
        for j in range(UNROLL):
            u = first + j
            q = qproj(u)
            oa = pv(0, zero)
            qk(u, q, 0)
            ob = pv(1, zero)
            outproj(u - 1, oa, ob)
            qk(u, q, 1)
            vt_scr[...] = v_v[head_of(u)].T
        return carry + 1

    count = lax.fori_loop(0, n_steady, steady, 0)

    for cp in mlp_copies():
        cp.wait()
    zero = jnp.full((8, LANES), count >> 20, I32).astype(U32)
    outproj(n_units - 1, pv(0, zero), pv(1, zero))
    finalize(n_q - 1)

    keys = key_scr[...]
    sub8 = lax.broadcasted_iota(I32, (TOPC, 1), 0)
    lane = lax.broadcasted_iota(I32, (TOPC, LANES), 1)
    top = jnp.zeros((TOPC, 1), F32)
    idxs = []
    for i in range(TOPC):
        mx = jnp.max(jnp.max(keys, axis=0, keepdims=True), axis=1, keepdims=True)
        keys = jnp.where(keys == mx, 0.0, keys)
        top = jnp.where(sub8 == i, mx, top)
        kb = lax.bitcast_convert_type(mx, I32)
        idxs.append(seq - 1 - (kb[0, 0] & (seq - 1)))
    kb = lax.bitcast_convert_type(top, I32)
    idx_col = seq - 1 - (kb & (seq - 1))
    order = (kb >> 11) & 0xFFFF
    rbits = jnp.where(order >= 32768, order - 32768, -1 - order) << 16
    r_sel = lax.bitcast_convert_type(rbits, F32)
    bases = [pl.multiple_of(ix & ~(LANES - 1), LANES) for ix in idxs]
    xs = jnp.zeros((TOPC, d), F32)
    for i in range(TOPC):
        pick = jnp.logical_and(sub8 == i, lane + bases[i] == idx_col)
        pick = jnp.where(pick, 1.0, 0.0).astype(BF16)
        xs = xs + lax.dot_general(pick, h2_scr[:, pl.ds(bases[i], LANES)], _NT,
                                  preferred_element_type=F32)
    xs = xs.astype(BF16)
    g = _rb(jnp.dot(xs, wg_v[...], preferred_element_type=F32))
    g = _rb(g * _rb(_sigmoid(g)))
    u = _rb(jnp.dot(xs, wu_v[...], preferred_element_type=F32))
    y = _rb(lax.dot_general((g * u).astype(BF16), wdt_v[...], _NT,
                            preferred_element_type=F32))
    y = _rb(y * _rb(_sigmoid(r_sel)))
    ypad = jnp.concatenate([y, jnp.zeros((LANES - TOPC, d), F32)], axis=0)
    yt = ypad.T.astype(BF16)
    idx_big = jnp.concatenate([idx_col, jnp.full((LANES - TOPC, 1), -1, I32)], axis=0)
    lane2 = lax.broadcasted_iota(I32, (LANES, LANES), 1)
    for blk in range(n_q):
        out_copy(blk).wait()
    for i in range(TOPC):
        place = jnp.where(lane2 + bases[i] == idx_big, 1.0, 0.0).astype(BF16)
        upd = jnp.dot(yt, place, preferred_element_type=F32)
        sl = pl.ds(bases[i], LANES)
        hm = _rb(h2_scr[:, sl].astype(F32) + upd)
        ot_v[:, sl] = (x1_scr[:, sl].astype(F32) + col_scr[3] * hm).astype(BF16)

    def fix_copy(i):
        sl = pl.ds(bases[i], LANES)
        return pltpu.make_async_copy(ot_v.at[:, sl], o_hbm.at[:, sl], fix_sems.at[i])

    fresh = []
    for i in range(TOPC):
        ok = True
        for j in range(i):
            ok = jnp.logical_and(ok, bases[i] != bases[j])
        fresh.append(ok)
    fix_copy(0).start()
    for i in range(1, TOPC):
        pl.when(fresh[i])(lambda i=i: fix_copy(i).start())
    fix_copy(0).wait()
    for i in range(1, TOPC):
        pl.when(fresh[i])(lambda i=i: fix_copy(i).wait())


@jax.jit
def pallas_adaLN_cond__gqa_block_cached__moe_arch_mod__prompt_kernel(
    A_x: jax.Array,
    A_k_cache: jax.Array,
    A_v_cache: jax.Array,
    A_wq: jax.Array,
    A_wo: jax.Array,
    B_x: jax.Array,
    B_w_r: jax.Array,
    B_w_gate: jax.Array,
    B_w_up: jax.Array,
    B_w_down: jax.Array,
    c: jax.Array,
    w_mod: jax.Array,
):
    b, seq, d = A_x.shape
    _, hkv, sk, dh = A_k_cache.shape
    assert b == 1 and dh == DH and HQ == 2 * hkv
    assert seq & (seq - 1) == 0 and seq <= 2048
    f = B_w_gate.shape[1]
    n_q = seq // TQ
    n_units = hkv * n_q
    assert (n_units - 1) % UNROLL == 0 and hkv & (hkv - 1) == 0 and 2 * UNROLL <= HEAD_SLOTS

    xt = A_x.reshape(seq, d).T
    wot = A_wo.T
    wdt = B_w_down.T
    k3 = A_k_cache.reshape(hkv, sk, dh)
    v3 = A_v_cache.reshape(hkv, sk, dh)

    vmem = pl.BlockSpec(memory_space=pltpu.VMEM)
    hbm = pl.BlockSpec(memory_space=pl.ANY)
    out_t = pl.pallas_call(
        functools.partial(_kernel, n_heads=hkv, n_q=n_q),
        in_specs=[
            hbm, hbm, hbm, hbm, hbm,
            vmem,
            hbm, hbm, hbm,
            vmem,
            hbm,
        ],
        out_specs=hbm,
        out_shape=jax.ShapeDtypeStruct((d, seq), BF16),
        scratch_shapes=[
            pltpu.VMEM((d, seq), BF16),
            pltpu.VMEM((hkv, sk, dh), BF16),
            pltpu.VMEM((hkv, sk, dh), BF16),
            pltpu.VMEM((hkv, d, 2 * dh), BF16),
            pltpu.VMEM((hkv, d, 2 * dh), BF16),
            pltpu.VMEM((d, 6 * d), BF16),
            pltpu.VMEM((d, f), BF16),
            pltpu.VMEM((d, f), BF16),
            pltpu.VMEM((d, f), BF16),
            pltpu.VMEM((d, seq), BF16),
            pltpu.VMEM((2, TQ, d), BF16),
            pltpu.VMEM((2, d, TQ), F32),
            pltpu.VMEM((2 * TQ // LANES, sk, LANES), F32),
            pltpu.VMEM((2 * TQ // LANES, 1, LANES), F32),
            pltpu.VMEM((dh, sk), BF16),
            pltpu.VMEM((8, d), F32),
            pltpu.VMEM((4, d, LANES), F32),
            pltpu.VMEM((n_q, TQ), F32),
            pltpu.VMEM((d, seq), BF16),
            pltpu.VMEM((d, seq), BF16),
            pltpu.SemaphoreType.DMA((4, HEAD_SLOTS)),
            pltpu.SemaphoreType.DMA((4,)),
            pltpu.SemaphoreType.DMA((3,)),
            pltpu.SemaphoreType.DMA((n_q,)),
            pltpu.SemaphoreType.DMA((TOPC,)),
        ],
        compiler_params=pltpu.CompilerParams(
            disable_bounds_checks=True,
            disable_semaphore_checks=True,
            vmem_limit_bytes=110 * 1024 * 1024,
        ),
    )(xt, k3, v3, A_wq, wot, B_w_r, B_w_gate, B_w_up, wdt, c, w_mod)
    return out_t.T.reshape(b, seq, d)
```

```python
import contextlib
import functools
import math
import os

import jax
import jax.numpy as jnp
from jax import lax
import jax.experimental.pallas as pl
import jax.experimental.pallas.tpu as pltpu

F32 = jnp.float32
BF16 = jnp.bfloat16
I32 = jnp.int32
U32 = jnp.uint32

HQ = 32
DH = 128
TOPC = 8
EPS = 1e-05
LANES = 128

TQ = int(os.environ.get("KP_TQ", "1024"))
TIE0 = int(os.environ.get("KP_TIE0", "2"))
NTIE = int(os.environ.get("KP_NTIE", "3"))
CH = int(os.environ.get("KP_CH", "512"))
FP = int(os.environ.get("KP_FP", "128"))
SCOPES = os.environ.get("KP_SCOPES", "") == "1"

_NT = (((1,), (1,)), ((), ()))


def _rb(x):
    return x.astype(BF16).astype(F32)


def _sigmoid(x):
    return 1.0 / (1.0 + jnp.exp(-x))


def _lanes(col, width):
    reps = width // LANES
    return col if reps == 1 else jnp.concatenate([col] * reps, axis=1)


def _scope(name):
    return jax.named_scope(name) if SCOPES else contextlib.nullcontext()


def _kernel(xt_hbm, k_hbm, v_hbm, wq_hbm, wot_hbm, wr_ref, wg_hbm, wu_hbm, wdt_hbm,
            c_ref, wmod_hbm, o_hbm,
            xt_v, k_v, v_v, wq_v, wot_v, wmod_v, wg_v, wu_v, wdt_v, ot_v,
            h_scr, acc_scr, st_scr, m_scr, vt_scr, mod_scr, col_scr, key_scr, h2_scr, x1_scr,
            head_sems, misc_sems, mlp_sems, out_sems, fix_sems,
            *, n_heads, n_q):
    n_units = n_heads * n_q
    d, seq = xt_v.shape
    sk = k_v.shape[1]
    nb = TQ // LANES
    nt = sk // LANES
    cb = CH // LANES
    qbits = n_q.bit_length() - 1
    qscale = (DH ** -0.5) * math.log2(math.e)

    def head_of(u):
        return u >> qbits

    def blk_of(u):
        return u & (n_q - 1)

    def head_copies(h):
        c2 = pl.ds(h * 2 * DH, 2 * DH)
        return (pltpu.make_async_copy(wq_hbm.at[:, c2], wq_v.at[h], head_sems.at[0, h]),
                pltpu.make_async_copy(k_hbm.at[h], k_v.at[h], head_sems.at[1, h]),
                pltpu.make_async_copy(v_hbm.at[h], v_v.at[h], head_sems.at[2, h]),
                pltpu.make_async_copy(wot_hbm.at[:, c2], wot_v.at[h], head_sems.at[3, h]))

    def col_copy(src, dst, lo, hi, sem):
        return pltpu.make_async_copy(src.at[:, lo:hi], dst.at[:, lo:hi], sem)

    x_first = col_copy(xt_hbm, xt_v, 0, CH, misc_sems.at[0])
    x_rest = col_copy(xt_hbm, xt_v, CH, seq, misc_sems.at[1])
    mod_first = col_copy(wmod_hbm, wmod_v, 0, 2 * d, misc_sems.at[2])
    mod_rest = col_copy(wmod_hbm, wmod_v, 2 * d, 6 * d, misc_sems.at[3])

    def mlp_copies():
        return (pltpu.make_async_copy(wg_hbm, wg_v, mlp_sems.at[0]),
                pltpu.make_async_copy(wu_hbm, wu_v, mlp_sems.at[1]),
                pltpu.make_async_copy(wdt_hbm, wdt_v, mlp_sems.at[2]))

    def silu_c():
        cc = c_ref[...].astype(F32)
        return jnp.broadcast_to((cc * _rb(_sigmoid(cc))).astype(BF16), (8, d))

    def ln1_norm(ch):
        x = xt_v[:, ch * CH:(ch + 1) * CH].astype(F32)
        mu = jnp.sum(x, axis=0, keepdims=True) * (1.0 / d)
        xc = x - mu
        var = jnp.sum(xc * xc, axis=0, keepdims=True) * (1.0 / d)
        return (xc * lax.rsqrt(var + EPS)).astype(BF16).T

    def h_rows(ch):
        r0 = (ch * CH) % TQ
        return ((ch * CH) // TQ, slice(r0, r0 + CH), slice(None))

    def ln1_mod(ch, ln):
        h_scr[h_rows(ch)] = (ln.astype(F32) * mod_scr[1:2, :] + mod_scr[0:1, :]).astype(BF16)

    def qproj(u, lo=0, hi=TQ):
        q = jnp.dot(h_scr[blk_of(u), lo:hi, :], wq_v[head_of(u)], preferred_element_type=F32)
        return (q * qscale).astype(BF16)

    def qk(u, q, j, b0=0):
        st = lax.dot_general(k_v[head_of(u)], q[:, j * DH:(j + 1) * DH], _NT,
                             preferred_element_type=F32)
        for i in range(q.shape[0] // LANES):
            blk = st[:, i * LANES:(i + 1) * LANES]
            st_scr[j * nb + b0 + i] = blk
            m_scr[j * nb + b0 + i] = jnp.max(blk, axis=0, keepdims=True)

    def pv(slots, zero):
        ps, ls, pairs = [], [], []
        for sl in slots:
            p = jnp.exp2(st_scr[sl] - m_scr[sl])
            accs = [None] * 4
            for tile in range(nt):
                for r0 in range(tile * LANES + LANES - 16, tile * LANES - 16, -16):
                    pair = p[r0:r0 + 8] + p[r0 + 8:r0 + 16]
                    pairs.append(pair)
                    a = accs[tile % 4]
                    accs[tile % 4] = pair if a is None else a + pair
            ls.append(jnp.sum((accs[0] + accs[1]) + (accs[2] + accs[3]), axis=0, keepdims=True))
            ps.append(p.astype(BF16))
        outs = []
        for i in range(len(slots)):
            vu = pltpu.bitcast(vt_scr[...], U32)
            tiles = []
            for c in range(nt):
                g = i * nt + c + 4
                rows = []
                for r in range(8):
                    x = vu[8 * r:8 * r + 8, c * LANES:(c + 1) * LANES]
                    if g < len(slots) * nt and TIE0 <= r < TIE0 + NTIE:
                        src = pairs[g * 8 + (r - TIE0)]
                        x = x | (lax.bitcast_convert_type(src, U32) & zero)
                    rows.append(x)
                tiles.append(jnp.concatenate(rows, axis=0))
            lhs = pltpu.bitcast(jnp.concatenate(tiles, axis=1), BF16)
            o = jnp.dot(lhs, ps[i], preferred_element_type=F32)
            outs.append((o * (1.0 / ls[i])).astype(BF16))
        return outs

    def outproj(u, oa, ob, lo=0):
        o2 = jnp.concatenate([jnp.concatenate(oa, axis=1), jnp.concatenate(ob, axis=1)], axis=0)
        contrib = jnp.dot(wot_v[head_of(u)], o2, preferred_element_type=F32)
        hi = lo + o2.shape[1]
        old = jnp.where(head_of(u) > 0, acc_scr[blk_of(u), :, lo:hi], 0.0)
        acc_scr[blk_of(u), :, lo:hi] = old + contrib

    def finalize(t0):
        cs = slice(t0, t0 + FP)
        x = xt_v[:, cs].astype(F32)
        att = acc_scr[t0 // TQ, :, t0 % TQ:t0 % TQ + FP]
        x1b = (x + _lanes(col_scr[0], FP) * att).astype(BF16)
        x1 = x1b.astype(F32)
        mu = jnp.sum(x1, axis=0, keepdims=True) * (1.0 / d)
        xc = x1 - mu
        var = jnp.sum(xc * xc, axis=0, keepdims=True) * (1.0 / d)
        inv = 1.0 / _rb(jnp.sqrt(_rb(_rb(var) + EPS)))
        ln = (x1 - _rb(mu)) * inv
        h2 = (ln * _lanes(col_scr[2], FP) + _lanes(col_scr[1], FP)).astype(BF16)
        ot_v[:, cs] = (x1 + _lanes(col_scr[3], FP) * h2.astype(F32)).astype(BF16)
        h2_scr[:, cs] = h2
        x1_scr[:, cs] = x1b
        wr = jnp.broadcast_to(wr_ref[...].reshape(1, d), (8, d))
        r = _rb(jnp.dot(wr, h2, preferred_element_type=F32)[0:1, :]) + 0.0
        bits = lax.bitcast_convert_type(r, I32) >> 16
        order = jnp.where(bits < 0, -1 - bits, bits + 32768)
        pos = t0 + lax.broadcasted_iota(I32, (1, FP), 1)
        key = (order << 11) + (seq - 1 - pos) + 0x20000000
        key_scr[t0 // FP:t0 // FP + 1, :] = lax.bitcast_convert_type(key, F32)

    wq0, k0, v0, wo0 = head_copies(0)
    x_first.start()
    mod_first.start()
    with _scope("w_x"):
        x_first.wait()
    wq0.start()
    h_scr[h_rows(0)] = ln1_norm(0)
    with _scope("w_wmod"):
        mod_first.wait()
    k0.start()
    x_rest.start()
    mod = _rb(jnp.dot(silu_c(), wmod_v[:, 0:2 * d], preferred_element_type=F32))
    mod_scr[0:1, :] = mod[0:1, 0:d]
    mod_scr[1:2, :] = _rb(1.0 + mod[0:1, d:2 * d])
    ln1_mod(0, h_scr[h_rows(0)])
    with _scope("w_wq"):
        wq0.wait()
    q = qproj(0, 0, CH)
    with _scope("w_k"):
        k0.wait()
    v0.start()
    qk(0, q, 0)
    with _scope("w_x2"):
        x_rest.wait()
        v0.wait()
    wo0.start()
    for cp in head_copies(1):
        cp.start()
    with _scope("qk0"):
        qk(0, q, 1)
        for ch in range(1, TQ // CH):
            ln1_mod(ch, ln1_norm(ch))
            q = qproj(0, ch * CH, (ch + 1) * CH)
            qk(0, q, 0, ch * cb)
            qk(0, q, 1, ch * cb)
        for ch in range(TQ // CH, seq // CH):
            ln1_mod(ch, ln1_norm(ch))
        vt_scr[...] = v_v[0].T

    groups = [list(range(2, 6)), list(range(6, 11)), list(range(11, n_heads))]

    def steady(u, carry):
        @pl.when(u <= 5)
        def _():
            @pl.when(u == 1)
            def _():
                wo0.wait()
                for cp in head_copies(1):
                    cp.wait()

            for i in range(len(groups) + 1):
                @pl.when(u == i + 1)
                def _():
                    if i > 0:
                        for h in groups[i - 1]:
                            for cp in head_copies(h):
                                cp.wait()
                    if i < len(groups):
                        for h in groups[i]:
                            for cp in head_copies(h):
                                cp.start()
                    else:
                        mod_rest.start()

            @pl.when(u == 5)
            def _():
                mod_rest.wait()
                for cp in mlp_copies():
                    cp.start()
                mod = _rb(jnp.dot(silu_c(), wmod_v[:, 2 * d:6 * d], preferred_element_type=F32))
                for j in range(4):
                    piece = mod[0:1, j * d:(j + 1) * d]
                    if j == 2:
                        piece = _rb(1.0 + piece)
                    col_scr[j] = jnp.broadcast_to(piece, (LANES, d)).T

        with _scope("body"):
            zero = jnp.full((8, LANES), u >> 20, I32).astype(U32)
            q = qproj(u)
            oa = pv(range(0, nb), zero)
            qk(u, q, 0)
            ob = pv(range(nb, 2 * nb), zero)
            outproj(u - 1, oa, ob)
            qk(u, q, 1)
            vt_scr[...] = v_v[head_of(u)].T
        return carry + 1

    count = lax.fori_loop(1, n_units, steady, 0)

    for cp in mlp_copies():
        cp.wait()
    with _scope("lastpv"):
        zero = jnp.full((8, LANES), count >> 20, I32).astype(U32)
        todo = list(range(0, seq - TQ, FP))
        nch = TQ // CH
        for ch in range(nch):
            share = -(-len(todo) // (2 * (nch - ch)))
            oa = pv(range(ch * cb, (ch + 1) * cb), zero)
            for t0 in todo[:share]:
                finalize(t0)
            ob = pv(range(nb + ch * cb, nb + (ch + 1) * cb), zero)
            for t0 in todo[share:2 * share]:
                finalize(t0)
            todo = todo[2 * share:]
            outproj(n_units - 1, oa, ob, ch * CH)
            todo += list(range(seq - TQ + ch * CH, seq - TQ + (ch + 1) * CH, FP))
        for t0 in todo:
            finalize(t0)
    out_all = pltpu.make_async_copy(ot_v, o_hbm, out_sems.at[0])
    out_all.start()

    keys = key_scr[...]
    sub8 = lax.broadcasted_iota(I32, (TOPC, 1), 0)
    lane = lax.broadcasted_iota(I32, (TOPC, LANES), 1)
    top = jnp.zeros((TOPC, 1), F32)
    idxs = []
    for i in range(TOPC):
        mx = jnp.max(jnp.max(keys, axis=0, keepdims=True), axis=1, keepdims=True)
        keys = jnp.where(keys == mx, 0.0, keys)
        top = jnp.where(sub8 == i, mx, top)
        kb = lax.bitcast_convert_type(mx, I32)
        idxs.append(seq - 1 - (kb[0, 0] & (seq - 1)))
    kb = lax.bitcast_convert_type(top, I32)
    idx_col = seq - 1 - (kb & (seq - 1))
    order = (kb >> 11) & 0xFFFF
    rbits = jnp.where(order >= 32768, order - 32768, -1 - order) << 16
    r_sel = lax.bitcast_convert_type(rbits, F32)
    bases = [pl.multiple_of(ix & ~(LANES - 1), LANES) for ix in idxs]
    xs = jnp.zeros((TOPC, d), F32)
    for i in range(TOPC):
        pick = jnp.logical_and(sub8 == i, lane + bases[i] == idx_col)
        pick = jnp.where(pick, 1.0, 0.0).astype(BF16)
        xs = xs + lax.dot_general(pick, h2_scr[:, pl.ds(bases[i], LANES)], _NT,
                                  preferred_element_type=F32)
    xs = xs.astype(BF16)
    g = _rb(jnp.dot(xs, wg_v[...], preferred_element_type=F32))
    g = _rb(g * _rb(_sigmoid(g)))
    u = _rb(jnp.dot(xs, wu_v[...], preferred_element_type=F32))
    y = _rb(lax.dot_general((g * u).astype(BF16), wdt_v[...], _NT,
                            preferred_element_type=F32))
    y = _rb(y * _rb(_sigmoid(r_sel)))
    ypad = jnp.concatenate([y, jnp.zeros((LANES - TOPC, d), F32)], axis=0)
    yt = ypad.T.astype(BF16)
    idx_big = jnp.concatenate([idx_col, jnp.full((LANES - TOPC, 1), -1, I32)], axis=0)
    lane2 = lax.broadcasted_iota(I32, (LANES, LANES), 1)
    out_all.wait()
    for i in range(TOPC):
        place = jnp.where(lane2 + bases[i] == idx_big, 1.0, 0.0).astype(BF16)
        upd = jnp.dot(yt, place, preferred_element_type=F32)
        sl = pl.ds(bases[i], LANES)
        hm = _rb(h2_scr[:, sl].astype(F32) + upd)
        ot_v[:, sl] = (x1_scr[:, sl].astype(F32) + col_scr[3] * hm).astype(BF16)

    def fix_copy(i):
        sl = pl.ds(bases[i], LANES)
        return pltpu.make_async_copy(ot_v.at[:, sl], o_hbm.at[:, sl], fix_sems.at[i])

    fresh = []
    for i in range(TOPC):
        ok = True
        for j in range(i):
            ok = jnp.logical_and(ok, bases[i] != bases[j])
        fresh.append(ok)
    fix_copy(0).start()
    for i in range(1, TOPC):
        pl.when(fresh[i])(lambda i=i: fix_copy(i).start())
    with _scope("w_fix"):
        fix_copy(0).wait()
        for i in range(1, TOPC):
            pl.when(fresh[i])(lambda i=i: fix_copy(i).wait())


@jax.jit
def pallas_adaLN_cond__gqa_block_cached__moe_arch_mod__prompt_kernel(
    A_x: jax.Array,
    A_k_cache: jax.Array,
    A_v_cache: jax.Array,
    A_wq: jax.Array,
    A_wo: jax.Array,
    B_x: jax.Array,
    B_w_r: jax.Array,
    B_w_gate: jax.Array,
    B_w_up: jax.Array,
    B_w_down: jax.Array,
    c: jax.Array,
    w_mod: jax.Array,
):
    b, seq, d = A_x.shape
    _, hkv, sk, dh = A_k_cache.shape
    assert b == 1 and dh == DH and HQ == 2 * hkv
    assert seq & (seq - 1) == 0 and seq <= 2048
    f = B_w_gate.shape[1]
    n_q = seq // TQ

    xt = A_x.reshape(seq, d).T
    wot = A_wo.T
    wdt = B_w_down.T
    k3 = A_k_cache.reshape(hkv, sk, dh)
    v3 = A_v_cache.reshape(hkv, sk, dh)

    vmem = pl.BlockSpec(memory_space=pltpu.VMEM)
    hbm = pl.BlockSpec(memory_space=pl.ANY)
    out_t = pl.pallas_call(
        functools.partial(_kernel, n_heads=hkv, n_q=n_q),
        in_specs=[
            hbm, hbm, hbm, hbm, hbm,
            vmem,
            hbm, hbm, hbm,
            vmem,
            hbm,
        ],
        out_specs=hbm,
        out_shape=jax.ShapeDtypeStruct((d, seq), BF16),
        scratch_shapes=[
            pltpu.VMEM((d, seq), BF16),
            pltpu.VMEM((hkv, sk, dh), BF16),
            pltpu.VMEM((hkv, sk, dh), BF16),
            pltpu.VMEM((hkv, d, 2 * dh), BF16),
            pltpu.VMEM((hkv, d, 2 * dh), BF16),
            pltpu.VMEM((d, 6 * d), BF16),
            pltpu.VMEM((d, f), BF16),
            pltpu.VMEM((d, f), BF16),
            pltpu.VMEM((d, f), BF16),
            pltpu.VMEM((d, seq), BF16),
            pltpu.VMEM((n_q, TQ, d), BF16),
            pltpu.VMEM((n_q, d, TQ), F32),
            pltpu.VMEM((2 * TQ // LANES, sk, LANES), F32),
            pltpu.VMEM((2 * TQ // LANES, 1, LANES), F32),
            pltpu.VMEM((dh, sk), BF16),
            pltpu.VMEM((8, d), F32),
            pltpu.VMEM((4, d, LANES), F32),
            pltpu.VMEM((seq // FP, FP), F32),
            pltpu.VMEM((d, seq), BF16),
            pltpu.VMEM((d, seq), BF16),
            pltpu.SemaphoreType.DMA((4, hkv)),
            pltpu.SemaphoreType.DMA((4,)),
            pltpu.SemaphoreType.DMA((3,)),
            pltpu.SemaphoreType.DMA((1,)),
            pltpu.SemaphoreType.DMA((TOPC,)),
        ],
        compiler_params=pltpu.CompilerParams(
            disable_bounds_checks=True,
            disable_semaphore_checks=True,
            vmem_limit_bytes=110 * 1024 * 1024,
        ),
    )(xt, k3, v3, A_wq, wot, B_w_r, B_w_gate, B_w_up, wdt, c, w_mod)
    return out_t.T.reshape(b, seq, d)
```

```python
import contextlib
import functools
import math
import os

import jax
import jax.numpy as jnp
from jax import lax
import jax.experimental.pallas as pl
import jax.experimental.pallas.tpu as pltpu

F32 = jnp.float32
BF16 = jnp.bfloat16
I32 = jnp.int32
U32 = jnp.uint32

HQ = 32
DH = 128
TOPC = 8
EPS = 1e-05
LANES = 128

TQ = int(os.environ.get("KP_TQ", "1024"))
TIE0 = int(os.environ.get("KP_TIE0", "2"))
NTIE = int(os.environ.get("KP_NTIE", "3"))
CH = int(os.environ.get("KP_CH", "512"))
FP = int(os.environ.get("KP_FP", "256"))
NM1 = int(os.environ.get("KP_NM1", "8"))
NM2 = int(os.environ.get("KP_NM2", "12"))
NM3 = int(os.environ.get("KP_NM3", "16"))
TLO = int(os.environ.get("KP_TLO", "8"))
PRIO = int(os.environ.get("KP_PRIO", "1"))
NF1 = int(os.environ.get("KP_NF1", "9"))
NF2 = int(os.environ.get("KP_NF2", "6"))
NF3 = int(os.environ.get("KP_NF3", "18"))
TAILB = int(os.environ.get("KP_TAILB", "2"))
SIDE_ROW = int(os.environ.get("KP_SIDE_ROW", "1"))
SCOPES = os.environ.get("KP_SCOPES", "") == "1"

_NT = (((1,), (1,)), ((), ()))


def _rb(x):
    return x.astype(BF16).astype(F32)


def _sigmoid(x):
    return 1.0 / (1.0 + jnp.exp(-x))


def _lanes(col, width):
    reps = width // LANES
    return col if reps == 1 else jnp.concatenate([col] * reps, axis=1)


def _fold(x):
    xi = lax.bitcast_convert_type(x, U32)
    tok = None
    for r in range(0, x.shape[0], 8):
        for c in range(0, x.shape[1] - LANES + 1, LANES):
            t = xi[r:r + 8, c:c + LANES]
            tok = t if tok is None else tok | t
    return tok


def _colsum(x, marks, nmarks):
    n = x.shape[0] // 8
    acc = x[0:8]
    for g in range(1, n):
        acc = acc + x[8 * g:8 * g + 8]
        if ((g + 1) * nmarks) % n == 0:
            marks.append(_fold(acc))
    return jnp.sum(acc, axis=0, keepdims=True)


def _tie_rows(lhs, toks, zero, lo, hi):
    if not toks:
        return lhs
    lu = pltpu.bitcast(lhs, U32)
    rows = [lu[8 * r:8 * r + 8] for r in range(lu.shape[0] // 8)]
    for i, tok in enumerate(toks):
        r = lo + ((i + 1) * (hi - lo)) // len(toks) - 1
        rows[r] = rows[r] | (tok & zero)
    return pltpu.bitcast(jnp.concatenate(rows, axis=0), BF16)


def _scope(name):
    return jax.named_scope(name) if SCOPES else contextlib.nullcontext()


def _kernel(xt_hbm, k_hbm, v_hbm, wq_hbm, wot_hbm, wr_ref, wg_hbm, wu_hbm, wdt_hbm,
            c_ref, wmod_hbm, o_hbm,
            xt_v, k_v, v_v, wq_v, wot_v, wmod_v, wg_v, wu_v, wdt_v, ot_v,
            h_scr, acc_scr, st_scr, m_scr, vt_scr, mod_scr, col_scr, key_scr, h2_scr, x1_scr,
            zero_scr,
            head_sems, misc_sems, mlp_sems, out_sems, fix_sems,
            *, n_heads, n_q):
    n_units = n_heads * n_q
    d, seq = xt_v.shape
    sk = k_v.shape[1]
    nb = TQ // LANES
    nt = sk // LANES
    cb = CH // LANES
    qbits = n_q.bit_length() - 1
    qscale = (DH ** -0.5) * math.log2(math.e)

    def head_of(u):
        return u >> qbits

    def blk_of(u):
        return u & (n_q - 1)

    def head_copies(h):
        c2 = pl.ds(h * 2 * DH, 2 * DH)
        return (pltpu.make_async_copy(wq_hbm.at[:, c2], wq_v.at[h], head_sems.at[0, h]),
                pltpu.make_async_copy(k_hbm.at[h], k_v.at[h], head_sems.at[1, h]),
                pltpu.make_async_copy(v_hbm.at[h], v_v.at[h], head_sems.at[2, h]),
                pltpu.make_async_copy(wot_hbm.at[:, c2], wot_v.at[h], head_sems.at[3, h]))

    def col_copy(src, dst, lo, hi, sem):
        return pltpu.make_async_copy(src.at[:, lo:hi], dst.at[:, lo:hi], sem)

    x_first = col_copy(xt_hbm, xt_v, 0, CH, misc_sems.at[0])
    x_second = col_copy(xt_hbm, xt_v, CH, 2 * CH, misc_sems.at[4])
    x_rest = col_copy(xt_hbm, xt_v, 2 * CH, seq, misc_sems.at[1])
    mod_first = col_copy(wmod_hbm, wmod_v, 0, 2 * d, misc_sems.at[2])
    mod_rest = col_copy(wmod_hbm, wmod_v, 2 * d, 6 * d, misc_sems.at[3])

    def mlp_copies():
        return (pltpu.make_async_copy(wg_hbm, wg_v, mlp_sems.at[0]),
                pltpu.make_async_copy(wu_hbm, wu_v, mlp_sems.at[1]),
                pltpu.make_async_copy(wdt_hbm, wdt_v, mlp_sems.at[2]))

    def silu_c():
        cc = c_ref[...].astype(F32)
        return jnp.broadcast_to((cc * _rb(_sigmoid(cc))).astype(BF16), (8, d))

    def ln1_norm(ch, marks):
        x = xt_v[:, ch * CH:(ch + 1) * CH].astype(F32)
        mu = _colsum(x, marks, NM1) * (1.0 / d)
        xc = x - mu
        var = _colsum(xc * xc, marks, NM2) * (1.0 / d)
        return (xc * lax.rsqrt(var + EPS)).astype(BF16).T

    def h_rows(ch):
        r0 = (ch * CH) % TQ
        return ((ch * CH) // TQ, slice(r0, r0 + CH), slice(None))

    def ln1_mod(ch, ln, marks):
        h = ln.astype(F32) * mod_scr[1:2, :] + mod_scr[0:1, :]
        h_scr[h_rows(ch)] = h.astype(BF16)
        step = CH // NM3
        for r in range(step - 8, CH, step):
            marks.append(_fold(h[r:r + 8]))

    def ln1(ch):
        marks = []
        ln1_mod(ch, ln1_norm(ch, marks), marks)
        return marks

    def qproj(u, lo=0, hi=TQ):
        q = jnp.dot(h_scr[blk_of(u), lo:hi, :], wq_v[head_of(u)], preferred_element_type=F32)
        return (q * qscale).astype(BF16)

    def qk_slots(u, q, qb0, slots, toks=(), zero=None):
        k = _tie_rows(k_v[head_of(u)], toks, zero, TLO, sk // 16)
        parts = []
        for sl in slots:
            j, r0 = sl // nb, (sl % nb - qb0) * LANES
            parts.append(q[r0:r0 + LANES, j * DH:(j + 1) * DH])
        st = lax.dot_general(k, jnp.concatenate(parts, axis=0), _NT,
                             preferred_element_type=F32)
        for i, sl in enumerate(slots):
            blk = st[:, i * LANES:(i + 1) * LANES]
            st_scr[sl] = blk
            m_scr[sl] = jnp.max(blk, axis=0, keepdims=True)

    def qk(u, q, j, b0=0, toks=(), zero=None):
        n = q.shape[0] // LANES
        qk_slots(u, q, b0, range(j * nb + b0, j * nb + b0 + n), toks, zero)

    def pv(slots, zero, toks=()):
        ps, ls, pairs = [], [], []
        for sl in slots:
            p = jnp.exp2(st_scr[sl] - m_scr[sl])
            accs = [None] * 4
            for tile in range(nt):
                for r0 in range(tile * LANES + LANES - 16, tile * LANES - 16, -16):
                    pair = p[r0:r0 + 8] + p[r0 + 8:r0 + 16]
                    pairs.append(pair)
                    a = accs[tile % 4]
                    accs[tile % 4] = pair if a is None else a + pair
            ls.append(jnp.sum((accs[0] + accs[1]) + (accs[2] + accs[3]), axis=0, keepdims=True))
            ps.append(p.astype(BF16))
        outs = []
        ntiles = len(slots) * nt
        side = {}
        for i, tok in enumerate(toks):
            side.setdefault(((i + 1) * ntiles) // len(toks) - 1, []).append(tok)
        for i in range(len(slots)):
            vu = pltpu.bitcast(vt_scr[...], U32)
            tiles = []
            for c in range(nt):
                g = i * nt + c + 4
                rows = []
                for r in range(8):
                    x = vu[8 * r:8 * r + 8, c * LANES:(c + 1) * LANES]
                    if g < len(slots) * nt and TIE0 <= r < TIE0 + NTIE:
                        src = pairs[g * 8 + (r - TIE0)]
                        x = x | (lax.bitcast_convert_type(src, U32) & zero)
                    if r == SIDE_ROW:
                        for tok in side.get(i * nt + c, ()):
                            x = x | (tok & zero)
                    rows.append(x)
                tiles.append(jnp.concatenate(rows, axis=0))
            lhs = pltpu.bitcast(jnp.concatenate(tiles, axis=1), BF16)
            o = jnp.dot(lhs, ps[i], preferred_element_type=F32)
            outs.append((o * (1.0 / ls[i])).astype(BF16))
        return outs

    def outproj(u, oa, ob, lo=0):
        o2 = jnp.concatenate([jnp.concatenate(oa, axis=1), jnp.concatenate(ob, axis=1)], axis=0)
        contrib = jnp.dot(wot_v[head_of(u)], o2, preferred_element_type=F32)
        hi = lo + o2.shape[1]
        old = jnp.where(head_of(u) > 0, acc_scr[blk_of(u), :, lo:hi], 0.0)
        acc_scr[blk_of(u), :, lo:hi] = old + contrib

    def finalize(t0):
        marks = []
        cs = slice(t0, t0 + FP)
        x = xt_v[:, cs].astype(F32)
        att = acc_scr[t0 // TQ, :, t0 % TQ:t0 % TQ + FP]
        x1b = (x + _lanes(col_scr[0], FP) * att).astype(BF16)
        x1_scr[:, cs] = x1b
        ot_v[:, cs] = x1b
        x1 = x1b.astype(F32)
        mu = _colsum(x1, marks, NF1) * (1.0 / d)
        mub = _rb(mu)
        xc = x1_scr[:, cs].astype(F32) - mub
        var = _colsum(xc * xc, marks, NF2) * (1.0 / d) - (mu - mub) * (mu - mub)
        inv = 1.0 / _rb(jnp.sqrt(_rb(_rb(jnp.maximum(var, 0.0)) + EPS)))
        x1 = ot_v[:, cs].astype(F32)
        xc = x1 - mub
        h2b = (xc * inv * _lanes(col_scr[2], FP) + _lanes(col_scr[1], FP)).astype(BF16)
        h2_scr[:, cs] = h2b
        h2 = h2b.astype(F32)
        out = x1 + _lanes(col_scr[3], FP) * h2
        ot_v[:, cs] = out.astype(BF16)
        rmarks = []
        r = _rb(_colsum(h2 * _lanes(col_scr[4], FP), rmarks, NF3)) + 0.0
        step = d // NF3
        for i, tok in enumerate(rmarks):
            marks.append(tok | _fold(out[i * step:(i + 1) * step]))
        bits = lax.bitcast_convert_type(r, I32) >> 16
        order = jnp.where(bits < 0, -1 - bits, bits + 32768)
        pos = t0 + lax.broadcasted_iota(I32, (1, FP), 1)
        key = (order << 11) + (seq - 1 - pos) + 0x20000000
        key_scr[t0 // FP:t0 // FP + 1, :] = lax.bitcast_convert_type(key, F32)
        return marks

    wq0, k0, v0, wo0 = head_copies(0)
    x_first.start()
    mod_first.start()
    if PRIO:
        wq0.start()
        k0.start(priority=1)
        x_second.start(priority=1)
    cbits = lax.bitcast_convert_type(c_ref[:, 0:LANES].astype(F32), U32)
    zero_scr[...] = jnp.broadcast_to(cbits & 0xFFFF, (8, LANES))
    with _scope("w_x"):
        x_first.wait()
    if not PRIO:
        wq0.start()
    h_scr[h_rows(0)] = ln1_norm(0, [])
    with _scope("w_wmod"):
        mod_first.wait()
    with _scope("w_wq"):
        wq0.wait()
    if not PRIO:
        k0.start()
        x_second.start()
    else:
        x_rest.start(priority=1)
        v0.start(priority=1)
    mod = _rb(jnp.dot(silu_c(), wmod_v[:, 0:2 * d], preferred_element_type=F32))
    mod_scr[0:1, :] = mod[0:1, 0:d]
    mod_scr[1:2, :] = _rb(1.0 + mod[0:1, d:2 * d])
    ln1_mod(0, h_scr[h_rows(0)], [])
    q0 = qproj(0, 0, CH)
    with _scope("w_k"):
        k0.wait()
        x_second.wait()
    if not PRIO:
        x_rest.start()
        v0.start()
    assert TQ == 2 * CH and seq == 4 * CH
    zero = zero_scr[...]
    qk(0, q0, 0, 0, ln1(1), zero)
    q1 = qproj(0, CH, 2 * CH)
    with _scope("w_x2"):
        x_rest.wait()
        v0.wait()
    wo0.start()
    for cp in head_copies(1):
        cp.start()
    with _scope("qk0"):
        zero = zero_scr[...]
        qk(0, q0, 1, 0, ln1(2), zero)
        qk(0, q1, 0, cb, ln1(3), zero)
        qk(0, q1, 1, cb)
        vt_scr[...] = v_v[0].T

    groups = [list(range(2, 6)), list(range(6, 11)), list(range(11, n_heads))]

    def steady(u, carry):
        @pl.when(u <= 5)
        def _():
            @pl.when(u == 1)
            def _():
                wo0.wait()
                for cp in head_copies(1):
                    cp.wait()

            for i in range(len(groups) + 1):
                @pl.when(u == i + 1)
                def _():
                    if i > 0:
                        for h in groups[i - 1]:
                            for cp in head_copies(h):
                                cp.wait()
                    if i < len(groups):
                        for h in groups[i]:
                            for cp in head_copies(h):
                                cp.start()
                    else:
                        mod_rest.start()

            @pl.when(u == 5)
            def _():
                mod_rest.wait()
                for cp in mlp_copies():
                    cp.start()
                mod = _rb(jnp.dot(silu_c(), wmod_v[:, 2 * d:6 * d], preferred_element_type=F32))
                for j in range(4):
                    piece = mod[0:1, j * d:(j + 1) * d]
                    if j == 2:
                        piece = _rb(1.0 + piece)
                    col_scr[j] = jnp.broadcast_to(piece, (LANES, d)).T
                wr = wr_ref[...].reshape(1, d).astype(F32)
                col_scr[4] = jnp.broadcast_to(wr, (LANES, d)).T

        with _scope("body"):
            zero = jnp.full((8, LANES), u >> 20, I32).astype(U32)
            q = qproj(u)
            oa = pv(range(0, nb), zero)
            qk(u, q, 0)
            ob = pv(range(nb, 2 * nb), zero)
            outproj(u - 1, oa, ob)
            qk(u, q, 1)
            vt_scr[...] = v_v[head_of(u)].T
        return carry + 1

    lax.fori_loop(1, n_units - 1, steady, 0)

    assert n_q == 2
    ul = n_units - 1
    mlp_g, mlp_u, mlp_d = mlp_copies()
    out_lo = col_copy(ot_v, o_hbm, 0, TQ, out_sems.at[0])
    out_hi = col_copy(ot_v, o_hbm, TQ, seq, out_sems.at[1])
    nb0 = nb - TAILB
    first = [j * nb + i for j in range(2) for i in range(nb0)]
    rest = [j * nb + i for j in range(2) for i in range(nb0, nb)]
    with _scope("e_pv30"):
        zero = zero_scr[...]
        q = qproj(ul)
        o = pv(range(2 * nb), zero)
        outproj(ul - 1, o[:nb], o[nb:])
    mlp_g.wait()
    with _scope("e_qk31a"):
        zero = zero_scr[...]
        toks = [tok for t0 in range(0, TQ, FP) for tok in finalize(t0)]
        ng = len(first) // 4
        for g in range(ng):
            qk_slots(ul, q, 0, first[4 * g:4 * g + 4],
                     toks[g * len(toks) // ng:(g + 1) * len(toks) // ng], zero)
    out_lo.start()
    mlp_u.wait()
    with _scope("e_pv31a"):
        o = pv(first, zero_scr[...])
        outproj(ul, o[:nb0], o[nb0:])
    mlp_d.wait()
    ready = list(range(TQ, TQ + nb0 * LANES, FP))
    with _scope("e_qk31b"):
        toks = [tok for t0 in ready[:-1] for tok in finalize(t0)]
        qk_slots(ul, q, 0, rest, toks, zero_scr[...])
    out_lo.wait()
    with _scope("e_pv31b"):
        o = pv(rest, zero_scr[...], finalize(ready[-1]))
        outproj(ul, o[:TAILB], o[TAILB:], nb0 * LANES)
        for t0 in range(TQ + nb0 * LANES, seq, FP):
            finalize(t0)
    out_hi.start()

    keys = key_scr[...]
    sub8 = lax.broadcasted_iota(I32, (TOPC, 1), 0)
    lane = lax.broadcasted_iota(I32, (TOPC, LANES), 1)
    top = jnp.zeros((TOPC, 1), F32)
    idxs = []
    for i in range(TOPC):
        mx = jnp.max(jnp.max(keys, axis=0, keepdims=True), axis=1, keepdims=True)
        keys = jnp.where(keys == mx, 0.0, keys)
        top = jnp.where(sub8 == i, mx, top)
        kb = lax.bitcast_convert_type(mx, I32)
        idxs.append(seq - 1 - (kb[0, 0] & (seq - 1)))
    kb = lax.bitcast_convert_type(top, I32)
    idx_col = seq - 1 - (kb & (seq - 1))
    order = (kb >> 11) & 0xFFFF
    rbits = jnp.where(order >= 32768, order - 32768, -1 - order) << 16
    r_sel = lax.bitcast_convert_type(rbits, F32)
    bases = [pl.multiple_of(ix & ~(LANES - 1), LANES) for ix in idxs]
    xs = jnp.zeros((TOPC, d), F32)
    for i in range(TOPC):
        pick = jnp.logical_and(sub8 == i, lane + bases[i] == idx_col)
        pick = jnp.where(pick, 1.0, 0.0).astype(BF16)
        xs = xs + lax.dot_general(pick, h2_scr[:, pl.ds(bases[i], LANES)], _NT,
                                  preferred_element_type=F32)
    xs = xs.astype(BF16)
    g = _rb(jnp.dot(xs, wg_v[...], preferred_element_type=F32))
    g = _rb(g * _rb(_sigmoid(g)))
    u = _rb(jnp.dot(xs, wu_v[...], preferred_element_type=F32))
    y = _rb(lax.dot_general((g * u).astype(BF16), wdt_v[...], _NT,
                            preferred_element_type=F32))
    y = _rb(y * _rb(_sigmoid(r_sel)))
    ypad = jnp.concatenate([y, jnp.zeros((LANES - TOPC, d), F32)], axis=0)
    yt = ypad.T.astype(BF16)
    idx_big = jnp.concatenate([idx_col, jnp.full((LANES - TOPC, 1), -1, I32)], axis=0)
    lane2 = lax.broadcasted_iota(I32, (LANES, LANES), 1)
    out_hi.wait()
    for i in range(TOPC):
        place = jnp.where(lane2 + bases[i] == idx_big, 1.0, 0.0).astype(BF16)
        upd = jnp.dot(yt, place, preferred_element_type=F32)
        sl = pl.ds(bases[i], LANES)
        hm = _rb(h2_scr[:, sl].astype(F32) + upd)
        ot_v[:, sl] = (x1_scr[:, sl].astype(F32) + col_scr[3] * hm).astype(BF16)

    def fix_copy(i):
        sl = pl.ds(bases[i], LANES)
        return pltpu.make_async_copy(ot_v.at[:, sl], o_hbm.at[:, sl], fix_sems.at[i])

    fresh = []
    for i in range(TOPC):
        ok = True
        for j in range(i):
            ok = jnp.logical_and(ok, bases[i] != bases[j])
        fresh.append(ok)
    fix_copy(0).start()
    for i in range(1, TOPC):
        pl.when(fresh[i])(lambda i=i: fix_copy(i).start())
    with _scope("w_fix"):
        fix_copy(0).wait()
        for i in range(1, TOPC):
            pl.when(fresh[i])(lambda i=i: fix_copy(i).wait())


@jax.jit
def pallas_adaLN_cond__gqa_block_cached__moe_arch_mod__prompt_kernel(
    A_x: jax.Array,
    A_k_cache: jax.Array,
    A_v_cache: jax.Array,
    A_wq: jax.Array,
    A_wo: jax.Array,
    B_x: jax.Array,
    B_w_r: jax.Array,
    B_w_gate: jax.Array,
    B_w_up: jax.Array,
    B_w_down: jax.Array,
    c: jax.Array,
    w_mod: jax.Array,
):
    b, seq, d = A_x.shape
    _, hkv, sk, dh = A_k_cache.shape
    assert b == 1 and dh == DH and HQ == 2 * hkv
    assert seq & (seq - 1) == 0 and seq <= 2048
    f = B_w_gate.shape[1]
    n_q = seq // TQ

    xt = A_x.reshape(seq, d).T
    wot = A_wo.T
    wdt = B_w_down.T
    k3 = A_k_cache.reshape(hkv, sk, dh)
    v3 = A_v_cache.reshape(hkv, sk, dh)

    vmem = pl.BlockSpec(memory_space=pltpu.VMEM)
    hbm = pl.BlockSpec(memory_space=pl.ANY)
    out_t = pl.pallas_call(
        functools.partial(_kernel, n_heads=hkv, n_q=n_q),
        in_specs=[
            hbm, hbm, hbm, hbm, hbm,
            vmem,
            hbm, hbm, hbm,
            vmem,
            hbm,
        ],
        out_specs=hbm,
        out_shape=jax.ShapeDtypeStruct((d, seq), BF16),
        scratch_shapes=[
            pltpu.VMEM((d, seq), BF16),
            pltpu.VMEM((hkv, sk, dh), BF16),
            pltpu.VMEM((hkv, sk, dh), BF16),
            pltpu.VMEM((hkv, d, 2 * dh), BF16),
            pltpu.VMEM((hkv, d, 2 * dh), BF16),
            pltpu.VMEM((d, 6 * d), BF16),
            pltpu.VMEM((d, f), BF16),
            pltpu.VMEM((d, f), BF16),
            pltpu.VMEM((d, f), BF16),
            pltpu.VMEM((d, seq), BF16),
            pltpu.VMEM((n_q, TQ, d), BF16),
            pltpu.VMEM((n_q, d, TQ), F32),
            pltpu.VMEM((2 * TQ // LANES, sk, LANES), F32),
            pltpu.VMEM((2 * TQ // LANES, 1, LANES), F32),
            pltpu.VMEM((dh, sk), BF16),
            pltpu.VMEM((8, d), F32),
            pltpu.VMEM((5, d, LANES), F32),
            pltpu.VMEM((seq // FP, FP), F32),
            pltpu.VMEM((d, seq), BF16),
            pltpu.VMEM((d, seq), BF16),
            pltpu.VMEM((8, LANES), U32),
            pltpu.SemaphoreType.DMA((4, hkv)),
            pltpu.SemaphoreType.DMA((5,)),
            pltpu.SemaphoreType.DMA((3,)),
            pltpu.SemaphoreType.DMA((2,)),
            pltpu.SemaphoreType.DMA((TOPC,)),
        ],
        compiler_params=pltpu.CompilerParams(
            disable_bounds_checks=True,
            disable_semaphore_checks=True,
            vmem_limit_bytes=110 * 1024 * 1024,
        ),
    )(xt, k3, v3, A_wq, wot, B_w_r, B_w_gate, B_w_up, wdt, c, w_mod)
    return out_t.T.reshape(b, seq, d)
```

```python
import contextlib
import functools
import math
import os

import jax
import jax.numpy as jnp
from jax import lax
import jax.experimental.pallas as pl
import jax.experimental.pallas.tpu as pltpu

F32 = jnp.float32
BF16 = jnp.bfloat16
I32 = jnp.int32
U32 = jnp.uint32

HQ = 32
DH = 128
TOPC = 8
EPS = 1e-05
LANES = 128

TB = 512
HG = 2
TIE0 = int(os.environ.get("KP_TIE0", "2"))
NTIE = int(os.environ.get("KP_NTIE", "3"))
SP = int(os.environ.get("KP_SP", "128"))
NM1 = int(os.environ.get("KP_NM1", "8"))
NM2 = int(os.environ.get("KP_NM2", "12"))
NM3 = int(os.environ.get("KP_NM3", "16"))
TLO = int(os.environ.get("KP_TLO", "8"))
NF1 = int(os.environ.get("KP_NF1", "9"))
NF2 = int(os.environ.get("KP_NF2", "6"))
NF3 = int(os.environ.get("KP_NF3", "18"))
NVT = int(os.environ.get("KP_NVT", "16"))
TAILB = int(os.environ.get("KP_TAILB", "2"))
SIDE_ROW = int(os.environ.get("KP_SIDE_ROW", "1"))
SCOPES = os.environ.get("KP_SCOPES", "") == "1"

_NT = (((1,), (1,)), ((), ()))


def _rb(x):
    return x.astype(BF16).astype(F32)


def _sigmoid(x):
    return 1.0 / (1.0 + jnp.exp(-x))


def _lanes(col, width):
    reps = width // LANES
    return col if reps == 1 else jnp.concatenate([col] * reps, axis=1)


def _fold(x):
    xi = lax.bitcast_convert_type(x, U32)
    tok = None
    for r in range(0, x.shape[0], 8):
        for c in range(0, x.shape[1] - LANES + 1, LANES):
            t = xi[r:r + 8, c:c + LANES]
            tok = t if tok is None else tok | t
    return tok


def _colsum(x, marks, nmarks):
    n = x.shape[0] // 8
    acc = x[0:8]
    for g in range(1, n):
        acc = acc + x[8 * g:8 * g + 8]
        if ((g + 1) * nmarks) % n == 0:
            marks.append(_fold(acc))
    return jnp.sum(acc, axis=0, keepdims=True)


def _tie_rows(lhs, toks, zero, lo, hi):
    if not toks:
        return lhs
    lu = pltpu.bitcast(lhs, U32)
    rows = [lu[8 * r:8 * r + 8] for r in range(lu.shape[0] // 8)]
    for i, tok in enumerate(toks):
        r = lo + ((i + 1) * (hi - lo)) // len(toks) - 1
        rows[r] = rows[r] | (tok & zero)
    return pltpu.bitcast(jnp.concatenate(rows, axis=0), BF16)


def _span(start, size):
    if isinstance(start, int):
        return pl.ds(start, size)
    return pl.ds(pl.multiple_of(start, LANES), size)


def _scope(name):
    return jax.named_scope(name) if SCOPES else contextlib.nullcontext()


def _kernel(xt_hbm, k_hbm, v_hbm, wq_hbm, wot_hbm, wr_ref, wg_hbm, wu_hbm, wdt_hbm,
            c_ref, wmod_hbm, o_hbm,
            xt_v, k_v, v_v, wq_v, wot_v, wmod_v, wg_v, wu_v, wdt_v, ot_v,
            h_scr, acc_scr, st_scr, m_scr, vt_scr, mod_scr, col_scr, key_scr, h2_scr, x1_scr,
            zero_scr,
            grp_sems, misc_sems, mlp_sems, out_sems, fix_sems,
            *, n_heads):
    d, seq = xt_v.shape
    sk = k_v.shape[1]
    n_grp = n_heads // HG
    n_blk = seq // TB
    n_units = n_grp * n_blk
    nb = TB // LANES
    nq = 2 * HG
    nt = sk // LANES
    gbits = n_grp.bit_length() - 1
    gw = nq * DH
    qscale = (DH ** -0.5) * math.log2(math.e)

    def grp_of(u):
        return u & (n_grp - 1)

    def blk_of(u):
        return u >> gbits

    def grp_copies(g):
        cs, hs = pl.ds(g * gw, gw), pl.ds(g * HG, HG)
        return (pltpu.make_async_copy(wq_hbm.at[:, cs], wq_v.at[g], grp_sems.at[0, g]),
                pltpu.make_async_copy(k_hbm.at[hs], k_v.at[hs], grp_sems.at[1, g]),
                pltpu.make_async_copy(v_hbm.at[hs], v_v.at[hs], grp_sems.at[2, g]),
                pltpu.make_async_copy(wot_hbm.at[:, cs], wot_v.at[g], grp_sems.at[3, g]))

    def col_copy(src, dst, lo, hi, sem):
        return pltpu.make_async_copy(src.at[:, lo:hi], dst.at[:, lo:hi], sem)

    x_first = col_copy(xt_hbm, xt_v, 0, TB, misc_sems.at[0])
    x_rest = col_copy(xt_hbm, xt_v, TB, seq, misc_sems.at[1])
    mod_first = col_copy(wmod_hbm, wmod_v, 0, 2 * d, misc_sems.at[2])
    mod_rest = col_copy(wmod_hbm, wmod_v, 2 * d, 6 * d, misc_sems.at[3])
    mlp_g = pltpu.make_async_copy(wg_hbm, wg_v, mlp_sems.at[0])
    mlp_u = pltpu.make_async_copy(wu_hbm, wu_v, mlp_sems.at[1])
    mlp_d = pltpu.make_async_copy(wdt_hbm, wdt_v, mlp_sems.at[2])
    out_lo = col_copy(ot_v, o_hbm, 0, seq - TB, out_sems.at[0])
    out_hi = col_copy(ot_v, o_hbm, seq - TB, seq, out_sems.at[1])

    def silu_c():
        cc = c_ref[...].astype(F32)
        return jnp.broadcast_to((cc * _rb(_sigmoid(cc))).astype(BF16), (8, d))

    def ln1_norm(t0, n, marks):
        x = xt_v[:, _span(t0, n)].astype(F32)
        mu = _colsum(x, marks, NM1) * (1.0 / d)
        xc = x - mu
        var = _colsum(xc * xc, marks, NM2) * (1.0 / d)
        return (xc * lax.rsqrt(var + EPS)).astype(BF16).T

    def ln1_mod(ln, slot, r0, marks):
        n = ln.shape[0]
        h = ln.astype(F32) * mod_scr[1:2, :] + mod_scr[0:1, :]
        h_scr[slot, _span(r0, n), :] = h.astype(BF16)
        step = max(n // NM3, 8)
        for r in range(step - 8, n, step):
            marks.append(_fold(h[r:r + 8]))

    def qproj(u):
        q = jnp.dot(h_scr[blk_of(u) & 1], wq_v[grp_of(u)], preferred_element_type=F32)
        return (q * qscale).astype(BF16)

    def qk(u, q, j, toks=(), zero=None):
        k = _tie_rows(k_v[grp_of(u) * HG + j // 2], toks, zero, TLO, sk // 16)
        st = lax.dot_general(k, q[:, j * DH:(j + 1) * DH], _NT,
                             preferred_element_type=F32)
        for i in range(nb):
            blk = st[:, i * LANES:(i + 1) * LANES]
            st_scr[j * nb + i] = blk
            m_scr[j * nb + i] = jnp.max(blk, axis=0, keepdims=True)

    def v_transpose(u, i, marks=None):
        vt = pltpu.bitcast(v_v[grp_of(u) * HG + i].T, U32)
        vt_scr[i] = vt
        if marks is not None:
            step = sk // NVT
            for c in range(step - LANES, sk, step):
                marks.append(vt[DH // 2 - 8:DH // 2, c:c + LANES])

    def pv(slots, zero, toks=()):
        ps, ls, pairs = [], [], []
        for sl in slots:
            p = jnp.exp2(st_scr[sl] - m_scr[sl])
            accs = [None] * 4
            for tile in range(nt):
                for r0 in range(tile * LANES + LANES - 16, tile * LANES - 16, -16):
                    pair = p[r0:r0 + 8] + p[r0 + 8:r0 + 16]
                    pairs.append(pair)
                    a = accs[tile % 4]
                    accs[tile % 4] = pair if a is None else a + pair
            ls.append(jnp.sum((accs[0] + accs[1]) + (accs[2] + accs[3]), axis=0, keepdims=True))
            ps.append(p.astype(BF16))
        outs = []
        ntiles = len(slots) * nt
        side = {}
        for i, tok in enumerate(toks):
            side.setdefault(((i + 1) * ntiles) // len(toks) - 1, []).append(tok)
        for i, sl in enumerate(slots):
            vu = vt_scr[sl // (2 * nb)]
            tiles = []
            for c in range(nt):
                g = i * nt + c + 4
                rows = []
                for r in range(8):
                    x = vu[8 * r:8 * r + 8, c * LANES:(c + 1) * LANES]
                    if g < ntiles and TIE0 <= r < TIE0 + NTIE:
                        src = pairs[g * 8 + (r - TIE0)]
                        x = x | (lax.bitcast_convert_type(src, U32) & zero)
                    if r == SIDE_ROW:
                        for tok in side.get(i * nt + c, ()):
                            x = x | (tok & zero)
                    rows.append(x)
                tiles.append(jnp.concatenate(rows, axis=0))
            lhs = pltpu.bitcast(jnp.concatenate(tiles, axis=1), BF16)
            o = jnp.dot(lhs, ps[i], preferred_element_type=F32)
            outs.append((o * (1.0 / ls[i])).astype(BF16))
        return outs

    def outproj(u, o, lo=0):
        w = len(o) // nq
        o2 = jnp.concatenate(
            [jnp.concatenate(o[j * w:(j + 1) * w], axis=1) for j in range(nq)], axis=0)
        contrib = jnp.dot(wot_v[grp_of(u)], o2, preferred_element_type=F32)
        hi = lo + w * LANES
        slot = blk_of(u) & 1
        old = jnp.where(grp_of(u) > 0, acc_scr[slot, :, lo:hi], 0.0)
        acc_scr[slot, :, lo:hi] = old + contrib

    def finalize(t0, slot, a0, dst, n):
        marks = []
        cs = _span(dst, n)
        x = xt_v[:, _span(t0, n)].astype(F32)
        att = acc_scr[slot, :, _span(a0, n)]
        x1b = (x + _lanes(col_scr[0], n) * att).astype(BF16)
        x1_scr[:, cs] = x1b
        ot_v[:, cs] = x1b
        mu = _colsum(x1b.astype(F32), marks, NF1) * (1.0 / d)
        mub = _rb(mu)
        xc = x1_scr[:, cs].astype(F32) - mub
        var = _colsum(xc * xc, marks, NF2) * (1.0 / d) - (mu - mub) * (mu - mub)
        inv = 1.0 / _rb(jnp.sqrt(_rb(_rb(jnp.maximum(var, 0.0)) + EPS)))
        step = d // NF3
        racc = None
        for r0 in range(0, d, step):
            rs = slice(r0, r0 + step)
            x1 = ot_v[rs, cs].astype(F32)
            h2b = ((x1 - mub) * inv * _lanes(col_scr[2, rs, :], n)
                   + _lanes(col_scr[1, rs, :], n)).astype(BF16)
            h2_scr[rs, cs] = h2b
            h2 = h2b.astype(F32)
            out = x1 + _lanes(col_scr[3, rs, :], n) * h2
            ot_v[rs, cs] = out.astype(BF16)
            rp = h2 * _lanes(col_scr[4, rs, :], n)
            for g in range(0, step, 8):
                racc = rp[g:g + 8] if racc is None else racc + rp[g:g + 8]
            marks.append(_fold(racc) | _fold(out))
        r = _rb(jnp.sum(racc, axis=0, keepdims=True)) + 0.0
        bits = lax.bitcast_convert_type(r, I32) >> 16
        order = jnp.where(bits < 0, -1 - bits, bits + 32768)
        pos = t0 + lax.broadcasted_iota(I32, (1, n), 1)
        key = lax.bitcast_convert_type((order << 11) + (seq - 1 - pos) + 0x20000000, F32)
        for i in range(n // LANES):
            key_scr[pl.ds(dst // LANES + i, 1), :] = key[:, i * LANES:(i + 1) * LANES]
        return marks

    wq0, k0, v0, wo0 = grp_copies(0)
    x_first.start()
    mod_first.start()
    wq0.start()
    k0.start(priority=1)
    cbits = lax.bitcast_convert_type(c_ref[:, 0:LANES].astype(F32), U32)
    zero_scr[...] = jnp.broadcast_to(cbits & 0xFFFF, (8, LANES))
    acc_scr[...] = jnp.zeros(acc_scr.shape, F32)
    col_scr[...] = jnp.zeros(col_scr.shape, F32)
    with _scope("w_x"):
        x_first.wait()
    h_scr[0] = ln1_norm(0, TB, [])
    with _scope("w_wmod"):
        mod_first.wait()
        wq0.wait()
    v0.start(priority=1)
    x_rest.start(priority=1)
    mod = _rb(jnp.dot(silu_c(), wmod_v[:, 0:2 * d], preferred_element_type=F32))
    mod_scr[0:1, :] = mod[0:1, 0:d]
    mod_scr[1:2, :] = _rb(1.0 + mod[0:1, d:2 * d])
    ln1_mod(h_scr[0], 0, 0, [])
    q = qproj(0)
    with _scope("w_k"):
        k0.wait()
        v0.wait()
    wo0.start()
    for cp in grp_copies(1):
        cp.start()
    with _scope("qk0"):
        zero = zero_scr[...]
        for j in range(nq):
            marks = []
            if j >= nq - HG:
                v_transpose(0, j - (nq - HG), marks)
            qk(0, q, j, marks, zero)

    loads = [[2, 3], [4, 5], [6, 7]]
    assert n_grp == 8 and HG == 2
    npc = TB // SP

    def steady(u, carry):
        @pl.when(u <= 5)
        def _():
            @pl.when(u == 1)
            def _():
                x_rest.wait()
                wo0.wait()
                for cp in grp_copies(1):
                    cp.wait()

            for i in range(len(loads) + 1):
                @pl.when(u == i + 1)
                def _():
                    if i > 0:
                        for g in loads[i - 1]:
                            for cp in grp_copies(g):
                                cp.wait()
                    if i < len(loads):
                        for g in loads[i]:
                            for cp in grp_copies(g):
                                cp.start()
                    else:
                        mod_rest.start()

            @pl.when(u == 5)
            def _():
                mod_rest.wait()
                mlp_g.start()
                mlp_u.start()
                mlp_d.start()
                mod = _rb(jnp.dot(silu_c(), wmod_v[:, 2 * d:6 * d], preferred_element_type=F32))
                for j in range(4):
                    piece = mod[0:1, j * d:(j + 1) * d]
                    if j == 2:
                        piece = _rb(1.0 + piece)
                    col_scr[j] = jnp.broadcast_to(piece, (LANES, d)).T
                wr = wr_ref[...].reshape(1, d).astype(F32)
                col_scr[4] = jnp.broadcast_to(wr, (LANES, d)).T

        with _scope("body"):
            zero = zero_scr[...]
            blk, g = blk_of(u), grp_of(u)
            off = ((g - 1) & (npc - 1)) * SP
            q = qproj(u)
            o = pv(range(0, 2 * nb), zero)
            live = jnp.logical_and(blk > 0, jnp.logical_and(g >= 1, g <= npc))
            t0 = jnp.maximum(blk - 1, 0) * TB + off
            qk(u, q, 0, finalize(t0, (blk + 1) & 1, off, jnp.where(live, t0, seq), SP), zero)
            marks = []
            ln = ln1_norm(jnp.minimum(blk + 1, n_blk - 1) * TB + off, SP, marks)
            ln1_mod(ln, (blk + 1) & 1, off, marks)
            qk(u, q, 1, marks, zero)
            o += pv(range(2 * nb, 4 * nb), zero)
            outproj(u - 1, o)
            marks = []
            v_transpose(u, 0, marks)
            qk(u, q, 2, marks, zero)
            marks = []
            v_transpose(u, 1, marks)
            qk(u, q, 3, marks, zero)
        return carry

    lax.fori_loop(1, n_units, steady, 0)

    ul = n_units - 1
    tl = seq - TB
    sl_last = (n_blk - 1) & 1
    nb0 = nb - TAILB
    out_lo.start()
    mlp_g.wait()
    mlp_u.wait()
    with _scope("e_pva"):
        outproj(ul, pv([j * nb + i for j in range(nq) for i in range(nb0)], zero_scr[...]))
    mlp_d.wait()
    with _scope("e_pvb"):
        toks = finalize(tl, sl_last, 0, tl, nb0 * LANES)
        o = pv([j * nb + i for j in range(nq) for i in range(nb0, nb)], zero_scr[...], toks)
        outproj(ul, o, nb0 * LANES)
        finalize(tl + nb0 * LANES, sl_last, nb0 * LANES, tl + nb0 * LANES, TAILB * LANES)

    keys = key_scr[0:seq // LANES, :]
    sub8 = lax.broadcasted_iota(I32, (TOPC, 1), 0)
    lane = lax.broadcasted_iota(I32, (TOPC, LANES), 1)
    top = jnp.zeros((TOPC, 1), F32)
    bases = []
    xs = jnp.zeros((TOPC, d), F32)
    for i in range(TOPC):
        mx = jnp.max(jnp.max(keys, axis=0, keepdims=True), axis=1, keepdims=True)
        keys = jnp.where(keys == mx, 0.0, keys)
        top = jnp.where(sub8 == i, mx, top)
        idx = seq - 1 - (lax.bitcast_convert_type(mx, I32) & (seq - 1))
        bases.append(pl.multiple_of(idx[0, 0] & ~(LANES - 1), LANES))
        pick = jnp.logical_and(sub8 == i, lane == (idx & (LANES - 1)))
        pick = jnp.where(pick, 1.0, 0.0).astype(BF16)
        xs = xs + lax.dot_general(pick, h2_scr[:, pl.ds(bases[i], LANES)], _NT,
                                  preferred_element_type=F32)
    kb = lax.bitcast_convert_type(top, I32)
    idx_col = seq - 1 - (kb & (seq - 1))
    order = (kb >> 11) & 0xFFFF
    rbits = jnp.where(order >= 32768, order - 32768, -1 - order) << 16
    r_sel = lax.bitcast_convert_type(rbits, F32)
    xs = xs.astype(BF16)
    out_hi.start()
    g = _rb(jnp.dot(xs, wg_v[...], preferred_element_type=F32))
    g = _rb(g * _rb(_sigmoid(g)))
    u = _rb(jnp.dot(xs, wu_v[...], preferred_element_type=F32))
    y = _rb(lax.dot_general((g * u).astype(BF16), wdt_v[...], _NT,
                            preferred_element_type=F32))
    y = _rb(y * _rb(_sigmoid(r_sel)))
    ypad = jnp.concatenate([y, jnp.zeros((LANES - TOPC, d), F32)], axis=0)
    yt = ypad.T.astype(BF16)
    idx_big = jnp.concatenate([idx_col, jnp.full((LANES - TOPC, 1), -1, I32)], axis=0)
    lane2 = lax.broadcasted_iota(I32, (LANES, LANES), 1)
    out_lo.wait()
    out_hi.wait()
    for i in range(TOPC):
        place = jnp.where(lane2 + bases[i] == idx_big, 1.0, 0.0).astype(BF16)
        upd = jnp.dot(yt, place, preferred_element_type=F32)
        sl = pl.ds(bases[i], LANES)
        hm = _rb(h2_scr[:, sl].astype(F32) + upd)
        ot_v[:, sl] = (x1_scr[:, sl].astype(F32) + col_scr[3] * hm).astype(BF16)

    def fix_copy(i):
        sl = pl.ds(bases[i], LANES)
        return pltpu.make_async_copy(ot_v.at[:, sl], o_hbm.at[:, sl], fix_sems.at[i])

    fresh = []
    for i in range(TOPC):
        ok = True
        for j in range(i):
            ok = jnp.logical_and(ok, bases[i] != bases[j])
        fresh.append(ok)
    fix_copy(0).start()
    for i in range(1, TOPC):
        pl.when(fresh[i])(lambda i=i: fix_copy(i).start())
    with _scope("w_fix"):
        fix_copy(0).wait()
        for i in range(1, TOPC):
            pl.when(fresh[i])(lambda i=i: fix_copy(i).wait())


@jax.jit
def pallas_adaLN_cond__gqa_block_cached__moe_arch_mod__prompt_kernel(
    A_x: jax.Array,
    A_k_cache: jax.Array,
    A_v_cache: jax.Array,
    A_wq: jax.Array,
    A_wo: jax.Array,
    B_x: jax.Array,
    B_w_r: jax.Array,
    B_w_gate: jax.Array,
    B_w_up: jax.Array,
    B_w_down: jax.Array,
    c: jax.Array,
    w_mod: jax.Array,
):
    b, seq, d = A_x.shape
    _, hkv, sk, dh = A_k_cache.shape
    assert b == 1 and dh == DH and HQ == 2 * hkv
    assert seq & (seq - 1) == 0 and seq <= 2048
    f = B_w_gate.shape[1]
    n_grp = hkv // HG
    gw = 2 * HG * dh
    n_slots = 2 * HG * TB // LANES

    xt = A_x.reshape(seq, d).T
    wot = A_wo.T
    wdt = B_w_down.T
    k3 = A_k_cache.reshape(hkv, sk, dh)
    v3 = A_v_cache.reshape(hkv, sk, dh)

    vmem = pl.BlockSpec(memory_space=pltpu.VMEM)
    hbm = pl.BlockSpec(memory_space=pl.ANY)
    out_t = pl.pallas_call(
        functools.partial(_kernel, n_heads=hkv),
        in_specs=[hbm, hbm, hbm, hbm, hbm, vmem, hbm, hbm, hbm, vmem, hbm],
        out_specs=hbm,
        out_shape=jax.ShapeDtypeStruct((d, seq), BF16),
        scratch_shapes=[
            pltpu.VMEM((d, seq), BF16),
            pltpu.VMEM((hkv, sk, dh), BF16),
            pltpu.VMEM((hkv, sk, dh), BF16),
            pltpu.VMEM((n_grp, d, gw), BF16),
            pltpu.VMEM((n_grp, d, gw), BF16),
            pltpu.VMEM((d, 6 * d), BF16),
            pltpu.VMEM((d, f), BF16),
            pltpu.VMEM((d, f), BF16),
            pltpu.VMEM((d, f), BF16),
            pltpu.VMEM((d, seq + SP), BF16),
            pltpu.VMEM((2, TB, d), BF16),
            pltpu.VMEM((2, d, TB), F32),
            pltpu.VMEM((n_slots, sk, LANES), F32),
            pltpu.VMEM((n_slots, 1, LANES), F32),
            pltpu.VMEM((HG, dh // 2, sk), U32),
            pltpu.VMEM((8, d), F32),
            pltpu.VMEM((5, d, LANES), F32),
            pltpu.VMEM(((seq + SP) // LANES + 7 & ~7, LANES), F32),
            pltpu.VMEM((d, seq + SP), BF16),
            pltpu.VMEM((d, seq + SP), BF16),
            pltpu.VMEM((8, LANES), U32),
            pltpu.SemaphoreType.DMA((4, n_grp)),
            pltpu.SemaphoreType.DMA((4,)),
            pltpu.SemaphoreType.DMA((3,)),
            pltpu.SemaphoreType.DMA((2,)),
            pltpu.SemaphoreType.DMA((TOPC,)),
        ],
        compiler_params=pltpu.CompilerParams(
            disable_bounds_checks=True,
            disable_semaphore_checks=True,
            vmem_limit_bytes=110 * 1024 * 1024,
        ),
    )(xt, k3, v3, A_wq, wot, B_w_r, B_w_gate, B_w_up, wdt, c, w_mod)
    return out_t.T.reshape(b, seq, d)
```

```python
import contextlib
import functools
import math
import os

import jax
import jax.numpy as jnp
from jax import lax
import jax.experimental.pallas as pl
import jax.experimental.pallas.tpu as pltpu

F32 = jnp.float32
BF16 = jnp.bfloat16
I32 = jnp.int32
U32 = jnp.uint32

HQ = 32
DH = 128
TOPC = 8
EPS = 1e-05
LANES = 128

TB = 512
HG = 2
TIE0 = int(os.environ.get("KP_TIE0", "2"))
NTIE = int(os.environ.get("KP_NTIE", "3"))
SP = int(os.environ.get("KP_SP", "128"))
NM1 = int(os.environ.get("KP_NM1", "8"))
NM2 = int(os.environ.get("KP_NM2", "12"))
NM3 = int(os.environ.get("KP_NM3", "16"))
TLO = int(os.environ.get("KP_TLO", "8"))
NF1 = int(os.environ.get("KP_NF1", "9"))
NF2 = int(os.environ.get("KP_NF2", "6"))
NF3 = int(os.environ.get("KP_NF3", "18"))
NVT = int(os.environ.get("KP_NVT", "16"))
TAILB = int(os.environ.get("KP_TAILB", "2"))
SIDE_ROW = int(os.environ.get("KP_SIDE_ROW", "1"))
SCOPES = os.environ.get("KP_SCOPES", "") == "1"

_NT = (((1,), (1,)), ((), ()))


def _rb(x):
    return x.astype(BF16).astype(F32)


def _sigmoid(x):
    return 1.0 / (1.0 + jnp.exp(-x))


def _lanes(col, width):
    reps = width // LANES
    return col if reps == 1 else jnp.concatenate([col] * reps, axis=1)


def _fold(x):
    xi = lax.bitcast_convert_type(x, U32)
    tok = None
    for r in range(0, x.shape[0], 8):
        for c in range(0, x.shape[1] - LANES + 1, LANES):
            t = xi[r:r + 8, c:c + LANES]
            tok = t if tok is None else tok | t
    return tok


def _colsum(x, marks, nmarks):
    n = x.shape[0] // 8
    acc = x[0:8]
    for g in range(1, n):
        acc = acc + x[8 * g:8 * g + 8]
        if ((g + 1) * nmarks) % n == 0:
            marks.append(_fold(acc))
    return jnp.sum(acc, axis=0, keepdims=True)


def _tie_rows(lhs, toks, zero, lo, hi):
    if not toks:
        return lhs
    lu = pltpu.bitcast(lhs, U32)
    rows = [lu[8 * r:8 * r + 8] for r in range(lu.shape[0] // 8)]
    for i, tok in enumerate(toks):
        r = lo + ((i + 1) * (hi - lo)) // len(toks) - 1
        rows[r] = rows[r] | (tok & zero)
    return pltpu.bitcast(jnp.concatenate(rows, axis=0), BF16)


def _span(start, size):
    if isinstance(start, int):
        return pl.ds(start, size)
    return pl.ds(pl.multiple_of(start, LANES), size)


def _scope(name):
    return jax.named_scope(name) if SCOPES else contextlib.nullcontext()


def _kernel(xt_hbm, k_hbm, v_hbm, wq_hbm, wot_hbm, wr_ref, wg_hbm, wu_hbm, wdt_hbm,
            c_ref, wmod_hbm, o_hbm,
            xt_v, k_v, v_v, wq_v, wot_v, wmod_v, wg_v, wu_v, wdt_v, ot_v,
            h_scr, acc_scr, st_scr, m_scr, vt_scr, mod_scr, col_scr, key_scr, h2_scr, x1_scr,
            zero_scr,
            grp_sems, misc_sems, mlp_sems, out_sems, fix_sems,
            *, n_heads):
    d, seq = xt_v.shape
    sk = k_v.shape[1]
    n_grp = n_heads // HG
    n_blk = seq // TB
    n_units = n_grp * n_blk
    nb = TB // LANES
    nq = 2 * HG
    nt = sk // LANES
    gbits = n_grp.bit_length() - 1
    gw = nq * DH
    qscale = (DH ** -0.5) * math.log2(math.e)

    def grp_of(u):
        return u & (n_grp - 1)

    def blk_of(u):
        return u >> gbits

    def grp_copies(g):
        cs, hs = pl.ds(g * gw, gw), pl.ds(g * HG, HG)
        return (pltpu.make_async_copy(wq_hbm.at[:, cs], wq_v.at[g], grp_sems.at[0, g]),
                pltpu.make_async_copy(k_hbm.at[hs], k_v.at[hs], grp_sems.at[1, g]),
                pltpu.make_async_copy(v_hbm.at[hs], v_v.at[hs], grp_sems.at[2, g]),
                pltpu.make_async_copy(wot_hbm.at[:, cs], wot_v.at[g], grp_sems.at[3, g]))

    def col_copy(src, dst, lo, hi, sem):
        return pltpu.make_async_copy(src.at[:, lo:hi], dst.at[:, lo:hi], sem)

    x_first = col_copy(xt_hbm, xt_v, 0, TB, misc_sems.at[0])
    x_rest = col_copy(xt_hbm, xt_v, TB, seq, misc_sems.at[1])
    mod_first = col_copy(wmod_hbm, wmod_v, 0, 2 * d, misc_sems.at[2])
    mod_rest = col_copy(wmod_hbm, wmod_v, 2 * d, 6 * d, misc_sems.at[3])
    mlp_g = pltpu.make_async_copy(wg_hbm, wg_v, mlp_sems.at[0])
    mlp_u = pltpu.make_async_copy(wu_hbm, wu_v, mlp_sems.at[1])
    mlp_d = pltpu.make_async_copy(wdt_hbm, wdt_v, mlp_sems.at[2])
    out_lo = col_copy(ot_v, o_hbm, 0, seq - TB, out_sems.at[0])
    out_hi = col_copy(ot_v, o_hbm, seq - TB, seq, out_sems.at[1])

    def silu_c():
        cc = c_ref[...].astype(F32)
        return jnp.broadcast_to((cc * _rb(_sigmoid(cc))).astype(BF16), (8, d))

    def ln1_norm(t0, n, marks):
        x = xt_v[:, _span(t0, n)].astype(F32)
        mu = _colsum(x, marks, NM1) * (1.0 / d)
        xc = x - mu
        var = _colsum(xc * xc, marks, NM2) * (1.0 / d)
        return (xc * lax.rsqrt(var + EPS)).astype(BF16).T

    def ln1_mod(ln, slot, r0, marks):
        n = ln.shape[0]
        h = ln.astype(F32) * mod_scr[1:2, :] + mod_scr[0:1, :]
        h_scr[slot, _span(r0, n), :] = h.astype(BF16)
        step = max(n // NM3, 8)
        for r in range(step - 8, n, step):
            marks.append(_fold(h[r:r + 8]))

    def qproj(u):
        q = jnp.dot(h_scr[blk_of(u) & 1], wq_v[grp_of(u)], preferred_element_type=F32)
        return (q * qscale).astype(BF16)

    def qk(u, q, j, toks=(), zero=None):
        k = _tie_rows(k_v[grp_of(u) * HG + j // 2], toks, zero, TLO, sk // 16)
        st = lax.dot_general(k, q[:, j * DH:(j + 1) * DH], _NT,
                             preferred_element_type=F32)
        for i in range(nb):
            blk = st[:, i * LANES:(i + 1) * LANES]
            st_scr[j * nb + i] = blk
            m_scr[j * nb + i] = jnp.max(blk, axis=0, keepdims=True)

    def v_transpose(u, i, marks=None):
        vt = pltpu.bitcast(v_v[grp_of(u) * HG + i].T, U32)
        vt_scr[i] = vt
        if marks is not None:
            step = sk // NVT
            for c in range(step - LANES, sk, step):
                marks.append(vt[DH // 2 - 8:DH // 2, c:c + LANES])

    def pv(slots, zero, toks=()):
        ps, ls, pairs = [], [], []
        for sl in slots:
            p = jnp.exp2(st_scr[sl] - m_scr[sl])
            accs = [None] * 4
            for tile in range(nt):
                for r0 in range(tile * LANES + LANES - 16, tile * LANES - 16, -16):
                    pair = p[r0:r0 + 8] + p[r0 + 8:r0 + 16]
                    pairs.append(pair)
                    a = accs[tile % 4]
                    accs[tile % 4] = pair if a is None else a + pair
            ls.append(jnp.sum((accs[0] + accs[1]) + (accs[2] + accs[3]), axis=0, keepdims=True))
            ps.append(p.astype(BF16))
        outs = []
        ntiles = len(slots) * nt
        side = {}
        for i, tok in enumerate(toks):
            side.setdefault(((i + 1) * ntiles) // len(toks) - 1, []).append(tok)
        for i, sl in enumerate(slots):
            vu = vt_scr[sl // (2 * nb)]
            tiles = []
            for c in range(nt):
                g = i * nt + c + 4
                rows = []
                for r in range(8):
                    x = vu[8 * r:8 * r + 8, c * LANES:(c + 1) * LANES]
                    if g < ntiles and TIE0 <= r < TIE0 + NTIE:
                        src = pairs[g * 8 + (r - TIE0)]
                        x = x | (lax.bitcast_convert_type(src, U32) & zero)
                    if r == SIDE_ROW:
                        for tok in side.get(i * nt + c, ()):
                            x = x | (tok & zero)
                    rows.append(x)
                tiles.append(jnp.concatenate(rows, axis=0))
            lhs = pltpu.bitcast(jnp.concatenate(tiles, axis=1), BF16)
            o = jnp.dot(lhs, ps[i], preferred_element_type=F32)
            outs.append((o * (1.0 / ls[i])).astype(BF16))
        return outs

    def outproj(u, o, lo=0):
        w = len(o) // nq
        o2 = jnp.concatenate(
            [jnp.concatenate(o[j * w:(j + 1) * w], axis=1) for j in range(nq)], axis=0)
        contrib = jnp.dot(wot_v[grp_of(u)], o2, preferred_element_type=F32)
        hi = lo + w * LANES
        slot = blk_of(u) & 1
        old = jnp.where(grp_of(u) > 0, acc_scr[slot, :, lo:hi], 0.0)
        acc_scr[slot, :, lo:hi] = old + contrib

    def finalize(t0, slot, a0, dst, n):
        marks = []
        cs = _span(dst, n)
        x = xt_v[:, _span(t0, n)].astype(F32)
        att = acc_scr[slot, :, _span(a0, n)]
        x1b = (x + _lanes(col_scr[0], n) * att).astype(BF16)
        x1_scr[:, cs] = x1b
        ot_v[:, cs] = x1b
        mu = _colsum(x1b.astype(F32), marks, NF1) * (1.0 / d)
        mub = _rb(mu)
        xc = x1_scr[:, cs].astype(F32) - mub
        var = _colsum(xc * xc, marks, NF2) * (1.0 / d) - (mu - mub) * (mu - mub)
        inv = 1.0 / _rb(jnp.sqrt(_rb(_rb(jnp.maximum(var, 0.0)) + EPS)))
        step = d // NF3
        racc = None
        for r0 in range(0, d, step):
            rs = slice(r0, r0 + step)
            x1 = ot_v[rs, cs].astype(F32)
            h2b = ((x1 - mub) * inv * _lanes(col_scr[2, rs, :], n)
                   + _lanes(col_scr[1, rs, :], n)).astype(BF16)
            h2_scr[rs, cs] = h2b
            h2 = h2b.astype(F32)
            out = x1 + _lanes(col_scr[3, rs, :], n) * h2
            ot_v[rs, cs] = out.astype(BF16)
            rp = h2 * _lanes(col_scr[4, rs, :], n)
            for g in range(0, step, 8):
                racc = rp[g:g + 8] if racc is None else racc + rp[g:g + 8]
            marks.append(_fold(racc) | _fold(out))
        r = _rb(jnp.sum(racc, axis=0, keepdims=True)) + 0.0
        bits = lax.bitcast_convert_type(r, I32) >> 16
        order = jnp.where(bits < 0, -1 - bits, bits + 32768)
        pos = t0 + lax.broadcasted_iota(I32, (1, n), 1)
        key = lax.bitcast_convert_type((order << 11) + (seq - 1 - pos) + 0x20000000, F32)
        for i in range(n // LANES):
            key_scr[pl.ds(dst // LANES + i, 1), :] = key[:, i * LANES:(i + 1) * LANES]
        return marks

    wq0, k0, v0, wo0 = grp_copies(0)
    wq1, k1, v1, wo1 = grp_copies(1)
    x_first.start()
    mod_first.start()
    wq0.start()
    k0.start(priority=1)
    cbits = lax.bitcast_convert_type(c_ref[:, 0:LANES].astype(F32), U32)
    zero_scr[...] = jnp.broadcast_to(cbits & 0xFFFF, (8, LANES))
    acc_scr[...] = jnp.zeros(acc_scr.shape, F32)
    col_scr[...] = jnp.zeros(col_scr.shape, F32)
    with _scope("w_x"):
        x_first.wait()
    h_scr[0] = ln1_norm(0, TB, [])
    with _scope("w_wmod"):
        mod_first.wait()
        wq0.wait()
    v0.start()
    wq1.start(priority=1)
    k1.start(priority=1)
    mod = _rb(jnp.dot(silu_c(), wmod_v[:, 0:2 * d], preferred_element_type=F32))
    mod_scr[0:1, :] = mod[0:1, 0:d]
    mod_scr[1:2, :] = _rb(1.0 + mod[0:1, d:2 * d])
    ln1_mod(h_scr[0], 0, 0, [])
    q = qproj(0)
    with _scope("w_k"):
        k0.wait()
        v0.wait()
    v1.start()
    wo0.start()
    with _scope("qk0"):
        zero = zero_scr[...]
        for j in range(nq):
            marks = []
            if j >= nq - HG:
                v_transpose(0, j - (nq - HG), marks)
            qk(0, q, j, marks, zero)

    assert n_grp == 8 and HG == 2
    loads = [[wq1, k1, v1, wo0],
             [wo1, *grp_copies(2), x_rest],
             [*grp_copies(3), *grp_copies(4)],
             [*grp_copies(5), *grp_copies(6)],
             [*grp_copies(7), mod_rest]]
    npc = TB // SP

    def steady(u, carry):
        @pl.when(u <= 5)
        def _():
            for i in range(1, len(loads)):
                @pl.when(u == i)
                def _():
                    for cp in loads[i - 1]:
                        cp.wait()
                    for cp in loads[i]:
                        cp.start()

            @pl.when(u == 5)
            def _():
                for cp in loads[-1]:
                    cp.wait()
                mlp_g.start()
                mlp_u.start()
                mlp_d.start()
                mod = _rb(jnp.dot(silu_c(), wmod_v[:, 2 * d:6 * d], preferred_element_type=F32))
                for j in range(4):
                    piece = mod[0:1, j * d:(j + 1) * d]
                    if j == 2:
                        piece = _rb(1.0 + piece)
                    col_scr[j] = jnp.broadcast_to(piece, (LANES, d)).T
                wr = wr_ref[...].reshape(1, d).astype(F32)
                col_scr[4] = jnp.broadcast_to(wr, (LANES, d)).T

        with _scope("body"):
            zero = zero_scr[...]
            blk, g = blk_of(u), grp_of(u)
            off = ((g - 1) & (npc - 1)) * SP
            q = qproj(u)
            o = pv(range(0, 2 * nb), zero)
            live = jnp.logical_and(blk > 0, jnp.logical_and(g >= 1, g <= npc))
            t0 = jnp.maximum(blk - 1, 0) * TB + off
            qk(u, q, 0, finalize(t0, (blk + 1) & 1, off, jnp.where(live, t0, seq), SP), zero)
            marks = []
            nxt = jnp.where(u >= 2, jnp.minimum(blk + 1, n_blk - 1), 0)
            ln = ln1_norm(nxt * TB + off, SP, marks)
            ln1_mod(ln, (blk + 1) & 1, off, marks)
            qk(u, q, 1, marks, zero)
            o += pv(range(2 * nb, 4 * nb), zero)
            outproj(u - 1, o)
            marks = []
            v_transpose(u, 0, marks)
            qk(u, q, 2, marks, zero)
            marks = []
            v_transpose(u, 1, marks)
            qk(u, q, 3, marks, zero)
        return carry

    lax.fori_loop(1, n_units, steady, 0)

    ul = n_units - 1
    tl = seq - TB
    sl_last = (n_blk - 1) & 1
    nb0 = nb - TAILB
    out_lo.start()
    mlp_g.wait()
    mlp_u.wait()
    with _scope("e_pva"):
        outproj(ul, pv([j * nb + i for j in range(nq) for i in range(nb0)], zero_scr[...]))
    mlp_d.wait()
    with _scope("e_pvb"):
        toks = finalize(tl, sl_last, 0, tl, nb0 * LANES)
        o = pv([j * nb + i for j in range(nq) for i in range(nb0, nb)], zero_scr[...], toks)
        outproj(ul, o, nb0 * LANES)
        finalize(tl + nb0 * LANES, sl_last, nb0 * LANES, tl + nb0 * LANES, TAILB * LANES)

    keys = key_scr[0:seq // LANES, :]
    sub8 = lax.broadcasted_iota(I32, (TOPC, 1), 0)
    lane = lax.broadcasted_iota(I32, (TOPC, LANES), 1)
    top = jnp.zeros((TOPC, 1), F32)
    bases = []
    xs = jnp.zeros((TOPC, d), F32)
    for i in range(TOPC):
        mx = jnp.max(jnp.max(keys, axis=0, keepdims=True), axis=1, keepdims=True)
        keys = jnp.where(keys == mx, 0.0, keys)
        top = jnp.where(sub8 == i, mx, top)
        idx = seq - 1 - (lax.bitcast_convert_type(mx, I32) & (seq - 1))
        bases.append(pl.multiple_of(idx[0, 0] & ~(LANES - 1), LANES))
        pick = jnp.logical_and(sub8 == i, lane == (idx & (LANES - 1)))
        pick = jnp.where(pick, 1.0, 0.0).astype(BF16)
        xs = xs + lax.dot_general(pick, h2_scr[:, pl.ds(bases[i], LANES)], _NT,
                                  preferred_element_type=F32)
    kb = lax.bitcast_convert_type(top, I32)
    idx_col = seq - 1 - (kb & (seq - 1))
    order = (kb >> 11) & 0xFFFF
    rbits = jnp.where(order >= 32768, order - 32768, -1 - order) << 16
    r_sel = lax.bitcast_convert_type(rbits, F32)
    xs = xs.astype(BF16)
    out_hi.start()
    g = _rb(jnp.dot(xs, wg_v[...], preferred_element_type=F32))
    g = _rb(g * _rb(_sigmoid(g)))
    u = _rb(jnp.dot(xs, wu_v[...], preferred_element_type=F32))
    y = _rb(lax.dot_general((g * u).astype(BF16), wdt_v[...], _NT,
                            preferred_element_type=F32))
    y = _rb(y * _rb(_sigmoid(r_sel)))
    ypad = jnp.concatenate([y, jnp.zeros((LANES - TOPC, d), F32)], axis=0)
    yt = ypad.T.astype(BF16)
    idx_big = jnp.concatenate([idx_col, jnp.full((LANES - TOPC, 1), -1, I32)], axis=0)
    lane2 = lax.broadcasted_iota(I32, (LANES, LANES), 1)
    out_lo.wait()
    out_hi.wait()
    for i in range(TOPC):
        place = jnp.where(lane2 + bases[i] == idx_big, 1.0, 0.0).astype(BF16)
        upd = jnp.dot(yt, place, preferred_element_type=F32)
        sl = pl.ds(bases[i], LANES)
        hm = _rb(h2_scr[:, sl].astype(F32) + upd)
        ot_v[:, sl] = (x1_scr[:, sl].astype(F32) + col_scr[3] * hm).astype(BF16)

    def fix_copy(i):
        sl = pl.ds(bases[i], LANES)
        return pltpu.make_async_copy(ot_v.at[:, sl], o_hbm.at[:, sl], fix_sems.at[i])

    fresh = []
    for i in range(TOPC):
        ok = True
        for j in range(i):
            ok = jnp.logical_and(ok, bases[i] != bases[j])
        fresh.append(ok)
    fix_copy(0).start()
    for i in range(1, TOPC):
        pl.when(fresh[i])(lambda i=i: fix_copy(i).start())
    with _scope("w_fix"):
        fix_copy(0).wait()
        for i in range(1, TOPC):
            pl.when(fresh[i])(lambda i=i: fix_copy(i).wait())


@jax.jit
def pallas_adaLN_cond__gqa_block_cached__moe_arch_mod__prompt_kernel(
    A_x: jax.Array,
    A_k_cache: jax.Array,
    A_v_cache: jax.Array,
    A_wq: jax.Array,
    A_wo: jax.Array,
    B_x: jax.Array,
    B_w_r: jax.Array,
    B_w_gate: jax.Array,
    B_w_up: jax.Array,
    B_w_down: jax.Array,
    c: jax.Array,
    w_mod: jax.Array,
):
    b, seq, d = A_x.shape
    _, hkv, sk, dh = A_k_cache.shape
    assert b == 1 and dh == DH and HQ == 2 * hkv
    assert seq & (seq - 1) == 0 and seq <= 2048
    f = B_w_gate.shape[1]
    n_grp = hkv // HG
    gw = 2 * HG * dh
    n_slots = 2 * HG * TB // LANES

    xt = A_x.reshape(seq, d).T
    wot = A_wo.T
    wdt = B_w_down.T
    k3 = A_k_cache.reshape(hkv, sk, dh)
    v3 = A_v_cache.reshape(hkv, sk, dh)

    vmem = pl.BlockSpec(memory_space=pltpu.VMEM)
    hbm = pl.BlockSpec(memory_space=pl.ANY)
    out_t = pl.pallas_call(
        functools.partial(_kernel, n_heads=hkv),
        in_specs=[hbm, hbm, hbm, hbm, hbm, vmem, hbm, hbm, hbm, vmem, hbm],
        out_specs=hbm,
        out_shape=jax.ShapeDtypeStruct((d, seq), BF16),
        scratch_shapes=[
            pltpu.VMEM((d, seq), BF16),
            pltpu.VMEM((hkv, sk, dh), BF16),
            pltpu.VMEM((hkv, sk, dh), BF16),
            pltpu.VMEM((n_grp, d, gw), BF16),
            pltpu.VMEM((n_grp, d, gw), BF16),
            pltpu.VMEM((d, 6 * d), BF16),
            pltpu.VMEM((d, f), BF16),
            pltpu.VMEM((d, f), BF16),
            pltpu.VMEM((d, f), BF16),
            pltpu.VMEM((d, seq + SP), BF16),
            pltpu.VMEM((2, TB, d), BF16),
            pltpu.VMEM((2, d, TB), F32),
            pltpu.VMEM((n_slots, sk, LANES), F32),
            pltpu.VMEM((n_slots, 1, LANES), F32),
            pltpu.VMEM((HG, dh // 2, sk), U32),
            pltpu.VMEM((8, d), F32),
            pltpu.VMEM((5, d, LANES), F32),
            pltpu.VMEM(((seq + SP) // LANES + 7 & ~7, LANES), F32),
            pltpu.VMEM((d, seq + SP), BF16),
            pltpu.VMEM((d, seq + SP), BF16),
            pltpu.VMEM((8, LANES), U32),
            pltpu.SemaphoreType.DMA((4, n_grp)),
            pltpu.SemaphoreType.DMA((4,)),
            pltpu.SemaphoreType.DMA((3,)),
            pltpu.SemaphoreType.DMA((2,)),
            pltpu.SemaphoreType.DMA((TOPC,)),
        ],
        compiler_params=pltpu.CompilerParams(
            disable_bounds_checks=True,
            disable_semaphore_checks=True,
            vmem_limit_bytes=110 * 1024 * 1024,
        ),
    )(xt, k3, v3, A_wq, wot, B_w_r, B_w_gate, B_w_up, wdt, c, w_mod)
    return out_t.T.reshape(b, seq, d)
```

```python
import contextlib
import functools
import math
import os

import jax
import jax.numpy as jnp
from jax import lax
import jax.experimental.pallas as pl
import jax.experimental.pallas.tpu as pltpu

F32 = jnp.float32
BF16 = jnp.bfloat16
I32 = jnp.int32
U32 = jnp.uint32

HQ = 32
DH = 128
TOPC = 8
EPS = 1e-05
LANES = 128

TB = 512
HG = 2
TIE0 = int(os.environ.get("KP_TIE0", "2"))
NTIE = int(os.environ.get("KP_NTIE", "3"))
SP = int(os.environ.get("KP_SP", "128"))
NM1 = int(os.environ.get("KP_NM1", "8"))
NM2 = int(os.environ.get("KP_NM2", "12"))
NM3 = int(os.environ.get("KP_NM3", "16"))
TLO = int(os.environ.get("KP_TLO", "8"))
NF1 = int(os.environ.get("KP_NF1", "9"))
NF2 = int(os.environ.get("KP_NF2", "6"))
NF3 = int(os.environ.get("KP_NF3", "18"))
NVT = int(os.environ.get("KP_NVT", "16"))
TAILB = int(os.environ.get("KP_TAILB", "2"))
SIDE_ROW = int(os.environ.get("KP_SIDE_ROW", "1"))
EDGES = [int(e) for e in os.environ.get("KP_EDGES", "0,128,256,384,512,576").split(",")]
SCOPES = os.environ.get("KP_SCOPES", "") == "1"

_NT = (((1,), (1,)), ((), ()))


def _rb(x):
    return x.astype(BF16).astype(F32)


def _sigmoid(x):
    return 1.0 / (1.0 + jnp.exp(-x))


def _lanes(col, width):
    reps = width // LANES
    return col if reps == 1 else jnp.concatenate([col] * reps, axis=1)


def _fold(x):
    xi = lax.bitcast_convert_type(x, U32)
    tok = None
    for r in range(0, x.shape[0], 8):
        for c in range(0, x.shape[1] - LANES + 1, LANES):
            t = xi[r:r + 8, c:c + LANES]
            tok = t if tok is None else tok | t
    return tok


def _colsum(x, marks, nmarks):
    n = x.shape[0] // 8
    acc = x[0:8]
    for g in range(1, n):
        acc = acc + x[8 * g:8 * g + 8]
        if ((g + 1) * nmarks) % n == 0:
            marks.append(_fold(acc))
    return jnp.sum(acc, axis=0, keepdims=True)


def _tie_rows(lhs, toks, zero, lo, hi):
    if not toks:
        return lhs
    lu = pltpu.bitcast(lhs, U32)
    rows = [lu[8 * r:8 * r + 8] for r in range(lu.shape[0] // 8)]
    for i, tok in enumerate(toks):
        r = lo + ((i + 1) * (hi - lo)) // len(toks) - 1
        rows[r] = rows[r] | (tok & zero)
    return pltpu.bitcast(jnp.concatenate(rows, axis=0), BF16)


def _span(start, size):
    if isinstance(start, int):
        return pl.ds(start, size)
    return pl.ds(pl.multiple_of(start, LANES), size)


def _scope(name):
    return jax.named_scope(name) if SCOPES else contextlib.nullcontext()


def _kernel(xt_hbm, k_hbm, v_hbm, wq_hbm, wot_hbm, wr_ref, wg_hbm, wu_hbm, wdt_hbm,
            c_ref, wmod_hbm, o_hbm,
            xt_v, k_v, v_v, wq_v, wot_v, wmod_v, wg_v, wu_v, wdt_v, ot_v,
            h_scr, acc_scr, st_scr, m_scr, vt_scr, mod_scr, col_scr, key_scr, h2_scr, x1_scr,
            zero_scr, fix_v,
            grp_sems, misc_sems, mlp_sems, out_sems, fix_sems,
            *, n_heads):
    d, seq = xt_v.shape
    sk = k_v.shape[1]
    n_grp = n_heads // HG
    n_blk = seq // TB
    n_units = n_grp * n_blk
    nb = TB // LANES
    nq = 2 * HG
    nt = sk // LANES
    gbits = n_grp.bit_length() - 1
    gw = nq * DH
    qscale = (DH ** -0.5) * math.log2(math.e)

    def grp_of(u):
        return u & (n_grp - 1)

    def blk_of(u):
        return u >> gbits

    def grp_copies(g):
        cs, hs = pl.ds(g * gw, gw), pl.ds(g * HG, HG)
        return (pltpu.make_async_copy(wq_hbm.at[:, cs], wq_v.at[g], grp_sems.at[0, g]),
                pltpu.make_async_copy(k_hbm.at[hs], k_v.at[hs], grp_sems.at[1, g]),
                pltpu.make_async_copy(v_hbm.at[hs], v_v.at[hs], grp_sems.at[2, g]),
                pltpu.make_async_copy(wot_hbm.at[:, cs], wot_v.at[g], grp_sems.at[3, g]))

    def col_copy(src, dst, lo, hi, sem):
        return pltpu.make_async_copy(src.at[:, lo:hi], dst.at[:, lo:hi], sem)

    x_first = col_copy(xt_hbm, xt_v, 0, TB, misc_sems.at[0])
    x_rest = col_copy(xt_hbm, xt_v, TB, seq, misc_sems.at[1])
    mod_first = col_copy(wmod_hbm, wmod_v, 0, 2 * d, misc_sems.at[2])
    mod_rest = col_copy(wmod_hbm, wmod_v, 2 * d, 6 * d, misc_sems.at[3])
    mlp_g = pltpu.make_async_copy(wg_hbm, wg_v, mlp_sems.at[0])
    mlp_u = pltpu.make_async_copy(wu_hbm, wu_v, mlp_sems.at[1])
    mlp_d = pltpu.make_async_copy(wdt_hbm, wdt_v, mlp_sems.at[2])
    out_lo = col_copy(ot_v, o_hbm, 0, seq - TB, out_sems.at[0])
    chunks = list(zip(EDGES[:-1], EDGES[1:]))
    out_hi = [pltpu.make_async_copy(ot_v.at[r0:r1, seq - TB:seq], o_hbm.at[r0:r1, seq - TB:seq],
                                    out_sems.at[1 + i]) for i, (r0, r1) in enumerate(chunks)]

    def silu_c():
        cc = c_ref[...].astype(F32)
        return jnp.broadcast_to((cc * _rb(_sigmoid(cc))).astype(BF16), (8, d))

    def ln1_norm(t0, n, marks):
        x = xt_v[:, _span(t0, n)].astype(F32)
        mu = _colsum(x, marks, NM1) * (1.0 / d)
        xc = x - mu
        var = _colsum(xc * xc, marks, NM2) * (1.0 / d)
        return (xc * lax.rsqrt(var + EPS)).astype(BF16).T

    def ln1_mod(ln, slot, r0, marks):
        n = ln.shape[0]
        h = ln.astype(F32) * mod_scr[1:2, :] + mod_scr[0:1, :]
        h_scr[slot, _span(r0, n), :] = h.astype(BF16)
        step = max(n // NM3, 8)
        for r in range(step - 8, n, step):
            marks.append(_fold(h[r:r + 8]))

    def qproj(u):
        q = jnp.dot(h_scr[blk_of(u) & 1], wq_v[grp_of(u)], preferred_element_type=F32)
        return (q * qscale).astype(BF16)

    def qk(u, q, j, toks=(), zero=None):
        k = _tie_rows(k_v[grp_of(u) * HG + j // 2], toks, zero, TLO, sk // 16)
        st = lax.dot_general(k, q[:, j * DH:(j + 1) * DH], _NT,
                             preferred_element_type=F32)
        for i in range(nb):
            blk = st[:, i * LANES:(i + 1) * LANES]
            st_scr[j * nb + i] = blk
            m_scr[j * nb + i] = jnp.max(blk, axis=0, keepdims=True)

    def v_transpose(u, i, marks=None):
        vt = pltpu.bitcast(v_v[grp_of(u) * HG + i].T, U32)
        vt_scr[i] = vt
        if marks is not None:
            step = sk // NVT
            for c in range(step - LANES, sk, step):
                marks.append(vt[DH // 2 - 8:DH // 2, c:c + LANES])

    def pv(slots, zero, toks=()):
        ps, ls, pairs = [], [], []
        for sl in slots:
            p = jnp.exp2(st_scr[sl] - m_scr[sl])
            accs = [None] * 4
            for tile in range(nt):
                for r0 in range(tile * LANES + LANES - 16, tile * LANES - 16, -16):
                    pair = p[r0:r0 + 8] + p[r0 + 8:r0 + 16]
                    pairs.append(pair)
                    a = accs[tile % 4]
                    accs[tile % 4] = pair if a is None else a + pair
            ls.append(jnp.sum((accs[0] + accs[1]) + (accs[2] + accs[3]), axis=0, keepdims=True))
            ps.append(p.astype(BF16))
        outs = []
        ntiles = len(slots) * nt
        side = {}
        for i, tok in enumerate(toks):
            side.setdefault(((i + 1) * ntiles) // len(toks) - 1, []).append(tok)
        for i, sl in enumerate(slots):
            vu = vt_scr[sl // (2 * nb)]
            tiles = []
            for c in range(nt):
                g = i * nt + c + 4
                rows = []
                for r in range(8):
                    x = vu[8 * r:8 * r + 8, c * LANES:(c + 1) * LANES]
                    if g < ntiles and TIE0 <= r < TIE0 + NTIE:
                        src = pairs[g * 8 + (r - TIE0)]
                        x = x | (lax.bitcast_convert_type(src, U32) & zero)
                    if r == SIDE_ROW:
                        for tok in side.get(i * nt + c, ()):
                            x = x | (tok & zero)
                    rows.append(x)
                tiles.append(jnp.concatenate(rows, axis=0))
            lhs = pltpu.bitcast(jnp.concatenate(tiles, axis=1), BF16)
            o = jnp.dot(lhs, ps[i], preferred_element_type=F32)
            outs.append((o * (1.0 / ls[i])).astype(BF16))
        return outs

    def outproj(u, o, lo=0):
        w = len(o) // nq
        o2 = jnp.concatenate(
            [jnp.concatenate(o[j * w:(j + 1) * w], axis=1) for j in range(nq)], axis=0)
        contrib = jnp.dot(wot_v[grp_of(u)], o2, preferred_element_type=F32)
        hi = lo + w * LANES
        slot = blk_of(u) & 1
        old = jnp.where(grp_of(u) > 0, acc_scr[slot, :, lo:hi], 0.0)
        acc_scr[slot, :, lo:hi] = old + contrib

    def finalize(t0, slot, a0, dst, n):
        marks = []
        cs = _span(dst, n)
        x = xt_v[:, _span(t0, n)].astype(F32)
        att = acc_scr[slot, :, _span(a0, n)]
        x1b = (x + _lanes(col_scr[0], n) * att).astype(BF16)
        x1_scr[:, cs] = x1b
        ot_v[:, cs] = x1b
        mu = _colsum(x1b.astype(F32), marks, NF1) * (1.0 / d)
        mub = _rb(mu)
        xc = x1_scr[:, cs].astype(F32) - mub
        var = _colsum(xc * xc, marks, NF2) * (1.0 / d) - (mu - mub) * (mu - mub)
        inv = 1.0 / _rb(jnp.sqrt(_rb(_rb(jnp.maximum(var, 0.0)) + EPS)))
        step = d // NF3
        racc = None
        for r0 in range(0, d, step):
            rs = slice(r0, r0 + step)
            x1 = ot_v[rs, cs].astype(F32)
            h2b = ((x1 - mub) * inv * _lanes(col_scr[2, rs, :], n)
                   + _lanes(col_scr[1, rs, :], n)).astype(BF16)
            h2_scr[rs, cs] = h2b
            h2 = h2b.astype(F32)
            out = x1 + _lanes(col_scr[3, rs, :], n) * h2
            ot_v[rs, cs] = out.astype(BF16)
            rp = h2 * _lanes(col_scr[4, rs, :], n)
            for g in range(0, step, 8):
                racc = rp[g:g + 8] if racc is None else racc + rp[g:g + 8]
            marks.append(_fold(racc) | _fold(out))
        r = _rb(jnp.sum(racc, axis=0, keepdims=True)) + 0.0
        bits = lax.bitcast_convert_type(r, I32) >> 16
        order = jnp.where(bits < 0, -1 - bits, bits + 32768)
        pos = t0 + lax.broadcasted_iota(I32, (1, n), 1)
        key = lax.bitcast_convert_type((order << 11) + (seq - 1 - pos) + 0x20000000, F32)
        for i in range(n // LANES):
            key_scr[pl.ds(dst // LANES + i, 1), :] = key[:, i * LANES:(i + 1) * LANES]
        return marks

    wq0, k0, v0, wo0 = grp_copies(0)
    wq1, k1, v1, wo1 = grp_copies(1)
    x_first.start()
    mod_first.start()
    wq0.start()
    k0.start(priority=1)
    cbits = lax.bitcast_convert_type(c_ref[:, 0:LANES].astype(F32), U32)
    zero_scr[...] = jnp.broadcast_to(cbits & 0xFFFF, (8, LANES))
    acc_scr[...] = jnp.zeros(acc_scr.shape, F32)
    col_scr[...] = jnp.zeros(col_scr.shape, F32)
    with _scope("w_x"):
        x_first.wait()
    h_scr[0] = ln1_norm(0, TB, [])
    with _scope("w_wmod"):
        mod_first.wait()
        wq0.wait()
    v0.start()
    wq1.start(priority=1)
    k1.start(priority=1)
    mod = _rb(jnp.dot(silu_c(), wmod_v[:, 0:2 * d], preferred_element_type=F32))
    mod_scr[0:1, :] = mod[0:1, 0:d]
    mod_scr[1:2, :] = _rb(1.0 + mod[0:1, d:2 * d])
    ln1_mod(h_scr[0], 0, 0, [])
    q = qproj(0)
    with _scope("w_k"):
        k0.wait()
        v0.wait()
    v1.start()
    wo0.start()
    with _scope("qk0"):
        zero = zero_scr[...]
        for j in range(nq):
            marks = []
            if j >= nq - HG:
                v_transpose(0, j - (nq - HG), marks)
            qk(0, q, j, marks, zero)

    assert n_grp == 8 and HG == 2
    loads = [[wq1, k1, v1, wo0],
             [wo1, *grp_copies(2), x_rest],
             [*grp_copies(3), *grp_copies(4)],
             [*grp_copies(5), *grp_copies(6)],
             [*grp_copies(7), mod_rest]]
    npc = TB // SP

    def steady(u, carry):
        @pl.when(u <= 5)
        def _():
            for i in range(1, len(loads)):
                @pl.when(u == i)
                def _():
                    for cp in loads[i - 1]:
                        cp.wait()
                    for cp in loads[i]:
                        cp.start()

            @pl.when(u == 5)
            def _():
                for cp in loads[-1]:
                    cp.wait()
                mlp_g.start()
                mlp_u.start()
                mlp_d.start()
                mod = _rb(jnp.dot(silu_c(), wmod_v[:, 2 * d:6 * d], preferred_element_type=F32))
                for j in range(4):
                    piece = mod[0:1, j * d:(j + 1) * d]
                    if j == 2:
                        piece = _rb(1.0 + piece)
                    col_scr[j] = jnp.broadcast_to(piece, (LANES, d)).T
                mod_scr[2:3, :] = piece
                wr = wr_ref[...].reshape(1, d).astype(F32)
                col_scr[4] = jnp.broadcast_to(wr, (LANES, d)).T

        with _scope("body"):
            zero = zero_scr[...]
            blk, g = blk_of(u), grp_of(u)
            off = ((g - 1) & (npc - 1)) * SP
            q = qproj(u)
            o = pv(range(0, 2 * nb), zero)
            live = jnp.logical_and(blk > 0, jnp.logical_and(g >= 1, g <= npc))
            t0 = jnp.maximum(blk - 1, 0) * TB + off
            qk(u, q, 0, finalize(t0, (blk + 1) & 1, off, jnp.where(live, t0, seq), SP), zero)
            marks = []
            nxt = jnp.where(u >= 2, jnp.minimum(blk + 1, n_blk - 1), 0)
            ln = ln1_norm(nxt * TB + off, SP, marks)
            ln1_mod(ln, (blk + 1) & 1, off, marks)
            qk(u, q, 1, marks, zero)
            o += pv(range(2 * nb, 4 * nb), zero)
            outproj(u - 1, o)
            marks = []
            v_transpose(u, 0, marks)
            qk(u, q, 2, marks, zero)
            marks = []
            v_transpose(u, 1, marks)
            qk(u, q, 3, marks, zero)
        return carry

    lax.fori_loop(1, n_units, steady, 0)

    ul = n_units - 1
    tl = seq - TB
    sl_last = (n_blk - 1) & 1
    nb0 = nb - TAILB
    out_lo.start()
    mlp_g.wait()
    mlp_u.wait()
    with _scope("e_pva"):
        outproj(ul, pv([j * nb + i for j in range(nq) for i in range(nb0)], zero_scr[...]))
    mlp_d.wait()
    with _scope("e_pvb"):
        toks = finalize(tl, sl_last, 0, tl, nb0 * LANES)
        o = pv([j * nb + i for j in range(nq) for i in range(nb0, nb)], zero_scr[...], toks)
        outproj(ul, o, nb0 * LANES)
        finalize(tl + nb0 * LANES, sl_last, nb0 * LANES, tl + nb0 * LANES, TAILB * LANES)

    keys = key_scr[0:seq // LANES, :]
    sub8 = lax.broadcasted_iota(I32, (TOPC, 1), 0)
    lane = lax.broadcasted_iota(I32, (TOPC, LANES), 1)
    top = jnp.zeros((TOPC, 1), F32)
    bases, idxs = [], []
    h2s = jnp.zeros((TOPC, d), F32)
    x1s = jnp.zeros((TOPC, d), F32)
    for i in range(TOPC):
        mx = jnp.max(jnp.max(keys, axis=0, keepdims=True), axis=1, keepdims=True)
        keys = jnp.where(keys == mx, 0.0, keys)
        top = jnp.where(sub8 == i, mx, top)
        idx = seq - 1 - (lax.bitcast_convert_type(mx, I32) & (seq - 1))
        bases.append(pl.multiple_of(idx[0, 0] & ~(LANES - 1), LANES))
        idxs.append(idx)
        pick = jnp.logical_and(sub8 == i, lane == (idx & (LANES - 1)))
        pick = jnp.where(pick, 1.0, 0.0).astype(BF16)
        sl = pl.ds(bases[i], LANES)
        h2s = h2s + lax.dot_general(pick, h2_scr[:, sl], _NT, preferred_element_type=F32)
        x1s = x1s + lax.dot_general(pick, x1_scr[:, sl], _NT, preferred_element_type=F32)
    order = (lax.bitcast_convert_type(top, I32) >> 11) & 0xFFFF
    rbits = jnp.where(order >= 32768, order - 32768, -1 - order) << 16
    gate = _rb(_sigmoid(lax.bitcast_convert_type(rbits, F32)))
    xs = h2s.astype(BF16)
    for cp in out_hi:
        cp.start()
    g = _rb(jnp.dot(xs, wg_v[...], preferred_element_type=F32))
    g = _rb(g * _rb(_sigmoid(g)))
    u = _rb(jnp.dot(xs, wu_v[...], preferred_element_type=F32))
    gu = (g * u).astype(BF16)

    last_use = []
    for i in range(TOPC):
        ok = True
        for j in range(i + 1, TOPC):
            ok = jnp.logical_and(ok, bases[i] != bases[j])
        last_use.append(ok)

    def down(r0, r1):
        y = _rb(lax.dot_general(gu, wdt_v[r0:r1, :], _NT, preferred_element_type=F32))
        hm = _rb(h2s[:, r0:r1] + _rb(y * gate))
        return x1s[:, r0:r1] + mod_scr[2:3, r0:r1] * hm

    def patch(r0, r1, new):
        n = r1 - r0
        pad = jnp.concatenate([new, jnp.zeros((LANES - TOPC, n), F32)], axis=0)
        cols = pltpu.bitcast(pad.T.astype(BF16), U32)
        col = [jnp.broadcast_to(cols[:, j:j + 1], (n // 2, LANES)) for j in range(TOPC)]
        for i in range(TOPC):
            res = pltpu.bitcast(ot_v[r0:r1, pl.ds(bases[i], LANES)], U32)
            tok = lane[0:1, :] + (idxs[i] & ~(LANES - 1))
            for j in range(i + 1):
                res = jnp.where(tok == idxs[j], col[j], res)
            fix_v[i, r0:r1, :] = pltpu.bitcast(res, BF16)

    def fix_copy(i, r0, r1):
        return pltpu.make_async_copy(fix_v.at[i, r0:r1, :],
                                     o_hbm.at[r0:r1, pl.ds(bases[i], LANES)], fix_sems.at[i])

    def for_last(fn):
        for i in range(TOPC - 1):
            pl.when(last_use[i])(functools.partial(fn, i))
        fn(TOPC - 1)

    new = down(*chunks[0])
    out_lo.wait()
    for ci, (r0, r1) in enumerate(chunks):
        out_hi[ci].wait()
        nxt = down(*chunks[ci + 1]) if ci + 1 < len(chunks) else None
        patch(r0, r1, new)
        for_last(lambda i: fix_copy(i, r0, r1).start())
        new = nxt
    with _scope("w_fix"):
        for r0, r1 in chunks:
            for_last(lambda i: fix_copy(i, r0, r1).wait())


@jax.jit
def pallas_adaLN_cond__gqa_block_cached__moe_arch_mod__prompt_kernel(
    A_x: jax.Array,
    A_k_cache: jax.Array,
    A_v_cache: jax.Array,
    A_wq: jax.Array,
    A_wo: jax.Array,
    B_x: jax.Array,
    B_w_r: jax.Array,
    B_w_gate: jax.Array,
    B_w_up: jax.Array,
    B_w_down: jax.Array,
    c: jax.Array,
    w_mod: jax.Array,
):
    b, seq, d = A_x.shape
    _, hkv, sk, dh = A_k_cache.shape
    assert b == 1 and dh == DH and HQ == 2 * hkv
    assert seq & (seq - 1) == 0 and seq <= 2048
    f = B_w_gate.shape[1]
    n_grp = hkv // HG
    gw = 2 * HG * dh
    n_slots = 2 * HG * TB // LANES

    xt = A_x.reshape(seq, d).T
    wot = A_wo.T
    wdt = B_w_down.T
    k3 = A_k_cache.reshape(hkv, sk, dh)
    v3 = A_v_cache.reshape(hkv, sk, dh)

    vmem = pl.BlockSpec(memory_space=pltpu.VMEM)
    hbm = pl.BlockSpec(memory_space=pl.ANY)
    out_t = pl.pallas_call(
        functools.partial(_kernel, n_heads=hkv),
        in_specs=[hbm, hbm, hbm, hbm, hbm, vmem, hbm, hbm, hbm, vmem, hbm],
        out_specs=hbm,
        out_shape=jax.ShapeDtypeStruct((d, seq), BF16),
        scratch_shapes=[
            pltpu.VMEM((d, seq), BF16),
            pltpu.VMEM((hkv, sk, dh), BF16),
            pltpu.VMEM((hkv, sk, dh), BF16),
            pltpu.VMEM((n_grp, d, gw), BF16),
            pltpu.VMEM((n_grp, d, gw), BF16),
            pltpu.VMEM((d, 6 * d), BF16),
            pltpu.VMEM((d, f), BF16),
            pltpu.VMEM((d, f), BF16),
            pltpu.VMEM((d, f), BF16),
            pltpu.VMEM((d, seq + SP), BF16),
            pltpu.VMEM((2, TB, d), BF16),
            pltpu.VMEM((2, d, TB), F32),
            pltpu.VMEM((n_slots, sk, LANES), F32),
            pltpu.VMEM((n_slots, 1, LANES), F32),
            pltpu.VMEM((HG, dh // 2, sk), U32),
            pltpu.VMEM((8, d), F32),
            pltpu.VMEM((5, d, LANES), F32),
            pltpu.VMEM(((seq + SP) // LANES + 7 & ~7, LANES), F32),
            pltpu.VMEM((d, seq + SP), BF16),
            pltpu.VMEM((d, seq + SP), BF16),
            pltpu.VMEM((8, LANES), U32),
            pltpu.VMEM((TOPC, d, LANES), BF16),
            pltpu.SemaphoreType.DMA((4, n_grp)),
            pltpu.SemaphoreType.DMA((4,)),
            pltpu.SemaphoreType.DMA((3,)),
            pltpu.SemaphoreType.DMA((len(EDGES),)),
            pltpu.SemaphoreType.DMA((TOPC,)),
        ],
        compiler_params=pltpu.CompilerParams(
            disable_bounds_checks=True,
            disable_semaphore_checks=True,
            vmem_limit_bytes=110 * 1024 * 1024,
        ),
    )(xt, k3, v3, A_wq, wot, B_w_r, B_w_gate, B_w_up, wdt, c, w_mod)
    return out_t.T.reshape(b, seq, d)
```

```python
import contextlib
import functools
import math
import os

import jax
import jax.numpy as jnp
from jax import lax
import jax.experimental.pallas as pl
import jax.experimental.pallas.tpu as pltpu

F32 = jnp.float32
BF16 = jnp.bfloat16
I32 = jnp.int32
U32 = jnp.uint32

HQ = 32
DH = 128
TOPC = 8
EPS = 1e-05
LANES = 128

TB = 512
HG = 2
TIE0 = int(os.environ.get("KP_TIE0", "2"))
NTIE = int(os.environ.get("KP_NTIE", "3"))
SP = int(os.environ.get("KP_SP", "128"))
NM1 = int(os.environ.get("KP_NM1", "8"))
NM2 = int(os.environ.get("KP_NM2", "12"))
NM3 = int(os.environ.get("KP_NM3", "16"))
TLO = int(os.environ.get("KP_TLO", "8"))
NF1 = int(os.environ.get("KP_NF1", "9"))
NF2 = int(os.environ.get("KP_NF2", "6"))
NF3 = int(os.environ.get("KP_NF3", "18"))
NVT = int(os.environ.get("KP_NVT", "16"))
TAILB = int(os.environ.get("KP_TAILB", "2"))
SIDE_ROW = int(os.environ.get("KP_SIDE_ROW", "6"))
EDGES = [int(e) for e in os.environ.get("KP_EDGES", "0,128,256,384,512,576").split(",")]
MODR = int(os.environ.get("KP_MODR", "384"))
SCOPES = os.environ.get("KP_SCOPES", "") == "1"

_NT = (((1,), (1,)), ((), ()))


def _rb(x):
    return x.astype(BF16).astype(F32)


def _sigmoid(x):
    return 1.0 / (1.0 + jnp.exp(-x))


def _lanes(col, width):
    reps = width // LANES
    return col if reps == 1 else jnp.concatenate([col] * reps, axis=1)


def _fold(x):
    xi = lax.bitcast_convert_type(x, U32)
    tok = None
    for r in range(0, x.shape[0], 8):
        for c in range(0, x.shape[1] - LANES + 1, LANES):
            t = xi[r:r + 8, c:c + LANES]
            tok = t if tok is None else tok | t
    return tok


def _colsum(x, marks, nmarks):
    n = x.shape[0] // 8
    acc = x[0:8]
    for g in range(1, n):
        acc = acc + x[8 * g:8 * g + 8]
        if ((g + 1) * nmarks) % n == 0:
            marks.append(_fold(acc))
    return jnp.sum(acc, axis=0, keepdims=True)


def _tie_rows(lhs, toks, zero, lo, hi):
    if not toks:
        return lhs
    lu = pltpu.bitcast(lhs, U32)
    rows = [lu[8 * r:8 * r + 8] for r in range(lu.shape[0] // 8)]
    for i, tok in enumerate(toks):
        r = lo + ((i + 1) * (hi - lo)) // len(toks) - 1
        rows[r] = rows[r] | (tok & zero)
    return pltpu.bitcast(jnp.concatenate(rows, axis=0), BF16)


def _span(start, size):
    if isinstance(start, int):
        return pl.ds(start, size)
    return pl.ds(pl.multiple_of(start, LANES), size)


def _scope(name):
    return jax.named_scope(name) if SCOPES else contextlib.nullcontext()


def _kernel(xt_hbm, k_hbm, v_hbm, wq_hbm, wot_hbm, wr_hbm, wg_hbm, wu_hbm, wdt_hbm,
            c_hbm, wmod_hbm, o_hbm,
            xt_v, k_v, v_v, wq_v, wot_v, wmod_v, wg_v, wu_v, wdt_v, ot_v,
            h_scr, acc_scr, st_scr, m_scr, vt_scr, mod_scr, col_scr, key_scr, h2_scr, x1_scr,
            zero_scr, fix_v, c_ref, wr_ref,
            grp_sems, misc_sems, mlp_sems, out_sems, fix_sems,
            *, n_heads):
    d, seq = xt_v.shape
    sk = k_v.shape[1]
    n_grp = n_heads // HG
    n_blk = seq // TB
    n_units = n_grp * n_blk
    nb = TB // LANES
    nq = 2 * HG
    nt = sk // LANES
    gbits = n_grp.bit_length() - 1
    gw = nq * DH
    qscale = (DH ** -0.5) * math.log2(math.e)

    def grp_of(u):
        return u & (n_grp - 1)

    def blk_of(u):
        return u >> gbits

    def grp_copies(g):
        cs, hs = pl.ds(g * gw, gw), pl.ds(g * HG, HG)
        return (pltpu.make_async_copy(wq_hbm.at[:, cs], wq_v.at[g], grp_sems.at[0, g]),
                pltpu.make_async_copy(k_hbm.at[hs], k_v.at[hs], grp_sems.at[1, g]),
                pltpu.make_async_copy(v_hbm.at[hs], v_v.at[hs], grp_sems.at[2, g]),
                pltpu.make_async_copy(wot_hbm.at[:, cs], wot_v.at[g], grp_sems.at[3, g]))

    def col_copy(src, dst, lo, hi, sem):
        return pltpu.make_async_copy(src.at[:, lo:hi], dst.at[:, lo:hi], sem)

    x_first = col_copy(xt_hbm, xt_v, 0, TB, misc_sems.at[0])
    x_rest = col_copy(xt_hbm, xt_v, TB, seq, misc_sems.at[1])
    mod_rows = [(0, MODR), (MODR, d)]
    mod_first = [pltpu.make_async_copy(wmod_hbm.at[r0:r1, 0:2 * d], wmod_v.at[r0:r1, 0:2 * d],
                                       misc_sems.at[8 + i]) for i, (r0, r1) in enumerate(mod_rows)]
    mod_rest = col_copy(wmod_hbm, wmod_v, 2 * d, 6 * d, misc_sems.at[3])
    mlp_g = pltpu.make_async_copy(wg_hbm, wg_v, mlp_sems.at[0])
    mlp_u = pltpu.make_async_copy(wu_hbm, wu_v, mlp_sems.at[1])
    mlp_d = pltpu.make_async_copy(wdt_hbm, wdt_v, mlp_sems.at[2])
    out_lo = col_copy(ot_v, o_hbm, 0, seq - TB, out_sems.at[0])
    chunks = list(zip(EDGES[:-1], EDGES[1:]))
    out_hi = [pltpu.make_async_copy(ot_v.at[r0:r1, seq - TB:seq], o_hbm.at[r0:r1, seq - TB:seq],
                                    out_sems.at[1 + i]) for i, (r0, r1) in enumerate(chunks)]

    def silu_c():
        cc = c_ref[...].astype(F32)
        return jnp.broadcast_to((cc * _rb(_sigmoid(cc))).astype(BF16), (8, d))

    def ln1_norm(t0, n, marks):
        x = xt_v[:, _span(t0, n)].astype(F32)
        mu = _colsum(x, marks, NM1) * (1.0 / d)
        xc = x - mu
        var = _colsum(xc * xc, marks, NM2) * (1.0 / d)
        return (xc * lax.rsqrt(var + EPS)).astype(BF16).T

    def ln1_mod(ln, slot, r0, marks):
        n = ln.shape[0]
        h = ln.astype(F32) * mod_scr[1:2, :] + mod_scr[0:1, :]
        h_scr[slot, _span(r0, n), :] = h.astype(BF16)
        step = max(n // NM3, 8)
        for r in range(step - 8, n, step):
            marks.append(_fold(h[r:r + 8]))

    def qproj(u, lo=0, hi=gw, parts=1):
        qs = []
        for r0 in range(0, TB, TB // parts):
            q = jnp.dot(h_scr[blk_of(u) & 1, r0:r0 + TB // parts, :], wq_v[grp_of(u), :, lo:hi],
                        preferred_element_type=F32)
            qs.append((q * qscale).astype(BF16))
        return jnp.concatenate(qs, axis=0)

    def qk(u, q, j, toks=(), zero=None):
        k = _tie_rows(k_v[grp_of(u) * HG + j // 2], toks, zero, TLO, sk // 16)
        st = lax.dot_general(k, q[:, j * DH:(j + 1) * DH], _NT,
                             preferred_element_type=F32)
        for i in range(nb):
            blk = st[:, i * LANES:(i + 1) * LANES]
            st_scr[j * nb + i] = blk
            m_scr[j * nb + i] = jnp.max(blk, axis=0, keepdims=True)

    def v_transpose(u, i, marks=None):
        vt = pltpu.bitcast(v_v[grp_of(u) * HG + i].T, U32)
        vt_scr[i] = vt
        if marks is not None:
            step = sk // NVT
            for c in range(step - LANES, sk, step):
                marks.append(vt[DH // 2 - 8:DH // 2, c:c + LANES])

    def pv(slots, zero, toks=()):
        ps, ls, pairs = [], [], []
        for sl in slots:
            p = jnp.exp2(st_scr[sl] - m_scr[sl])
            accs = [None] * 4
            for tile in range(nt):
                for r0 in range(tile * LANES + LANES - 16, tile * LANES - 16, -16):
                    pair = p[r0:r0 + 8] + p[r0 + 8:r0 + 16]
                    pairs.append(pair)
                    a = accs[tile % 4]
                    accs[tile % 4] = pair if a is None else a + pair
            ls.append(jnp.sum((accs[0] + accs[1]) + (accs[2] + accs[3]), axis=0, keepdims=True))
            ps.append(p.astype(BF16))
        outs = []
        ntiles = len(slots) * nt
        side = {}
        for i, tok in enumerate(toks):
            side.setdefault(((i + 1) * ntiles) // len(toks) - 1, []).append(tok)
        for i, sl in enumerate(slots):
            vu = vt_scr[sl // (2 * nb)]
            tiles = []
            for c in range(nt):
                g = i * nt + c + 4
                rows = []
                for r in range(8):
                    x = vu[8 * r:8 * r + 8, c * LANES:(c + 1) * LANES]
                    if g < ntiles and TIE0 <= r < TIE0 + NTIE:
                        src = pairs[g * 8 + (r - TIE0)]
                        x = x | (lax.bitcast_convert_type(src, U32) & zero)
                    if r == SIDE_ROW:
                        for tok in side.get(i * nt + c, ()):
                            x = x | (tok & zero)
                    rows.append(x)
                tiles.append(jnp.concatenate(rows, axis=0))
            lhs = pltpu.bitcast(jnp.concatenate(tiles, axis=1), BF16)
            o = jnp.dot(lhs, ps[i], preferred_element_type=F32)
            outs.append((o * (1.0 / ls[i])).astype(BF16))
        return outs

    def outproj(u, o, lo=0):
        w = len(o) // nq
        o2 = jnp.concatenate(
            [jnp.concatenate(o[j * w:(j + 1) * w], axis=1) for j in range(nq)], axis=0)
        contrib = jnp.dot(wot_v[grp_of(u)], o2, preferred_element_type=F32)
        hi = lo + w * LANES
        slot = blk_of(u) & 1
        old = jnp.where(grp_of(u) > 0, acc_scr[slot, :, lo:hi], 0.0)
        acc_scr[slot, :, lo:hi] = old + contrib

    def finalize(t0, slot, a0, dst, n):
        marks = []
        cs = _span(dst, n)
        x = xt_v[:, _span(t0, n)].astype(F32)
        att = acc_scr[slot, :, _span(a0, n)]
        x1b = (x + _lanes(col_scr[0], n) * att).astype(BF16)
        x1_scr[:, cs] = x1b
        ot_v[:, cs] = x1b
        mu = _colsum(x1b.astype(F32), marks, NF1) * (1.0 / d)
        mub = _rb(mu)
        xc = x1_scr[:, cs].astype(F32) - mub
        var = _colsum(xc * xc, marks, NF2) * (1.0 / d) - (mu - mub) * (mu - mub)
        inv = 1.0 / _rb(jnp.sqrt(_rb(_rb(jnp.maximum(var, 0.0)) + EPS)))
        step = d // NF3
        racc = None
        for r0 in range(0, d, step):
            rs = slice(r0, r0 + step)
            x1 = ot_v[rs, cs].astype(F32)
            h2b = ((x1 - mub) * inv * _lanes(col_scr[2, rs, :], n)
                   + _lanes(col_scr[1, rs, :], n)).astype(BF16)
            h2_scr[rs, cs] = h2b
            h2 = h2b.astype(F32)
            out = x1 + _lanes(col_scr[3, rs, :], n) * h2
            ot_v[rs, cs] = out.astype(BF16)
            rp = h2 * _lanes(col_scr[4, rs, :], n)
            for g in range(0, step, 8):
                racc = rp[g:g + 8] if racc is None else racc + rp[g:g + 8]
            marks.append(_fold(racc) | _fold(out))
        r = _rb(jnp.sum(racc, axis=0, keepdims=True)) + 0.0
        bits = lax.bitcast_convert_type(r, I32) >> 16
        order = jnp.where(bits < 0, -1 - bits, bits + 32768)
        pos = t0 + lax.broadcasted_iota(I32, (1, n), 1)
        key = lax.bitcast_convert_type((order << 11) + (seq - 1 - pos) + 0x20000000, F32)
        for i in range(n // LANES):
            key_scr[pl.ds(dst // LANES + i, 1), :] = key[:, i * LANES:(i + 1) * LANES]
        return marks

    hw = gw // 2
    wq0a = pltpu.make_async_copy(wq_hbm.at[:, 0:hw], wq_v.at[0, :, 0:hw], grp_sems.at[0, 0])
    wq0b = pltpu.make_async_copy(wq_hbm.at[:, hw:gw], wq_v.at[0, :, hw:gw], misc_sems.at[4])
    k0a = pltpu.make_async_copy(k_hbm.at[0], k_v.at[0], grp_sems.at[1, 0])
    k0b = pltpu.make_async_copy(k_hbm.at[1], k_v.at[1], misc_sems.at[5])
    v0 = pltpu.make_async_copy(v_hbm.at[0:HG], v_v.at[0:HG], grp_sems.at[2, 0])
    wo0 = pltpu.make_async_copy(wot_hbm.at[:, 0:gw], wot_v.at[0], grp_sems.at[3, 0])
    wq1, k1, v1, wo1 = grp_copies(1)
    c_copy = pltpu.make_async_copy(c_hbm, c_ref, misc_sems.at[6])
    wr_copy = pltpu.make_async_copy(wr_hbm, wr_ref, misc_sems.at[7])
    c_copy.start()
    wr_copy.start()
    x_first.start()
    mod_first[0].start()
    mod_first[1].start()
    wq0a.start()
    acc_scr[1] = jnp.zeros((d, TB), F32)
    col_scr[...] = jnp.zeros(col_scr.shape, F32)
    with _scope("w_x"):
        c_copy.wait()
        wr_copy.wait()
        x_first.wait()
    cbits = lax.bitcast_convert_type(c_ref[:, 0:LANES].astype(F32), U32)
    zero_scr[...] = jnp.broadcast_to(cbits & 0xFFFF, (8, LANES))
    h_scr[0] = ln1_norm(0, TB, [])
    sc = silu_c()
    with _scope("w_wmod"):
        mod_first[0].wait()
    mod = jnp.dot(sc[:, 0:MODR], wmod_v[0:MODR, 0:2 * d], preferred_element_type=F32)
    with _scope("w_wmod2"):
        mod_first[1].wait()
    wq0b.start()
    k0a.start()
    k0b.start(priority=1)
    v0.start(priority=1)
    mod = _rb(mod + jnp.dot(sc[:, MODR:d], wmod_v[MODR:d, 0:2 * d], preferred_element_type=F32))
    mod_scr[0:1, :] = mod[0:1, 0:d]
    mod_scr[1:2, :] = _rb(1.0 + mod[0:1, d:2 * d])
    with _scope("w_wq"):
        wq0a.wait()
    ln1_mod(h_scr[0], 0, 0, [])
    qa = qproj(0, 0, hw, 2)
    with _scope("w_k"):
        wq0b.wait()
        k0a.wait()
    wq1.start(priority=1)
    k1.start(priority=1)
    q = jnp.concatenate([qa, qproj(0, hw, gw, 2)], axis=1)
    qk(0, q, 0)
    qk(0, q, 1)
    with _scope("w_v"):
        k0b.wait()
        v0.wait()
    v1.start()
    wo0.start()
    with _scope("qk0"):
        zero = zero_scr[...]
        for i in range(HG):
            marks = []
            v_transpose(0, i, marks)
            qk(0, q, nq - HG + i, marks, zero)

    assert n_grp == 8 and HG == 2
    loads = [[wq1, k1, v1, wo0],
             [wo1, *grp_copies(2), x_rest],
             [*grp_copies(3), *grp_copies(4)],
             [*grp_copies(5), *grp_copies(6)],
             [*grp_copies(7), mod_rest]]
    npc = TB // SP

    def steady(u, carry):
        @pl.when(u <= 5)
        def _():
            for i in range(1, len(loads)):
                @pl.when(u == i)
                def _():
                    for cp in loads[i - 1]:
                        cp.wait()
                    for cp in loads[i]:
                        cp.start()

            @pl.when(u == 5)
            def _():
                for cp in loads[-1]:
                    cp.wait()
                mlp_g.start()
                mlp_u.start()
                mlp_d.start()
                mod = _rb(jnp.dot(silu_c(), wmod_v[:, 2 * d:6 * d], preferred_element_type=F32))
                for j in range(4):
                    piece = mod[0:1, j * d:(j + 1) * d]
                    if j == 2:
                        piece = _rb(1.0 + piece)
                    col_scr[j] = jnp.broadcast_to(piece, (LANES, d)).T
                mod_scr[2:3, :] = piece
                wr = wr_ref[...].reshape(1, d).astype(F32)
                col_scr[4] = jnp.broadcast_to(wr, (LANES, d)).T

        with _scope("body"):
            zero = zero_scr[...]
            blk, g = blk_of(u), grp_of(u)
            off = ((g - 1) & (npc - 1)) * SP
            q = qproj(u)
            o = pv(range(0, 2 * nb), zero)
            live = jnp.logical_and(blk > 0, jnp.logical_and(g >= 1, g <= npc))
            t0 = jnp.maximum(blk - 1, 0) * TB + off
            qk(u, q, 0, finalize(t0, (blk + 1) & 1, off, jnp.where(live, t0, seq), SP), zero)
            marks = []
            nxt = jnp.where(u >= 2, jnp.minimum(blk + 1, n_blk - 1), 0)
            ln = ln1_norm(nxt * TB + off, SP, marks)
            ln1_mod(ln, (blk + 1) & 1, off, marks)
            qk(u, q, 1, marks, zero)
            o += pv(range(2 * nb, 4 * nb), zero)
            outproj(u - 1, o)
            marks = []
            v_transpose(u, 0, marks)
            qk(u, q, 2, marks, zero)
            marks = []
            v_transpose(u, 1, marks)
            qk(u, q, 3, marks, zero)
        return carry

    lax.fori_loop(1, n_units, steady, 0)

    ul = n_units - 1
    tl = seq - TB
    sl_last = (n_blk - 1) & 1
    nb0 = nb - TAILB
    out_lo.start()
    mlp_g.wait()
    mlp_u.wait()
    with _scope("e_pva"):
        outproj(ul, pv([j * nb + i for j in range(nq) for i in range(nb0)], zero_scr[...]))
    mlp_d.wait()
    with _scope("e_pvb"):
        toks = finalize(tl, sl_last, 0, tl, nb0 * LANES)
        o = pv([j * nb + i for j in range(nq) for i in range(nb0, nb)], zero_scr[...], toks)
        outproj(ul, o, nb0 * LANES)
        finalize(tl + nb0 * LANES, sl_last, nb0 * LANES, tl + nb0 * LANES, TAILB * LANES)

    keys = key_scr[0:seq // LANES, :]
    sub8 = lax.broadcasted_iota(I32, (TOPC, 1), 0)
    lane = lax.broadcasted_iota(I32, (TOPC, LANES), 1)
    top = jnp.zeros((TOPC, 1), F32)
    bases, idxs = [], []
    h2s = jnp.zeros((TOPC, d), F32)
    x1s = jnp.zeros((TOPC, d), F32)
    for i in range(TOPC):
        mx = jnp.max(jnp.max(keys, axis=0, keepdims=True), axis=1, keepdims=True)
        keys = jnp.where(keys == mx, 0.0, keys)
        top = jnp.where(sub8 == i, mx, top)
        idx = seq - 1 - (lax.bitcast_convert_type(mx, I32) & (seq - 1))
        bases.append(pl.multiple_of(idx[0, 0] & ~(LANES - 1), LANES))
        idxs.append(idx)
        pick = jnp.logical_and(sub8 == i, lane == (idx & (LANES - 1)))
        pick = jnp.where(pick, 1.0, 0.0).astype(BF16)
        sl = pl.ds(bases[i], LANES)
        h2s = h2s + lax.dot_general(pick, h2_scr[:, sl], _NT, preferred_element_type=F32)
        x1s = x1s + lax.dot_general(pick, x1_scr[:, sl], _NT, preferred_element_type=F32)
    order = (lax.bitcast_convert_type(top, I32) >> 11) & 0xFFFF
    rbits = jnp.where(order >= 32768, order - 32768, -1 - order) << 16
    gate = _rb(_sigmoid(lax.bitcast_convert_type(rbits, F32)))
    xs = h2s.astype(BF16)
    for cp in out_hi:
        cp.start()
    g = _rb(jnp.dot(xs, wg_v[...], preferred_element_type=F32))
    g = _rb(g * _rb(_sigmoid(g)))
    u = _rb(jnp.dot(xs, wu_v[...], preferred_element_type=F32))
    gu = (g * u).astype(BF16)

    last_use = []
    for i in range(TOPC):
        ok = True
        for j in range(i + 1, TOPC):
            ok = jnp.logical_and(ok, bases[i] != bases[j])
        last_use.append(ok)

    def down(r0, r1):
        y = _rb(lax.dot_general(gu, wdt_v[r0:r1, :], _NT, preferred_element_type=F32))
        hm = _rb(h2s[:, r0:r1] + _rb(y * gate))
        return x1s[:, r0:r1] + mod_scr[2:3, r0:r1] * hm

    def patch(r0, r1, new):
        n = r1 - r0
        pad = jnp.concatenate([new, jnp.zeros((LANES - TOPC, n), F32)], axis=0)
        cols = pltpu.bitcast(pad.T.astype(BF16), U32)
        col = [jnp.broadcast_to(cols[:, j:j + 1], (n // 2, LANES)) for j in range(TOPC)]
        for i in range(TOPC):
            res = pltpu.bitcast(ot_v[r0:r1, pl.ds(bases[i], LANES)], U32)
            tok = lane[0:1, :] + (idxs[i] & ~(LANES - 1))
            for j in range(i + 1):
                res = jnp.where(tok == idxs[j], col[j], res)
            fix_v[i, r0:r1, :] = pltpu.bitcast(res, BF16)

    def fix_copy(i, r0, r1):
        return pltpu.make_async_copy(fix_v.at[i, r0:r1, :],
                                     o_hbm.at[r0:r1, pl.ds(bases[i], LANES)], fix_sems.at[i])

    def for_last(fn):
        for i in range(TOPC - 1):
            pl.when(last_use[i])(functools.partial(fn, i))
        fn(TOPC - 1)

    new = down(*chunks[0])
    out_lo.wait()
    for ci, (r0, r1) in enumerate(chunks):
        out_hi[ci].wait()
        nxt = down(*chunks[ci + 1]) if ci + 1 < len(chunks) else None
        patch(r0, r1, new)
        for_last(lambda i: fix_copy(i, r0, r1).start())
        new = nxt
    with _scope("w_fix"):
        for r0, r1 in chunks:
            for_last(lambda i: fix_copy(i, r0, r1).wait())


@jax.jit
def pallas_adaLN_cond__gqa_block_cached__moe_arch_mod__prompt_kernel(
    A_x: jax.Array,
    A_k_cache: jax.Array,
    A_v_cache: jax.Array,
    A_wq: jax.Array,
    A_wo: jax.Array,
    B_x: jax.Array,
    B_w_r: jax.Array,
    B_w_gate: jax.Array,
    B_w_up: jax.Array,
    B_w_down: jax.Array,
    c: jax.Array,
    w_mod: jax.Array,
):
    b, seq, d = A_x.shape
    _, hkv, sk, dh = A_k_cache.shape
    assert b == 1 and dh == DH and HQ == 2 * hkv
    assert seq & (seq - 1) == 0 and seq <= 2048
    f = B_w_gate.shape[1]
    n_grp = hkv // HG
    gw = 2 * HG * dh
    n_slots = 2 * HG * TB // LANES

    xt = A_x.reshape(seq, d).T
    wot = A_wo.T
    wdt = B_w_down.T
    k3 = A_k_cache.reshape(hkv, sk, dh)
    v3 = A_v_cache.reshape(hkv, sk, dh)

    hbm = pl.BlockSpec(memory_space=pl.ANY)
    out_t = pl.pallas_call(
        functools.partial(_kernel, n_heads=hkv),
        in_specs=[hbm] * 11,
        out_specs=hbm,
        out_shape=jax.ShapeDtypeStruct((d, seq), BF16),
        scratch_shapes=[
            pltpu.VMEM((d, seq), BF16),
            pltpu.VMEM((hkv, sk, dh), BF16),
            pltpu.VMEM((hkv, sk, dh), BF16),
            pltpu.VMEM((n_grp, d, gw), BF16),
            pltpu.VMEM((n_grp, d, gw), BF16),
            pltpu.VMEM((d, 6 * d), BF16),
            pltpu.VMEM((d, f), BF16),
            pltpu.VMEM((d, f), BF16),
            pltpu.VMEM((d, f), BF16),
            pltpu.VMEM((d, seq + SP), BF16),
            pltpu.VMEM((2, TB, d), BF16),
            pltpu.VMEM((2, d, TB), F32),
            pltpu.VMEM((n_slots, sk, LANES), F32),
            pltpu.VMEM((n_slots, 1, LANES), F32),
            pltpu.VMEM((HG, dh // 2, sk), U32),
            pltpu.VMEM((8, d), F32),
            pltpu.VMEM((5, d, LANES), F32),
            pltpu.VMEM(((seq + SP) // LANES + 7 & ~7, LANES), F32),
            pltpu.VMEM((d, seq + SP), BF16),
            pltpu.VMEM((d, seq + SP), BF16),
            pltpu.VMEM((8, LANES), U32),
            pltpu.VMEM((TOPC, d, LANES), BF16),
            pltpu.VMEM((1, d), BF16),
            pltpu.VMEM((d,), BF16),
            pltpu.SemaphoreType.DMA((4, n_grp)),
            pltpu.SemaphoreType.DMA((10,)),
            pltpu.SemaphoreType.DMA((3,)),
            pltpu.SemaphoreType.DMA((len(EDGES),)),
            pltpu.SemaphoreType.DMA((TOPC,)),
        ],
        compiler_params=pltpu.CompilerParams(
            disable_bounds_checks=True,
            disable_semaphore_checks=True,
            vmem_limit_bytes=110 * 1024 * 1024,
        ),
    )(xt, k3, v3, A_wq, wot, B_w_r, B_w_gate, B_w_up, wdt, c, w_mod)
    return out_t.T.reshape(b, seq, d)
```

```python
import contextlib
import functools
import math
import os

import jax
import jax.numpy as jnp
from jax import lax
import jax.experimental.pallas as pl
import jax.experimental.pallas.tpu as pltpu

F32 = jnp.float32
BF16 = jnp.bfloat16
I32 = jnp.int32
U32 = jnp.uint32

HQ = 32
DH = 128
TOPC = 8
EPS = 1e-05
LANES = 128

TB = 512
HG = 2
TIE0 = int(os.environ.get("KP_TIE0", "2"))
NTIE = int(os.environ.get("KP_NTIE", "3"))
SP = int(os.environ.get("KP_SP", "128"))
NM1 = int(os.environ.get("KP_NM1", "8"))
NM2 = int(os.environ.get("KP_NM2", "12"))
NM3 = int(os.environ.get("KP_NM3", "16"))
TLO = int(os.environ.get("KP_TLO", "8"))
NF1 = int(os.environ.get("KP_NF1", "9"))
NF2 = int(os.environ.get("KP_NF2", "6"))
NF3 = int(os.environ.get("KP_NF3", "18"))
NVT = int(os.environ.get("KP_NVT", "16"))
TAILB = int(os.environ.get("KP_TAILB", "2"))
SIDE_ROW = int(os.environ.get("KP_SIDE_ROW", "6"))
EDGES = [int(e) for e in os.environ.get("KP_EDGES", "0,128,256,384,512,576").split(",")]
MODR = int(os.environ.get("KP_MODR", "384"))
MP = int(os.environ.get("KP_MP", "384"))
NMP = int(os.environ.get("KP_NMP", "12"))
SCOPES = os.environ.get("KP_SCOPES", "") == "1"

_NT = (((1,), (1,)), ((), ()))


def _rb(x):
    return x.astype(BF16).astype(F32)


def _sigmoid(x):
    return 1.0 / (1.0 + jnp.exp(-x))


def _lanes(col, width):
    reps = width // LANES
    return col if reps == 1 else jnp.concatenate([col] * reps, axis=1)


def _fold(x):
    xi = lax.bitcast_convert_type(x, U32)
    tok = None
    for r in range(0, x.shape[0], 8):
        for c in range(0, x.shape[1] - LANES + 1, LANES):
            t = xi[r:r + 8, c:c + LANES]
            tok = t if tok is None else tok | t
    return tok


def _colsum(x, marks, nmarks):
    n = x.shape[0] // 8
    acc = x[0:8]
    for g in range(1, n):
        acc = acc + x[8 * g:8 * g + 8]
        if ((g + 1) * nmarks) % n == 0:
            marks.append(_fold(acc))
    return jnp.sum(acc, axis=0, keepdims=True)


def _tie_rows(lhs, toks, zero, lo, hi):
    if not toks:
        return lhs
    lu = pltpu.bitcast(lhs, U32)
    rows = [lu[8 * r:8 * r + 8] for r in range(lu.shape[0] // 8)]
    for i, tok in enumerate(toks):
        r = lo + ((i + 1) * (hi - lo)) // len(toks) - 1
        rows[r] = rows[r] | (tok & zero)
    return pltpu.bitcast(jnp.concatenate(rows, axis=0), BF16)


def _span(start, size):
    if isinstance(start, int):
        return pl.ds(start, size)
    return pl.ds(pl.multiple_of(start, LANES), size)


def _scope(name):
    return jax.named_scope(name) if SCOPES else contextlib.nullcontext()


def _kernel(xt_hbm, k_hbm, v_hbm, wq_hbm, wot_hbm, wr_hbm, wg_hbm, wu_hbm, wdt_hbm,
            c_hbm, wmod_hbm, o_hbm,
            xt_v, k_v, v_v, wq_v, wot_v, wmod_v, wg_v, wu_v, wdt_v, ot_v,
            h_scr, acc_scr, st_scr, m_scr, vt_scr, mod_scr, col_scr, key_scr, h2_scr, x1_scr,
            zero_scr, fix_v, c_ref, wr_ref, row_scr,
            grp_sems, misc_sems, mlp_sems, out_sems, fix_sems,
            *, n_heads):
    d, seq = xt_v.shape
    sk = k_v.shape[1]
    n_grp = n_heads // HG
    n_blk = seq // TB
    n_units = n_grp * n_blk
    nb = TB // LANES
    nq = 2 * HG
    nt = sk // LANES
    gbits = n_grp.bit_length() - 1
    gw = nq * DH
    qscale = (DH ** -0.5) * math.log2(math.e)

    def grp_of(u):
        return u & (n_grp - 1)

    def blk_of(u):
        return u >> gbits

    def grp_copies(g):
        cs, hs = pl.ds(g * gw, gw), pl.ds(g * HG, HG)
        return (pltpu.make_async_copy(wq_hbm.at[:, cs], wq_v.at[g], grp_sems.at[0, g]),
                pltpu.make_async_copy(k_hbm.at[hs], k_v.at[hs], grp_sems.at[1, g]),
                pltpu.make_async_copy(v_hbm.at[hs], v_v.at[hs], grp_sems.at[2, g]),
                pltpu.make_async_copy(wot_hbm.at[:, cs], wot_v.at[g], grp_sems.at[3, g]))

    def col_copy(src, dst, lo, hi, sem):
        return pltpu.make_async_copy(src.at[:, lo:hi], dst.at[:, lo:hi], sem)

    x_first = col_copy(xt_hbm, xt_v, 0, TB, misc_sems.at[0])
    x_rest = col_copy(xt_hbm, xt_v, TB, seq, misc_sems.at[1])
    mod_rows = [(0, MODR), (MODR, d)]
    mod_first = [pltpu.make_async_copy(wmod_hbm.at[r0:r1, 0:2 * d], wmod_v.at[r0:r1, 0:2 * d],
                                       misc_sems.at[8 + i]) for i, (r0, r1) in enumerate(mod_rows)]
    mod_rest = col_copy(wmod_hbm, wmod_v, 2 * d, 6 * d, misc_sems.at[3])
    mlp_g = pltpu.make_async_copy(wg_hbm, wg_v, mlp_sems.at[0])
    mlp_u = pltpu.make_async_copy(wu_hbm, wu_v, mlp_sems.at[1])
    mlp_d = pltpu.make_async_copy(wdt_hbm, wdt_v, mlp_sems.at[2])
    out_lo = col_copy(ot_v, o_hbm, 0, seq - TB, out_sems.at[0])
    chunks = list(zip(EDGES[:-1], EDGES[1:]))
    out_hi = [pltpu.make_async_copy(ot_v.at[r0:r1, seq - TB:seq], o_hbm.at[r0:r1, seq - TB:seq],
                                    out_sems.at[1 + i]) for i, (r0, r1) in enumerate(chunks)]

    def silu_c():
        cc = c_ref[...].astype(F32)
        return jnp.broadcast_to((cc * _rb(_sigmoid(cc))).astype(BF16), (8, d))

    def ln1_norm(t0, n, marks):
        x = xt_v[:, _span(t0, n)].astype(F32)
        mu = _colsum(x, marks, NM1) * (1.0 / d)
        xc = x - mu
        var = _colsum(xc * xc, marks, NM2) * (1.0 / d)
        return (xc * lax.rsqrt(var + EPS)).astype(BF16).T

    def ln1_mod(ln, slot, r0, marks):
        n = ln.shape[0]
        h = ln.astype(F32) * mod_scr[1:2, :] + mod_scr[0:1, :]
        h_scr[slot, _span(r0, n), :] = h.astype(BF16)
        step = max(n // NM3, 8)
        for r in range(step - 8, n, step):
            marks.append(_fold(h[r:r + 8]))

    def mod_piece(src, dst, marks):
        w = wmod_v[:, _span(src, MP)].astype(F32)
        row = _rb(_colsum(w * _lanes(col_scr[5 * d:6 * d, :], MP), marks, NMP))
        pos = dst + lax.broadcasted_iota(I32, (1, MP), 1)
        is_cb = jnp.logical_and(pos >= 2 * d, pos < 3 * d)
        row = jnp.where(is_cb, _rb(1.0 + row), row)
        row_scr[:, _span(dst, MP)] = row
        col = jnp.broadcast_to(row, (LANES, MP)).T
        col_scr[_span(dst, MP), :] = col
        for r in range(LANES - 8, MP, LANES):
            marks.append(lax.bitcast_convert_type(col[r:r + 8], U32))

    def qproj(u, lo=0, hi=gw, parts=1):
        qs = []
        for r0 in range(0, TB, TB // parts):
            q = jnp.dot(h_scr[blk_of(u) & 1, r0:r0 + TB // parts, :], wq_v[grp_of(u), :, lo:hi],
                        preferred_element_type=F32)
            qs.append((q * qscale).astype(BF16))
        return jnp.concatenate(qs, axis=0)

    def qk(u, q, j, toks=(), zero=None):
        k = _tie_rows(k_v[grp_of(u) * HG + j // 2], toks, zero, TLO, sk // 16)
        st = lax.dot_general(k, q[:, j * DH:(j + 1) * DH], _NT,
                             preferred_element_type=F32)
        for i in range(nb):
            blk = st[:, i * LANES:(i + 1) * LANES]
            st_scr[j * nb + i] = blk
            m_scr[j * nb + i] = jnp.max(blk, axis=0, keepdims=True)

    def v_transpose(u, i, marks=None):
        vt = pltpu.bitcast(v_v[grp_of(u) * HG + i].T, U32)
        vt_scr[i] = vt
        if marks is not None:
            step = sk // NVT
            for c in range(step - LANES, sk, step):
                marks.append(vt[DH // 2 - 8:DH // 2, c:c + LANES])

    def pv(slots, zero, toks=()):
        ps, ls, pairs = [], [], []
        for sl in slots:
            p = jnp.exp2(st_scr[sl] - m_scr[sl])
            accs = [None] * 4
            for tile in range(nt):
                for r0 in range(tile * LANES + LANES - 16, tile * LANES - 16, -16):
                    pair = p[r0:r0 + 8] + p[r0 + 8:r0 + 16]
                    pairs.append(pair)
                    a = accs[tile % 4]
                    accs[tile % 4] = pair if a is None else a + pair
            ls.append(jnp.sum((accs[0] + accs[1]) + (accs[2] + accs[3]), axis=0, keepdims=True))
            ps.append(p.astype(BF16))
        outs = []
        ntiles = len(slots) * nt
        side = {}
        for i, tok in enumerate(toks):
            side.setdefault(((i + 1) * ntiles) // len(toks) - 1, []).append(tok)
        for i, sl in enumerate(slots):
            vu = vt_scr[sl // (2 * nb)]
            tiles = []
            for c in range(nt):
                g = i * nt + c + 4
                rows = []
                for r in range(8):
                    x = vu[8 * r:8 * r + 8, c * LANES:(c + 1) * LANES]
                    if g < ntiles and TIE0 <= r < TIE0 + NTIE:
                        src = pairs[g * 8 + (r - TIE0)]
                        x = x | (lax.bitcast_convert_type(src, U32) & zero)
                    if r == SIDE_ROW:
                        for tok in side.get(i * nt + c, ()):
                            x = x | (tok & zero)
                    rows.append(x)
                tiles.append(jnp.concatenate(rows, axis=0))
            lhs = pltpu.bitcast(jnp.concatenate(tiles, axis=1), BF16)
            o = jnp.dot(lhs, ps[i], preferred_element_type=F32)
            outs.append((o * (1.0 / ls[i])).astype(BF16))
        return outs

    def outproj(u, o, lo=0):
        w = len(o) // nq
        o2 = jnp.concatenate(
            [jnp.concatenate(o[j * w:(j + 1) * w], axis=1) for j in range(nq)], axis=0)
        contrib = jnp.dot(wot_v[grp_of(u)], o2, preferred_element_type=F32)
        hi = lo + w * LANES
        slot = blk_of(u) & 1
        old = jnp.where(grp_of(u) > 0, acc_scr[slot, :, lo:hi], 0.0)
        acc_scr[slot, :, lo:hi] = old + contrib

    def finalize(t0, slot, a0, dst, n):
        marks = []
        cs = _span(dst, n)
        x = xt_v[:, _span(t0, n)].astype(F32)
        att = acc_scr[slot, :, _span(a0, n)]
        x1b = (x + _lanes(col_scr[0:d, :], n) * att).astype(BF16)
        x1_scr[:, cs] = x1b
        ot_v[:, cs] = x1b
        mu = _colsum(x1b.astype(F32), marks, NF1) * (1.0 / d)
        mub = _rb(mu)
        xc = x1_scr[:, cs].astype(F32) - mub
        var = _colsum(xc * xc, marks, NF2) * (1.0 / d) - (mu - mub) * (mu - mub)
        inv = 1.0 / _rb(jnp.sqrt(_rb(_rb(jnp.maximum(var, 0.0)) + EPS)))
        step = d // NF3
        racc = None
        for r0 in range(0, d, step):
            rs = slice(r0, r0 + step)
            x1 = ot_v[rs, cs].astype(F32)
            h2b = ((x1 - mub) * inv * _lanes(col_scr[2 * d + r0:2 * d + r0 + step, :], n)
                   + _lanes(col_scr[d + r0:d + r0 + step, :], n)).astype(BF16)
            h2_scr[rs, cs] = h2b
            h2 = h2b.astype(F32)
            out = x1 + _lanes(col_scr[3 * d + r0:3 * d + r0 + step, :], n) * h2
            ot_v[rs, cs] = out.astype(BF16)
            rp = h2 * _lanes(col_scr[4 * d + r0:4 * d + r0 + step, :], n)
            for g in range(0, step, 8):
                racc = rp[g:g + 8] if racc is None else racc + rp[g:g + 8]
            marks.append(_fold(racc) | _fold(out))
        r = _rb(jnp.sum(racc, axis=0, keepdims=True)) + 0.0
        bits = lax.bitcast_convert_type(r, I32) >> 16
        order = jnp.where(bits < 0, -1 - bits, bits + 32768)
        pos = t0 + lax.broadcasted_iota(I32, (1, n), 1)
        key = lax.bitcast_convert_type((order << 11) + (seq - 1 - pos) + 0x20000000, F32)
        for i in range(n // LANES):
            key_scr[pl.ds(dst // LANES + i, 1), :] = key[:, i * LANES:(i + 1) * LANES]
        return marks

    hw = gw // 2
    wq0a = pltpu.make_async_copy(wq_hbm.at[:, 0:hw], wq_v.at[0, :, 0:hw], grp_sems.at[0, 0])
    wq0b = pltpu.make_async_copy(wq_hbm.at[:, hw:gw], wq_v.at[0, :, hw:gw], misc_sems.at[4])
    k0a = pltpu.make_async_copy(k_hbm.at[0], k_v.at[0], grp_sems.at[1, 0])
    k0b = pltpu.make_async_copy(k_hbm.at[1], k_v.at[1], misc_sems.at[5])
    v0 = pltpu.make_async_copy(v_hbm.at[0:HG], v_v.at[0:HG], grp_sems.at[2, 0])
    wo0 = pltpu.make_async_copy(wot_hbm.at[:, 0:gw], wot_v.at[0], grp_sems.at[3, 0])
    wq1, k1, v1, wo1 = grp_copies(1)
    c_copy = pltpu.make_async_copy(c_hbm, c_ref, misc_sems.at[6])
    wr_copy = pltpu.make_async_copy(wr_hbm, wr_ref, misc_sems.at[7])
    c_copy.start()
    wr_copy.start()
    x_first.start()
    mod_first[0].start()
    mod_first[1].start()
    wq0a.start()
    acc_scr[1] = jnp.zeros((d, TB), F32)
    col_scr[0:4 * d, :] = jnp.zeros((4 * d, LANES), F32)
    with _scope("w_x"):
        c_copy.wait()
        wr_copy.wait()
        x_first.wait()
    cbits = lax.bitcast_convert_type(c_ref[:, 0:LANES].astype(F32), U32)
    zero_scr[...] = jnp.broadcast_to(cbits & 0xFFFF, (8, LANES))
    h_scr[0] = ln1_norm(0, TB, [])
    sc = silu_c()
    wr = wr_ref[...].reshape(1, d).astype(F32)
    col_scr[4 * d:5 * d, :] = jnp.broadcast_to(wr, (LANES, d)).T
    col_scr[5 * d:6 * d, :] = jnp.broadcast_to(sc[0:1, :].astype(F32), (LANES, d)).T
    with _scope("w_wmod"):
        mod_first[0].wait()
    mod = jnp.dot(sc[:, 0:MODR], wmod_v[0:MODR, 0:2 * d], preferred_element_type=F32)
    with _scope("w_wmod2"):
        mod_first[1].wait()
    wq0b.start()
    k0a.start()
    k0b.start(priority=1)
    v0.start(priority=1)
    mod = _rb(mod + jnp.dot(sc[:, MODR:d], wmod_v[MODR:d, 0:2 * d], preferred_element_type=F32))
    mod_scr[0:1, :] = mod[0:1, 0:d]
    mod_scr[1:2, :] = _rb(1.0 + mod[0:1, d:2 * d])
    with _scope("w_wq"):
        wq0a.wait()
    ln1_mod(h_scr[0], 0, 0, [])
    qa = qproj(0, 0, hw, 2)
    with _scope("w_k"):
        wq0b.wait()
        k0a.wait()
    wq1.start(priority=1)
    k1.start(priority=1)
    q = jnp.concatenate([qa, qproj(0, hw, gw, 2)], axis=1)
    qk(0, q, 0)
    qk(0, q, 1)
    with _scope("w_v"):
        k0b.wait()
        v0.wait()
    v1.start()
    wo0.start()
    with _scope("qk0"):
        zero = zero_scr[...]
        for i in range(HG):
            marks = []
            v_transpose(0, i, marks)
            qk(0, q, nq - HG + i, marks, zero)

    assert n_grp == 8 and HG == 2
    loads = [[wq1, k1, v1, wo0],
             [wo1, *grp_copies(2), mod_rest, x_rest],
             [*grp_copies(3), *grp_copies(4), *grp_copies(5)],
             [*grp_copies(6), *grp_copies(7)],
             [mlp_g, mlp_u, mlp_d]]
    npc = TB // SP
    nmp = 4 * d // MP

    def manage(i):
        for cp in loads[i - 1]:
            cp.wait()
        for cp in loads[i]:
            cp.start()

    def steady(u, carry):
        def manage_u(_, c):
            for i in range(1, len(loads)):
                pl.when(u == i)(functools.partial(manage, i))
            return c

        lax.fori_loop(0, jnp.where(u < len(loads), 1, 0), manage_u, 0)

        with _scope("body"):
            zero = zero_scr[...]
            blk, g = blk_of(u), grp_of(u)
            off = ((g - 1) & (npc - 1)) * SP
            q = qproj(u)
            o = pv(range(0, 2 * nb), zero)
            live = jnp.logical_and(blk > 0, jnp.logical_and(g >= 1, g <= npc))
            t0 = jnp.maximum(blk - 1, 0) * TB + off
            qk(u, q, 0, finalize(t0, (blk + 1) & 1, off, jnp.where(live, t0, seq), SP), zero)
            marks = []
            nxt = jnp.where(u >= 2, jnp.minimum(blk + 1, n_blk - 1), 0)
            ln = ln1_norm(nxt * TB + off, SP, marks)
            ln1_mod(ln, (blk + 1) & 1, off, marks)
            qk(u, q, 1, marks, zero)
            o += pv(range(2 * nb, 4 * nb), zero)
            outproj(u - 1, o)
            marks = []
            v_transpose(u, 0, marks)
            mp = jnp.clip(u - 2, 0, nmp - 1) * MP
            mmarks = []
            mod_piece(jnp.where(u >= 2, 2 * d + mp, 0), mp, mmarks)
            marks = [a | b for a, b in zip(marks, mmarks + [mmarks[-1]] * len(marks))]
            qk(u, q, 2, marks, zero)
            marks = []
            v_transpose(u, 1, marks)
            qk(u, q, 3, marks, zero)
        return carry

    lax.fori_loop(1, n_units, steady, 0)

    ul = n_units - 1
    tl = seq - TB
    sl_last = (n_blk - 1) & 1
    nb0 = nb - TAILB
    out_lo.start()
    mlp_g.wait()
    mlp_u.wait()
    with _scope("e_pva"):
        mod_scr[2:3, :] = row_scr[:, 3 * d:4 * d]
        outproj(ul, pv([j * nb + i for j in range(nq) for i in range(nb0)], zero_scr[...]))
    mlp_d.wait()
    with _scope("e_pvb"):
        toks = finalize(tl, sl_last, 0, tl, nb0 * LANES)
        o = pv([j * nb + i for j in range(nq) for i in range(nb0, nb)], zero_scr[...], toks)
        outproj(ul, o, nb0 * LANES)
        finalize(tl + nb0 * LANES, sl_last, nb0 * LANES, tl + nb0 * LANES, TAILB * LANES)

    keys = key_scr[0:seq // LANES, :]
    sub8 = lax.broadcasted_iota(I32, (TOPC, 1), 0)
    lane = lax.broadcasted_iota(I32, (TOPC, LANES), 1)
    top = jnp.zeros((TOPC, 1), F32)
    bases, idxs = [], []
    h2s = jnp.zeros((TOPC, d), F32)
    x1s = jnp.zeros((TOPC, d), F32)
    for i in range(TOPC):
        mx = jnp.max(jnp.max(keys, axis=0, keepdims=True), axis=1, keepdims=True)
        keys = jnp.where(keys == mx, 0.0, keys)
        top = jnp.where(sub8 == i, mx, top)
        idx = seq - 1 - (lax.bitcast_convert_type(mx, I32) & (seq - 1))
        bases.append(pl.multiple_of(idx[0, 0] & ~(LANES - 1), LANES))
        idxs.append(idx)
        pick = jnp.logical_and(sub8 == i, lane == (idx & (LANES - 1)))
        pick = jnp.where(pick, 1.0, 0.0).astype(BF16)
        sl = pl.ds(bases[i], LANES)
        h2s = h2s + lax.dot_general(pick, h2_scr[:, sl], _NT, preferred_element_type=F32)
        x1s = x1s + lax.dot_general(pick, x1_scr[:, sl], _NT, preferred_element_type=F32)
    order = (lax.bitcast_convert_type(top, I32) >> 11) & 0xFFFF
    rbits = jnp.where(order >= 32768, order - 32768, -1 - order) << 16
    gate = _rb(_sigmoid(lax.bitcast_convert_type(rbits, F32)))
    xs = h2s.astype(BF16)
    for cp in out_hi:
        cp.start()
    g = _rb(jnp.dot(xs, wg_v[...], preferred_element_type=F32))
    g = _rb(g * _rb(_sigmoid(g)))
    u = _rb(jnp.dot(xs, wu_v[...], preferred_element_type=F32))
    gu = (g * u).astype(BF16)

    last_use = []
    for i in range(TOPC):
        ok = True
        for j in range(i + 1, TOPC):
            ok = jnp.logical_and(ok, bases[i] != bases[j])
        last_use.append(ok)

    def down(r0, r1):
        y = _rb(lax.dot_general(gu, wdt_v[r0:r1, :], _NT, preferred_element_type=F32))
        hm = _rb(h2s[:, r0:r1] + _rb(y * gate))
        return x1s[:, r0:r1] + mod_scr[2:3, r0:r1] * hm

    def patch(r0, r1, new):
        n = r1 - r0
        pad = jnp.concatenate([new, jnp.zeros((LANES - TOPC, n), F32)], axis=0)
        cols = pltpu.bitcast(pad.T.astype(BF16), U32)
        col = [jnp.broadcast_to(cols[:, j:j + 1], (n // 2, LANES)) for j in range(TOPC)]
        for i in range(TOPC):
            res = pltpu.bitcast(ot_v[r0:r1, pl.ds(bases[i], LANES)], U32)
            tok = lane[0:1, :] + (idxs[i] & ~(LANES - 1))
            for j in range(i + 1):
                res = jnp.where(tok == idxs[j], col[j], res)
            fix_v[i, r0:r1, :] = pltpu.bitcast(res, BF16)

    def fix_copy(i, r0, r1):
        return pltpu.make_async_copy(fix_v.at[i, r0:r1, :],
                                     o_hbm.at[r0:r1, pl.ds(bases[i], LANES)], fix_sems.at[i])

    def for_last(fn):
        for i in range(TOPC - 1):
            pl.when(last_use[i])(functools.partial(fn, i))
        fn(TOPC - 1)

    new = down(*chunks[0])
    out_lo.wait()
    for ci, (r0, r1) in enumerate(chunks):
        out_hi[ci].wait()
        nxt = down(*chunks[ci + 1]) if ci + 1 < len(chunks) else None
        patch(r0, r1, new)
        for_last(lambda i: fix_copy(i, r0, r1).start())
        new = nxt
    with _scope("w_fix"):
        for r0, r1 in chunks:
            for_last(lambda i: fix_copy(i, r0, r1).wait())


@jax.jit
def pallas_adaLN_cond__gqa_block_cached__moe_arch_mod__prompt_kernel(
    A_x: jax.Array,
    A_k_cache: jax.Array,
    A_v_cache: jax.Array,
    A_wq: jax.Array,
    A_wo: jax.Array,
    B_x: jax.Array,
    B_w_r: jax.Array,
    B_w_gate: jax.Array,
    B_w_up: jax.Array,
    B_w_down: jax.Array,
    c: jax.Array,
    w_mod: jax.Array,
):
    b, seq, d = A_x.shape
    _, hkv, sk, dh = A_k_cache.shape
    assert b == 1 and dh == DH and HQ == 2 * hkv
    assert seq & (seq - 1) == 0 and seq <= 2048
    f = B_w_gate.shape[1]
    n_grp = hkv // HG
    gw = 2 * HG * dh
    n_slots = 2 * HG * TB // LANES

    xt = A_x.reshape(seq, d).T
    wot = A_wo.T
    wdt = B_w_down.T
    k3 = A_k_cache.reshape(hkv, sk, dh)
    v3 = A_v_cache.reshape(hkv, sk, dh)

    hbm = pl.BlockSpec(memory_space=pl.ANY)
    out_t = pl.pallas_call(
        functools.partial(_kernel, n_heads=hkv),
        in_specs=[hbm] * 11,
        out_specs=hbm,
        out_shape=jax.ShapeDtypeStruct((d, seq), BF16),
        scratch_shapes=[
            pltpu.VMEM((d, seq), BF16),
            pltpu.VMEM((hkv, sk, dh), BF16),
            pltpu.VMEM((hkv, sk, dh), BF16),
            pltpu.VMEM((n_grp, d, gw), BF16),
            pltpu.VMEM((n_grp, d, gw), BF16),
            pltpu.VMEM((d, 6 * d), BF16),
            pltpu.VMEM((d, f), BF16),
            pltpu.VMEM((d, f), BF16),
            pltpu.VMEM((d, f), BF16),
            pltpu.VMEM((d, seq + SP), BF16),
            pltpu.VMEM((2, TB, d), BF16),
            pltpu.VMEM((2, d, TB), F32),
            pltpu.VMEM((n_slots, sk, LANES), F32),
            pltpu.VMEM((n_slots, 1, LANES), F32),
            pltpu.VMEM((HG, dh // 2, sk), U32),
            pltpu.VMEM((8, d), F32),
            pltpu.VMEM((6 * d, LANES), F32),
            pltpu.VMEM(((seq + SP) // LANES + 7 & ~7, LANES), F32),
            pltpu.VMEM((d, seq + SP), BF16),
            pltpu.VMEM((d, seq + SP), BF16),
            pltpu.VMEM((8, LANES), U32),
            pltpu.VMEM((TOPC, d, LANES), BF16),
            pltpu.VMEM((1, d), BF16),
            pltpu.VMEM((d,), BF16),
            pltpu.VMEM((1, 4 * d), F32),
            pltpu.SemaphoreType.DMA((4, n_grp)),
            pltpu.SemaphoreType.DMA((10,)),
            pltpu.SemaphoreType.DMA((3,)),
            pltpu.SemaphoreType.DMA((len(EDGES),)),
            pltpu.SemaphoreType.DMA((TOPC,)),
        ],
        compiler_params=pltpu.CompilerParams(
            disable_bounds_checks=True,
            disable_semaphore_checks=True,
            vmem_limit_bytes=110 * 1024 * 1024,
        ),
    )(xt, k3, v3, A_wq, wot, B_w_r, B_w_gate, B_w_up, wdt, c, w_mod)
    return out_t.T.reshape(b, seq, d)
```

```python
import contextlib
import functools
import math
import os

import jax
import jax.numpy as jnp
from jax import lax
import jax.experimental.pallas as pl
import jax.experimental.pallas.tpu as pltpu

F32 = jnp.float32
BF16 = jnp.bfloat16
I32 = jnp.int32
U32 = jnp.uint32

HQ = 32
DH = 128
TOPC = 8
EPS = 1e-05
LANES = 128

TB = 512
HG = 2
TIE0 = int(os.environ.get("KP_TIE0", "2"))
NTIE = int(os.environ.get("KP_NTIE", "3"))
SP = int(os.environ.get("KP_SP", "128"))
NM1 = int(os.environ.get("KP_NM1", "8"))
NM2 = int(os.environ.get("KP_NM2", "12"))
NM3 = int(os.environ.get("KP_NM3", "16"))
TLO = int(os.environ.get("KP_TLO", "8"))
NF1 = int(os.environ.get("KP_NF1", "9"))
NF2 = int(os.environ.get("KP_NF2", "6"))
NF3 = int(os.environ.get("KP_NF3", "18"))
NVT = int(os.environ.get("KP_NVT", "16"))
TAILB = int(os.environ.get("KP_TAILB", "2"))
SIDE_ROW = int(os.environ.get("KP_SIDE_ROW", "6"))
EDGES = [int(e) for e in os.environ.get("KP_EDGES", "0,128,256,384,512,576").split(",")]
MODR = int(os.environ.get("KP_MODR", "384"))
MP = int(os.environ.get("KP_MP", "384"))
NMP = int(os.environ.get("KP_NMP", "12"))
WP = 256
SCOPES = os.environ.get("KP_SCOPES", "") == "1"

_NT = (((1,), (1,)), ((), ()))


def _rb(x):
    return x.astype(BF16).astype(F32)


def _sigmoid(x):
    return 1.0 / (1.0 + jnp.exp(-x))


def _lanes(col, width):
    reps = width // LANES
    return col if reps == 1 else jnp.concatenate([col] * reps, axis=1)


def _fold(x):
    xi = lax.bitcast_convert_type(x, U32)
    tok = None
    for r in range(0, x.shape[0], 8):
        for c in range(0, x.shape[1] - LANES + 1, LANES):
            t = xi[r:r + 8, c:c + LANES]
            tok = t if tok is None else tok | t
    return tok


def _colsum(x, marks, nmarks):
    n = x.shape[0] // 8
    acc = x[0:8]
    for g in range(1, n):
        acc = acc + x[8 * g:8 * g + 8]
        if ((g + 1) * nmarks) % n == 0:
            marks.append(_fold(acc))
    return jnp.sum(acc, axis=0, keepdims=True)


def _tie_rows(lhs, toks, zero, lo, hi):
    if not toks:
        return lhs
    lu = pltpu.bitcast(lhs, U32)
    rows = [lu[8 * r:8 * r + 8] for r in range(lu.shape[0] // 8)]
    for i, tok in enumerate(toks):
        r = lo + ((i + 1) * (hi - lo)) // len(toks) - 1
        rows[r] = rows[r] | (tok & zero)
    return pltpu.bitcast(jnp.concatenate(rows, axis=0), BF16)


def _merge(a, b):
    keyed = [((i + 1) / len(a), t) for i, t in enumerate(a)]
    keyed += [((i + 1) / len(b), t) for i, t in enumerate(b)]
    return [t for _, t in sorted(keyed, key=lambda kv: kv[0])]


def _span(start, size):
    if isinstance(start, int):
        return pl.ds(start, size)
    return pl.ds(pl.multiple_of(start, LANES), size)


def _scope(name):
    return jax.named_scope(name) if SCOPES else contextlib.nullcontext()


def _kernel(xt_hbm, k_hbm, v_hbm, wq_hbm, wot_hbm, wr_hbm, wg_hbm, wu_hbm, wdt_hbm,
            c_hbm, wmod_hbm, o_hbm,
            xt_v, k_v, v_v, wq_v, wot_v, wmod_v, wg_v, wu_v, wdt_v, ot_v,
            h_scr, acc_scr, st_scr, m_scr, vt_scr, mod_scr, col_scr, key_scr, h2_scr, x1_scr,
            zero_scr, fix_v, c_ref, wr_ref, row_scr, wd_scr,
            grp_sems, misc_sems, mlp_sems, out_sems, fix_sems,
            *, n_heads):
    d, seq = xt_v.shape
    sk = k_v.shape[1]
    n_grp = n_heads // HG
    n_blk = seq // TB
    n_units = n_grp * n_blk
    nb = TB // LANES
    nq = 2 * HG
    nt = sk // LANES
    gbits = n_grp.bit_length() - 1
    gw = nq * DH
    qscale = (DH ** -0.5) * math.log2(math.e)

    def grp_of(u):
        return u & (n_grp - 1)

    def blk_of(u):
        return u >> gbits

    def grp_copies(g):
        cs, hs = pl.ds(g * gw, gw), pl.ds(g * HG, HG)
        return (pltpu.make_async_copy(wq_hbm.at[:, cs], wq_v.at[g], grp_sems.at[0, g]),
                pltpu.make_async_copy(k_hbm.at[hs], k_v.at[hs], grp_sems.at[1, g]),
                pltpu.make_async_copy(v_hbm.at[hs], v_v.at[hs], grp_sems.at[2, g]),
                pltpu.make_async_copy(wot_hbm.at[:, cs], wot_v.at[g], grp_sems.at[3, g]))

    def col_copy(src, dst, lo, hi, sem):
        return pltpu.make_async_copy(src.at[:, lo:hi], dst.at[:, lo:hi], sem)

    x_first = col_copy(xt_hbm, xt_v, 0, TB, misc_sems.at[0])
    x_rest = col_copy(xt_hbm, xt_v, TB, seq, misc_sems.at[1])
    mod_rows = [(0, MODR), (MODR, d)]
    mod_first = [pltpu.make_async_copy(wmod_hbm.at[r0:r1, 0:2 * d], wmod_v.at[r0:r1, 0:2 * d],
                                       misc_sems.at[8 + i]) for i, (r0, r1) in enumerate(mod_rows)]
    mod_rest = col_copy(wmod_hbm, wmod_v, 2 * d, 6 * d, misc_sems.at[3])
    mlp_g = pltpu.make_async_copy(wg_hbm, wg_v, mlp_sems.at[0])
    mlp_u = pltpu.make_async_copy(wu_hbm, wu_v, mlp_sems.at[1])
    ff = wdt_hbm.shape[1]
    mlp_d = pltpu.make_async_copy(wdt_hbm, wdt_v.at[:, 0:ff], mlp_sems.at[2])
    out_lo = col_copy(ot_v, o_hbm, 0, seq - TB, out_sems.at[0])
    chunks = list(zip(EDGES[:-1], EDGES[1:]))
    out_hi = [pltpu.make_async_copy(ot_v.at[r0:r1, seq - TB:seq], o_hbm.at[r0:r1, seq - TB:seq],
                                    out_sems.at[1 + i]) for i, (r0, r1) in enumerate(chunks)]

    def silu_c():
        cc = c_ref[...].astype(F32)
        return jnp.broadcast_to((cc * _rb(_sigmoid(cc))).astype(BF16), (8, d))

    def ln1_norm(t0, n, marks):
        x = xt_v[:, _span(t0, n)].astype(F32)
        mu = _colsum(x, marks, NM1) * (1.0 / d)
        xc = x - mu
        var = _colsum(xc * xc, marks, NM2) * (1.0 / d)
        return (xc * lax.rsqrt(var + EPS)).astype(BF16).T

    def ln1_mod(ln, slot, r0, marks):
        n = ln.shape[0]
        h = ln.astype(F32) * mod_scr[1:2, :] + mod_scr[0:1, :]
        h_scr[slot, _span(r0, n), :] = h.astype(BF16)
        step = max(n // NM3, 8)
        for r in range(step - 8, n, step):
            marks.append(_fold(h[r:r + 8]))

    def mod_piece(src, dst, marks):
        w = wmod_v[:, _span(src, MP)].astype(F32)
        row = _rb(_colsum(w * _lanes(col_scr[5 * d:6 * d, :], MP), marks, NMP))
        pos = dst + lax.broadcasted_iota(I32, (1, MP), 1)
        is_cb = jnp.logical_and(pos >= 2 * d, pos < 3 * d)
        row = jnp.where(is_cb, _rb(1.0 + row), row)
        row_scr[:, _span(dst, MP)] = row
        col = jnp.broadcast_to(row, (LANES, MP)).T
        col_scr[_span(dst, MP), :] = col
        for r in range(LANES - 8, MP, LANES):
            marks.append(lax.bitcast_convert_type(col[r:r + 8], U32))

    def wd_piece(src, dst, marks):
        w = pltpu.bitcast(wdt_v[:, _span(src, WP)].T, U32)
        wd_scr[pl.ds(pl.multiple_of(dst // 2, WP // 2), WP // 2), :] = w
        for r in range(56, WP // 2, 64):
            for c in range(0, d - LANES + 1, LANES):
                marks.append(w[r:r + 8, c:c + LANES])

    def qproj(u, lo=0, hi=gw, parts=1):
        qs = []
        for r0 in range(0, TB, TB // parts):
            q = jnp.dot(h_scr[blk_of(u) & 1, r0:r0 + TB // parts, :], wq_v[grp_of(u), :, lo:hi],
                        preferred_element_type=F32)
            qs.append((q * qscale).astype(BF16))
        return jnp.concatenate(qs, axis=0)

    def qk(u, q, j, toks=(), zero=None):
        k = _tie_rows(k_v[grp_of(u) * HG + j // 2], toks, zero, TLO, sk // 16)
        st = lax.dot_general(k, q[:, j * DH:(j + 1) * DH], _NT,
                             preferred_element_type=F32)
        for i in range(nb):
            blk = st[:, i * LANES:(i + 1) * LANES]
            st_scr[j * nb + i] = blk
            m_scr[j * nb + i] = jnp.max(blk, axis=0, keepdims=True)

    def v_transpose(u, i, marks=None):
        vt = pltpu.bitcast(v_v[grp_of(u) * HG + i].T, U32)
        vt_scr[i] = vt
        if marks is not None:
            step = sk // NVT
            for c in range(step - LANES, sk, step):
                marks.append(vt[DH // 2 - 8:DH // 2, c:c + LANES])

    def pv(slots, zero, toks=()):
        ps, ls, pairs = [], [], []
        for sl in slots:
            p = jnp.exp2(st_scr[sl] - m_scr[sl])
            accs = [None] * 4
            for tile in range(nt):
                for r0 in range(tile * LANES + LANES - 16, tile * LANES - 16, -16):
                    pair = p[r0:r0 + 8] + p[r0 + 8:r0 + 16]
                    pairs.append(pair)
                    a = accs[tile % 4]
                    accs[tile % 4] = pair if a is None else a + pair
            ls.append(jnp.sum((accs[0] + accs[1]) + (accs[2] + accs[3]), axis=0, keepdims=True))
            ps.append(p.astype(BF16))
        outs = []
        ntiles = len(slots) * nt
        side = {}
        for i, tok in enumerate(toks):
            side.setdefault(((i + 1) * ntiles) // len(toks) - 1, []).append(tok)
        for i, sl in enumerate(slots):
            vu = vt_scr[sl // (2 * nb)]
            tiles = []
            for c in range(nt):
                g = i * nt + c + 4
                rows = []
                for r in range(8):
                    x = vu[8 * r:8 * r + 8, c * LANES:(c + 1) * LANES]
                    if g < ntiles and TIE0 <= r < TIE0 + NTIE:
                        src = pairs[g * 8 + (r - TIE0)]
                        x = x | (lax.bitcast_convert_type(src, U32) & zero)
                    if r == SIDE_ROW:
                        for tok in side.get(i * nt + c, ()):
                            x = x | (tok & zero)
                    rows.append(x)
                tiles.append(jnp.concatenate(rows, axis=0))
            lhs = pltpu.bitcast(jnp.concatenate(tiles, axis=1), BF16)
            o = jnp.dot(lhs, ps[i], preferred_element_type=F32)
            outs.append((o * (1.0 / ls[i])).astype(BF16))
        return outs

    def outproj(u, o, lo=0):
        w = len(o) // nq
        o2 = jnp.concatenate(
            [jnp.concatenate(o[j * w:(j + 1) * w], axis=1) for j in range(nq)], axis=0)
        contrib = jnp.dot(wot_v[grp_of(u)], o2, preferred_element_type=F32)
        hi = lo + w * LANES
        slot = blk_of(u) & 1
        old = jnp.where(grp_of(u) > 0, acc_scr[slot, :, lo:hi], 0.0)
        acc_scr[slot, :, lo:hi] = old + contrib

    def finalize(t0, slot, a0, dst, n):
        marks = []
        cs = _span(dst, n)
        x = xt_v[:, _span(t0, n)].astype(F32)
        att = acc_scr[slot, :, _span(a0, n)]
        x1b = (x + _lanes(col_scr[0:d, :], n) * att).astype(BF16)
        x1_scr[:, cs] = x1b
        ot_v[:, cs] = x1b
        mu = _colsum(x1b.astype(F32), marks, NF1) * (1.0 / d)
        mub = _rb(mu)
        xc = x1_scr[:, cs].astype(F32) - mub
        var = _colsum(xc * xc, marks, NF2) * (1.0 / d) - (mu - mub) * (mu - mub)
        inv = 1.0 / _rb(jnp.sqrt(_rb(_rb(jnp.maximum(var, 0.0)) + EPS)))
        step = d // NF3
        racc = None
        for r0 in range(0, d, step):
            rs = slice(r0, r0 + step)
            x1 = ot_v[rs, cs].astype(F32)
            h2b = ((x1 - mub) * inv * _lanes(col_scr[2 * d + r0:2 * d + r0 + step, :], n)
                   + _lanes(col_scr[d + r0:d + r0 + step, :], n)).astype(BF16)
            h2_scr[rs, cs] = h2b
            h2 = h2b.astype(F32)
            out = x1 + _lanes(col_scr[3 * d + r0:3 * d + r0 + step, :], n) * h2
            ot_v[rs, cs] = out.astype(BF16)
            rp = h2 * _lanes(col_scr[4 * d + r0:4 * d + r0 + step, :], n)
            for g in range(0, step, 8):
                racc = rp[g:g + 8] if racc is None else racc + rp[g:g + 8]
            marks.append(_fold(racc) | _fold(out))
        r = _rb(jnp.sum(racc, axis=0, keepdims=True)) + 0.0
        bits = lax.bitcast_convert_type(r, I32) >> 16
        order = jnp.where(bits < 0, -1 - bits, bits + 32768)
        pos = t0 + lax.broadcasted_iota(I32, (1, n), 1)
        key = lax.bitcast_convert_type((order << 11) + (seq - 1 - pos) + 0x20000000, F32)
        for i in range(n // LANES):
            key_scr[pl.ds(dst // LANES + i, 1), :] = key[:, i * LANES:(i + 1) * LANES]
        return marks

    hw = gw // 2
    wq0a = pltpu.make_async_copy(wq_hbm.at[:, 0:hw], wq_v.at[0, :, 0:hw], grp_sems.at[0, 0])
    wq0b = pltpu.make_async_copy(wq_hbm.at[:, hw:gw], wq_v.at[0, :, hw:gw], misc_sems.at[4])
    k0a = pltpu.make_async_copy(k_hbm.at[0], k_v.at[0], grp_sems.at[1, 0])
    k0b = pltpu.make_async_copy(k_hbm.at[1], k_v.at[1], misc_sems.at[5])
    v0 = pltpu.make_async_copy(v_hbm.at[0:HG], v_v.at[0:HG], grp_sems.at[2, 0])
    wo0 = pltpu.make_async_copy(wot_hbm.at[:, 0:gw], wot_v.at[0], grp_sems.at[3, 0])
    wq1, k1, v1, wo1 = grp_copies(1)
    c_copy = pltpu.make_async_copy(c_hbm, c_ref, misc_sems.at[6])
    wr_copy = pltpu.make_async_copy(wr_hbm, wr_ref, misc_sems.at[7])
    c_copy.start()
    wr_copy.start()
    x_first.start()
    mod_first[0].start()
    mod_first[1].start()
    wq0a.start()
    acc_scr[1] = jnp.zeros((d, TB), F32)
    col_scr[0:4 * d, :] = jnp.zeros((4 * d, LANES), F32)
    wdt_v[:, ff:ff + WP] = jnp.zeros((d, WP), BF16)
    with _scope("w_x"):
        c_copy.wait()
        wr_copy.wait()
        x_first.wait()
    cbits = lax.bitcast_convert_type(c_ref[:, 0:LANES].astype(F32), U32)
    zero_scr[...] = jnp.broadcast_to(cbits & 0xFFFF, (8, LANES))
    h_scr[0] = ln1_norm(0, TB, [])
    sc = silu_c()
    wr = wr_ref[...].reshape(1, d).astype(F32)
    col_scr[4 * d:5 * d, :] = jnp.broadcast_to(wr, (LANES, d)).T
    col_scr[5 * d:6 * d, :] = jnp.broadcast_to(sc[0:1, :].astype(F32), (LANES, d)).T
    with _scope("w_wmod"):
        mod_first[0].wait()
    mod = jnp.dot(sc[:, 0:MODR], wmod_v[0:MODR, 0:2 * d], preferred_element_type=F32)
    with _scope("w_wmod2"):
        mod_first[1].wait()
    wq0b.start()
    k0a.start()
    k0b.start(priority=1)
    v0.start(priority=1)
    mod = _rb(mod + jnp.dot(sc[:, MODR:d], wmod_v[MODR:d, 0:2 * d], preferred_element_type=F32))
    mod_scr[0:1, :] = mod[0:1, 0:d]
    mod_scr[1:2, :] = _rb(1.0 + mod[0:1, d:2 * d])
    with _scope("w_wq"):
        wq0a.wait()
    ln1_mod(h_scr[0], 0, 0, [])
    qa = qproj(0, 0, hw, 2)
    with _scope("w_k"):
        wq0b.wait()
        k0a.wait()
    wq1.start(priority=1)
    k1.start(priority=1)
    q = jnp.concatenate([qa, qproj(0, hw, gw, 2)], axis=1)
    qk(0, q, 0)
    qk(0, q, 1)
    with _scope("w_v"):
        k0b.wait()
        v0.wait()
    v1.start()
    wo0.start()
    with _scope("qk0"):
        zero = zero_scr[...]
        for i in range(HG):
            marks = []
            v_transpose(0, i, marks)
            qk(0, q, nq - HG + i, marks, zero)

    assert n_grp == 8 and HG == 2
    loads = [[wq1, k1, v1, wo0],
             [wo1, *grp_copies(2), mod_rest, x_rest],
             [*grp_copies(3), *grp_copies(4), *grp_copies(5)],
             [*grp_copies(6), *grp_copies(7)],
             [mlp_d],
             [mlp_g, mlp_u]]
    wd0 = len(loads) - 1
    npc = TB // SP
    nmp = 4 * d // MP

    def manage(i):
        for cp in loads[i - 1]:
            cp.wait()
        for cp in loads[i]:
            cp.start()

    def steady(u, carry):
        def manage_u(_, c):
            for i in range(1, len(loads)):
                pl.when(u == i)(functools.partial(manage, i))
            return c

        lax.fori_loop(0, jnp.where(u < len(loads), 1, 0), manage_u, 0)

        with _scope("body"):
            zero = zero_scr[...]
            blk, g = blk_of(u), grp_of(u)
            off = ((g - 1) & (npc - 1)) * SP
            q = qproj(u)
            o = pv(range(0, 2 * nb), zero)
            live = jnp.logical_and(blk > 0, jnp.logical_and(g >= 1, g <= npc))
            t0 = jnp.maximum(blk - 1, 0) * TB + off
            marks = finalize(t0, (blk + 1) & 1, off, jnp.where(live, t0, seq), SP)
            wp = jnp.clip(u - wd0, 0, ff // WP - 1) * WP
            wmarks = []
            wd_piece(jnp.where(u >= wd0, wp, ff), wp, wmarks)
            qk(u, q, 0, _merge(marks, wmarks), zero)
            marks = []
            nxt = jnp.where(u >= 2, jnp.minimum(blk + 1, n_blk - 1), 0)
            ln = ln1_norm(nxt * TB + off, SP, marks)
            ln1_mod(ln, (blk + 1) & 1, off, marks)
            qk(u, q, 1, marks, zero)
            o += pv(range(2 * nb, 4 * nb), zero)
            outproj(u - 1, o)
            marks = []
            v_transpose(u, 0, marks)
            mp = jnp.clip(u - 2, 0, nmp - 1) * MP
            mmarks = []
            mod_piece(jnp.where(u >= 2, 2 * d + mp, 0), mp, mmarks)
            qk(u, q, 2, _merge(marks, mmarks), zero)
            marks = []
            v_transpose(u, 1, marks)
            qk(u, q, 3, marks, zero)
        return carry

    lax.fori_loop(1, n_units, steady, 0)

    ul = n_units - 1
    tl = seq - TB
    sl_last = (n_blk - 1) & 1
    nb0 = nb - TAILB
    out_lo.start()
    mlp_g.wait()
    with _scope("e_pva"):
        mod_scr[2:3, :] = row_scr[:, 3 * d:4 * d]
        outproj(ul, pv([j * nb + i for j in range(nq) for i in range(nb0)], zero_scr[...]))
    mlp_u.wait()
    with _scope("e_pvb"):
        toks = finalize(tl, sl_last, 0, tl, nb0 * LANES)
        o = pv([j * nb + i for j in range(nq) for i in range(nb0, nb)], zero_scr[...], toks)
        outproj(ul, o, nb0 * LANES)
        finalize(tl + nb0 * LANES, sl_last, nb0 * LANES, tl + nb0 * LANES, TAILB * LANES)

    keys = key_scr[0:seq // LANES, :]
    sub8 = lax.broadcasted_iota(I32, (TOPC, 1), 0)
    lane = lax.broadcasted_iota(I32, (TOPC, LANES), 1)
    top = jnp.zeros((TOPC, 1), F32)
    bases, idxs = [], []
    h2s = jnp.zeros((TOPC, d), F32)
    x1s = jnp.zeros((TOPC, d), F32)
    for i in range(TOPC):
        mx = jnp.max(jnp.max(keys, axis=0, keepdims=True), axis=1, keepdims=True)
        keys = jnp.where(keys == mx, 0.0, keys)
        top = jnp.where(sub8 == i, mx, top)
        idx = seq - 1 - (lax.bitcast_convert_type(mx, I32) & (seq - 1))
        bases.append(pl.multiple_of(idx[0, 0] & ~(LANES - 1), LANES))
        idxs.append(idx)
        pick = jnp.logical_and(sub8 == i, lane == (idx & (LANES - 1)))
        pick = jnp.where(pick, 1.0, 0.0).astype(BF16)
        sl = pl.ds(bases[i], LANES)
        h2s = h2s + lax.dot_general(pick, h2_scr[:, sl], _NT, preferred_element_type=F32)
        x1s = x1s + lax.dot_general(pick, x1_scr[:, sl], _NT, preferred_element_type=F32)
    order = (lax.bitcast_convert_type(top, I32) >> 11) & 0xFFFF
    rbits = jnp.where(order >= 32768, order - 32768, -1 - order) << 16
    gate = _rb(_sigmoid(lax.bitcast_convert_type(rbits, F32)))
    xs = h2s.astype(BF16)
    for cp in out_hi:
        cp.start()
    g = _rb(jnp.dot(xs, wg_v[...], preferred_element_type=F32))
    g = _rb(g * _rb(_sigmoid(g)))
    u = _rb(jnp.dot(xs, wu_v[...], preferred_element_type=F32))
    gu = (g * u).astype(BF16)

    last_use = []
    for i in range(TOPC):
        ok = True
        for j in range(i + 1, TOPC):
            ok = jnp.logical_and(ok, bases[i] != bases[j])
        last_use.append(ok)

    def down(r0, r1):
        wd = pltpu.bitcast(wd_scr[:, r0:r1], BF16)
        y = _rb(jnp.dot(gu, wd, preferred_element_type=F32))
        hm = _rb(h2s[:, r0:r1] + _rb(y * gate))
        return x1s[:, r0:r1] + mod_scr[2:3, r0:r1] * hm

    def patch(r0, r1, new):
        n = r1 - r0
        pad = jnp.concatenate([new, jnp.zeros((LANES - TOPC, n), F32)], axis=0)
        cols = pltpu.bitcast(pad.T.astype(BF16), U32)
        col = [jnp.broadcast_to(cols[:, j:j + 1], (n // 2, LANES)) for j in range(TOPC)]
        for i in range(TOPC):
            res = pltpu.bitcast(ot_v[r0:r1, pl.ds(bases[i], LANES)], U32)
            tok = lane[0:1, :] + (idxs[i] & ~(LANES - 1))
            for j in range(i + 1):
                res = jnp.where(tok == idxs[j], col[j], res)
            fix_v[i, r0:r1, :] = pltpu.bitcast(res, BF16)

    def fix_copy(i, r0, r1):
        return pltpu.make_async_copy(fix_v.at[i, r0:r1, :],
                                     o_hbm.at[r0:r1, pl.ds(bases[i], LANES)], fix_sems.at[i])

    def for_last(fn):
        for i in range(TOPC - 1):
            pl.when(last_use[i])(functools.partial(fn, i))
        fn(TOPC - 1)

    new = down(*chunks[0])
    out_lo.wait()
    for ci, (r0, r1) in enumerate(chunks):
        out_hi[ci].wait()
        nxt = down(*chunks[ci + 1]) if ci + 1 < len(chunks) else None
        patch(r0, r1, new)
        for_last(lambda i: fix_copy(i, r0, r1).start())
        new = nxt
    with _scope("w_fix"):
        for r0, r1 in chunks:
            for_last(lambda i: fix_copy(i, r0, r1).wait())


@jax.jit
def pallas_adaLN_cond__gqa_block_cached__moe_arch_mod__prompt_kernel(
    A_x: jax.Array,
    A_k_cache: jax.Array,
    A_v_cache: jax.Array,
    A_wq: jax.Array,
    A_wo: jax.Array,
    B_x: jax.Array,
    B_w_r: jax.Array,
    B_w_gate: jax.Array,
    B_w_up: jax.Array,
    B_w_down: jax.Array,
    c: jax.Array,
    w_mod: jax.Array,
):
    b, seq, d = A_x.shape
    _, hkv, sk, dh = A_k_cache.shape
    assert b == 1 and dh == DH and HQ == 2 * hkv
    assert seq & (seq - 1) == 0 and seq <= 2048
    f = B_w_gate.shape[1]
    n_grp = hkv // HG
    gw = 2 * HG * dh
    n_slots = 2 * HG * TB // LANES

    xt = A_x.reshape(seq, d).T
    wot = A_wo.T
    wdt = B_w_down.T
    k3 = A_k_cache.reshape(hkv, sk, dh)
    v3 = A_v_cache.reshape(hkv, sk, dh)

    hbm = pl.BlockSpec(memory_space=pl.ANY)
    out_t = pl.pallas_call(
        functools.partial(_kernel, n_heads=hkv),
        in_specs=[hbm] * 11,
        out_specs=hbm,
        out_shape=jax.ShapeDtypeStruct((d, seq), BF16),
        scratch_shapes=[
            pltpu.VMEM((d, seq), BF16),
            pltpu.VMEM((hkv, sk, dh), BF16),
            pltpu.VMEM((hkv, sk, dh), BF16),
            pltpu.VMEM((n_grp, d, gw), BF16),
            pltpu.VMEM((n_grp, d, gw), BF16),
            pltpu.VMEM((d, 6 * d), BF16),
            pltpu.VMEM((d, f), BF16),
            pltpu.VMEM((d, f), BF16),
            pltpu.VMEM((d, f + WP), BF16),
            pltpu.VMEM((d, seq + SP), BF16),
            pltpu.VMEM((2, TB, d), BF16),
            pltpu.VMEM((2, d, TB), F32),
            pltpu.VMEM((n_slots, sk, LANES), F32),
            pltpu.VMEM((n_slots, 1, LANES), F32),
            pltpu.VMEM((HG, dh // 2, sk), U32),
            pltpu.VMEM((8, d), F32),
            pltpu.VMEM((6 * d, LANES), F32),
            pltpu.VMEM(((seq + SP) // LANES + 7 & ~7, LANES), F32),
            pltpu.VMEM((d, seq + SP), BF16),
            pltpu.VMEM((d, seq + SP), BF16),
            pltpu.VMEM((8, LANES), U32),
            pltpu.VMEM((TOPC, d, LANES), BF16),
            pltpu.VMEM((1, d), BF16),
            pltpu.VMEM((d,), BF16),
            pltpu.VMEM((1, 4 * d), F32),
            pltpu.VMEM((f // 2, d), U32),
            pltpu.SemaphoreType.DMA((4, n_grp)),
            pltpu.SemaphoreType.DMA((10,)),
            pltpu.SemaphoreType.DMA((3,)),
            pltpu.SemaphoreType.DMA((len(EDGES),)),
            pltpu.SemaphoreType.DMA((TOPC,)),
        ],
        compiler_params=pltpu.CompilerParams(
            disable_bounds_checks=True,
            disable_semaphore_checks=True,
            vmem_limit_bytes=110 * 1024 * 1024,
        ),
    )(xt, k3, v3, A_wq, wot, B_w_r, B_w_gate, B_w_up, wdt, c, w_mod)
    return out_t.T.reshape(b, seq, d)
```

```python
import contextlib
import functools
import math
import os

import jax
import jax.numpy as jnp
from jax import lax
import jax.experimental.pallas as pl
import jax.experimental.pallas.tpu as pltpu

F32 = jnp.float32
BF16 = jnp.bfloat16
I32 = jnp.int32
U32 = jnp.uint32

HQ = 32
DH = 128
TOPC = 8
EPS = 1e-05
LANES = 128

TB = 512
HG = 2
TIE0 = int(os.environ.get("KP_TIE0", "2"))
NTIE = int(os.environ.get("KP_NTIE", "3"))
SP = int(os.environ.get("KP_SP", "128"))
NM1 = int(os.environ.get("KP_NM1", "8"))
NM2 = int(os.environ.get("KP_NM2", "12"))
NM3 = int(os.environ.get("KP_NM3", "16"))
TLO = int(os.environ.get("KP_TLO", "8"))
NF1 = int(os.environ.get("KP_NF1", "9"))
NF2 = int(os.environ.get("KP_NF2", "6"))
NF3 = int(os.environ.get("KP_NF3", "18"))
NVT = int(os.environ.get("KP_NVT", "16"))
TAILB = int(os.environ.get("KP_TAILB", "2"))
SIDE_ROW = int(os.environ.get("KP_SIDE_ROW", "6"))
EDGES = [int(e) for e in os.environ.get("KP_EDGES", "0,128,256,384,512,576").split(",")]
MODR = int(os.environ.get("KP_MODR", "384"))
MP = int(os.environ.get("KP_MP", "384"))
NMP = int(os.environ.get("KP_NMP", "12"))
WP = 256
REMF = int(os.environ.get("KP_REMF", "1"))
DEFM = int(os.environ.get("KP_DEFM", "1"))
SCOPES = os.environ.get("KP_SCOPES", "") == "1"

_NT = (((1,), (1,)), ((), ()))


def _rb(x):
    return x.astype(BF16).astype(F32)


def _sigmoid(x):
    return 1.0 / (1.0 + jnp.exp(-x))


def _lanes(col, width):
    reps = width // LANES
    return col if reps == 1 else jnp.concatenate([col] * reps, axis=1)


def _fold(x):
    xi = lax.bitcast_convert_type(x, U32)
    tok = None
    for r in range(0, x.shape[0], 8):
        for c in range(0, x.shape[1] - LANES + 1, LANES):
            t = xi[r:r + 8, c:c + LANES]
            tok = t if tok is None else tok | t
    return tok


def _colsum(x, marks, nmarks):
    n = x.shape[0] // 8
    acc = x[0:8]
    for g in range(1, n):
        acc = acc + x[8 * g:8 * g + 8]
        if ((g + 1) * nmarks) % n == 0:
            marks.append(_fold(acc))
    return jnp.sum(acc, axis=0, keepdims=True)


def _tie_rows(lhs, toks, zero, lo, hi):
    if not toks:
        return lhs
    lu = pltpu.bitcast(lhs, U32)
    rows = [lu[8 * r:8 * r + 8] for r in range(lu.shape[0] // 8)]
    for i, tok in enumerate(toks):
        r = lo + ((i + 1) * (hi - lo)) // len(toks) - 1
        rows[r] = rows[r] | (tok & zero)
    return pltpu.bitcast(jnp.concatenate(rows, axis=0), BF16)


def _merge(a, b):
    keyed = [((i + 1) / len(a), t) for i, t in enumerate(a)]
    keyed += [((i + 1) / len(b), t) for i, t in enumerate(b)]
    return [t for _, t in sorted(keyed, key=lambda kv: kv[0])]


def _span(start, size):
    if isinstance(start, int):
        return pl.ds(start, size)
    return pl.ds(pl.multiple_of(start, LANES), size)


def _scope(name):
    return jax.named_scope(name) if SCOPES else contextlib.nullcontext()


def _kernel(xt_hbm, k_hbm, v_hbm, wq_hbm, wot_hbm, wr_hbm, wg_hbm, wu_hbm, wdt_hbm,
            c_hbm, wmod_hbm, o_hbm,
            xt_v, k_v, v_v, wq_v, wot_v, wmod_v, wg_v, wu_v, wdt_v, ot_v,
            h_scr, acc_scr, st_scr, m_scr, vt_scr, mod_scr, col_scr, key_scr, h2_scr, x1_scr,
            zero_scr, fix_v, c_ref, wr_ref, row_scr, wd_scr,
            grp_sems, misc_sems, mlp_sems, out_sems, fix_sems,
            *, n_heads):
    d, seq = xt_v.shape
    sk = k_v.shape[1]
    n_grp = n_heads // HG
    n_blk = seq // TB
    n_units = n_grp * n_blk
    nb = TB // LANES
    nq = 2 * HG
    nt = sk // LANES
    gbits = n_grp.bit_length() - 1
    gw = nq * DH
    qscale = (DH ** -0.5) * math.log2(math.e)

    def grp_of(u):
        return u & (n_grp - 1)

    def blk_of(u):
        return u >> gbits

    def grp_copies(g):
        cs, hs = pl.ds(g * gw, gw), pl.ds(g * HG, HG)
        return (pltpu.make_async_copy(wq_hbm.at[:, cs], wq_v.at[g], grp_sems.at[0, g]),
                pltpu.make_async_copy(k_hbm.at[hs], k_v.at[hs], grp_sems.at[1, g]),
                pltpu.make_async_copy(v_hbm.at[hs], v_v.at[hs], grp_sems.at[2, g]),
                pltpu.make_async_copy(wot_hbm.at[:, cs], wot_v.at[g], grp_sems.at[3, g]))

    def col_copy(src, dst, lo, hi, sem):
        return pltpu.make_async_copy(src.at[:, lo:hi], dst.at[:, lo:hi], sem)

    x_first = col_copy(xt_hbm, xt_v, 0, TB, misc_sems.at[0])
    x_rest = col_copy(xt_hbm, xt_v, TB, seq, misc_sems.at[1])
    mod_rows = [(0, MODR), (MODR, d)]
    mod_first = [pltpu.make_async_copy(wmod_hbm.at[r0:r1, 0:2 * d], wmod_v.at[r0:r1, 0:2 * d],
                                       misc_sems.at[8 + i]) for i, (r0, r1) in enumerate(mod_rows)]
    mod_rest = col_copy(wmod_hbm, wmod_v, 2 * d, 6 * d, misc_sems.at[3])
    mlp_g = pltpu.make_async_copy(wg_hbm, wg_v, mlp_sems.at[0])
    mlp_u = pltpu.make_async_copy(wu_hbm, wu_v, mlp_sems.at[1])
    ff = wdt_hbm.shape[1]
    mlp_d = pltpu.make_async_copy(wdt_hbm, wdt_v.at[:, 0:ff], mlp_sems.at[2])
    out_lo = col_copy(ot_v, o_hbm, 0, seq - TB, out_sems.at[0])
    chunks = list(zip(EDGES[:-1], EDGES[1:]))
    out_hi = [pltpu.make_async_copy(ot_v.at[r0:r1, seq - TB:seq], o_hbm.at[r0:r1, seq - TB:seq],
                                    out_sems.at[1 + i]) for i, (r0, r1) in enumerate(chunks)]

    def silu_c():
        cc = c_ref[...].astype(F32)
        return jnp.broadcast_to((cc * _rb(_sigmoid(cc))).astype(BF16), (8, d))

    def ln1_norm(t0, n, marks):
        x = xt_v[:, _span(t0, n)].astype(F32)
        mu = _colsum(x, marks, NM1) * (1.0 / d)
        xc = x - mu
        var = _colsum(xc * xc, marks, NM2) * (1.0 / d)
        return (xc * lax.rsqrt(var + EPS)).astype(BF16).T

    def ln1_mod(ln, slot, r0, marks):
        n = ln.shape[0]
        h = ln.astype(F32) * mod_scr[1:2, :] + mod_scr[0:1, :]
        h_scr[slot, _span(r0, n), :] = h.astype(BF16)
        step = max(n // NM3, 8)
        for r in range(step - 8, n, step):
            marks.append(_fold(h[r:r + 8]))

    def mod_piece(src, dst, marks):
        w = wmod_v[:, _span(src, MP)].astype(F32)
        row = _rb(_colsum(w * _lanes(col_scr[5 * d:6 * d, :], MP), marks, NMP))
        pos = dst + lax.broadcasted_iota(I32, (1, MP), 1)
        is_cb = jnp.logical_and(pos >= 2 * d, pos < 3 * d)
        row = jnp.where(is_cb, _rb(1.0 + row), row)
        row_scr[:, _span(dst, MP)] = row
        col = jnp.broadcast_to(row, (LANES, MP)).T
        col_scr[_span(dst, MP), :] = col
        for r in range(LANES - 8, MP, LANES):
            marks.append(lax.bitcast_convert_type(col[r:r + 8], U32))

    def wd_piece(src, dst, marks):
        w = pltpu.bitcast(wdt_v[:, _span(src, WP)].T, U32)
        wd_scr[pl.ds(pl.multiple_of(dst // 2, WP // 2), WP // 2), :] = w
        for r in range(56, WP // 2, 64):
            for c in range(0, d - LANES + 1, LANES):
                marks.append(w[r:r + 8, c:c + LANES])

    def qproj(u, lo=0, hi=gw, parts=1):
        qs = []
        for r0 in range(0, TB, TB // parts):
            rs, dm = slice(r0, r0 + TB // parts), d - d % LANES
            if REMF:
                q = jnp.dot(h_scr[blk_of(u) & 1, rs, dm:d], wq_v[grp_of(u), dm:d, lo:hi],
                            preferred_element_type=F32)
                q = jnp.dot(h_scr[blk_of(u) & 1, rs, 0:dm], wq_v[grp_of(u), 0:dm, lo:hi],
                            preferred_element_type=F32) + q
            else:
                q = jnp.dot(h_scr[blk_of(u) & 1, rs, :], wq_v[grp_of(u), :, lo:hi],
                            preferred_element_type=F32)
            qs.append((q * qscale).astype(BF16))
        return jnp.concatenate(qs, axis=0)

    def qk(u, q, j, toks=(), zero=None):
        k = _tie_rows(k_v[grp_of(u) * HG + j // 2], toks, zero, TLO, sk // 16)
        st = lax.dot_general(k, q[:, j * DH:(j + 1) * DH], _NT,
                             preferred_element_type=F32)
        for i in range(nb):
            blk = st[:, i * LANES:(i + 1) * LANES]
            st_scr[j * nb + i] = blk
            if DEFM:
                m_scr[j * nb + i] = jnp.max(blk.reshape(sk // 8, 8, LANES), axis=0)
            else:
                m_scr[j * nb + i, 0:1] = jnp.max(blk, axis=0, keepdims=True)

    def v_transpose(u, i, marks=None):
        vt = pltpu.bitcast(v_v[grp_of(u) * HG + i].T, U32)
        vt_scr[i] = vt
        if marks is not None:
            step = sk // NVT
            for c in range(step - LANES, sk, step):
                marks.append(vt[DH // 2 - 8:DH // 2, c:c + LANES])

    def pv(slots, zero, toks=()):
        ps, ls, pairs = [], [], []
        for sl in slots:
            m = jnp.max(m_scr[sl], axis=0, keepdims=True) if DEFM else m_scr[sl, 0:1]
            p = jnp.exp2(st_scr[sl] - m)
            accs = [None] * 4
            for tile in range(nt):
                for r0 in range(tile * LANES + LANES - 16, tile * LANES - 16, -16):
                    pair = p[r0:r0 + 8] + p[r0 + 8:r0 + 16]
                    pairs.append(pair)
                    a = accs[tile % 4]
                    accs[tile % 4] = pair if a is None else a + pair
            ls.append(jnp.sum((accs[0] + accs[1]) + (accs[2] + accs[3]), axis=0, keepdims=True))
            ps.append(p.astype(BF16))
        outs = []
        ntiles = len(slots) * nt
        side = {}
        for i, tok in enumerate(toks):
            side.setdefault(((i + 1) * ntiles) // len(toks) - 1, []).append(tok)
        for i, sl in enumerate(slots):
            vu = vt_scr[sl // (2 * nb)]
            tiles = []
            for c in range(nt):
                g = i * nt + c + 4
                rows = []
                for r in range(8):
                    x = vu[8 * r:8 * r + 8, c * LANES:(c + 1) * LANES]
                    if g < ntiles and TIE0 <= r < TIE0 + NTIE:
                        src = pairs[g * 8 + (r - TIE0)]
                        x = x | (lax.bitcast_convert_type(src, U32) & zero)
                    if r == SIDE_ROW:
                        for tok in side.get(i * nt + c, ()):
                            x = x | (tok & zero)
                    rows.append(x)
                tiles.append(jnp.concatenate(rows, axis=0))
            lhs = pltpu.bitcast(jnp.concatenate(tiles, axis=1), BF16)
            o = jnp.dot(lhs, ps[i], preferred_element_type=F32)
            outs.append((o * (1.0 / ls[i])).astype(BF16))
        return outs

    def outproj(u, o, lo=0):
        w = len(o) // nq
        o2 = jnp.concatenate(
            [jnp.concatenate(o[j * w:(j + 1) * w], axis=1) for j in range(nq)], axis=0)
        contrib = jnp.dot(wot_v[grp_of(u)], o2, preferred_element_type=F32)
        hi = lo + w * LANES
        slot = blk_of(u) & 1
        old = jnp.where(grp_of(u) > 0, acc_scr[slot, :, lo:hi], 0.0)
        acc_scr[slot, :, lo:hi] = old + contrib

    def finalize(t0, slot, a0, dst, n):
        marks = []
        cs = _span(dst, n)
        x = xt_v[:, _span(t0, n)].astype(F32)
        att = acc_scr[slot, :, _span(a0, n)]
        x1b = (x + _lanes(col_scr[0:d, :], n) * att).astype(BF16)
        x1_scr[:, cs] = x1b
        ot_v[:, cs] = x1b
        mu = _colsum(x1b.astype(F32), marks, NF1) * (1.0 / d)
        mub = _rb(mu)
        xc = x1_scr[:, cs].astype(F32) - mub
        var = _colsum(xc * xc, marks, NF2) * (1.0 / d) - (mu - mub) * (mu - mub)
        inv = 1.0 / _rb(jnp.sqrt(_rb(_rb(jnp.maximum(var, 0.0)) + EPS)))
        step = d // NF3
        racc = None
        for r0 in range(0, d, step):
            rs = slice(r0, r0 + step)
            x1 = ot_v[rs, cs].astype(F32)
            h2b = ((x1 - mub) * inv * _lanes(col_scr[2 * d + r0:2 * d + r0 + step, :], n)
                   + _lanes(col_scr[d + r0:d + r0 + step, :], n)).astype(BF16)
            h2_scr[rs, cs] = h2b
            h2 = h2b.astype(F32)
            out = x1 + _lanes(col_scr[3 * d + r0:3 * d + r0 + step, :], n) * h2
            ot_v[rs, cs] = out.astype(BF16)
            rp = h2 * _lanes(col_scr[4 * d + r0:4 * d + r0 + step, :], n)
            for g in range(0, step, 8):
                racc = rp[g:g + 8] if racc is None else racc + rp[g:g + 8]
            marks.append(_fold(racc) | _fold(out))
        r = _rb(jnp.sum(racc, axis=0, keepdims=True)) + 0.0
        bits = lax.bitcast_convert_type(r, I32) >> 16
        order = jnp.where(bits < 0, -1 - bits, bits + 32768)
        pos = t0 + lax.broadcasted_iota(I32, (1, n), 1)
        key = lax.bitcast_convert_type((order << 11) + (seq - 1 - pos) + 0x20000000, F32)
        for i in range(n // LANES):
            key_scr[pl.ds(dst // LANES + i, 1), :] = key[:, i * LANES:(i + 1) * LANES]
        return marks

    hw = gw // 2
    wq0a = pltpu.make_async_copy(wq_hbm.at[:, 0:hw], wq_v.at[0, :, 0:hw], grp_sems.at[0, 0])
    wq0b = pltpu.make_async_copy(wq_hbm.at[:, hw:gw], wq_v.at[0, :, hw:gw], misc_sems.at[4])
    k0a = pltpu.make_async_copy(k_hbm.at[0], k_v.at[0], grp_sems.at[1, 0])
    k0b = pltpu.make_async_copy(k_hbm.at[1], k_v.at[1], misc_sems.at[5])
    v0 = pltpu.make_async_copy(v_hbm.at[0:HG], v_v.at[0:HG], grp_sems.at[2, 0])
    wo0 = pltpu.make_async_copy(wot_hbm.at[:, 0:gw], wot_v.at[0], grp_sems.at[3, 0])
    wq1, k1, v1, wo1 = grp_copies(1)
    c_copy = pltpu.make_async_copy(c_hbm, c_ref, misc_sems.at[6])
    wr_copy = pltpu.make_async_copy(wr_hbm, wr_ref, misc_sems.at[7])
    c_copy.start()
    wr_copy.start()
    x_first.start()
    mod_first[0].start()
    mod_first[1].start()
    wq0a.start()
    acc_scr[1] = jnp.zeros((d, TB), F32)
    col_scr[0:4 * d, :] = jnp.zeros((4 * d, LANES), F32)
    wdt_v[:, ff:ff + WP] = jnp.zeros((d, WP), BF16)
    with _scope("w_x"):
        c_copy.wait()
        wr_copy.wait()
        x_first.wait()
    cbits = lax.bitcast_convert_type(c_ref[:, 0:LANES].astype(F32), U32)
    zero_scr[...] = jnp.broadcast_to(cbits & 0xFFFF, (8, LANES))
    h_scr[0] = ln1_norm(0, TB, [])
    sc = silu_c()
    wr = wr_ref[...].reshape(1, d).astype(F32)
    col_scr[4 * d:5 * d, :] = jnp.broadcast_to(wr, (LANES, d)).T
    col_scr[5 * d:6 * d, :] = jnp.broadcast_to(sc[0:1, :].astype(F32), (LANES, d)).T
    with _scope("w_wmod"):
        mod_first[0].wait()
    mod = jnp.dot(sc[:, 0:MODR], wmod_v[0:MODR, 0:2 * d], preferred_element_type=F32)
    with _scope("w_wmod2"):
        mod_first[1].wait()
    wq0b.start()
    k0a.start()
    k0b.start(priority=1)
    v0.start(priority=1)
    mod = _rb(mod + jnp.dot(sc[:, MODR:d], wmod_v[MODR:d, 0:2 * d], preferred_element_type=F32))
    mod_scr[0:1, :] = mod[0:1, 0:d]
    mod_scr[1:2, :] = _rb(1.0 + mod[0:1, d:2 * d])
    with _scope("w_wq"):
        wq0a.wait()
    ln1_mod(h_scr[0], 0, 0, [])
    qa = qproj(0, 0, hw, 2)
    with _scope("w_k"):
        wq0b.wait()
        k0a.wait()
    wq1.start(priority=1)
    k1.start(priority=1)
    q = jnp.concatenate([qa, qproj(0, hw, gw, 2)], axis=1)
    qk(0, q, 0)
    qk(0, q, 1)
    with _scope("w_v"):
        k0b.wait()
        v0.wait()
    v1.start()
    wo0.start()
    with _scope("qk0"):
        zero = zero_scr[...]
        for i in range(HG):
            marks = []
            v_transpose(0, i, marks)
            qk(0, q, nq - HG + i, marks, zero)

    assert n_grp == 8 and HG == 2
    loads = [[wq1, k1, v1, wo0],
             [wo1, *grp_copies(2), mod_rest, x_rest],
             [*grp_copies(3), *grp_copies(4), *grp_copies(5)],
             [*grp_copies(6), *grp_copies(7)],
             [mlp_d],
             [mlp_g, mlp_u]]
    wd0 = len(loads) - 1
    npc = TB // SP
    nmp = 4 * d // MP

    def manage(i):
        for cp in loads[i - 1]:
            cp.wait()
        for cp in loads[i]:
            cp.start()

    def steady(u, carry):
        with _scope("body"):
            zero = zero_scr[...]
            blk, g = blk_of(u), grp_of(u)
            off = ((g - 1) & (npc - 1)) * SP
            q = qproj(u)
            o = pv(range(0, 2 * nb), zero)
            live = jnp.logical_and(blk > 0, jnp.logical_and(g >= 1, g <= npc))
            t0 = jnp.maximum(blk - 1, 0) * TB + off
            marks = finalize(t0, (blk + 1) & 1, off, jnp.where(live, t0, seq), SP)
            wp = jnp.clip(u - wd0, 0, ff // WP - 1) * WP
            wmarks = []
            wd_piece(jnp.where(u >= wd0, wp, ff), wp, wmarks)
            qk(u, q, 0, _merge(marks, wmarks), zero)
            marks = []
            nxt = jnp.where(u >= 2, jnp.minimum(blk + 1, n_blk - 1), 0)
            ln = ln1_norm(nxt * TB + off, SP, marks)
            ln1_mod(ln, (blk + 1) & 1, off, marks)
            qk(u, q, 1, marks, zero)
            o += pv(range(2 * nb, 4 * nb), zero)
            outproj(u - 1, o)
            marks = []
            v_transpose(u, 0, marks)
            mp = jnp.clip(u - 2, 0, nmp - 1) * MP
            mmarks = []
            mod_piece(jnp.where(u >= 2, 2 * d + mp, 0), mp, mmarks)
            qk(u, q, 2, _merge(marks, mmarks), zero)
            marks = []
            v_transpose(u, 1, marks)
            qk(u, q, 3, marks, zero)
        return carry

    def stage(i, carry):
        for k in range(1, len(loads)):
            pl.when(i == k)(functools.partial(manage, k))
        return lax.fori_loop(i, jnp.where(i < len(loads) - 1, i + 1, n_units), steady, carry)

    lax.fori_loop(1, len(loads), stage, 0)

    ul = n_units - 1
    tl = seq - TB
    sl_last = (n_blk - 1) & 1
    nb0 = nb - TAILB
    out_lo.start()
    mlp_g.wait()
    with _scope("e_pva"):
        mod_scr[2:3, :] = row_scr[:, 3 * d:4 * d]
        outproj(ul, pv([j * nb + i for j in range(nq) for i in range(nb0)], zero_scr[...]))
    mlp_u.wait()
    with _scope("e_pvb"):
        toks = finalize(tl, sl_last, 0, tl, nb0 * LANES)
        o = pv([j * nb + i for j in range(nq) for i in range(nb0, nb)], zero_scr[...], toks)
        outproj(ul, o, nb0 * LANES)
        finalize(tl + nb0 * LANES, sl_last, nb0 * LANES, tl + nb0 * LANES, TAILB * LANES)

    keys = key_scr[0:seq // LANES, :]
    sub8 = lax.broadcasted_iota(I32, (TOPC, 1), 0)
    lane = lax.broadcasted_iota(I32, (TOPC, LANES), 1)
    top = jnp.zeros((TOPC, 1), F32)
    bases, idxs = [], []
    h2s = jnp.zeros((TOPC, d), F32)
    picks = []
    for i in range(TOPC):
        mx = jnp.max(jnp.max(keys, axis=0, keepdims=True), axis=1, keepdims=True)
        keys = jnp.where(keys == mx, 0.0, keys)
        top = jnp.where(sub8 == i, mx, top)
        idx = seq - 1 - (lax.bitcast_convert_type(mx, I32) & (seq - 1))
        bases.append(pl.multiple_of(idx[0, 0] & ~(LANES - 1), LANES))
        idxs.append(idx)
        pick = jnp.logical_and(sub8 == i, lane == (idx & (LANES - 1)))
        pick = jnp.where(pick, 1.0, 0.0).astype(BF16)
        sl = pl.ds(bases[i], LANES)
        h2s = h2s + lax.dot_general(pick, h2_scr[:, sl], _NT, preferred_element_type=F32)
        picks.append(pick)
    order = (lax.bitcast_convert_type(top, I32) >> 11) & 0xFFFF
    rbits = jnp.where(order >= 32768, order - 32768, -1 - order) << 16
    gate = _rb(_sigmoid(lax.bitcast_convert_type(rbits, F32)))
    xs = h2s.astype(BF16)
    for cp in out_hi:
        cp.start()
    g = _rb(jnp.dot(xs, wg_v[...], preferred_element_type=F32))
    g = _rb(g * _rb(_sigmoid(g)))
    u = _rb(jnp.dot(xs, wu_v[...], preferred_element_type=F32))
    gu = (g * u).astype(BF16)

    last_use = []
    for i in range(TOPC):
        ok = True
        for j in range(i + 1, TOPC):
            ok = jnp.logical_and(ok, bases[i] != bases[j])
        last_use.append(ok)

    def down(r0, r1):
        x1p = jnp.concatenate([x1_scr[r0:r1, pl.ds(bases[i], LANES)] for i in range(TOPC)], axis=1)
        x1s = lax.dot_general(jnp.concatenate(picks, axis=1), x1p, _NT,
                              preferred_element_type=F32)
        wd = pltpu.bitcast(wd_scr[:, r0:r1], BF16)
        y = _rb(jnp.dot(gu, wd, preferred_element_type=F32))
        hm = _rb(h2s[:, r0:r1] + _rb(y * gate))
        return x1s + mod_scr[2:3, r0:r1] * hm

    def patch(r0, r1, new):
        n = r1 - r0
        pad = jnp.concatenate([new, jnp.zeros((LANES - TOPC, n), F32)], axis=0)
        cols = pltpu.bitcast(pad.T.astype(BF16), U32)
        col = [jnp.broadcast_to(cols[:, j:j + 1], (n // 2, LANES)) for j in range(TOPC)]
        for i in range(TOPC):
            res = pltpu.bitcast(ot_v[r0:r1, pl.ds(bases[i], LANES)], U32)
            tok = lane[0:1, :] + (idxs[i] & ~(LANES - 1))
            for j in range(i + 1):
                res = jnp.where(tok == idxs[j], col[j], res)
            fix_v[i, r0:r1, :] = pltpu.bitcast(res, BF16)

    def fix_copy(i, r0, r1):
        return pltpu.make_async_copy(fix_v.at[i, r0:r1, :],
                                     o_hbm.at[r0:r1, pl.ds(bases[i], LANES)], fix_sems.at[i])

    def for_last(fn):
        for i in range(TOPC - 1):
            pl.when(last_use[i])(functools.partial(fn, i))
        fn(TOPC - 1)

    new = down(*chunks[0])
    out_lo.wait()
    for ci, (r0, r1) in enumerate(chunks):
        out_hi[ci].wait()
        nxt = down(*chunks[ci + 1]) if ci + 1 < len(chunks) else None
        patch(r0, r1, new)
        for_last(lambda i: fix_copy(i, r0, r1).start())
        new = nxt
    with _scope("w_fix"):
        for r0, r1 in chunks:
            for_last(lambda i: fix_copy(i, r0, r1).wait())


@jax.jit
def pallas_adaLN_cond__gqa_block_cached__moe_arch_mod__prompt_kernel(
    A_x: jax.Array,
    A_k_cache: jax.Array,
    A_v_cache: jax.Array,
    A_wq: jax.Array,
    A_wo: jax.Array,
    B_x: jax.Array,
    B_w_r: jax.Array,
    B_w_gate: jax.Array,
    B_w_up: jax.Array,
    B_w_down: jax.Array,
    c: jax.Array,
    w_mod: jax.Array,
):
    b, seq, d = A_x.shape
    _, hkv, sk, dh = A_k_cache.shape
    assert b == 1 and dh == DH and HQ == 2 * hkv
    assert seq & (seq - 1) == 0 and seq <= 2048
    f = B_w_gate.shape[1]
    n_grp = hkv // HG
    gw = 2 * HG * dh
    n_slots = 2 * HG * TB // LANES

    xt = A_x.reshape(seq, d).T
    wot = A_wo.T
    wdt = B_w_down.T
    k3 = A_k_cache.reshape(hkv, sk, dh)
    v3 = A_v_cache.reshape(hkv, sk, dh)

    hbm = pl.BlockSpec(memory_space=pl.ANY)
    out_t = pl.pallas_call(
        functools.partial(_kernel, n_heads=hkv),
        in_specs=[hbm] * 11,
        out_specs=hbm,
        out_shape=jax.ShapeDtypeStruct((d, seq), BF16),
        scratch_shapes=[
            pltpu.VMEM((d, seq), BF16),
            pltpu.VMEM((hkv, sk, dh), BF16),
            pltpu.VMEM((hkv, sk, dh), BF16),
            pltpu.VMEM((n_grp, d, gw), BF16),
            pltpu.VMEM((n_grp, d, gw), BF16),
            pltpu.VMEM((d, 6 * d), BF16),
            pltpu.VMEM((d, f), BF16),
            pltpu.VMEM((d, f), BF16),
            pltpu.VMEM((d, f + WP), BF16),
            pltpu.VMEM((d, seq + SP), BF16),
            pltpu.VMEM((2, TB, d), BF16),
            pltpu.VMEM((2, d, TB), F32),
            pltpu.VMEM((n_slots, sk, LANES), F32),
            pltpu.VMEM((n_slots, 8, LANES), F32),
            pltpu.VMEM((HG, dh // 2, sk), U32),
            pltpu.VMEM((8, d), F32),
            pltpu.VMEM((6 * d, LANES), F32),
            pltpu.VMEM(((seq + SP) // LANES + 7 & ~7, LANES), F32),
            pltpu.VMEM((d, seq + SP), BF16),
            pltpu.VMEM((d, seq + SP), BF16),
            pltpu.VMEM((8, LANES), U32),
            pltpu.VMEM((TOPC, d, LANES), BF16),
            pltpu.VMEM((1, d), BF16),
            pltpu.VMEM((d,), BF16),
            pltpu.VMEM((1, 4 * d), F32),
            pltpu.VMEM((f // 2, d), U32),
            pltpu.SemaphoreType.DMA((4, n_grp)),
            pltpu.SemaphoreType.DMA((10,)),
            pltpu.SemaphoreType.DMA((3,)),
            pltpu.SemaphoreType.DMA((len(EDGES),)),
            pltpu.SemaphoreType.DMA((TOPC,)),
        ],
        compiler_params=pltpu.CompilerParams(
            disable_bounds_checks=True,
            disable_semaphore_checks=True,
            vmem_limit_bytes=110 * 1024 * 1024,
        ),
    )(xt, k3, v3, A_wq, wot, B_w_r, B_w_gate, B_w_up, wdt, c, w_mod)
    return out_t.T.reshape(b, seq, d)
```

```python
import contextlib
import functools
import math
import os

import jax
import jax.numpy as jnp
from jax import lax
import jax.experimental.pallas as pl
import jax.experimental.pallas.tpu as pltpu

F32 = jnp.float32
BF16 = jnp.bfloat16
I32 = jnp.int32
U32 = jnp.uint32

HQ = 32
DH = 128
TOPC = 8
EPS = 1e-05
LANES = 128

TB = 512
HG = 2
TIE0 = int(os.environ.get("KP_TIE0", "2"))
NTIE = int(os.environ.get("KP_NTIE", "3"))
SP = int(os.environ.get("KP_SP", "128"))
NM1 = int(os.environ.get("KP_NM1", "8"))
NM2 = int(os.environ.get("KP_NM2", "12"))
NM3 = int(os.environ.get("KP_NM3", "16"))
TLO = int(os.environ.get("KP_TLO", "8"))
NF1 = int(os.environ.get("KP_NF1", "9"))
NF2 = int(os.environ.get("KP_NF2", "6"))
NF3 = int(os.environ.get("KP_NF3", "18"))
NVT = int(os.environ.get("KP_NVT", "16"))
TAILB = int(os.environ.get("KP_TAILB", "2"))
SIDE_ROW = int(os.environ.get("KP_SIDE_ROW", "6"))
EDGES = [int(e) for e in os.environ.get("KP_EDGES", "0,128,256,384,512,576").split(",")]
MODC = int(os.environ.get("KP_MODC", "384"))
MP = int(os.environ.get("KP_MP", "384"))
NMP = int(os.environ.get("KP_NMP", "12"))
WP = 256
REMF = int(os.environ.get("KP_REMF", "1"))
DEFM = int(os.environ.get("KP_DEFM", "1"))
KAP = int(os.environ.get("KP_KAP", "0"))
LATEKV = int(os.environ.get("KP_LATEKV", "1"))
EARLYMOD = int(os.environ.get("KP_EARLYMOD", "0"))
SCOPES = os.environ.get("KP_SCOPES", "") == "1"

_NT = (((1,), (1,)), ((), ()))


def _rb(x):
    return x.astype(BF16).astype(F32)


def _sigmoid(x):
    return 1.0 / (1.0 + jnp.exp(-x))


def _lanes(col, width):
    reps = width // LANES
    return col if reps == 1 else jnp.concatenate([col] * reps, axis=1)


def _fold(x):
    xi = lax.bitcast_convert_type(x, U32)
    tok = None
    for r in range(0, x.shape[0], 8):
        for c in range(0, x.shape[1] - LANES + 1, LANES):
            t = xi[r:r + 8, c:c + LANES]
            tok = t if tok is None else tok | t
    return tok


def _colsum(x, marks, nmarks):
    n = x.shape[0] // 8
    acc = x[0:8]
    for g in range(1, n):
        acc = acc + x[8 * g:8 * g + 8]
        if ((g + 1) * nmarks) % n == 0:
            marks.append(_fold(acc))
    return jnp.sum(acc, axis=0, keepdims=True)


def _tie_rows(lhs, toks, zero, lo, hi):
    if not toks:
        return lhs
    lu = pltpu.bitcast(lhs, U32)
    rows = [lu[8 * r:8 * r + 8] for r in range(lu.shape[0] // 8)]
    for i, tok in enumerate(toks):
        r = lo + ((i + 1) * (hi - lo)) // len(toks) - 1
        rows[r] = rows[r] | (tok & zero)
    return pltpu.bitcast(jnp.concatenate(rows, axis=0), BF16)


def _merge(a, b):
    keyed = [((i + 1) / len(a), t) for i, t in enumerate(a)]
    keyed += [((i + 1) / len(b), t) for i, t in enumerate(b)]
    return [t for _, t in sorted(keyed, key=lambda kv: kv[0])]


def _span(start, size):
    if isinstance(start, int):
        return pl.ds(start, size)
    return pl.ds(pl.multiple_of(start, LANES), size)


def _scope(name):
    return jax.named_scope(name) if SCOPES else contextlib.nullcontext()


def _kernel(xt_hbm, k_hbm, v_hbm, wq_hbm, wot_hbm, wr_hbm, wg_hbm, wu_hbm, wdt_hbm,
            c_hbm, wmod_hbm, o_hbm,
            xt_v, k_v, v_v, wq_v, wot_v, wmod_v, wg_v, wu_v, wdt_v, ot_v,
            h_scr, acc_scr, st_scr, m_scr, vt_scr, mod_scr, col_scr, key_scr, h2_scr, x1_scr,
            zero_scr, fix_v, c_ref, wr_ref, row_scr, wd_scr, h2l_scr,
            grp_sems, misc_sems, mlp_sems, out_sems, fix_sems,
            *, n_heads):
    d, seq = xt_v.shape
    sk = k_v.shape[1]
    n_grp = n_heads // HG
    n_blk = seq // TB
    n_units = n_grp * n_blk
    nb = TB // LANES
    nq = 2 * HG
    nt = sk // LANES
    gbits = n_grp.bit_length() - 1
    gw = nq * DH
    qscale = (DH ** -0.5) * math.log2(math.e)

    def grp_of(u):
        return u & (n_grp - 1)

    def blk_of(u):
        return u >> gbits

    def grp_copies(g, n=1):
        cs, hs, ps = pl.ds(g * gw, n * gw), pl.ds(g * HG, n * HG), pl.ds((g - 1) * gw, n * gw)
        return (pltpu.make_async_copy(wq_hbm.at[:, cs], wq_v.at[:, cs], grp_sems.at[0, g]),
                pltpu.make_async_copy(k_hbm.at[hs], k_v.at[hs], grp_sems.at[1, g]),
                pltpu.make_async_copy(v_hbm.at[hs], v_v.at[hs], grp_sems.at[2, g]),
                pltpu.make_async_copy(wot_hbm.at[:, ps], wot_v.at[:, ps], grp_sems.at[3, g]))

    def col_copy(src, dst, lo, hi, sem):
        return pltpu.make_async_copy(src.at[:, lo:hi], dst.at[:, lo:hi], sem)

    x_first = col_copy(xt_hbm, xt_v, 0, TB, misc_sems.at[0])
    x_rest = col_copy(xt_hbm, xt_v, TB, seq, misc_sems.at[1])
    mod_first = [col_copy(wmod_hbm, wmod_v, MODC, 2 * d, misc_sems.at[8]),
                 col_copy(wmod_hbm, wmod_v, 0, MODC, misc_sems.at[9])]
    mod_rest = col_copy(wmod_hbm, wmod_v, 2 * d, 6 * d, misc_sems.at[3])
    mlp_g = pltpu.make_async_copy(wg_hbm, wg_v, mlp_sems.at[0])
    mlp_u = pltpu.make_async_copy(wu_hbm, wu_v, mlp_sems.at[1])
    ff = wdt_hbm.shape[1]
    mlp_d = pltpu.make_async_copy(wdt_hbm, wdt_v.at[:, 0:ff], mlp_sems.at[2])
    out_lo = col_copy(ot_v, o_hbm, 0, seq - TB, out_sems.at[0])
    chunks = list(zip(EDGES[:-1], EDGES[1:]))
    out_hi = [pltpu.make_async_copy(ot_v.at[r0:r1, seq - TB:seq], o_hbm.at[r0:r1, seq - TB:seq],
                                    out_sems.at[1 + i]) for i, (r0, r1) in enumerate(chunks)]

    def silu_c():
        cc = c_ref[...].astype(F32)
        return jnp.broadcast_to((cc * _rb(_sigmoid(cc))).astype(BF16), (8, d))

    def ln1_norm(t0, n, marks):
        x = xt_v[:, _span(t0, n)].astype(F32)
        mu = _colsum(x, marks, NM1) * (1.0 / d)
        xc = x - mu
        var = _colsum(xc * xc, marks, NM2) * (1.0 / d)
        return (xc * lax.rsqrt(var + EPS)).astype(BF16).T

    def ln1_mod(ln, slot, r0, marks):
        n = ln.shape[0]
        h = ln.astype(F32) * mod_scr[1:2, :] + mod_scr[0:1, :]
        h_scr[slot, _span(r0, n), :] = h.astype(BF16)
        step = max(n // NM3, 8)
        for r in range(step - 8, n, step):
            marks.append(_fold(h[r:r + 8]))

    def mod_piece(src, dst, marks):
        w = wmod_v[:, _span(src, MP)].astype(F32)
        row = _rb(_colsum(w * _lanes(col_scr[5 * d:6 * d, :], MP), marks, NMP))
        pos = dst + lax.broadcasted_iota(I32, (1, MP), 1)
        is_cb = jnp.logical_and(pos >= 2 * d, pos < 3 * d)
        row = jnp.where(is_cb, _rb(1.0 + row), row)
        row_scr[:, _span(dst, MP)] = row
        col = jnp.broadcast_to(row, (LANES, MP)).T
        col_scr[_span(dst, MP), :] = col
        for r in range(LANES - 8, MP, LANES):
            marks.append(lax.bitcast_convert_type(col[r:r + 8], U32))

    def wd_piece(src, dst, marks):
        w = pltpu.bitcast(wdt_v[:, _span(src, WP)].T, U32)
        wd_scr[pl.ds(pl.multiple_of(dst // 2, WP // 2), WP // 2), :] = w
        for r in range(56, WP // 2, 64):
            for c in range(0, d - LANES + 1, LANES):
                marks.append(w[r:r + 8, c:c + LANES])

    def qproj(u, lo=0, hi=gw, parts=1):
        qs = []
        ws = _span(grp_of(u) * gw + lo, hi - lo)
        for r0 in range(0, TB, TB // parts):
            rs, dm = slice(r0, r0 + TB // parts), d - d % LANES
            if REMF:
                q = jnp.dot(h_scr[blk_of(u) & 1, rs, dm:d], wq_v[dm:d, ws],
                            preferred_element_type=F32)
                q = jnp.dot(h_scr[blk_of(u) & 1, rs, 0:dm], wq_v[0:dm, ws],
                            preferred_element_type=F32) + q
            else:
                q = jnp.dot(h_scr[blk_of(u) & 1, rs, :], wq_v[:, ws],
                            preferred_element_type=F32)
            qs.append((q * qscale).astype(BF16))
        return jnp.concatenate(qs, axis=0)

    def qk(u, q, j, toks=(), zero=None):
        k = _tie_rows(k_v[grp_of(u) * HG + j // 2], toks, zero, TLO, sk // 16)
        st = lax.dot_general(k, q[:, j * DH:(j + 1) * DH], _NT,
                             preferred_element_type=F32)
        for i in range(nb):
            blk = st[:, i * LANES:(i + 1) * LANES]
            st_scr[j * nb + i] = blk
            if DEFM:
                m_scr[j * nb + i] = jnp.max(blk.reshape(sk // 8, 8, LANES), axis=0)
            else:
                m_scr[j * nb + i, 0:1] = jnp.max(blk, axis=0, keepdims=True)

    def v_transpose(u, i, marks=None):
        vt = pltpu.bitcast(v_v[grp_of(u) * HG + i].T, U32)
        vt_scr[i] = vt
        if marks is not None:
            step = sk // NVT
            for c in range(step - LANES, sk, step):
                marks.append(vt[DH // 2 - 8:DH // 2, c:c + LANES])

    def pv(slots, zero, toks=()):
        ps, ls, pairs = [], [], []
        for sl in slots:
            m = jnp.max(m_scr[sl], axis=0, keepdims=True) if DEFM else m_scr[sl, 0:1]
            p = jnp.exp2(st_scr[sl] - m)
            accs = [None] * 4
            for tile in range(nt):
                for r0 in range(tile * LANES + LANES - 16, tile * LANES - 16, -16):
                    pair = p[r0:r0 + 8] + p[r0 + 8:r0 + 16]
                    pairs.append(pair)
                    a = accs[tile % 4]
                    accs[tile % 4] = pair if a is None else a + pair
            ls.append(jnp.sum((accs[0] + accs[1]) + (accs[2] + accs[3]), axis=0, keepdims=True))
            ps.append(p.astype(BF16))
        outs = []
        ntiles = len(slots) * nt
        side = {}
        for i, tok in enumerate(toks):
            side.setdefault(((i + 1) * ntiles) // len(toks) - 1, []).append(tok)
        for i, sl in enumerate(slots):
            vu = vt_scr[sl // (2 * nb)]
            tiles = []
            for c in range(nt):
                g = i * nt + c + 4
                rows = []
                for r in range(8):
                    x = vu[8 * r:8 * r + 8, c * LANES:(c + 1) * LANES]
                    if g < ntiles and TIE0 <= r < TIE0 + NTIE:
                        src = pairs[g * 8 + (r - TIE0)]
                        x = x | (lax.bitcast_convert_type(src, U32) & zero)
                    if r == SIDE_ROW:
                        for tok in side.get(i * nt + c, ()):
                            x = x | (tok & zero)
                    rows.append(x)
                tiles.append(jnp.concatenate(rows, axis=0))
            lhs = pltpu.bitcast(jnp.concatenate(tiles, axis=1), BF16)
            o = jnp.dot(lhs, ps[i], preferred_element_type=F32)
            outs.append((o * (1.0 / ls[i])).astype(BF16))
        return outs

    def outproj(u, o, lo=0):
        w = len(o) // nq
        o2 = jnp.concatenate(
            [jnp.concatenate(o[j * w:(j + 1) * w], axis=1) for j in range(nq)], axis=0)
        contrib = jnp.dot(wot_v[:, _span(grp_of(u) * gw, gw)], o2, preferred_element_type=F32)
        hi = lo + w * LANES
        slot = blk_of(u) & 1
        old = jnp.where(grp_of(u) > 0, acc_scr[slot, :, lo:hi], 0.0)
        acc_scr[slot, :, lo:hi] = old + contrib

    def router_keys(racc, t0):
        r = _rb(jnp.sum(racc, axis=0, keepdims=True)) + 0.0
        bits = lax.bitcast_convert_type(r, I32) >> 16
        order = jnp.where(bits < 0, -1 - bits, bits + 32768)
        pos = t0 + lax.broadcasted_iota(I32, r.shape, 1)
        return lax.bitcast_convert_type((order << 11) + (seq - 1 - pos) + 0x20000000, F32)

    def finalize(t0, slot, a0, dst, n, keys_out=None):
        marks = []
        cs = _span(dst, n)
        x = xt_v[:, _span(t0, n)].astype(F32)
        att = acc_scr[slot, :, _span(a0, n)]
        x1b = (x + _lanes(col_scr[0:d, :], n) * att).astype(BF16)
        x1_scr[:, cs] = x1b
        ot_v[:, cs] = x1b
        mu = _colsum(x1b.astype(F32), marks, NF1) * (1.0 / d)
        mub = _rb(mu)
        xc = x1_scr[:, cs].astype(F32) - mub
        var = _colsum(xc * xc, marks, NF2) * (1.0 / d) - (mu - mub) * (mu - mub)
        inv = 1.0 / _rb(jnp.sqrt(_rb(_rb(jnp.maximum(var, 0.0)) + EPS)))
        step = d // NF3
        racc = None
        for r0 in range(0, d, step):
            rs = slice(r0, r0 + step)
            x1 = ot_v[rs, cs].astype(F32)
            h2b = ((x1 - mub) * inv * _lanes(col_scr[2 * d + r0:2 * d + r0 + step, :], n)
                   + _lanes(col_scr[d + r0:d + r0 + step, :], n)).astype(BF16)
            if keys_out is None:
                h2_scr[rs, cs] = h2b
            else:
                h2l_scr[rs, :] = h2b
            h2 = h2b.astype(F32)
            out = x1 + _lanes(col_scr[3 * d + r0:3 * d + r0 + step, :], n) * h2
            ot_v[rs, cs] = out.astype(BF16)
            rp = h2 * _lanes(col_scr[4 * d + r0:4 * d + r0 + step, :], n)
            for g in range(0, step, 8):
                racc = rp[g:g + 8] if racc is None else racc + rp[g:g + 8]
            marks.append(_fold(racc) | _fold(out))
        if keys_out is not None:
            keys_out.append(racc)
            return marks
        key = router_keys(racc, t0)
        for i in range(n // LANES):
            key_scr[pl.ds(dst // LANES + i, 1), :] = key[:, i * LANES:(i + 1) * LANES]
        return marks

    hw = gw // 2
    wq0a = col_copy(wq_hbm, wq_v, 0, hw, grp_sems.at[0, 0])
    wq0b = col_copy(wq_hbm, wq_v, hw, gw, misc_sems.at[4])
    k0a = pltpu.make_async_copy(k_hbm.at[0], k_v.at[0], grp_sems.at[1, 0])
    k0b = pltpu.make_async_copy(k_hbm.at[1], k_v.at[1], misc_sems.at[5])
    v0 = pltpu.make_async_copy(v_hbm.at[0:HG], v_v.at[0:HG], grp_sems.at[2, 0])
    wq1, k1, v1, wo0 = grp_copies(1)
    wo_last = col_copy(wot_hbm, wot_v, (n_grp - 1) * gw, n_grp * gw, grp_sems.at[3, 0])
    c_copy = pltpu.make_async_copy(c_hbm, c_ref, misc_sems.at[6])
    wr_copy = pltpu.make_async_copy(wr_hbm, wr_ref, misc_sems.at[7])
    c_copy.start()
    wr_copy.start()
    x_first.start()
    mod_first[0].start()
    mod_first[1].start()
    wq0a.start()
    wq0b.start()
    acc_scr[1] = jnp.zeros((d, TB), F32)
    col_scr[0:4 * d, :] = jnp.zeros((4 * d, LANES), F32)
    wdt_v[:, ff:ff + WP] = jnp.zeros((d, WP), BF16)
    with _scope("w_x"):
        c_copy.wait()
        wr_copy.wait()
        x_first.wait()
    cbits = lax.bitcast_convert_type(c_ref[:, 0:LANES].astype(F32), U32)
    zero_scr[...] = jnp.broadcast_to(cbits & 0xFFFF, (8, LANES))
    h_scr[0] = ln1_norm(0, TB, [])
    sc = silu_c()
    wr = wr_ref[...].reshape(1, d).astype(F32)
    col_scr[4 * d:5 * d, :] = jnp.broadcast_to(wr, (LANES, d)).T
    col_scr[5 * d:6 * d, :] = jnp.broadcast_to(sc[0:1, :].astype(F32), (LANES, d)).T
    with _scope("w_wmod"):
        mod_first[0].wait()
    mod = _rb(jnp.dot(sc, wmod_v[:, MODC:2 * d], preferred_element_type=F32))
    mod_scr[0:1, MODC:d] = mod[0:1, 0:d - MODC]
    mod_scr[1:2, :] = _rb(1.0 + mod[0:1, d - MODC:2 * d - MODC])
    with _scope("w_wmod2"):
        mod_first[1].wait()
    k0a.start(priority=KAP)
    if not LATEKV:
        k0b.start(priority=1)
        v0.start(priority=1)
    mod_scr[0:1, 0:MODC] = _rb(jnp.dot(sc, wmod_v[:, 0:MODC], preferred_element_type=F32))[0:1]
    if EARLYMOD:
        ln1_mod(h_scr[0], 0, 0, [])
    with _scope("w_wq"):
        wq0a.wait()
    if LATEKV:
        k0b.start(priority=1)
        v0.start(priority=1)
    if not EARLYMOD:
        ln1_mod(h_scr[0], 0, 0, [])
    qa = qproj(0, 0, hw, 2)
    with _scope("w_k"):
        wq0b.wait()
        k0a.wait()
    wq1.start(priority=1)
    k1.start(priority=1)
    q = jnp.concatenate([qa, qproj(0, hw, gw, 2)], axis=1)
    qk(0, q, 0)
    qk(0, q, 1)
    with _scope("w_v"):
        k0b.wait()
        v0.wait()
    v1.start()
    wo0.start()
    with _scope("qk0"):
        zero = zero_scr[...]
        for i in range(HG):
            marks = []
            v_transpose(0, i, marks)
            qk(0, q, nq - HG + i, marks, zero)

    assert n_grp == 8 and HG == 2
    loads = [[wq1, k1, v1, wo0],
             [*grp_copies(2), mod_rest, x_rest],
             [*grp_copies(3, 3)],
             [*grp_copies(6, 2), wo_last],
             [mlp_d],
             [mlp_g, mlp_u]]
    wd0 = len(loads) - 1
    npc = TB // SP
    nmp = 4 * d // MP

    def manage(i):
        for cp in loads[i - 1]:
            cp.wait()
        for cp in loads[i]:
            cp.start()

    def steady(u, carry):
        with _scope("body"):
            zero = zero_scr[...]
            blk, g = blk_of(u), grp_of(u)
            off = ((g - 1) & (npc - 1)) * SP
            q = qproj(u)
            o = pv(range(0, 2 * nb), zero)
            live = jnp.logical_and(blk > 0, jnp.logical_and(g >= 1, g <= npc))
            t0 = jnp.maximum(blk - 1, 0) * TB + off
            marks = finalize(t0, (blk + 1) & 1, off, jnp.where(live, t0, seq), SP)
            wp = jnp.clip(u - wd0, 0, ff // WP - 1) * WP
            wmarks = []
            wd_piece(jnp.where(u >= wd0, wp, ff), wp, wmarks)
            qk(u, q, 0, _merge(marks, wmarks), zero)
            marks = []
            nxt = jnp.where(u >= 2, jnp.minimum(blk + 1, n_blk - 1), 0)
            ln = ln1_norm(nxt * TB + off, SP, marks)
            ln1_mod(ln, (blk + 1) & 1, off, marks)
            qk(u, q, 1, marks, zero)
            o += pv(range(2 * nb, 4 * nb), zero)
            outproj(u - 1, o)
            marks = []
            v_transpose(u, 0, marks)
            mp = jnp.clip(u - 2, 0, nmp - 1) * MP
            mmarks = []
            mod_piece(jnp.where(u >= 2, 2 * d + mp, 0), mp, mmarks)
            qk(u, q, 2, _merge(marks, mmarks), zero)
            marks = []
            v_transpose(u, 1, marks)
            qk(u, q, 3, marks, zero)
        return carry

    def stage(i, carry):
        for k in range(1, len(loads)):
            pl.when(i == k)(functools.partial(manage, k))
        return lax.fori_loop(i, jnp.where(i < len(loads) - 1, i + 1, n_units), steady, carry)

    lax.fori_loop(1, len(loads), stage, 0)

    ul = n_units - 1
    tl = seq - TB
    sl_last = (n_blk - 1) & 1
    nb0 = nb - TAILB
    with _scope("e_pva"):
        mod_scr[2:3, :] = row_scr[:, 3 * d:4 * d]
        outproj(ul, pv([j * nb + i for j in range(nq) for i in range(nb0)], zero_scr[...]))
    mlp_g.wait()
    mlp_u.wait()
    out_lo.start()
    with _scope("e_pvb"):
        toks = finalize(tl, sl_last, 0, tl, nb0 * LANES)
        o = pv([j * nb + i for j in range(nq) for i in range(nb0, nb)], zero_scr[...], toks)
        outproj(ul, o, nb0 * LANES)

    nl = TAILB * LANES
    sub8 = lax.broadcasted_iota(I32, (TOPC, 1), 0)
    lane = lax.broadcasted_iota(I32, (TOPC, LANES), 1)

    def key_index(k):
        return seq - 1 - (lax.bitcast_convert_type(k, I32) & (seq - 1))

    keys = key_scr[0:seq // LANES, :]
    piece = lax.broadcasted_iota(I32, (seq // LANES, 1), 0)
    keys = jnp.where(piece < (seq - nl) // LANES, keys, 0.0)
    ecol = jnp.zeros((TOPC, LANES), F32)
    erow = jnp.zeros((1, LANES), F32)
    h2e = jnp.zeros((TOPC, d), F32)
    late = []
    marks = finalize(seq - nl, sl_last, TB - nl, seq - nl, nl, late)
    zero = zero_scr[...]
    pace = dict(zip([int(v) for v in os.environ.get("KP_PG", "2,4,5,6,7").split(",")],
                    [int(v) for v in os.environ.get("KP_PM", "8,14,18,23,27").split(",")]))
    for i in range(TOPC):
        mx = jnp.max(jnp.max(keys, axis=0, keepdims=True), axis=1, keepdims=True)
        keys = jnp.where(keys == mx, 0.0, keys)
        ecol = jnp.where(sub8 == i, mx, ecol)
        erow = jnp.where(lane[0:1] == i, mx, erow)
        idx = key_index(mx)
        pick = jnp.logical_and(sub8 == i, lane == (idx & (LANES - 1)))
        sl = pl.ds(pl.multiple_of(idx[0, 0] & ~(LANES - 1), LANES), LANES)
        pick = jnp.where(pick, 1.0, 0.0)
        if i in pace:
            pick = lax.bitcast_convert_type(
                lax.bitcast_convert_type(pick, U32) | (marks[pace[i]] & zero), F32)
        h2e = h2e + lax.dot_general(pick.astype(BF16), h2_scr[:, sl], _NT,
                                    preferred_element_type=F32)

    racc = lax.bitcast_convert_type(late[0], U32)
    if os.environ.get("KP_AFTER", "0") == "1":
        racc = racc | _lanes(_fold(h2e) & zero, nl)
    late = [router_keys(lax.bitcast_convert_type(racc, F32), seq - nl)]
    krow = jnp.concatenate([late[0], erow], axis=1)
    kcol = jnp.concatenate([jnp.broadcast_to(late[0], (LANES, nl)).T, ecol], axis=0)
    cnt = [None] * 4
    for g in range(kcol.shape[0] // 8):
        one = jnp.where(_lanes(kcol[8 * g:8 * g + 8], nl + LANES) > krow, 1.0, 0.0)
        cnt[g % 4] = one if cnt[g % 4] is None else cnt[g % 4] + one
    rank = jnp.sum((cnt[0] + cnt[1]) + (cnt[2] + cnt[3]), axis=0, keepdims=True)
    chosen = rank == sub8.astype(F32)
    onehot = jnp.where(chosen, 1.0, 0.0).astype(BF16)
    h2pad = jnp.concatenate([h2e, jnp.zeros((TOPC, d), F32)], axis=0).astype(BF16)
    h2s = (jnp.dot(onehot[:, nl:nl + 2 * TOPC], h2pad, preferred_element_type=F32)
           + lax.dot_general(onehot[:, 0:nl], h2l_scr[...], _NT,
                             preferred_element_type=F32))
    top = jnp.max(jnp.where(chosen, krow, 0.0), axis=1, keepdims=True)
    idx_col = key_index(top)
    idxs = [idx_col[i:i + 1] for i in range(TOPC)]
    bases = [pl.multiple_of(idx_col[i, 0] & ~(LANES - 1), LANES) for i in range(TOPC)]
    hit = lane == (idx_col & (LANES - 1))
    picks = [jnp.where(jnp.logical_and(sub8 == i, hit), 1.0, 0.0).astype(BF16)
             for i in range(TOPC)]
    order = (lax.bitcast_convert_type(top, I32) >> 11) & 0xFFFF
    rbits = jnp.where(order >= 32768, order - 32768, -1 - order) << 16
    gate = _rb(_sigmoid(lax.bitcast_convert_type(rbits, F32)))
    xs = h2s.astype(BF16)
    for cp in out_hi:
        cp.start()
    g = _rb(jnp.dot(xs, wg_v[...], preferred_element_type=F32))
    g = _rb(g * _rb(_sigmoid(g)))
    u = _rb(jnp.dot(xs, wu_v[...], preferred_element_type=F32))
    gu = (g * u).astype(BF16)

    last_use = []
    for i in range(TOPC):
        ok = True
        for j in range(i + 1, TOPC):
            ok = jnp.logical_and(ok, bases[i] != bases[j])
        last_use.append(ok)

    def down(r0, r1):
        x1p = jnp.concatenate([x1_scr[r0:r1, pl.ds(bases[i], LANES)] for i in range(TOPC)], axis=1)
        x1s = lax.dot_general(jnp.concatenate(picks, axis=1), x1p, _NT,
                              preferred_element_type=F32)
        wd = pltpu.bitcast(wd_scr[:, r0:r1], BF16)
        y = _rb(jnp.dot(gu, wd, preferred_element_type=F32))
        hm = _rb(h2s[:, r0:r1] + _rb(y * gate))
        return x1s + mod_scr[2:3, r0:r1] * hm

    def patch(r0, r1, new):
        n = r1 - r0
        pad = jnp.concatenate([new, jnp.zeros((LANES - TOPC, n), F32)], axis=0)
        cols = pltpu.bitcast(pad.T.astype(BF16), U32)
        col = [jnp.broadcast_to(cols[:, j:j + 1], (n // 2, LANES)) for j in range(TOPC)]
        for i in range(TOPC):
            res = pltpu.bitcast(ot_v[r0:r1, pl.ds(bases[i], LANES)], U32)
            tok = lane[0:1, :] + (idxs[i] & ~(LANES - 1))
            for j in range(i + 1):
                res = jnp.where(tok == idxs[j], col[j], res)
            fix_v[i, r0:r1, :] = pltpu.bitcast(res, BF16)

    def fix_copy(i, r0, r1):
        return pltpu.make_async_copy(fix_v.at[i, r0:r1, :],
                                     o_hbm.at[r0:r1, pl.ds(bases[i], LANES)], fix_sems.at[i])

    def for_last(fn):
        for i in range(TOPC - 1):
            pl.when(last_use[i])(functools.partial(fn, i))
        fn(TOPC - 1)

    new = down(*chunks[0])
    out_lo.wait()
    for ci, (r0, r1) in enumerate(chunks):
        out_hi[ci].wait()
        nxt = down(*chunks[ci + 1]) if ci + 1 < len(chunks) else None
        patch(r0, r1, new)
        for_last(lambda i: fix_copy(i, r0, r1).start())
        new = nxt
    with _scope("w_fix"):
        for r0, r1 in chunks:
            for_last(lambda i: fix_copy(i, r0, r1).wait())


@jax.jit
def pallas_adaLN_cond__gqa_block_cached__moe_arch_mod__prompt_kernel(
    A_x: jax.Array,
    A_k_cache: jax.Array,
    A_v_cache: jax.Array,
    A_wq: jax.Array,
    A_wo: jax.Array,
    B_x: jax.Array,
    B_w_r: jax.Array,
    B_w_gate: jax.Array,
    B_w_up: jax.Array,
    B_w_down: jax.Array,
    c: jax.Array,
    w_mod: jax.Array,
):
    b, seq, d = A_x.shape
    _, hkv, sk, dh = A_k_cache.shape
    assert b == 1 and dh == DH and HQ == 2 * hkv
    assert seq & (seq - 1) == 0 and seq <= 2048
    f = B_w_gate.shape[1]
    n_grp = hkv // HG
    gw = 2 * HG * dh
    n_slots = 2 * HG * TB // LANES

    xt = A_x.reshape(seq, d).T
    wot = A_wo.T
    wdt = B_w_down.T
    k3 = A_k_cache.reshape(hkv, sk, dh)
    v3 = A_v_cache.reshape(hkv, sk, dh)

    hbm = pl.BlockSpec(memory_space=pl.ANY)
    out_t = pl.pallas_call(
        functools.partial(_kernel, n_heads=hkv),
        in_specs=[hbm] * 11,
        out_specs=hbm,
        out_shape=jax.ShapeDtypeStruct((d, seq), BF16),
        scratch_shapes=[
            pltpu.VMEM((d, seq), BF16),
            pltpu.VMEM((hkv, sk, dh), BF16),
            pltpu.VMEM((hkv, sk, dh), BF16),
            pltpu.VMEM((d, n_grp * gw), BF16),
            pltpu.VMEM((d, n_grp * gw), BF16),
            pltpu.VMEM((d, 6 * d), BF16),
            pltpu.VMEM((d, f), BF16),
            pltpu.VMEM((d, f), BF16),
            pltpu.VMEM((d, f + WP), BF16),
            pltpu.VMEM((d, seq + SP), BF16),
            pltpu.VMEM((2, TB, d), BF16),
            pltpu.VMEM((2, d, TB), F32),
            pltpu.VMEM((n_slots, sk, LANES), F32),
            pltpu.VMEM((n_slots, 8, LANES), F32),
            pltpu.VMEM((HG, dh // 2, sk), U32),
            pltpu.VMEM((8, d), F32),
            pltpu.VMEM((6 * d, LANES), F32),
            pltpu.VMEM(((seq + SP) // LANES + 7 & ~7, LANES), F32),
            pltpu.VMEM((d, seq + SP), BF16),
            pltpu.VMEM((d, seq + SP), BF16),
            pltpu.VMEM((8, LANES), U32),
            pltpu.VMEM((TOPC, d, LANES), BF16),
            pltpu.VMEM((1, d), BF16),
            pltpu.VMEM((d,), BF16),
            pltpu.VMEM((1, 4 * d), F32),
            pltpu.VMEM((f // 2, d), U32),
            pltpu.VMEM((d, TAILB * LANES), BF16),
            pltpu.SemaphoreType.DMA((4, n_grp)),
            pltpu.SemaphoreType.DMA((10,)),
            pltpu.SemaphoreType.DMA((3,)),
            pltpu.SemaphoreType.DMA((len(EDGES),)),
            pltpu.SemaphoreType.DMA((TOPC,)),
        ],
        compiler_params=pltpu.CompilerParams(
            disable_bounds_checks=True,
            disable_semaphore_checks=True,
            vmem_limit_bytes=110 * 1024 * 1024,
        ),
    )(xt, k3, v3, A_wq, wot, B_w_r, B_w_gate, B_w_up, wdt, c, w_mod)
    return out_t.T.reshape(b, seq, d)
```

```python
import contextlib
import functools
import math
import os

import jax
import jax.numpy as jnp
from jax import lax
import jax.experimental.pallas as pl
import jax.experimental.pallas.tpu as pltpu

F32 = jnp.float32
BF16 = jnp.bfloat16
I32 = jnp.int32
U32 = jnp.uint32

HQ = 32
DH = 128
TOPC = 8
EPS = 1e-05
EPS_BF16 = 1.0013580322265625e-05
LANES = 128

TB = 512
HG = 2
TIE0 = int(os.environ.get("KP_TIE0", "2"))
NTIE = int(os.environ.get("KP_NTIE", "3"))
SP = int(os.environ.get("KP_SP", "128"))
NM1 = int(os.environ.get("KP_NM1", "8"))
NM2 = int(os.environ.get("KP_NM2", "12"))
NM3 = int(os.environ.get("KP_NM3", "16"))
TLO = int(os.environ.get("KP_TLO", "8"))
NF1 = int(os.environ.get("KP_NF1", "9"))
NF2 = int(os.environ.get("KP_NF2", "6"))
NF3 = int(os.environ.get("KP_NF3", "18"))
NVT = int(os.environ.get("KP_NVT", "16"))
TAILB = int(os.environ.get("KP_TAILB", "2"))
SIDE_ROW = int(os.environ.get("KP_SIDE_ROW", "6"))
EDGES = [int(e) for e in os.environ.get("KP_EDGES", "0,128,256,384,512,576").split(",")]
MODC = int(os.environ.get("KP_MODC", "384"))
MP = int(os.environ.get("KP_MP", "384"))
NMP = int(os.environ.get("KP_NMP", "12"))
WP = 256
REMF = int(os.environ.get("KP_REMF", "1"))
DEFM = int(os.environ.get("KP_DEFM", "1"))
KAP = int(os.environ.get("KP_KAP", "0"))
LATEKV = int(os.environ.get("KP_LATEKV", "1"))
EARLYMOD = int(os.environ.get("KP_EARLYMOD", "0"))
SCOPES = os.environ.get("KP_SCOPES", "") == "1"

_NT = (((1,), (1,)), ((), ()))


def _rb(x):
    return x.astype(BF16).astype(F32)


def _sigmoid(x):
    return 1.0 / (1.0 + jnp.exp(-x))


def _lanes(col, width):
    reps = width // LANES
    return col if reps == 1 else jnp.concatenate([col] * reps, axis=1)


def _fold(x):
    xi = lax.bitcast_convert_type(x, U32)
    tok = None
    for r in range(0, x.shape[0], 8):
        for c in range(0, x.shape[1] - LANES + 1, LANES):
            t = xi[r:r + 8, c:c + LANES]
            tok = t if tok is None else tok | t
    return tok


def _colsum(x, marks, nmarks):
    n = x.shape[0] // 8
    acc = x[0:8]
    for g in range(1, n):
        acc = acc + x[8 * g:8 * g + 8]
        if ((g + 1) * nmarks) % n == 0:
            marks.append(_fold(acc))
    return jnp.sum(acc, axis=0, keepdims=True)


def _tie_rows(lhs, toks, zero, lo, hi):
    if not toks:
        return lhs
    lu = pltpu.bitcast(lhs, U32)
    rows = [lu[8 * r:8 * r + 8] for r in range(lu.shape[0] // 8)]
    for i, tok in enumerate(toks):
        r = lo + ((i + 1) * (hi - lo)) // len(toks) - 1
        rows[r] = rows[r] | (tok & zero)
    return pltpu.bitcast(jnp.concatenate(rows, axis=0), BF16)


def _merge(a, b):
    keyed = [((i + 1) / len(a), t) for i, t in enumerate(a)]
    keyed += [((i + 1) / len(b), t) for i, t in enumerate(b)]
    return [t for _, t in sorted(keyed, key=lambda kv: kv[0])]


def _span(start, size):
    if isinstance(start, int):
        return pl.ds(start, size)
    return pl.ds(pl.multiple_of(start, LANES), size)


def _scope(name):
    return jax.named_scope(name) if SCOPES else contextlib.nullcontext()


def _kernel(xt_hbm, k_hbm, v_hbm, wq_hbm, wot_hbm, wr_hbm, wg_hbm, wu_hbm, wdt_hbm,
            c_hbm, wmod_hbm, o_hbm,
            xt_v, k_v, v_v, wq_v, wot_v, wmod_v, wg_v, wu_v, wdt_v, ot_v,
            h_scr, acc_scr, st_scr, m_scr, vt_scr, mod_scr, col_scr, key_scr, h2_scr, x1_scr,
            zero_scr, fix_v, c_ref, wr_ref, row_scr, wd_scr, h2l_scr,
            grp_sems, misc_sems, mlp_sems, out_sems, fix_sems,
            *, n_heads):
    d, seq = xt_v.shape
    sk = k_v.shape[1]
    n_grp = n_heads // HG
    n_blk = seq // TB
    n_units = n_grp * n_blk
    nb = TB // LANES
    nq = 2 * HG
    nt = sk // LANES
    gbits = n_grp.bit_length() - 1
    gw = nq * DH
    qscale = (DH ** -0.5) * math.log2(math.e)

    def grp_of(u):
        return u & (n_grp - 1)

    def blk_of(u):
        return u >> gbits

    def grp_copies(g, n=1):
        cs, hs, ps = pl.ds(g * gw, n * gw), pl.ds(g * HG, n * HG), pl.ds((g - 1) * gw, n * gw)
        return (pltpu.make_async_copy(wq_hbm.at[:, cs], wq_v.at[:, cs], grp_sems.at[0, g]),
                pltpu.make_async_copy(k_hbm.at[hs], k_v.at[hs], grp_sems.at[1, g]),
                pltpu.make_async_copy(v_hbm.at[hs], v_v.at[hs], grp_sems.at[2, g]),
                pltpu.make_async_copy(wot_hbm.at[:, ps], wot_v.at[:, ps], grp_sems.at[3, g]))

    def col_copy(src, dst, lo, hi, sem):
        return pltpu.make_async_copy(src.at[:, lo:hi], dst.at[:, lo:hi], sem)

    x_first = col_copy(xt_hbm, xt_v, 0, TB, misc_sems.at[0])
    x_rest = col_copy(xt_hbm, xt_v, TB, seq, misc_sems.at[1])
    mod_first = [col_copy(wmod_hbm, wmod_v, MODC, 2 * d, misc_sems.at[8]),
                 col_copy(wmod_hbm, wmod_v, 0, MODC, misc_sems.at[9])]
    mod_rest = col_copy(wmod_hbm, wmod_v, 2 * d, 6 * d, misc_sems.at[3])
    mlp_g = pltpu.make_async_copy(wg_hbm, wg_v, mlp_sems.at[0])
    mlp_u = pltpu.make_async_copy(wu_hbm, wu_v, mlp_sems.at[1])
    ff = wdt_hbm.shape[1]
    mlp_d = pltpu.make_async_copy(wdt_hbm, wdt_v.at[:, 0:ff], mlp_sems.at[2])
    out_lo = col_copy(ot_v, o_hbm, 0, seq - TB, out_sems.at[0])
    chunks = list(zip(EDGES[:-1], EDGES[1:]))
    out_hi = [pltpu.make_async_copy(ot_v.at[r0:r1, seq - TB:seq], o_hbm.at[r0:r1, seq - TB:seq],
                                    out_sems.at[1 + i]) for i, (r0, r1) in enumerate(chunks)]

    def silu_c():
        cc = c_ref[...].astype(F32)
        return jnp.broadcast_to((cc * _rb(_sigmoid(cc))).astype(BF16), (8, d))

    def ln1_norm(t0, n, marks):
        x = xt_v[:, _span(t0, n)].astype(F32)
        mu = _colsum(x, marks, NM1) * (1.0 / d)
        xc = x - mu
        var = _colsum(xc * xc, marks, NM2) * (1.0 / d)
        return (xc * lax.rsqrt(var + EPS)).astype(BF16).T

    def ln1_mod(ln, slot, r0, marks):
        n = ln.shape[0]
        h = ln.astype(F32) * mod_scr[1:2, :] + mod_scr[0:1, :]
        h_scr[slot, _span(r0, n), :] = h.astype(BF16)
        step = max(n // NM3, 8)
        for r in range(step - 8, n, step):
            marks.append(_fold(h[r:r + 8]))

    def mod_piece(src, dst, marks):
        w = wmod_v[:, _span(src, MP)].astype(F32)
        row = _rb(_colsum(w * _lanes(col_scr[5 * d:6 * d, :], MP), marks, NMP))
        pos = dst + lax.broadcasted_iota(I32, (1, MP), 1)
        is_cb = jnp.logical_and(pos >= 2 * d, pos < 3 * d)
        row = jnp.where(is_cb, _rb(1.0 + row), row)
        row_scr[:, _span(dst, MP)] = row
        col = jnp.broadcast_to(row, (LANES, MP)).T
        col_scr[_span(dst, MP), :] = col
        for r in range(LANES - 8, MP, LANES):
            marks.append(lax.bitcast_convert_type(col[r:r + 8], U32))

    def wd_piece(src, dst, marks):
        w = pltpu.bitcast(wdt_v[:, _span(src, WP)].T, U32)
        wd_scr[pl.ds(pl.multiple_of(dst // 2, WP // 2), WP // 2), :] = w
        for r in range(56, WP // 2, 64):
            for c in range(0, d - LANES + 1, LANES):
                marks.append(w[r:r + 8, c:c + LANES])

    def qproj(u, lo=0, hi=gw, parts=1):
        qs = []
        ws = _span(grp_of(u) * gw + lo, hi - lo)
        for r0 in range(0, TB, TB // parts):
            rs, dm = slice(r0, r0 + TB // parts), d - d % LANES
            if REMF:
                q = jnp.dot(h_scr[blk_of(u) & 1, rs, dm:d], wq_v[dm:d, ws],
                            preferred_element_type=F32)
                q = jnp.dot(h_scr[blk_of(u) & 1, rs, 0:dm], wq_v[0:dm, ws],
                            preferred_element_type=F32) + q
            else:
                q = jnp.dot(h_scr[blk_of(u) & 1, rs, :], wq_v[:, ws],
                            preferred_element_type=F32)
            qs.append((q * qscale).astype(BF16))
        return jnp.concatenate(qs, axis=0)

    def qk(u, q, j, toks=(), zero=None):
        k = _tie_rows(k_v[grp_of(u) * HG + j // 2], toks, zero, TLO, sk // 16)
        st = lax.dot_general(k, q[:, j * DH:(j + 1) * DH], _NT,
                             preferred_element_type=F32)
        for i in range(nb):
            blk = st[:, i * LANES:(i + 1) * LANES]
            st_scr[j * nb + i] = blk
            if DEFM:
                m_scr[j * nb + i] = jnp.max(blk.reshape(sk // 8, 8, LANES), axis=0)
            else:
                m_scr[j * nb + i, 0:1] = jnp.max(blk, axis=0, keepdims=True)

    def v_transpose(u, i, marks=None):
        vt = pltpu.bitcast(v_v[grp_of(u) * HG + i].T, U32)
        vt_scr[i] = vt
        if marks is not None:
            step = sk // NVT
            for c in range(step - LANES, sk, step):
                marks.append(vt[DH // 2 - 8:DH // 2, c:c + LANES])

    def pv(slots, zero, toks=()):
        ps, ls, pairs = [], [], []
        for sl in slots:
            m = jnp.max(m_scr[sl], axis=0, keepdims=True) if DEFM else m_scr[sl, 0:1]
            p = jnp.exp2(st_scr[sl] - m)
            accs = [None] * 4
            for tile in range(nt):
                for r0 in range(tile * LANES + LANES - 16, tile * LANES - 16, -16):
                    pair = p[r0:r0 + 8] + p[r0 + 8:r0 + 16]
                    pairs.append(pair)
                    a = accs[tile % 4]
                    accs[tile % 4] = pair if a is None else a + pair
            ls.append(jnp.sum((accs[0] + accs[1]) + (accs[2] + accs[3]), axis=0, keepdims=True))
            ps.append(p.astype(BF16))
        outs = []
        ntiles = len(slots) * nt
        side = {}
        for i, tok in enumerate(toks):
            side.setdefault(((i + 1) * ntiles) // len(toks) - 1, []).append(tok)
        for i, sl in enumerate(slots):
            vu = vt_scr[sl // (2 * nb)]
            tiles = []
            for c in range(nt):
                g = i * nt + c + 4
                rows = []
                for r in range(8):
                    x = vu[8 * r:8 * r + 8, c * LANES:(c + 1) * LANES]
                    if g < ntiles and TIE0 <= r < TIE0 + NTIE:
                        src = pairs[g * 8 + (r - TIE0)]
                        x = x | (lax.bitcast_convert_type(src, U32) & zero)
                    if r == SIDE_ROW:
                        for tok in side.get(i * nt + c, ()):
                            x = x | (tok & zero)
                    rows.append(x)
                tiles.append(jnp.concatenate(rows, axis=0))
            lhs = pltpu.bitcast(jnp.concatenate(tiles, axis=1), BF16)
            o = jnp.dot(lhs, ps[i], preferred_element_type=F32)
            outs.append((o * (1.0 / ls[i])).astype(BF16))
        return outs

    def outproj(u, o, lo=0):
        w = len(o) // nq
        o2 = jnp.concatenate(
            [jnp.concatenate(o[j * w:(j + 1) * w], axis=1) for j in range(nq)], axis=0)
        contrib = jnp.dot(wot_v[:, _span(grp_of(u) * gw, gw)], o2, preferred_element_type=F32)
        hi = lo + w * LANES
        slot = blk_of(u) & 1
        old = jnp.where(grp_of(u) > 0, acc_scr[slot, :, lo:hi], 0.0)
        acc_scr[slot, :, lo:hi] = old + contrib

    def router_keys(racc, t0):
        r = _rb(jnp.sum(racc, axis=0, keepdims=True)) + 0.0
        bits = lax.bitcast_convert_type(r, I32) >> 16
        order = jnp.where(bits < 0, -1 - bits, bits + 32768)
        pos = t0 + lax.broadcasted_iota(I32, r.shape, 1)
        return lax.bitcast_convert_type((order << 11) + (seq - 1 - pos) + 0x20000000, F32)

    def finalize(t0, slot, a0, dst, n, keys_out=None):
        marks = []
        cs = _span(dst, n)
        x = xt_v[:, _span(t0, n)].astype(F32)
        att = acc_scr[slot, :, _span(a0, n)]
        x1b = (x + _lanes(col_scr[0:d, :], n) * att).astype(BF16)
        x1_scr[:, cs] = x1b
        ot_v[:, cs] = x1b
        mu = _colsum(x1b.astype(F32), marks, NF1) * (1.0 / d)
        mub = _rb(mu)
        xc = x1_scr[:, cs].astype(F32) - mub
        var = _colsum(xc * xc, marks, NF2) * (1.0 / d) - (mu - mub) * (mu - mub)
        inv = 1.0 / _rb(jnp.sqrt(_rb(_rb(jnp.maximum(var, 0.0)) + EPS_BF16)))
        step = d // NF3
        racc = None
        for r0 in range(0, d, step):
            rs = slice(r0, r0 + step)
            x1 = ot_v[rs, cs].astype(F32)
            ln = _rb(_rb(x1 - mub) * inv)
            h2b = (_rb(ln * _lanes(col_scr[2 * d + r0:2 * d + r0 + step, :], n))
                   + _lanes(col_scr[d + r0:d + r0 + step, :], n)).astype(BF16)
            if keys_out is None:
                h2_scr[rs, cs] = h2b
            else:
                h2l_scr[rs, :] = h2b
            h2 = h2b.astype(F32)
            out = x1 + _lanes(col_scr[3 * d + r0:3 * d + r0 + step, :], n) * h2
            ot_v[rs, cs] = out.astype(BF16)
            rp = h2 * _lanes(col_scr[4 * d + r0:4 * d + r0 + step, :], n)
            for g in range(0, step, 8):
                racc = rp[g:g + 8] if racc is None else racc + rp[g:g + 8]
            marks.append(_fold(racc) | _fold(out))
        if keys_out is not None:
            keys_out.append(racc)
            return marks
        key = router_keys(racc, t0)
        for i in range(n // LANES):
            key_scr[pl.ds(dst // LANES + i, 1), :] = key[:, i * LANES:(i + 1) * LANES]
        return marks

    hw = gw // 2
    wq0a = col_copy(wq_hbm, wq_v, 0, hw, grp_sems.at[0, 0])
    wq0b = col_copy(wq_hbm, wq_v, hw, gw, misc_sems.at[4])
    k0a = pltpu.make_async_copy(k_hbm.at[0], k_v.at[0], grp_sems.at[1, 0])
    k0b = pltpu.make_async_copy(k_hbm.at[1], k_v.at[1], misc_sems.at[5])
    v0 = pltpu.make_async_copy(v_hbm.at[0:HG], v_v.at[0:HG], grp_sems.at[2, 0])
    wq1, k1, v1, wo0 = grp_copies(1)
    wo_last = col_copy(wot_hbm, wot_v, (n_grp - 1) * gw, n_grp * gw, grp_sems.at[3, 0])
    c_copy = pltpu.make_async_copy(c_hbm, c_ref, misc_sems.at[6])
    wr_copy = pltpu.make_async_copy(wr_hbm, wr_ref, misc_sems.at[7])
    c_copy.start()
    wr_copy.start()
    x_first.start()
    mod_first[0].start()
    mod_first[1].start()
    wq0a.start()
    wq0b.start()
    acc_scr[1] = jnp.zeros((d, TB), F32)
    col_scr[0:4 * d, :] = jnp.zeros((4 * d, LANES), F32)
    wdt_v[:, ff:ff + WP] = jnp.zeros((d, WP), BF16)
    with _scope("w_x"):
        c_copy.wait()
        wr_copy.wait()
        x_first.wait()
    cbits = lax.bitcast_convert_type(c_ref[:, 0:LANES].astype(F32), U32)
    zero_scr[...] = jnp.broadcast_to(cbits & 0xFFFF, (8, LANES))
    h_scr[0] = ln1_norm(0, TB, [])
    sc = silu_c()
    wr = wr_ref[...].reshape(1, d).astype(F32)
    col_scr[4 * d:5 * d, :] = jnp.broadcast_to(wr, (LANES, d)).T
    col_scr[5 * d:6 * d, :] = jnp.broadcast_to(sc[0:1, :].astype(F32), (LANES, d)).T
    with _scope("w_wmod"):
        mod_first[0].wait()
    mod = _rb(jnp.dot(sc, wmod_v[:, MODC:2 * d], preferred_element_type=F32))
    mod_scr[0:1, MODC:d] = mod[0:1, 0:d - MODC]
    mod_scr[1:2, :] = _rb(1.0 + mod[0:1, d - MODC:2 * d - MODC])
    with _scope("w_wmod2"):
        mod_first[1].wait()
    k0a.start(priority=KAP)
    if not LATEKV:
        k0b.start(priority=1)
        v0.start(priority=1)
    mod_scr[0:1, 0:MODC] = _rb(jnp.dot(sc, wmod_v[:, 0:MODC], preferred_element_type=F32))[0:1]
    if EARLYMOD:
        ln1_mod(h_scr[0], 0, 0, [])
    with _scope("w_wq"):
        wq0a.wait()
    if LATEKV:
        k0b.start(priority=1)
        v0.start(priority=1)
    if not EARLYMOD:
        ln1_mod(h_scr[0], 0, 0, [])
    qa = qproj(0, 0, hw, 2)
    with _scope("w_k"):
        wq0b.wait()
        k0a.wait()
    wq1.start(priority=1)
    k1.start(priority=1)
    q = jnp.concatenate([qa, qproj(0, hw, gw, 2)], axis=1)
    qk(0, q, 0)
    qk(0, q, 1)
    with _scope("w_v"):
        k0b.wait()
        v0.wait()
    v1.start()
    wo0.start()
    with _scope("qk0"):
        zero = zero_scr[...]
        for i in range(HG):
            marks = []
            v_transpose(0, i, marks)
            qk(0, q, nq - HG + i, marks, zero)

    assert n_grp == 8 and HG == 2
    loads = [[wq1, k1, v1, wo0],
             [*grp_copies(2), mod_rest, x_rest],
             [*grp_copies(3, 3)],
             [*grp_copies(6, 2), wo_last],
             [mlp_d],
             [mlp_g, mlp_u]]
    wd0 = len(loads) - 1
    npc = TB // SP
    nmp = 4 * d // MP

    def manage(i):
        for cp in loads[i - 1]:
            cp.wait()
        for cp in loads[i]:
            cp.start()

    def steady(u, carry):
        with _scope("body"):
            zero = zero_scr[...]
            blk, g = blk_of(u), grp_of(u)
            off = ((g - 1) & (npc - 1)) * SP
            q = qproj(u)
            o = pv(range(0, 2 * nb), zero)
            live = jnp.logical_and(blk > 0, jnp.logical_and(g >= 1, g <= npc))
            t0 = jnp.maximum(blk - 1, 0) * TB + off
            marks = finalize(t0, (blk + 1) & 1, off, jnp.where(live, t0, seq), SP)
            wp = jnp.clip(u - wd0, 0, ff // WP - 1) * WP
            wmarks = []
            wd_piece(jnp.where(u >= wd0, wp, ff), wp, wmarks)
            qk(u, q, 0, _merge(marks, wmarks), zero)
            marks = []
            nxt = jnp.where(u >= 2, jnp.minimum(blk + 1, n_blk - 1), 0)
            ln = ln1_norm(nxt * TB + off, SP, marks)
            ln1_mod(ln, (blk + 1) & 1, off, marks)
            qk(u, q, 1, marks, zero)
            o += pv(range(2 * nb, 4 * nb), zero)
            outproj(u - 1, o)
            marks = []
            v_transpose(u, 0, marks)
            mp = jnp.clip(u - 2, 0, nmp - 1) * MP
            mmarks = []
            mod_piece(jnp.where(u >= 2, 2 * d + mp, 0), mp, mmarks)
            qk(u, q, 2, _merge(marks, mmarks), zero)
            marks = []
            v_transpose(u, 1, marks)
            qk(u, q, 3, marks, zero)
        return carry

    def stage(i, carry):
        for k in range(1, len(loads)):
            pl.when(i == k)(functools.partial(manage, k))
        return lax.fori_loop(i, jnp.where(i < len(loads) - 1, i + 1, n_units), steady, carry)

    lax.fori_loop(1, len(loads), stage, 0)

    ul = n_units - 1
    tl = seq - TB
    sl_last = (n_blk - 1) & 1
    nb0 = nb - TAILB
    with _scope("e_pva"):
        mod_scr[2:3, :] = row_scr[:, 3 * d:4 * d]
        outproj(ul, pv([j * nb + i for j in range(nq) for i in range(nb0)], zero_scr[...]))
    mlp_g.wait()
    mlp_u.wait()
    out_lo.start()
    with _scope("e_pvb"):
        toks = finalize(tl, sl_last, 0, tl, nb0 * LANES)
        o = pv([j * nb + i for j in range(nq) for i in range(nb0, nb)], zero_scr[...], toks)
        outproj(ul, o, nb0 * LANES)

    nl = TAILB * LANES
    sub8 = lax.broadcasted_iota(I32, (TOPC, 1), 0)
    lane = lax.broadcasted_iota(I32, (TOPC, LANES), 1)

    def key_index(k):
        return seq - 1 - (lax.bitcast_convert_type(k, I32) & (seq - 1))

    keys = key_scr[0:seq // LANES, :]
    piece = lax.broadcasted_iota(I32, (seq // LANES, 1), 0)
    keys = jnp.where(piece < (seq - nl) // LANES, keys, 0.0)
    ecol = jnp.zeros((TOPC, LANES), F32)
    erow = jnp.zeros((1, LANES), F32)
    h2e = jnp.zeros((TOPC, d), F32)
    late = []
    marks = finalize(seq - nl, sl_last, TB - nl, seq - nl, nl, late)
    zero = zero_scr[...]
    pace = dict(zip([int(v) for v in os.environ.get("KP_PG", "2,4,5,6,7").split(",")],
                    [int(v) for v in os.environ.get("KP_PM", "8,14,18,23,27").split(",")]))
    for i in range(TOPC):
        mx = jnp.max(jnp.max(keys, axis=0, keepdims=True), axis=1, keepdims=True)
        keys = jnp.where(keys == mx, 0.0, keys)
        ecol = jnp.where(sub8 == i, mx, ecol)
        erow = jnp.where(lane[0:1] == i, mx, erow)
        idx = key_index(mx)
        pick = jnp.logical_and(sub8 == i, lane == (idx & (LANES - 1)))
        sl = pl.ds(pl.multiple_of(idx[0, 0] & ~(LANES - 1), LANES), LANES)
        pick = jnp.where(pick, 1.0, 0.0)
        if i in pace:
            pick = lax.bitcast_convert_type(
                lax.bitcast_convert_type(pick, U32) | (marks[pace[i]] & zero), F32)
        h2e = h2e + lax.dot_general(pick.astype(BF16), h2_scr[:, sl], _NT,
                                    preferred_element_type=F32)

    racc = lax.bitcast_convert_type(late[0], U32)
    if os.environ.get("KP_AFTER", "0") == "1":
        racc = racc | _lanes(_fold(h2e) & zero, nl)
    late = [router_keys(lax.bitcast_convert_type(racc, F32), seq - nl)]
    krow = jnp.concatenate([late[0], erow], axis=1)
    kcol = jnp.concatenate([jnp.broadcast_to(late[0], (LANES, nl)).T, ecol], axis=0)
    cnt = [None] * 4
    for g in range(kcol.shape[0] // 8):
        one = jnp.where(_lanes(kcol[8 * g:8 * g + 8], nl + LANES) > krow, 1.0, 0.0)
        cnt[g % 4] = one if cnt[g % 4] is None else cnt[g % 4] + one
    rank = jnp.sum((cnt[0] + cnt[1]) + (cnt[2] + cnt[3]), axis=0, keepdims=True)
    chosen = rank == sub8.astype(F32)
    onehot = jnp.where(chosen, 1.0, 0.0).astype(BF16)
    h2pad = jnp.concatenate([h2e, jnp.zeros((TOPC, d), F32)], axis=0).astype(BF16)
    h2s = (jnp.dot(onehot[:, nl:nl + 2 * TOPC], h2pad, preferred_element_type=F32)
           + lax.dot_general(onehot[:, 0:nl], h2l_scr[...], _NT,
                             preferred_element_type=F32))
    top = jnp.max(jnp.where(chosen, krow, 0.0), axis=1, keepdims=True)
    idx_col = key_index(top)
    idxs = [idx_col[i:i + 1] for i in range(TOPC)]
    bases = [pl.multiple_of(idx_col[i, 0] & ~(LANES - 1), LANES) for i in range(TOPC)]
    hit = lane == (idx_col & (LANES - 1))
    picks = [jnp.where(jnp.logical_and(sub8 == i, hit), 1.0, 0.0).astype(BF16)
             for i in range(TOPC)]
    order = (lax.bitcast_convert_type(top, I32) >> 11) & 0xFFFF
    rbits = jnp.where(order >= 32768, order - 32768, -1 - order) << 16
    gate = _rb(_sigmoid(lax.bitcast_convert_type(rbits, F32)))
    xs = h2s.astype(BF16)
    for cp in out_hi:
        cp.start()
    g = _rb(jnp.dot(xs, wg_v[...], preferred_element_type=F32))
    g = _rb(g * _rb(_sigmoid(g)))
    u = _rb(jnp.dot(xs, wu_v[...], preferred_element_type=F32))
    gu = (g * u).astype(BF16)

    last_use = []
    for i in range(TOPC):
        ok = True
        for j in range(i + 1, TOPC):
            ok = jnp.logical_and(ok, bases[i] != bases[j])
        last_use.append(ok)

    def down(r0, r1):
        x1p = jnp.concatenate([x1_scr[r0:r1, pl.ds(bases[i], LANES)] for i in range(TOPC)], axis=1)
        x1s = lax.dot_general(jnp.concatenate(picks, axis=1), x1p, _NT,
                              preferred_element_type=F32)
        wd = pltpu.bitcast(wd_scr[:, r0:r1], BF16)
        y = _rb(jnp.dot(gu, wd, preferred_element_type=F32))
        hm = _rb(h2s[:, r0:r1] + _rb(y * gate))
        return x1s + mod_scr[2:3, r0:r1] * hm

    def patch(r0, r1, new):
        n = r1 - r0
        pad = jnp.concatenate([new, jnp.zeros((LANES - TOPC, n), F32)], axis=0)
        cols = pltpu.bitcast(pad.T.astype(BF16), U32)
        col = [jnp.broadcast_to(cols[:, j:j + 1], (n // 2, LANES)) for j in range(TOPC)]
        for i in range(TOPC):
            res = pltpu.bitcast(ot_v[r0:r1, pl.ds(bases[i], LANES)], U32)
            tok = lane[0:1, :] + (idxs[i] & ~(LANES - 1))
            for j in range(i + 1):
                res = jnp.where(tok == idxs[j], col[j], res)
            fix_v[i, r0:r1, :] = pltpu.bitcast(res, BF16)

    def fix_copy(i, r0, r1):
        return pltpu.make_async_copy(fix_v.at[i, r0:r1, :],
                                     o_hbm.at[r0:r1, pl.ds(bases[i], LANES)], fix_sems.at[i])

    def for_last(fn):
        for i in range(TOPC - 1):
            pl.when(last_use[i])(functools.partial(fn, i))
        fn(TOPC - 1)

    new = down(*chunks[0])
    out_lo.wait()
    for ci, (r0, r1) in enumerate(chunks):
        out_hi[ci].wait()
        nxt = down(*chunks[ci + 1]) if ci + 1 < len(chunks) else None
        patch(r0, r1, new)
        for_last(lambda i: fix_copy(i, r0, r1).start())
        new = nxt
    with _scope("w_fix"):
        for r0, r1 in chunks:
            for_last(lambda i: fix_copy(i, r0, r1).wait())


@jax.jit
def pallas_adaLN_cond__gqa_block_cached__moe_arch_mod__prompt_kernel(
    A_x: jax.Array,
    A_k_cache: jax.Array,
    A_v_cache: jax.Array,
    A_wq: jax.Array,
    A_wo: jax.Array,
    B_x: jax.Array,
    B_w_r: jax.Array,
    B_w_gate: jax.Array,
    B_w_up: jax.Array,
    B_w_down: jax.Array,
    c: jax.Array,
    w_mod: jax.Array,
):
    b, seq, d = A_x.shape
    _, hkv, sk, dh = A_k_cache.shape
    assert b == 1 and dh == DH and HQ == 2 * hkv
    assert seq & (seq - 1) == 0 and seq <= 2048
    f = B_w_gate.shape[1]
    n_grp = hkv // HG
    gw = 2 * HG * dh
    n_slots = 2 * HG * TB // LANES

    xt = A_x.reshape(seq, d).T
    wot = A_wo.T
    wdt = B_w_down.T
    k3 = A_k_cache.reshape(hkv, sk, dh)
    v3 = A_v_cache.reshape(hkv, sk, dh)

    hbm = pl.BlockSpec(memory_space=pl.ANY)
    out_t = pl.pallas_call(
        functools.partial(_kernel, n_heads=hkv),
        in_specs=[hbm] * 11,
        out_specs=hbm,
        out_shape=jax.ShapeDtypeStruct((d, seq), BF16),
        scratch_shapes=[
            pltpu.VMEM((d, seq), BF16),
            pltpu.VMEM((hkv, sk, dh), BF16),
            pltpu.VMEM((hkv, sk, dh), BF16),
            pltpu.VMEM((d, n_grp * gw), BF16),
            pltpu.VMEM((d, n_grp * gw), BF16),
            pltpu.VMEM((d, 6 * d), BF16),
            pltpu.VMEM((d, f), BF16),
            pltpu.VMEM((d, f), BF16),
            pltpu.VMEM((d, f + WP), BF16),
            pltpu.VMEM((d, seq + SP), BF16),
            pltpu.VMEM((2, TB, d), BF16),
            pltpu.VMEM((2, d, TB), F32),
            pltpu.VMEM((n_slots, sk, LANES), F32),
            pltpu.VMEM((n_slots, 8, LANES), F32),
            pltpu.VMEM((HG, dh // 2, sk), U32),
            pltpu.VMEM((8, d), F32),
            pltpu.VMEM((6 * d, LANES), F32),
            pltpu.VMEM(((seq + SP) // LANES + 7 & ~7, LANES), F32),
            pltpu.VMEM((d, seq + SP), BF16),
            pltpu.VMEM((d, seq + SP), BF16),
            pltpu.VMEM((8, LANES), U32),
            pltpu.VMEM((TOPC, d, LANES), BF16),
            pltpu.VMEM((1, d), BF16),
            pltpu.VMEM((d,), BF16),
            pltpu.VMEM((1, 4 * d), F32),
            pltpu.VMEM((f // 2, d), U32),
            pltpu.VMEM((d, TAILB * LANES), BF16),
            pltpu.SemaphoreType.DMA((4, n_grp)),
            pltpu.SemaphoreType.DMA((10,)),
            pltpu.SemaphoreType.DMA((3,)),
            pltpu.SemaphoreType.DMA((len(EDGES),)),
            pltpu.SemaphoreType.DMA((TOPC,)),
        ],
        compiler_params=pltpu.CompilerParams(
            disable_bounds_checks=True,
            disable_semaphore_checks=True,
            vmem_limit_bytes=110 * 1024 * 1024,
        ),
    )(xt, k3, v3, A_wq, wot, B_w_r, B_w_gate, B_w_up, wdt, c, w_mod)
    return out_t.T.reshape(b, seq, d)
```

```python
import contextlib
import functools
import math
import os

import jax
import jax.numpy as jnp
from jax import lax
import jax.experimental.pallas as pl
import jax.experimental.pallas.tpu as pltpu

F32 = jnp.float32
BF16 = jnp.bfloat16
I32 = jnp.int32
U32 = jnp.uint32

HQ = 32
DH = 128
TOPC = 8
EPS = 1e-05
EPS_BF16 = 1.0013580322265625e-05
LANES = 128

TB = 512
HG = 2
TIE0 = int(os.environ.get("KP_TIE0", "2"))
NTIE = int(os.environ.get("KP_NTIE", "3"))
SP = int(os.environ.get("KP_SP", "128"))
NM1 = int(os.environ.get("KP_NM1", "8"))
NM2 = int(os.environ.get("KP_NM2", "12"))
NM3 = int(os.environ.get("KP_NM3", "16"))
TLO = int(os.environ.get("KP_TLO", "8"))
NF1 = int(os.environ.get("KP_NF1", "9"))
NF2 = int(os.environ.get("KP_NF2", "6"))
NF3 = int(os.environ.get("KP_NF3", "18"))
NVT = int(os.environ.get("KP_NVT", "16"))
TAILB = int(os.environ.get("KP_TAILB", "2"))
SIDE_ROW = int(os.environ.get("KP_SIDE_ROW", "6"))
EDGES = [int(e) for e in os.environ.get("KP_EDGES", "0,128,256,384,512,576").split(",")]
MODC = int(os.environ.get("KP_MODC", "384"))
MP = int(os.environ.get("KP_MP", "384"))
NMP = int(os.environ.get("KP_NMP", "12"))
WP = 256
REMF = int(os.environ.get("KP_REMF", "1"))
DEFM = int(os.environ.get("KP_DEFM", "1"))
KAP = int(os.environ.get("KP_KAP", "0"))
LATEKV = int(os.environ.get("KP_LATEKV", "1"))
EARLYMOD = int(os.environ.get("KP_EARLYMOD", "0"))
SCOPES = os.environ.get("KP_SCOPES", "") == "1"

_NT = (((1,), (1,)), ((), ()))


def _rb(x):
    return x.astype(BF16).astype(F32)


def _sigmoid(x):
    return 1.0 / (1.0 + jnp.exp(-x))


def _lanes(col, width):
    reps = width // LANES
    return col if reps == 1 else jnp.concatenate([col] * reps, axis=1)


def _fold(x):
    xi = lax.bitcast_convert_type(x, U32)
    tok = None
    for r in range(0, x.shape[0], 8):
        for c in range(0, x.shape[1] - LANES + 1, LANES):
            t = xi[r:r + 8, c:c + LANES]
            tok = t if tok is None else tok | t
    return tok


def _colsum(x, marks, nmarks):
    n = x.shape[0] // 8
    acc = x[0:8]
    for g in range(1, n):
        acc = acc + x[8 * g:8 * g + 8]
        if ((g + 1) * nmarks) % n == 0:
            marks.append(_fold(acc))
    return jnp.sum(acc, axis=0, keepdims=True)


def _tie_rows(lhs, toks, zero, lo, hi):
    if not toks:
        return lhs
    lu = pltpu.bitcast(lhs, U32)
    rows = [lu[8 * r:8 * r + 8] for r in range(lu.shape[0] // 8)]
    for i, tok in enumerate(toks):
        r = lo + ((i + 1) * (hi - lo)) // len(toks) - 1
        rows[r] = rows[r] | (tok & zero)
    return pltpu.bitcast(jnp.concatenate(rows, axis=0), BF16)


def _merge(a, b):
    keyed = [((i + 1) / len(a), t) for i, t in enumerate(a)]
    keyed += [((i + 1) / len(b), t) for i, t in enumerate(b)]
    return [t for _, t in sorted(keyed, key=lambda kv: kv[0])]


def _span(start, size):
    if isinstance(start, int):
        return pl.ds(start, size)
    return pl.ds(pl.multiple_of(start, LANES), size)


def _scope(name):
    return jax.named_scope(name) if SCOPES else contextlib.nullcontext()


def _kernel(xt_hbm, k_hbm, v_hbm, wq_hbm, wot_hbm, wr_hbm, wg_hbm, wu_hbm, wdt_hbm,
            c_hbm, wmod_hbm, o_hbm,
            xt_v, k_v, v_v, wq_v, wot_v, wmod_v, wg_v, wu_v, wdt_v, ot_v,
            h_scr, acc_scr, st_scr, m_scr, vt_scr, mod_scr, col_scr, key_scr, h2_scr, x1_scr,
            zero_scr, fix_v, c_ref, wr_ref, row_scr, wd_scr, h2l_scr,
            grp_sems, misc_sems, mlp_sems, out_sems, fix_sems,
            *, n_heads):
    d, seq = xt_v.shape
    sk = k_v.shape[1]
    n_grp = n_heads // HG
    n_blk = seq // TB
    n_units = n_grp * n_blk
    nb = TB // LANES
    nq = 2 * HG
    nt = sk // LANES
    gbits = n_grp.bit_length() - 1
    gw = nq * DH
    qscale = (DH ** -0.5) * math.log2(math.e)

    def grp_of(u):
        return u & (n_grp - 1)

    def blk_of(u):
        return u >> gbits

    def grp_copies(g, n=1):
        cs, hs, ps = pl.ds(g * gw, n * gw), pl.ds(g * HG, n * HG), pl.ds((g - 1) * gw, n * gw)
        return (pltpu.make_async_copy(wq_hbm.at[:, cs], wq_v.at[:, cs], grp_sems.at[0, g]),
                pltpu.make_async_copy(k_hbm.at[hs], k_v.at[hs], grp_sems.at[1, g]),
                pltpu.make_async_copy(v_hbm.at[hs], v_v.at[hs], grp_sems.at[2, g]),
                pltpu.make_async_copy(wot_hbm.at[:, ps], wot_v.at[:, ps], grp_sems.at[3, g]))

    def col_copy(src, dst, lo, hi, sem):
        return pltpu.make_async_copy(src.at[:, lo:hi], dst.at[:, lo:hi], sem)

    x_first = col_copy(xt_hbm, xt_v, 0, TB, misc_sems.at[0])
    x_rest = col_copy(xt_hbm, xt_v, TB, seq, misc_sems.at[1])
    mod_first = [col_copy(wmod_hbm, wmod_v, MODC, 2 * d, misc_sems.at[8]),
                 col_copy(wmod_hbm, wmod_v, 0, MODC, misc_sems.at[9])]
    mod_rest = col_copy(wmod_hbm, wmod_v, 2 * d, 6 * d, misc_sems.at[3])
    mlp_g = pltpu.make_async_copy(wg_hbm, wg_v, mlp_sems.at[0])
    mlp_u = pltpu.make_async_copy(wu_hbm, wu_v, mlp_sems.at[1])
    ff = wdt_hbm.shape[1]
    mlp_d = pltpu.make_async_copy(wdt_hbm, wdt_v.at[:, 0:ff], mlp_sems.at[2])
    out_lo = col_copy(ot_v, o_hbm, 0, seq - TB, out_sems.at[0])
    chunks = list(zip(EDGES[:-1], EDGES[1:]))
    out_hi = [pltpu.make_async_copy(ot_v.at[r0:r1, seq - TB:seq], o_hbm.at[r0:r1, seq - TB:seq],
                                    out_sems.at[1 + i]) for i, (r0, r1) in enumerate(chunks)]

    def silu_c():
        cc = c_ref[...].astype(F32)
        return jnp.broadcast_to((cc * _rb(_sigmoid(cc))).astype(BF16), (8, d))

    def ln1_norm(t0, n, marks):
        x = xt_v[:, _span(t0, n)].astype(F32)
        mu = _colsum(x, marks, NM1) * (1.0 / d)
        xc = x - mu
        var = _colsum(xc * xc, marks, NM2) * (1.0 / d)
        return (xc * lax.rsqrt(var + EPS)).astype(BF16).T

    def ln1_mod(ln, slot, r0, marks):
        n = ln.shape[0]
        h = ln.astype(F32) * mod_scr[1:2, :] + mod_scr[0:1, :]
        h_scr[slot, _span(r0, n), :] = h.astype(BF16)
        step = max(n // NM3, 8)
        for r in range(step - 8, n, step):
            marks.append(_fold(h[r:r + 8]))

    def mod_piece(src, dst, marks):
        w = wmod_v[:, _span(src, MP)].astype(F32)
        row = _rb(_colsum(w * _lanes(col_scr[5 * d:6 * d, :], MP), marks, NMP))
        pos = dst + lax.broadcasted_iota(I32, (1, MP), 1)
        is_cb = jnp.logical_and(pos >= 2 * d, pos < 3 * d)
        row = jnp.where(is_cb, _rb(1.0 + row), row)
        row_scr[:, _span(dst, MP)] = row
        col = jnp.broadcast_to(row, (LANES, MP)).T
        col_scr[_span(dst, MP), :] = col
        for r in range(LANES - 8, MP, LANES):
            marks.append(lax.bitcast_convert_type(col[r:r + 8], U32))

    def wd_piece(src, dst, marks):
        w = pltpu.bitcast(wdt_v[:, _span(src, WP)].T, U32)
        wd_scr[pl.ds(pl.multiple_of(dst // 2, WP // 2), WP // 2), :] = w
        for r in range(56, WP // 2, 64):
            for c in range(0, d - LANES + 1, LANES):
                marks.append(w[r:r + 8, c:c + LANES])

    def qproj(u, lo=0, hi=gw, parts=1):
        qs = []
        ws = _span(grp_of(u) * gw + lo, hi - lo)
        for r0 in range(0, TB, TB // parts):
            rs, dm = slice(r0, r0 + TB // parts), d - d % LANES
            if REMF:
                q = jnp.dot(h_scr[blk_of(u) & 1, rs, dm:d], wq_v[dm:d, ws],
                            preferred_element_type=F32)
                q = jnp.dot(h_scr[blk_of(u) & 1, rs, 0:dm], wq_v[0:dm, ws],
                            preferred_element_type=F32) + q
            else:
                q = jnp.dot(h_scr[blk_of(u) & 1, rs, :], wq_v[:, ws],
                            preferred_element_type=F32)
            qs.append((q * qscale).astype(BF16))
        return jnp.concatenate(qs, axis=0)

    def qk(u, q, j, toks=(), zero=None):
        k = _tie_rows(k_v[grp_of(u) * HG + j // 2], toks, zero, TLO, sk // 16)
        st = lax.dot_general(k, q[:, j * DH:(j + 1) * DH], _NT,
                             preferred_element_type=F32)
        for i in range(nb):
            blk = st[:, i * LANES:(i + 1) * LANES]
            st_scr[j * nb + i] = blk
            if DEFM:
                m_scr[j * nb + i] = jnp.max(blk.reshape(sk // 8, 8, LANES), axis=0)
            else:
                m_scr[j * nb + i, 0:1] = jnp.max(blk, axis=0, keepdims=True)

    def v_transpose(u, i, marks=None):
        vt = pltpu.bitcast(v_v[grp_of(u) * HG + i].T, U32)
        vt_scr[i] = vt
        if marks is not None:
            step = sk // NVT
            for c in range(step - LANES, sk, step):
                marks.append(vt[DH // 2 - 8:DH // 2, c:c + LANES])

    def pv(slots, zero, toks=()):
        ps, ls, pairs = [], [], []
        for sl in slots:
            m = jnp.max(m_scr[sl], axis=0, keepdims=True) if DEFM else m_scr[sl, 0:1]
            p = jnp.exp2(st_scr[sl] - m)
            accs = [None] * 4
            for tile in range(nt):
                for r0 in range(tile * LANES + LANES - 16, tile * LANES - 16, -16):
                    pair = p[r0:r0 + 8] + p[r0 + 8:r0 + 16]
                    pairs.append(pair)
                    a = accs[tile % 4]
                    accs[tile % 4] = pair if a is None else a + pair
            ls.append(jnp.sum((accs[0] + accs[1]) + (accs[2] + accs[3]), axis=0, keepdims=True))
            ps.append(p.astype(BF16))
        outs = []
        ntiles = len(slots) * nt
        side = {}
        for i, tok in enumerate(toks):
            side.setdefault(((i + 1) * ntiles) // len(toks) - 1, []).append(tok)
        for i, sl in enumerate(slots):
            vu = vt_scr[sl // (2 * nb)]
            tiles = []
            for c in range(nt):
                g = i * nt + c + 4
                rows = []
                for r in range(8):
                    x = vu[8 * r:8 * r + 8, c * LANES:(c + 1) * LANES]
                    if g < ntiles and TIE0 <= r < TIE0 + NTIE:
                        src = pairs[g * 8 + (r - TIE0)]
                        x = x | (lax.bitcast_convert_type(src, U32) & zero)
                    if r == SIDE_ROW:
                        for tok in side.get(i * nt + c, ()):
                            x = x | (tok & zero)
                    rows.append(x)
                tiles.append(jnp.concatenate(rows, axis=0))
            lhs = pltpu.bitcast(jnp.concatenate(tiles, axis=1), BF16)
            o = jnp.dot(lhs, ps[i], preferred_element_type=F32)
            outs.append((o * (1.0 / ls[i])).astype(BF16))
        return outs

    def outproj(u, o, lo=0):
        w = len(o) // nq
        o2 = jnp.concatenate(
            [jnp.concatenate(o[j * w:(j + 1) * w], axis=1) for j in range(nq)], axis=0)
        contrib = jnp.dot(wot_v[:, _span(grp_of(u) * gw, gw)], o2, preferred_element_type=F32)
        hi = lo + w * LANES
        slot = blk_of(u) & 1
        old = jnp.where(grp_of(u) > 0, acc_scr[slot, :, lo:hi], 0.0)
        acc_scr[slot, :, lo:hi] = old + contrib

    def router_keys(racc, t0):
        r = _rb(jnp.sum(racc, axis=0, keepdims=True)) + 0.0
        bits = lax.bitcast_convert_type(r, I32) >> 16
        order = jnp.where(bits < 0, -1 - bits, bits + 32768)
        pos = t0 + lax.broadcasted_iota(I32, r.shape, 1)
        return lax.bitcast_convert_type((order << 11) + (seq - 1 - pos) + 0x20000000, F32)

    def finalize(t0, slot, a0, dst, n, keys_out=None):
        marks = []
        cs = _span(dst, n)
        x = xt_v[:, _span(t0, n)].astype(F32)
        att = acc_scr[slot, :, _span(a0, n)]
        x1b = (x + _lanes(col_scr[0:d, :], n) * att).astype(BF16)
        x1_scr[:, cs] = x1b
        ot_v[:, cs] = x1b
        mu = _colsum(x1b.astype(F32), marks, NF1) * (1.0 / d)
        mub = _rb(mu)
        xc = x1_scr[:, cs].astype(F32) - mub
        var = _colsum(xc * xc, marks, NF2) * (1.0 / d) - (mu - mub) * (mu - mub)
        inv = 1.0 / _rb(jnp.sqrt(_rb(_rb(jnp.maximum(var, 0.0)) + EPS_BF16)))
        step = d // NF3
        racc = None
        for r0 in range(0, d, step):
            rs = slice(r0, r0 + step)
            x1 = ot_v[rs, cs].astype(F32)
            ln = _rb(_rb(x1 - mub) * inv)
            h2b = (_rb(ln * _lanes(col_scr[2 * d + r0:2 * d + r0 + step, :], n))
                   + _lanes(col_scr[d + r0:d + r0 + step, :], n)).astype(BF16)
            if keys_out is None:
                h2_scr[rs, cs] = h2b
            else:
                h2l_scr[rs, :] = h2b
            h2 = h2b.astype(F32)
            out = x1 + _lanes(col_scr[3 * d + r0:3 * d + r0 + step, :], n) * h2
            ot_v[rs, cs] = out.astype(BF16)
            rp = h2 * _lanes(col_scr[4 * d + r0:4 * d + r0 + step, :], n)
            for g in range(0, step, 8):
                racc = rp[g:g + 8] if racc is None else racc + rp[g:g + 8]
            marks.append(_fold(racc) | _fold(out))
        if keys_out is not None:
            keys_out.append(racc)
            return marks
        key = router_keys(racc, t0)
        for i in range(n // LANES):
            key_scr[pl.ds(dst // LANES + i, 1), :] = key[:, i * LANES:(i + 1) * LANES]
        return marks

    hw = gw // 2
    wq0a = col_copy(wq_hbm, wq_v, 0, hw, grp_sems.at[0, 0])
    wq0b = col_copy(wq_hbm, wq_v, hw, gw, misc_sems.at[4])
    k0a = pltpu.make_async_copy(k_hbm.at[0], k_v.at[0], grp_sems.at[1, 0])
    k0b = pltpu.make_async_copy(k_hbm.at[1], k_v.at[1], misc_sems.at[5])
    v0 = pltpu.make_async_copy(v_hbm.at[0:HG], v_v.at[0:HG], grp_sems.at[2, 0])
    wq1, k1, v1, wo0 = grp_copies(1)
    wo_last = col_copy(wot_hbm, wot_v, (n_grp - 1) * gw, n_grp * gw, grp_sems.at[3, 0])
    c_copy = pltpu.make_async_copy(c_hbm, c_ref, misc_sems.at[6])
    wr_copy = pltpu.make_async_copy(wr_hbm, wr_ref, misc_sems.at[7])
    c_copy.start()
    wr_copy.start()
    x_first.start()
    mod_first[0].start()
    mod_first[1].start()
    wq0a.start()
    wq0b.start()
    acc_scr[1] = jnp.zeros((d, TB), F32)
    col_scr[0:4 * d, :] = jnp.zeros((4 * d, LANES), F32)
    wdt_v[:, ff:ff + WP] = jnp.zeros((d, WP), BF16)
    with _scope("w_x"):
        c_copy.wait()
        wr_copy.wait()
        x_first.wait()
    cbits = lax.bitcast_convert_type(c_ref[:, 0:LANES].astype(F32), U32)
    zero_scr[...] = jnp.broadcast_to(cbits & 0xFFFF, (8, LANES))
    h_scr[0] = ln1_norm(0, TB, [])
    sc = silu_c()
    wr = wr_ref[...].reshape(1, d).astype(F32)
    col_scr[4 * d:5 * d, :] = jnp.broadcast_to(wr, (LANES, d)).T
    col_scr[5 * d:6 * d, :] = jnp.broadcast_to(sc[0:1, :].astype(F32), (LANES, d)).T
    with _scope("w_wmod"):
        mod_first[0].wait()
    mod = _rb(jnp.dot(sc, wmod_v[:, MODC:2 * d], preferred_element_type=F32))
    mod_scr[0:1, MODC:d] = mod[0:1, 0:d - MODC]
    mod_scr[1:2, :] = _rb(1.0 + mod[0:1, d - MODC:2 * d - MODC])
    with _scope("w_wmod2"):
        mod_first[1].wait()
    k0a.start(priority=KAP)
    if not LATEKV:
        k0b.start(priority=1)
        v0.start(priority=1)
    mod_scr[0:1, 0:MODC] = _rb(jnp.dot(sc, wmod_v[:, 0:MODC], preferred_element_type=F32))[0:1]
    if EARLYMOD:
        ln1_mod(h_scr[0], 0, 0, [])
    with _scope("w_wq"):
        wq0a.wait()
    if LATEKV:
        k0b.start(priority=1)
        v0.start(priority=1)
    if not EARLYMOD:
        ln1_mod(h_scr[0], 0, 0, [])
    qa = qproj(0, 0, hw, 2)
    with _scope("w_k"):
        wq0b.wait()
        k0a.wait()
    wq1.start(priority=1)
    k1.start(priority=1)
    q = jnp.concatenate([qa, qproj(0, hw, gw, 2)], axis=1)
    qk(0, q, 0)
    qk(0, q, 1)
    with _scope("w_v"):
        k0b.wait()
        v0.wait()
    v1.start()
    wo0.start()
    with _scope("qk0"):
        zero = zero_scr[...]
        for i in range(HG):
            marks = []
            v_transpose(0, i, marks)
            qk(0, q, nq - HG + i, marks, zero)

    assert n_grp == 8 and HG == 2
    loads = [[wq1, k1, v1, wo0],
             [*grp_copies(2), mod_rest, x_rest],
             [*grp_copies(3, 3)],
             [*grp_copies(6, 2), wo_last],
             [mlp_d],
             [mlp_g, mlp_u]]
    wd0 = len(loads) - 1
    npc = TB // SP
    nmp = 4 * d // MP

    def manage(i):
        for cp in loads[i - 1]:
            cp.wait()
        for cp in loads[i]:
            cp.start()

    def steady(u, carry):
        with _scope("body"):
            zero = zero_scr[...]
            blk, g = blk_of(u), grp_of(u)
            off = ((g - 1) & (npc - 1)) * SP
            q = qproj(u)
            o = pv(range(0, 2 * nb), zero)
            live = jnp.logical_and(blk > 0, jnp.logical_and(g >= 1, g <= npc))
            t0 = jnp.maximum(blk - 1, 0) * TB + off
            marks = finalize(t0, (blk + 1) & 1, off, jnp.where(live, t0, seq), SP)
            wp = jnp.clip(u - wd0, 0, ff // WP - 1) * WP
            wmarks = []
            wd_piece(jnp.where(u >= wd0, wp, ff), wp, wmarks)
            qk(u, q, 0, _merge(marks, wmarks), zero)
            marks = []
            nxt = jnp.where(u >= 2, jnp.minimum(blk + 1, n_blk - 1), 0)
            ln = ln1_norm(nxt * TB + off, SP, marks)
            ln1_mod(ln, (blk + 1) & 1, off, marks)
            qk(u, q, 1, marks, zero)
            o += pv(range(2 * nb, 4 * nb), zero)
            outproj(u - 1, o)
            marks = []
            v_transpose(u, 0, marks)
            mp = jnp.clip(u - 2, 0, nmp - 1) * MP
            mmarks = []
            mod_piece(jnp.where(u >= 2, 2 * d + mp, 0), mp, mmarks)
            qk(u, q, 2, _merge(marks, mmarks), zero)
            marks = []
            v_transpose(u, 1, marks)
            qk(u, q, 3, marks, zero)
        return carry

    def stage(i, carry):
        for k in range(1, len(loads)):
            pl.when(i == k)(functools.partial(manage, k))
        return lax.fori_loop(i, jnp.where(i < len(loads) - 1, i + 1, n_units), steady, carry)

    lax.fori_loop(1, len(loads), stage, 0)

    ul = n_units - 1
    tl = seq - TB
    sl_last = (n_blk - 1) & 1
    nb0 = nb - TAILB
    with _scope("e_pva"):
        mod_scr[2:3, :] = row_scr[:, 3 * d:4 * d]
        outproj(ul, pv([j * nb + i for j in range(nq) for i in range(nb0)], zero_scr[...]))
    mlp_g.wait()
    mlp_u.wait()
    out_lo.start()
    with _scope("e_pvb"):
        toks = finalize(tl, sl_last, 0, tl, nb0 * LANES)
        o = pv([j * nb + i for j in range(nq) for i in range(nb0, nb)], zero_scr[...], toks)
        outproj(ul, o, nb0 * LANES)

    nl = TAILB * LANES
    sub8 = lax.broadcasted_iota(I32, (TOPC, 1), 0)
    lane = lax.broadcasted_iota(I32, (TOPC, LANES), 1)

    def key_index(k):
        return seq - 1 - (lax.bitcast_convert_type(k, I32) & (seq - 1))

    def piece_base(idx, limit):
        return pl.multiple_of(jnp.clip(idx >> 7, 0, limit // LANES - 1) * LANES, LANES)

    keys = key_scr[0:seq // LANES, :]
    piece = lax.broadcasted_iota(I32, (seq // LANES, 1), 0)
    keys = jnp.where(piece < (seq - nl) // LANES, keys, 0.0)
    ecol = jnp.zeros((TOPC, LANES), F32)
    erow = jnp.zeros((1, LANES), F32)
    h2e = jnp.zeros((TOPC, d), F32)
    late = []
    marks = finalize(seq - nl, sl_last, TB - nl, seq - nl, nl, late)
    zero = zero_scr[...]
    pace = dict(zip([int(v) for v in os.environ.get("KP_PG", "2,4,5,6,7").split(",")],
                    [int(v) for v in os.environ.get("KP_PM", "8,14,18,23,27").split(",")]))
    for i in range(TOPC):
        mx = jnp.max(jnp.max(keys, axis=0, keepdims=True), axis=1, keepdims=True)
        keys = jnp.where(keys == mx, 0.0, keys)
        ecol = jnp.where(sub8 == i, mx, ecol)
        erow = jnp.where(lane[0:1] == i, mx, erow)
        idx = key_index(mx)
        pick = jnp.logical_and(sub8 == i, lane == (idx & (LANES - 1)))
        sl = pl.ds(piece_base(idx[0, 0], seq - nl), LANES)
        pick = jnp.where(pick, 1.0, 0.0)
        if i in pace:
            pick = lax.bitcast_convert_type(
                lax.bitcast_convert_type(pick, U32) | (marks[pace[i]] & zero), F32)
        h2e = h2e + lax.dot_general(pick.astype(BF16), h2_scr[:, sl], _NT,
                                    preferred_element_type=F32)

    late = [router_keys(late[0], seq - nl)]
    krow = jnp.concatenate([late[0], erow], axis=1)
    kcol = jnp.concatenate([jnp.broadcast_to(late[0], (LANES, nl)).T, ecol], axis=0)
    cnt = [None] * 4
    for g in range(kcol.shape[0] // 8):
        one = jnp.where(_lanes(kcol[8 * g:8 * g + 8], nl + LANES) > krow, 1.0, 0.0)
        cnt[g % 4] = one if cnt[g % 4] is None else cnt[g % 4] + one
    rank = jnp.sum((cnt[0] + cnt[1]) + (cnt[2] + cnt[3]), axis=0, keepdims=True)
    chosen = rank == sub8.astype(F32)
    onehot = jnp.where(chosen, 1.0, 0.0).astype(BF16)
    h2pad = jnp.concatenate([h2e, jnp.zeros((TOPC, d), F32)], axis=0).astype(BF16)
    h2s = (jnp.dot(onehot[:, nl:nl + 2 * TOPC], h2pad, preferred_element_type=F32)
           + lax.dot_general(onehot[:, 0:nl], h2l_scr[...], _NT,
                             preferred_element_type=F32))
    top = jnp.max(jnp.where(chosen, krow, 0.0), axis=1, keepdims=True)
    idx_col = key_index(top)
    idxs = [idx_col[i:i + 1] for i in range(TOPC)]
    bases = [piece_base(idx_col[i, 0], seq) for i in range(TOPC)]
    hit = lane == (idx_col & (LANES - 1))
    picks = [jnp.where(jnp.logical_and(sub8 == i, hit), 1.0, 0.0).astype(BF16)
             for i in range(TOPC)]
    order = (lax.bitcast_convert_type(top, I32) >> 11) & 0xFFFF
    rbits = jnp.where(order >= 32768, order - 32768, -1 - order) << 16
    gate = _rb(_sigmoid(lax.bitcast_convert_type(rbits, F32)))
    xs = h2s.astype(BF16)
    for cp in out_hi:
        cp.start()
    g = _rb(jnp.dot(xs, wg_v[...], preferred_element_type=F32))
    g = _rb(g * _rb(_sigmoid(g)))
    u = _rb(jnp.dot(xs, wu_v[...], preferred_element_type=F32))
    gu = (g * u).astype(BF16)

    last_use = []
    for i in range(TOPC):
        ok = True
        for j in range(i + 1, TOPC):
            ok = jnp.logical_and(ok, bases[i] != bases[j])
        last_use.append(ok)

    def down(r0, r1):
        x1p = jnp.concatenate([x1_scr[r0:r1, pl.ds(bases[i], LANES)] for i in range(TOPC)], axis=1)
        x1s = lax.dot_general(jnp.concatenate(picks, axis=1), x1p, _NT,
                              preferred_element_type=F32)
        wd = pltpu.bitcast(wd_scr[:, r0:r1], BF16)
        y = _rb(jnp.dot(gu, wd, preferred_element_type=F32))
        hm = _rb(h2s[:, r0:r1] + _rb(y * gate))
        return x1s + mod_scr[2:3, r0:r1] * hm

    def patch(r0, r1, new):
        n = r1 - r0
        pad = jnp.concatenate([new, jnp.zeros((LANES - TOPC, n), F32)], axis=0)
        cols = pltpu.bitcast(pad.T.astype(BF16), U32)
        col = [jnp.broadcast_to(cols[:, j:j + 1], (n // 2, LANES)) for j in range(TOPC)]
        for i in range(TOPC):
            res = pltpu.bitcast(ot_v[r0:r1, pl.ds(bases[i], LANES)], U32)
            tok = lane[0:1, :] + (idxs[i] & ~(LANES - 1))
            for j in range(i + 1):
                res = jnp.where(tok == idxs[j], col[j], res)
            fix_v[i, r0:r1, :] = pltpu.bitcast(res, BF16)

    def fix_copy(i, r0, r1):
        return pltpu.make_async_copy(fix_v.at[i, r0:r1, :],
                                     o_hbm.at[r0:r1, pl.ds(bases[i], LANES)], fix_sems.at[i])

    def for_last(fn):
        for i in range(TOPC - 1):
            pl.when(last_use[i])(functools.partial(fn, i))
        fn(TOPC - 1)

    new = down(*chunks[0])
    out_lo.wait()
    for ci, (r0, r1) in enumerate(chunks):
        out_hi[ci].wait()
        nxt = down(*chunks[ci + 1]) if ci + 1 < len(chunks) else None
        patch(r0, r1, new)
        for_last(lambda i: fix_copy(i, r0, r1).start())
        new = nxt
    with _scope("w_fix"):
        for r0, r1 in chunks:
            for_last(lambda i: fix_copy(i, r0, r1).wait())


@jax.jit
def pallas_adaLN_cond__gqa_block_cached__moe_arch_mod__prompt_kernel(
    A_x: jax.Array,
    A_k_cache: jax.Array,
    A_v_cache: jax.Array,
    A_wq: jax.Array,
    A_wo: jax.Array,
    B_x: jax.Array,
    B_w_r: jax.Array,
    B_w_gate: jax.Array,
    B_w_up: jax.Array,
    B_w_down: jax.Array,
    c: jax.Array,
    w_mod: jax.Array,
):
    b, seq, d = A_x.shape
    _, hkv, sk, dh = A_k_cache.shape
    assert b == 1 and dh == DH and HQ == 2 * hkv
    assert seq & (seq - 1) == 0 and seq <= 2048
    f = B_w_gate.shape[1]
    n_grp = hkv // HG
    gw = 2 * HG * dh
    n_slots = 2 * HG * TB // LANES

    xt = A_x.reshape(seq, d).T
    wot = A_wo.T
    wdt = B_w_down.T
    k3 = A_k_cache.reshape(hkv, sk, dh)
    v3 = A_v_cache.reshape(hkv, sk, dh)

    hbm = pl.BlockSpec(memory_space=pl.ANY)
    out_t = pl.pallas_call(
        functools.partial(_kernel, n_heads=hkv),
        in_specs=[hbm] * 11,
        out_specs=hbm,
        out_shape=jax.ShapeDtypeStruct((d, seq), BF16),
        scratch_shapes=[
            pltpu.VMEM((d, seq), BF16),
            pltpu.VMEM((hkv, sk, dh), BF16),
            pltpu.VMEM((hkv, sk, dh), BF16),
            pltpu.VMEM((d, n_grp * gw), BF16),
            pltpu.VMEM((d, n_grp * gw), BF16),
            pltpu.VMEM((d, 6 * d), BF16),
            pltpu.VMEM((d, f), BF16),
            pltpu.VMEM((d, f), BF16),
            pltpu.VMEM((d, f + WP), BF16),
            pltpu.VMEM((d, seq + SP), BF16),
            pltpu.VMEM((2, TB, d), BF16),
            pltpu.VMEM((2, d, TB), F32),
            pltpu.VMEM((n_slots, sk, LANES), F32),
            pltpu.VMEM((n_slots, 8, LANES), F32),
            pltpu.VMEM((HG, dh // 2, sk), U32),
            pltpu.VMEM((8, d), F32),
            pltpu.VMEM((6 * d, LANES), F32),
            pltpu.VMEM(((seq + SP) // LANES + 7 & ~7, LANES), F32),
            pltpu.VMEM((d, seq + SP), BF16),
            pltpu.VMEM((d, seq + SP), BF16),
            pltpu.VMEM((8, LANES), U32),
            pltpu.VMEM((TOPC, d, LANES), BF16),
            pltpu.VMEM((1, d), BF16),
            pltpu.VMEM((d,), BF16),
            pltpu.VMEM((1, 4 * d), F32),
            pltpu.VMEM((f // 2, d), U32),
            pltpu.VMEM((d, TAILB * LANES), BF16),
            pltpu.SemaphoreType.DMA((4, n_grp)),
            pltpu.SemaphoreType.DMA((10,)),
            pltpu.SemaphoreType.DMA((3,)),
            pltpu.SemaphoreType.DMA((len(EDGES),)),
            pltpu.SemaphoreType.DMA((TOPC,)),
        ],
        compiler_params=pltpu.CompilerParams(
            disable_bounds_checks=True,
            disable_semaphore_checks=True,
            vmem_limit_bytes=110 * 1024 * 1024,
        ),
    )(xt, k3, v3, A_wq, wot, B_w_r, B_w_gate, B_w_up, wdt, c, w_mod)
    return out_t.T.reshape(b, seq, d)
```

```python
import contextlib
import functools
import math
import os

import jax
import jax.numpy as jnp
from jax import lax
import jax.experimental.pallas as pl
import jax.experimental.pallas.tpu as pltpu

F32 = jnp.float32
BF16 = jnp.bfloat16
I32 = jnp.int32
U32 = jnp.uint32

HQ = 32
DH = 128
TOPC = 8
EPS = 1e-05
EPS_BF16 = 1.0013580322265625e-05
LANES = 128

TB = 512
HG = 2
TIE0 = int(os.environ.get("KP_TIE0", "2"))
NTIE = int(os.environ.get("KP_NTIE", "3"))
SP = int(os.environ.get("KP_SP", "128"))
NM1 = int(os.environ.get("KP_NM1", "8"))
NM2 = int(os.environ.get("KP_NM2", "12"))
NM3 = int(os.environ.get("KP_NM3", "16"))
TLO = int(os.environ.get("KP_TLO", "8"))
NF1 = int(os.environ.get("KP_NF1", "9"))
NF2 = int(os.environ.get("KP_NF2", "6"))
NF3 = int(os.environ.get("KP_NF3", "18"))
NVT = int(os.environ.get("KP_NVT", "16"))
TAILB = int(os.environ.get("KP_TAILB", "2"))
SIDE_ROW = int(os.environ.get("KP_SIDE_ROW", "6"))
EDGES = [int(e) for e in os.environ.get("KP_EDGES", "0,128,256,384,512,576").split(",")]
MODC = int(os.environ.get("KP_MODC", "384"))
MP = int(os.environ.get("KP_MP", "384"))
NMP = int(os.environ.get("KP_NMP", "12"))
WP = 256
REMF = int(os.environ.get("KP_REMF", "1"))
DEFM = int(os.environ.get("KP_DEFM", "1"))
KAP = int(os.environ.get("KP_KAP", "0"))
LATEKV = int(os.environ.get("KP_LATEKV", "1"))
EARLYMOD = int(os.environ.get("KP_EARLYMOD", "0"))
NR = int(os.environ.get("KP_NR", "2"))
RG = int(os.environ.get("KP_RG", "1"))
KS = int(os.environ.get("KP_KS", "4"))
HS = int(os.environ.get("KP_HS", "2"))
QLO = int(os.environ.get("KP_QLO", "4"))
CUTS = [int(v) for v in os.environ.get("KP_CUTS", "0,1,4,10,10,17,24,28,32").split(",")]
SCOPES = os.environ.get("KP_SCOPES", "") == "1"

_NT = (((1,), (1,)), ((), ()))


def _rb(x):
    return x.astype(BF16).astype(F32)


def _sigmoid(x):
    return 1.0 / (1.0 + jnp.exp(-x))


def _lanes(col, width):
    reps = width // LANES
    return col if reps == 1 else jnp.concatenate([col] * reps, axis=1)


def _fold(x):
    xi = lax.bitcast_convert_type(x, U32)
    tok = None
    for r in range(0, x.shape[0], 8):
        for c in range(0, x.shape[1] - LANES + 1, LANES):
            t = xi[r:r + 8, c:c + LANES]
            tok = t if tok is None else tok | t
    return tok


def _colsum(x, marks, nmarks):
    n = x.shape[0] // 8
    acc = x[0:8]
    for g in range(1, n):
        acc = acc + x[8 * g:8 * g + 8]
        if ((g + 1) * nmarks) % n == 0:
            marks.append(_fold(acc))
    return jnp.sum(acc, axis=0, keepdims=True)


def _tie_rows(lhs, toks, zero, lo, hi, c0=0):
    if not toks:
        return lhs
    lu = pltpu.bitcast(lhs, U32)
    rows = [lu[8 * r:8 * r + 8] for r in range(lu.shape[0] // 8)]
    for i, tok in enumerate(toks):
        r = lo + ((i + 1) * (hi - lo)) // len(toks) - 1
        head = rows[r][:, c0:c0 + LANES] | (tok & zero)
        rows[r] = head if lu.shape[1] == LANES else jnp.concatenate(
            [head, rows[r][:, LANES:]], axis=1)
    return pltpu.bitcast(jnp.concatenate(rows, axis=0), BF16)


def _merge(a, b):
    keyed = [((i + 1) / len(a), t) for i, t in enumerate(a)]
    keyed += [((i + 1) / len(b), t) for i, t in enumerate(b)]
    return [t for _, t in sorted(keyed, key=lambda kv: kv[0])]


def _span(start, size):
    if isinstance(start, int):
        return pl.ds(start, size)
    return pl.ds(pl.multiple_of(start, LANES), size)


def _scope(name):
    return jax.named_scope(name) if SCOPES else contextlib.nullcontext()


def _kernel(xt_hbm, k_hbm, v_hbm, wq_hbm, wot_hbm, wr_hbm, wg_hbm, wu_hbm, wdt_hbm,
            c_hbm, wmod_hbm, o_hbm,
            xt_v, k_v, v_v, wq_v, wot_v, wmod_v, wg_v, wu_v, wdt_v, ot_v,
            h_scr, acc_scr, st_scr, m_scr, vt_scr, mod_scr, col_scr, key_scr, h2_scr, x1_scr,
            zero_scr, fix_v, c_ref, wr_ref, row_scr, wd_scr, h2l_scr, hb_scr, wb_scr, rem_scr, wrem_v,
            grp_sems, misc_sems, mlp_sems, out_sems, fix_sems,
            *, n_heads):
    d, seq = xt_v.shape
    sk = k_v.shape[1]
    n_grp = n_heads // HG
    n_blk = seq // TB
    n_units = n_grp * n_blk
    nb = TB // LANES
    nq = 2 * HG
    nt = sk // LANES
    gbits = n_grp.bit_length() - 1
    gw = nq * DH
    qscale = (DH ** -0.5) * math.log2(math.e)

    def grp_of(u):
        return u & (n_grp - 1)

    def blk_of(u):
        return u >> gbits

    def grp_copies(g, n=1):
        hs = pl.ds(g * HG, n * HG)
        return (*[pltpu.make_async_copy(wq_hbm.at[:, pl.ds(i * gw, gw)], wq_v.at[i],
                                        grp_sems.at[0, i]) for i in range(g, g + n)],
                pltpu.make_async_copy(k_hbm.at[hs], k_v.at[hs], grp_sems.at[1, g]),
                pltpu.make_async_copy(v_hbm.at[hs], v_v.at[hs], grp_sems.at[2, g]),
                *[pltpu.make_async_copy(wot_hbm.at[:, pl.ds((i - 1) * gw, gw)], wot_v.at[i - 1],
                                        grp_sems.at[3, i]) for i in range(g, g + n)])

    def col_copy(src, dst, lo, hi, sem):
        return pltpu.make_async_copy(src.at[:, lo:hi], dst.at[:, lo:hi], sem)

    x_first = col_copy(xt_hbm, xt_v, 0, TB, misc_sems.at[0])
    x_rest = col_copy(xt_hbm, xt_v, TB, seq, misc_sems.at[1])
    mod_first = [col_copy(wmod_hbm, wmod_v, MODC, 2 * d, misc_sems.at[8]),
                 col_copy(wmod_hbm, wmod_v, 0, MODC, misc_sems.at[9])]
    mod_rest = col_copy(wmod_hbm, wmod_v, 2 * d, 6 * d, misc_sems.at[3])
    mlp_g = pltpu.make_async_copy(wg_hbm, wg_v, mlp_sems.at[0])
    mlp_u = pltpu.make_async_copy(wu_hbm, wu_v, mlp_sems.at[1])
    ff = wdt_hbm.shape[1]
    mlp_d = pltpu.make_async_copy(wdt_hbm, wdt_v.at[:, 0:ff], mlp_sems.at[2])
    out_lo = col_copy(ot_v, o_hbm, 0, seq - TB, out_sems.at[0])
    chunks = list(zip(EDGES[:-1], EDGES[1:]))
    out_hi = [pltpu.make_async_copy(ot_v.at[r0:r1, seq - TB:seq], o_hbm.at[r0:r1, seq - TB:seq],
                                    out_sems.at[1 + i]) for i, (r0, r1) in enumerate(chunks)]

    def silu_c():
        cc = c_ref[...].astype(F32)
        return jnp.broadcast_to((cc * _rb(_sigmoid(cc))).astype(BF16), (8, d))

    def ln1_norm(t0, n, marks):
        x = xt_v[:, _span(t0, n)].astype(F32)
        mu = _colsum(x, marks, NM1) * (1.0 / d)
        xc = x - mu
        var = _colsum(xc * xc, marks, NM2) * (1.0 / d)
        return (xc * lax.rsqrt(var + EPS)).astype(BF16).T

    def ln1_mod(ln, slot, r0, marks):
        n = ln.shape[0]
        h = ln.astype(F32) * mod_scr[1:2, :] + mod_scr[0:1, :]
        h_scr[slot, _span(r0, n), :] = h.astype(BF16)
        step = max(n // NM3, 8)
        for r in range(step - 8, n, step):
            marks.append(_fold(h[r:r + 8]))

    def mod_piece(src, dst, marks, z):
        w = wmod_v[:, _span(src, MP)].astype(F32)
        row = _rb(_colsum(w * _lanes(col_scr[5 * d:6 * d, :], MP), marks, NMP))
        row = lax.bitcast_convert_type(
            lax.bitcast_convert_type(row, U32) | _lanes(z[0:1], MP), F32)
        pos = dst + lax.broadcasted_iota(I32, (1, MP), 1)
        is_cb = jnp.logical_and(pos >= 2 * d, pos < 3 * d)
        row = jnp.where(is_cb, _rb(1.0 + row), row)
        row_scr[:, _span(dst, MP)] = row
        col = jnp.broadcast_to(row, (LANES, MP)).T
        col_scr[_span(dst, MP), :] = col
        for r in range(LANES - 8, MP, LANES):
            marks.append(lax.bitcast_convert_type(col[r:r + 8], U32))

    def wd_piece(src, dst, marks):
        w = pltpu.bitcast(wdt_v[:, _span(src, WP)].T, U32)
        wd_scr[pl.ds(pl.multiple_of(dst // 2, WP // 2), WP // 2), :] = w
        for r in range(56, WP // 2, 64):
            for c in range(0, d - LANES + 1, LANES):
                marks.append(w[r:r + 8, c:c + LANES])

    dm = d - d % LANES
    kr = d - dm
    nr = NR * LANES

    def hb_piece(slot, r0, marks, z=None):
        hu = pltpu.bitcast(h_scr[slot, _span(r0, SP), dm:d], U32)
        if z is not None:
            hu = hu | jnp.concatenate([z[:, 0:kr]] * (SP // 16), axis=0)
        rows = pl.ds(r0 // 2 if isinstance(r0, int) else pl.multiple_of(r0 // 2, SP // 2), SP // 2)
        for k in range(kr):
            col = jnp.broadcast_to(hu[:, k:k + 1], (SP // 2, LANES))
            hb_scr[slot, k, rows, :] = col
            if (k + 1) % HS == 0:
                marks.append(col[SP // 2 - 8:SP // 2])

    def wb_piece(u, toks, zero):
        w = lax.bitcast_convert_type(wrem_v[:, _span(grp_of(u) * gw, nr)].astype(F32), U32)
        for k in range(kr):
            row = jnp.broadcast_to(w[k:k + 1], (8, nr))
            if toks:
                row = row | _lanes(toks[k * len(toks) // kr] & zero, nr)
            wb_scr[k] = lax.bitcast_convert_type(row, F32)

    pend = []

    def rem_flush(st, zero, mine):
        old = len(pend) - mine
        for i, (p0, acc) in enumerate(pend):
            if i < old:
                rl = 8 * ((i + 1) * 200 // (old + 1))
            else:
                rl = 8 * min(16 + (i - old + 1) * 224 // mine, 236)
            tok = lax.bitcast_convert_type(st[rl:rl + 8, 0:LANES], U32)
            z = jnp.concatenate([_lanes(tok & zero, NR * LANES)] * (2 * RG), axis=0)
            rem_scr[16 * p0:16 * (p0 + RG), :] = lax.bitcast_convert_type(
                lax.bitcast_convert_type(acc, U32) | z, F32)
        pend.clear()

    def rem_piece(slot, gsel, g0, g1, marks):
        for p0 in range(g0, g1, RG):
            acc = None
            for k in range(kr):
                hb = pltpu.bitcast(hb_scr[slot, k, 8 * p0:8 * (p0 + RG), :], BF16).astype(F32)
                w = wb_scr[k]
                wt = jnp.concatenate([w] * (2 * RG), axis=0)
                t = _lanes(hb, NR * LANES) * wt
                acc = t if acc is None else acc + t
                if (k + 1) % KS == 0:
                    marks.append(_fold(acc))
            pend.append((p0, acc))

    def qproj2(u, toks, zero):
        h = h_scr[blk_of(u) & 1]
        wr2 = wq_v[grp_of(u), dm:d, nr:gw]
        q = jnp.concatenate([jnp.dot(h[r0:r0 + TB // 2, dm:d], wr2, preferred_element_type=F32)
                             for r0 in (0, TB // 2)], axis=0)
        r = jnp.concatenate([rem_scr[...], q], axis=1)
        outs = []
        for i in range(nq):
            tk = toks[i * len(toks) // nq:(i + 1) * len(toks) // nq]
            hm = _tie_rows(h[:, 0:dm], tk, zero, 0, TB // 16)
            q = jnp.dot(hm, wq_v[grp_of(u), 0:dm, i * DH:(i + 1) * DH],
                        preferred_element_type=F32) + r[:, i * DH:(i + 1) * DH]
            outs.append((q * qscale).astype(BF16))
        return jnp.concatenate(outs, axis=1)

    def qproj(u, lo=0, hi=gw, parts=1):
        qs = []
        for r0 in range(0, TB, TB // parts):
            rs = slice(r0, r0 + TB // parts)
            if REMF:
                q = jnp.dot(h_scr[blk_of(u) & 1, rs, dm:d], wq_v[grp_of(u), dm:d, lo:hi],
                            preferred_element_type=F32)
                q = jnp.dot(h_scr[blk_of(u) & 1, rs, 0:dm], wq_v[grp_of(u), 0:dm, lo:hi],
                            preferred_element_type=F32) + q
            else:
                q = jnp.dot(h_scr[blk_of(u) & 1, rs, :], wq_v[grp_of(u), :, lo:hi],
                            preferred_element_type=F32)
            qs.append((q * qscale).astype(BF16))
        return jnp.concatenate(qs, axis=0)

    def qk(u, q, j, toks=(), zero=None, mine=0):
        k = _tie_rows(k_v[grp_of(u) * HG + j // 2], toks, zero, TLO, int(os.environ.get('KP_THI', '120')))
        st = lax.dot_general(k, q[:, j * DH:(j + 1) * DH], _NT,
                             preferred_element_type=F32)
        if pend:
            rem_flush(st, zero, mine)
        for i in range(nb):
            blk = st[:, i * LANES:(i + 1) * LANES]
            st_scr[j * nb + i] = blk
            if DEFM:
                m_scr[j * nb + i] = jnp.max(blk.reshape(sk // 8, 8, LANES), axis=0)
            else:
                m_scr[j * nb + i, 0:1] = jnp.max(blk, axis=0, keepdims=True)
        rl = int(os.environ.get("KP_RL", "1800"))
        return lax.bitcast_convert_type(st[rl:rl + 8, 0:LANES], U32)

    def v_transpose(u, i, marks=None):
        vt = pltpu.bitcast(v_v[grp_of(u) * HG + i].T, U32)
        vt_scr[i] = vt
        if marks is not None:
            step = sk // NVT
            for c in range(step - LANES, sk, step):
                marks.append(vt[DH // 2 - 8:DH // 2, c:c + LANES])

    def pv(slots, zero, toks=()):
        ps, ls, pairs = [], [], []
        for sl in slots:
            m = jnp.max(m_scr[sl], axis=0, keepdims=True) if DEFM else m_scr[sl, 0:1]
            p = jnp.exp2(st_scr[sl] - m)
            accs = [None] * 4
            for tile in range(nt):
                for r0 in range(tile * LANES + LANES - 16, tile * LANES - 16, -16):
                    pair = p[r0:r0 + 8] + p[r0 + 8:r0 + 16]
                    pairs.append(pair)
                    a = accs[tile % 4]
                    accs[tile % 4] = pair if a is None else a + pair
            ls.append(jnp.sum((accs[0] + accs[1]) + (accs[2] + accs[3]), axis=0, keepdims=True))
            ps.append(p.astype(BF16))
        outs = []
        ntiles = len(slots) * nt
        side = {}
        for i, tok in enumerate(toks):
            side.setdefault(((i + 1) * ntiles) // len(toks) - 1, []).append(tok)
        for i, sl in enumerate(slots):
            vu = vt_scr[sl // (2 * nb)]
            tiles = []
            for c in range(nt):
                g = i * nt + c + 4
                rows = []
                for r in range(8):
                    x = vu[8 * r:8 * r + 8, c * LANES:(c + 1) * LANES]
                    if g < ntiles and TIE0 <= r < TIE0 + NTIE:
                        src = pairs[g * 8 + (r - TIE0)]
                        x = x | (lax.bitcast_convert_type(src, U32) & zero)
                    if r == SIDE_ROW:
                        for tok in side.get(i * nt + c, ()):
                            x = x | (tok & zero)
                    rows.append(x)
                tiles.append(jnp.concatenate(rows, axis=0))
            lhs = pltpu.bitcast(jnp.concatenate(tiles, axis=1), BF16)
            o = jnp.dot(lhs, ps[i], preferred_element_type=F32)
            outs.append((o * (1.0 / ls[i])).astype(BF16))
        return outs

    def outproj_tied(u, o, toks, zero):
        slot = blk_of(u) & 1
        for i in range(nb):
            o2 = jnp.concatenate([o[j * nb + i] for j in range(nq)], axis=0)
            tk = toks[i * len(toks) // nb:(i + 1) * len(toks) // nb]
            wo = _tie_rows(wot_v[grp_of(u)], tk, zero, 0, d // 16)
            contrib = jnp.dot(wo, o2, preferred_element_type=F32)
            cs = slice(i * LANES, (i + 1) * LANES)
            old = jnp.where(grp_of(u) > 0, acc_scr[slot, :, cs], 0.0)
            acc_scr[slot, :, cs] = old + contrib

    def outproj(u, o, lo=0):
        w = len(o) // nq
        o2 = jnp.concatenate(
            [jnp.concatenate(o[j * w:(j + 1) * w], axis=1) for j in range(nq)], axis=0)
        contrib = jnp.dot(wot_v[grp_of(u)], o2, preferred_element_type=F32)
        hi = lo + w * LANES
        slot = blk_of(u) & 1
        old = jnp.where(grp_of(u) > 0, acc_scr[slot, :, lo:hi], 0.0)
        acc_scr[slot, :, lo:hi] = old + contrib

    def router_keys(racc, t0):
        r = _rb(jnp.sum(racc, axis=0, keepdims=True)) + 0.0
        bits = lax.bitcast_convert_type(r, I32) >> 16
        order = jnp.where(bits < 0, -1 - bits, bits + 32768)
        pos = t0 + lax.broadcasted_iota(I32, r.shape, 1)
        return lax.bitcast_convert_type((order << 11) + (seq - 1 - pos) + 0x20000000, F32)

    def finalize(t0, slot, a0, dst, n, keys_out=None):
        marks = []
        cs = _span(dst, n)
        x = xt_v[:, _span(t0, n)].astype(F32)
        att = acc_scr[slot, :, _span(a0, n)]
        x1b = (x + _lanes(col_scr[0:d, :], n) * att).astype(BF16)
        x1_scr[:, cs] = x1b
        ot_v[:, cs] = x1b
        mu = _colsum(x1b.astype(F32), marks, NF1) * (1.0 / d)
        mub = _rb(mu)
        xc = x1_scr[:, cs].astype(F32) - mub
        var = _colsum(xc * xc, marks, NF2) * (1.0 / d) - (mu - mub) * (mu - mub)
        inv = 1.0 / _rb(jnp.sqrt(_rb(_rb(jnp.maximum(var, 0.0)) + EPS_BF16)))
        step = d // NF3
        racc = None
        for r0 in range(0, d, step):
            rs = slice(r0, r0 + step)
            x1 = ot_v[rs, cs].astype(F32)
            ln = _rb(_rb(x1 - mub) * inv)
            h2b = (_rb(ln * _lanes(col_scr[2 * d + r0:2 * d + r0 + step, :], n))
                   + _lanes(col_scr[d + r0:d + r0 + step, :], n)).astype(BF16)
            if keys_out is None:
                h2_scr[rs, cs] = h2b
            else:
                h2l_scr[rs, :] = h2b
            h2 = h2b.astype(F32)
            out = x1 + _lanes(col_scr[3 * d + r0:3 * d + r0 + step, :], n) * h2
            ot_v[rs, cs] = out.astype(BF16)
            rp = h2 * _lanes(col_scr[4 * d + r0:4 * d + r0 + step, :], n)
            for g in range(0, step, 8):
                racc = rp[g:g + 8] if racc is None else racc + rp[g:g + 8]
            marks.append(_fold(racc) | _fold(out))
        if keys_out is not None:
            keys_out.append(racc)
            return marks
        key = router_keys(racc, t0)
        for i in range(n // LANES):
            key_scr[pl.ds(dst // LANES + i, 1), :] = key[:, i * LANES:(i + 1) * LANES]
        return marks

    hw = gw // 2
    wq0a = col_copy(wq_hbm, wq_v.at[0], 0, hw, grp_sems.at[0, 0])
    wq0b = col_copy(wq_hbm, wq_v.at[0], hw, gw, misc_sems.at[4])
    k0a = pltpu.make_async_copy(k_hbm.at[0], k_v.at[0], grp_sems.at[1, 0])
    k0b = pltpu.make_async_copy(k_hbm.at[1], k_v.at[1], misc_sems.at[5])
    v0 = pltpu.make_async_copy(v_hbm.at[0:HG], v_v.at[0:HG], grp_sems.at[2, 0])
    wq1, k1, v1, wo0 = grp_copies(1)
    wo_last = pltpu.make_async_copy(wot_hbm.at[:, (n_grp - 1) * gw:n_grp * gw],
                                    wot_v.at[n_grp - 1], grp_sems.at[3, 0])
    wrem_copy = pltpu.make_async_copy(wq_hbm.at[dm:d, :], wrem_v, misc_sems.at[2])
    c_copy = pltpu.make_async_copy(c_hbm, c_ref, misc_sems.at[6])
    wr_copy = pltpu.make_async_copy(wr_hbm, wr_ref, misc_sems.at[7])
    c_copy.start()
    wr_copy.start()
    x_first.start()
    mod_first[0].start()
    mod_first[1].start()
    wq0a.start()
    wq0b.start()
    acc_scr[1] = jnp.zeros((d, TB), F32)
    col_scr[0:4 * d, :] = jnp.zeros((4 * d, LANES), F32)
    wdt_v[:, ff:ff + WP] = jnp.zeros((d, WP), BF16)
    with _scope("w_x"):
        c_copy.wait()
        wr_copy.wait()
        x_first.wait()
    cbits = lax.bitcast_convert_type(c_ref[:, 0:LANES].astype(F32), U32)
    zero_scr[...] = jnp.broadcast_to(cbits & 0xFFFF, (8, LANES))
    h_scr[0] = ln1_norm(0, TB, [])
    sc = silu_c()
    wr = wr_ref[...].reshape(1, d).astype(F32)
    col_scr[4 * d:5 * d, :] = jnp.broadcast_to(wr, (LANES, d)).T
    col_scr[5 * d:6 * d, :] = jnp.broadcast_to(sc[0:1, :].astype(F32), (LANES, d)).T
    with _scope("w_wmod"):
        mod_first[0].wait()
    mod = _rb(jnp.dot(sc, wmod_v[:, MODC:2 * d], preferred_element_type=F32))
    mod_scr[0:1, MODC:d] = mod[0:1, 0:d - MODC]
    mod_scr[1:2, :] = _rb(1.0 + mod[0:1, d - MODC:2 * d - MODC])
    with _scope("w_wmod2"):
        mod_first[1].wait()
    k0a.start(priority=KAP)
    if not LATEKV:
        k0b.start(priority=1)
        v0.start(priority=1)
    mod_scr[0:1, 0:MODC] = _rb(jnp.dot(sc, wmod_v[:, 0:MODC], preferred_element_type=F32))[0:1]
    if EARLYMOD:
        ln1_mod(h_scr[0], 0, 0, [])
    with _scope("w_wq"):
        wq0a.wait()
    if LATEKV:
        k0b.start(priority=1)
        v0.start(priority=1)
        wrem_copy.start(priority=1)
    if not EARLYMOD:
        ln1_mod(h_scr[0], 0, 0, [])
    qa = qproj(0, 0, hw, 2)
    with _scope("w_k"):
        wq0b.wait()
        k0a.wait()
    wq1.start(priority=1)
    k1.start(priority=1)
    q = jnp.concatenate([qa, qproj(0, hw, gw, 2)], axis=1)
    zero = zero_scr[...]
    for j in range(2):
        marks = []
        hb_piece(0, j * SP, marks)
        qk(0, q, j, marks, zero)
    with _scope("w_v"):
        k0b.wait()
        v0.wait()
        wrem_copy.wait()
    v1.start()
    wo0.start()
    with _scope("qk0"):
        zero = zero_scr[...]
        for i in range(HG):
            marks, hm = [], []
            v_transpose(0, i, marks)
            hb_piece(0, (2 + i) * SP, hm)
            if i == 0:
                wb_piece(2, hm, zero)
                rem_scr[...] = jnp.concatenate(
                    [jnp.dot(h_scr[0, r0:r0 + TB // 2, dm:d], wrem_v[:, gw:gw + nr],
                             preferred_element_type=F32) for r0 in (0, TB // 2)], axis=0)
            qk(0, q, nq - HG + i, _merge(marks, hm), zero)

    assert n_grp == 8 and HG == 2
    loads = [[wq1, k1, v1, wo0],
             [*grp_copies(2), mod_rest, x_rest],
             [*grp_copies(3, 3)],
             [*grp_copies(6, 2), wo_last],
             [mlp_d],
             [mlp_g, mlp_u]]
    wd0 = len(loads) - 1
    npc = TB // SP
    nmp = 4 * d // MP

    def manage(i):
        for cp in loads[i - 1]:
            cp.wait()
        for cp in loads[i]:
            cp.start()

    def steady(u, carry):
        with _scope("body"):
            zero = zero_scr[...]
            blk, g = blk_of(u), grp_of(u)
            off = ((g - 1) & (npc - 1)) * SP
            cuts = CUTS
            def rem(j, mk):
                rm = []
                rem_piece(blk_of(u + 1) & 1, (u + 1) & 1, cuts[j], cuts[j + 1], rm)
                return (_merge(mk, rm) if mk else rm) if rm else mk
            q = qproj2(u, rem(5, []), zero)
            o = pv(range(0, 2 * nb), zero, rem(6, []))
            live = jnp.logical_and(blk > 0, jnp.logical_and(g >= 1, g <= npc))
            t0 = jnp.maximum(blk - 1, 0) * TB + off
            marks = finalize(t0, (blk + 1) & 1, off, jnp.where(live, t0, seq), SP)
            wp = jnp.clip(u - wd0, 0, ff // WP - 1) * WP
            wmarks = []
            wd_piece(jnp.where(u >= wd0, wp, ff), wp, wmarks)
            qk(u, q, 0, rem(0, _merge(marks, wmarks)), zero, (cuts[1] - cuts[0]) // RG)
            marks = []
            nxt = jnp.where(u >= 2, jnp.minimum(blk + 1, n_blk - 1), 0)
            ln = ln1_norm(nxt * TB + off, SP, marks)
            ln1_mod(ln, (blk + 1) & 1, off, marks)
            mp = jnp.clip(u - 2, 0, nmp - 1) * MP
            mmarks = []
            mod_piece(jnp.where(u >= 2, 2 * d + mp, 0), mp, mmarks,
                      marks[int(os.environ.get("KP_MREL", "-1"))] & zero)
            nk = int(os.environ.get("KP_MKEEP", "2"))
            marks = _merge(marks[:-nk], mmarks[:NMP]) + marks[-nk:]
            qk(u, q, 1, rem(1, marks), zero, (cuts[2] - cuts[1]) // RG)
            o += pv(range(2 * nb, 4 * nb), zero, rem(7, []))
            rm = []
            rem_piece(blk_of(u + 1) & 1, (u + 1) & 1, cuts[4], cuts[5], rm)
            outproj_tied(u - 1, o, rm, zero)
            marks = []
            v_transpose(u, 0, marks)
            v_transpose(u, 1, marks)
            rel = qk(u, q, 2, rem(2, marks), zero, (cuts[3] - cuts[2]) // RG)
            hm = []
            hb_piece((blk + 1) & 1, off, hm, rel & zero)
            wb_piece(u + 2, hm, zero)
            qk(u, q, 3, hm, zero)
        return carry

    def stage(i, carry):
        for k in range(1, len(loads)):
            pl.when(i == k)(functools.partial(manage, k))
        return lax.fori_loop(i, jnp.where(i < len(loads) - 1, i + 1, n_units), steady, carry)

    lax.fori_loop(1, len(loads), stage, 0)

    ul = n_units - 1
    tl = seq - TB
    sl_last = (n_blk - 1) & 1
    nb0 = nb - TAILB
    with _scope("e_pva"):
        mod_scr[2:3, :] = row_scr[:, 3 * d:4 * d]
        outproj(ul, pv([j * nb + i for j in range(nq) for i in range(nb0)], zero_scr[...]))
    mlp_g.wait()
    mlp_u.wait()
    out_lo.start()
    with _scope("e_pvb"):
        toks = finalize(tl, sl_last, 0, tl, nb0 * LANES)
        o = pv([j * nb + i for j in range(nq) for i in range(nb0, nb)], zero_scr[...], toks)
        outproj(ul, o, nb0 * LANES)

    nl = TAILB * LANES
    sub8 = lax.broadcasted_iota(I32, (TOPC, 1), 0)
    lane = lax.broadcasted_iota(I32, (TOPC, LANES), 1)

    def key_index(k):
        return seq - 1 - (lax.bitcast_convert_type(k, I32) & (seq - 1))

    def piece_base(idx, limit):
        return pl.multiple_of(jnp.clip(idx >> 7, 0, limit // LANES - 1) * LANES, LANES)

    keys = key_scr[0:seq // LANES, :]
    piece = lax.broadcasted_iota(I32, (seq // LANES, 1), 0)
    keys = jnp.where(piece < (seq - nl) // LANES, keys, 0.0)
    ecol = jnp.zeros((TOPC, LANES), F32)
    erow = jnp.zeros((1, LANES), F32)
    h2e = jnp.zeros((TOPC, d), F32)
    late = []
    marks = finalize(seq - nl, sl_last, TB - nl, seq - nl, nl, late)
    zero = zero_scr[...]
    pace = dict(zip([int(v) for v in os.environ.get("KP_PG", "2,4,5,6,7").split(",")],
                    [int(v) for v in os.environ.get("KP_PM", "8,14,18,23,27").split(",")]))
    for i in range(TOPC):
        mx = jnp.max(jnp.max(keys, axis=0, keepdims=True), axis=1, keepdims=True)
        keys = jnp.where(keys == mx, 0.0, keys)
        ecol = jnp.where(sub8 == i, mx, ecol)
        erow = jnp.where(lane[0:1] == i, mx, erow)
        idx = key_index(mx)
        pick = jnp.logical_and(sub8 == i, lane == (idx & (LANES - 1)))
        sl = pl.ds(piece_base(idx[0, 0], seq - nl), LANES)
        pick = jnp.where(pick, 1.0, 0.0)
        if i in pace:
            pick = lax.bitcast_convert_type(
                lax.bitcast_convert_type(pick, U32) | (marks[pace[i]] & zero), F32)
        h2e = h2e + lax.dot_general(pick.astype(BF16), h2_scr[:, sl], _NT,
                                    preferred_element_type=F32)

    late = [router_keys(late[0], seq - nl)]
    krow = jnp.concatenate([late[0], erow], axis=1)
    kcol = jnp.concatenate([jnp.broadcast_to(late[0], (LANES, nl)).T, ecol], axis=0)
    cnt = [None] * 4
    for g in range(kcol.shape[0] // 8):
        one = jnp.where(_lanes(kcol[8 * g:8 * g + 8], nl + LANES) > krow, 1.0, 0.0)
        cnt[g % 4] = one if cnt[g % 4] is None else cnt[g % 4] + one
    rank = jnp.sum((cnt[0] + cnt[1]) + (cnt[2] + cnt[3]), axis=0, keepdims=True)
    chosen = rank == sub8.astype(F32)
    onehot = jnp.where(chosen, 1.0, 0.0).astype(BF16)
    h2pad = jnp.concatenate([h2e, jnp.zeros((TOPC, d), F32)], axis=0).astype(BF16)
    h2s = (jnp.dot(onehot[:, nl:nl + 2 * TOPC], h2pad, preferred_element_type=F32)
           + lax.dot_general(onehot[:, 0:nl], h2l_scr[...], _NT,
                             preferred_element_type=F32))
    top = jnp.max(jnp.where(chosen, krow, 0.0), axis=1, keepdims=True)
    idx_col = key_index(top)
    idxs = [idx_col[i:i + 1] for i in range(TOPC)]
    bases = [piece_base(idx_col[i, 0], seq) for i in range(TOPC)]
    hit = lane == (idx_col & (LANES - 1))
    picks = [jnp.where(jnp.logical_and(sub8 == i, hit), 1.0, 0.0).astype(BF16)
             for i in range(TOPC)]
    order = (lax.bitcast_convert_type(top, I32) >> 11) & 0xFFFF
    rbits = jnp.where(order >= 32768, order - 32768, -1 - order) << 16
    gate = _rb(_sigmoid(lax.bitcast_convert_type(rbits, F32)))
    xs = h2s.astype(BF16)
    for cp in out_hi:
        cp.start()
    g = _rb(jnp.dot(xs, wg_v[...], preferred_element_type=F32))
    g = _rb(g * _rb(_sigmoid(g)))
    u = _rb(jnp.dot(xs, wu_v[...], preferred_element_type=F32))
    gu = (g * u).astype(BF16)

    last_use = []
    for i in range(TOPC):
        ok = True
        for j in range(i + 1, TOPC):
            ok = jnp.logical_and(ok, bases[i] != bases[j])
        last_use.append(ok)

    def down(r0, r1):
        x1p = jnp.concatenate([x1_scr[r0:r1, pl.ds(bases[i], LANES)] for i in range(TOPC)], axis=1)
        x1s = lax.dot_general(jnp.concatenate(picks, axis=1), x1p, _NT,
                              preferred_element_type=F32)
        wd = pltpu.bitcast(wd_scr[:, r0:r1], BF16)
        y = _rb(jnp.dot(gu, wd, preferred_element_type=F32))
        hm = _rb(h2s[:, r0:r1] + _rb(y * gate))
        return x1s + mod_scr[2:3, r0:r1] * hm

    def patch(r0, r1, new):
        n = r1 - r0
        pad = jnp.concatenate([new, jnp.zeros((LANES - TOPC, n), F32)], axis=0)
        cols = pltpu.bitcast(pad.T.astype(BF16), U32)
        col = [jnp.broadcast_to(cols[:, j:j + 1], (n // 2, LANES)) for j in range(TOPC)]
        for i in range(TOPC):
            res = pltpu.bitcast(ot_v[r0:r1, pl.ds(bases[i], LANES)], U32)
            tok = lane[0:1, :] + (idxs[i] & ~(LANES - 1))
            for j in range(i + 1):
                res = jnp.where(tok == idxs[j], col[j], res)
            fix_v[i, r0:r1, :] = pltpu.bitcast(res, BF16)

    def fix_copy(i, r0, r1):
        return pltpu.make_async_copy(fix_v.at[i, r0:r1, :],
                                     o_hbm.at[r0:r1, pl.ds(bases[i], LANES)], fix_sems.at[i])

    def for_last(fn):
        for i in range(TOPC - 1):
            pl.when(last_use[i])(functools.partial(fn, i))
        fn(TOPC - 1)

    new = down(*chunks[0])
    out_lo.wait()
    for ci, (r0, r1) in enumerate(chunks):
        out_hi[ci].wait()
        nxt = down(*chunks[ci + 1]) if ci + 1 < len(chunks) else None
        patch(r0, r1, new)
        for_last(lambda i: fix_copy(i, r0, r1).start())
        new = nxt
    with _scope("w_fix"):
        for r0, r1 in chunks:
            for_last(lambda i: fix_copy(i, r0, r1).wait())


@jax.jit
def pallas_adaLN_cond__gqa_block_cached__moe_arch_mod__prompt_kernel(
    A_x: jax.Array,
    A_k_cache: jax.Array,
    A_v_cache: jax.Array,
    A_wq: jax.Array,
    A_wo: jax.Array,
    B_x: jax.Array,
    B_w_r: jax.Array,
    B_w_gate: jax.Array,
    B_w_up: jax.Array,
    B_w_down: jax.Array,
    c: jax.Array,
    w_mod: jax.Array,
):
    b, seq, d = A_x.shape
    _, hkv, sk, dh = A_k_cache.shape
    assert b == 1 and dh == DH and HQ == 2 * hkv
    assert seq & (seq - 1) == 0 and seq <= 2048
    f = B_w_gate.shape[1]
    n_grp = hkv // HG
    gw = 2 * HG * dh
    n_slots = 2 * HG * TB // LANES

    xt = A_x.reshape(seq, d).T
    wot = A_wo.T
    wdt = B_w_down.T
    k3 = A_k_cache.reshape(hkv, sk, dh)
    v3 = A_v_cache.reshape(hkv, sk, dh)

    hbm = pl.BlockSpec(memory_space=pl.ANY)
    out_t = pl.pallas_call(
        functools.partial(_kernel, n_heads=hkv),
        in_specs=[hbm] * 11,
        out_specs=hbm,
        out_shape=jax.ShapeDtypeStruct((d, seq), BF16),
        scratch_shapes=[
            pltpu.VMEM((d, seq), BF16),
            pltpu.VMEM((hkv, sk, dh), BF16),
            pltpu.VMEM((hkv, sk, dh), BF16),
            pltpu.VMEM((n_grp, d, gw), BF16),
            pltpu.VMEM((n_grp, d, gw), BF16),
            pltpu.VMEM((d, 6 * d), BF16),
            pltpu.VMEM((d, f), BF16),
            pltpu.VMEM((d, f), BF16),
            pltpu.VMEM((d, f + WP), BF16),
            pltpu.VMEM((d, seq + SP), BF16),
            pltpu.VMEM((2, TB, d), BF16),
            pltpu.VMEM((2, d, TB), F32),
            pltpu.VMEM((n_slots, sk, LANES), F32),
            pltpu.VMEM((n_slots, 8, LANES), F32),
            pltpu.VMEM((HG, dh // 2, sk), U32),
            pltpu.VMEM((8, d), F32),
            pltpu.VMEM((6 * d, LANES), F32),
            pltpu.VMEM(((seq + SP) // LANES + 7 & ~7, LANES), F32),
            pltpu.VMEM((d, seq + SP), BF16),
            pltpu.VMEM((d, seq + SP), BF16),
            pltpu.VMEM((8, LANES), U32),
            pltpu.VMEM((TOPC, d, LANES), BF16),
            pltpu.VMEM((1, d), BF16),
            pltpu.VMEM((d,), BF16),
            pltpu.VMEM((1, 4 * d), F32),
            pltpu.VMEM((f // 2, d), U32),
            pltpu.VMEM((d, TAILB * LANES), BF16),
            pltpu.VMEM((2, d % LANES, TB // 2, LANES), U32),
            pltpu.VMEM((d % LANES, 8, NR * LANES), F32),
            pltpu.VMEM((TB, NR * LANES), F32),
            pltpu.VMEM((d % LANES, n_grp * gw), BF16),
            pltpu.SemaphoreType.DMA((4, n_grp)),
            pltpu.SemaphoreType.DMA((10,)),
            pltpu.SemaphoreType.DMA((3,)),
            pltpu.SemaphoreType.DMA((len(EDGES),)),
            pltpu.SemaphoreType.DMA((TOPC,)),
        ],
        compiler_params=pltpu.CompilerParams(
            disable_bounds_checks=True,
            disable_semaphore_checks=True,
            vmem_limit_bytes=120 * 1024 * 1024,
        ),
    )(xt, k3, v3, A_wq, wot, B_w_r, B_w_gate, B_w_up, wdt, c, w_mod)
    return out_t.T.reshape(b, seq, d)
```

```python
import contextlib
import functools
import math
import os

import jax
import jax.numpy as jnp
from jax import lax
import jax.experimental.pallas as pl
import jax.experimental.pallas.tpu as pltpu

F32 = jnp.float32
BF16 = jnp.bfloat16
I32 = jnp.int32
U32 = jnp.uint32

HQ = 32
DH = 128
TOPC = 8
EPS = 1e-05
EPS_BF16 = 1.0013580322265625e-05
LANES = 128

TB = 512
HG = 2
TIE0 = int(os.environ.get("KP_TIE0", "2"))
NTIE = int(os.environ.get("KP_NTIE", "3"))
SP = int(os.environ.get("KP_SP", "128"))
NM1 = int(os.environ.get("KP_NM1", "8"))
NM2 = int(os.environ.get("KP_NM2", "12"))
NM3 = int(os.environ.get("KP_NM3", "16"))
TLO = int(os.environ.get("KP_TLO", "8"))
NF1 = int(os.environ.get("KP_NF1", "9"))
NF2 = int(os.environ.get("KP_NF2", "6"))
NF3 = int(os.environ.get("KP_NF3", "18"))
NVT = int(os.environ.get("KP_NVT", "16"))
TAILB = int(os.environ.get("KP_TAILB", "2"))
SIDE_ROW = int(os.environ.get("KP_SIDE_ROW", "6"))
EDGES = [int(e) for e in os.environ.get("KP_EDGES", "0,128,256,384,512,576").split(",")]
MODC = int(os.environ.get("KP_MODC", "384"))
MP = int(os.environ.get("KP_MP", "384"))
NMP = int(os.environ.get("KP_NMP", "12"))
WP = 256
REMF = int(os.environ.get("KP_REMF", "1"))
DEFM = int(os.environ.get("KP_DEFM", "1"))
KAP = int(os.environ.get("KP_KAP", "0"))
LATEKV = int(os.environ.get("KP_LATEKV", "1"))
EARLYMOD = int(os.environ.get("KP_EARLYMOD", "0"))
RV = int(os.environ.get("KP_RV", "320"))
HP = 64
KS = int(os.environ.get("KP_KS", "4"))
KSPLIT = int(os.environ.get("KP_KSPLIT", "2"))
HS = int(os.environ.get("KP_HS", "2"))
THI = int(os.environ.get("KP_THI", "120"))
OPN = int(os.environ.get("KP_OPN", "2"))
LNREL = int(os.environ.get("KP_LNREL", "1200"))
_sh = [int(v) for v in os.environ.get("KP_SH", "7,2,3,5,2,7,7,4").split(",")]
SHARES = [sum(_sh[:i]) for i in range(len(_sh) + 1)]
SCOPES = os.environ.get("KP_SCOPES", "") == "1"

_NT = (((1,), (1,)), ((), ()))


def _rb(x):
    return x.astype(BF16).astype(F32)


def _sigmoid(x):
    return 1.0 / (1.0 + jnp.exp(-x))


def _lanes(col, width):
    reps = width // LANES
    return col if reps == 1 else jnp.concatenate([col] * reps, axis=1)


def _fold(x):
    xi = lax.bitcast_convert_type(x, U32)
    tok = None
    for r in range(0, x.shape[0], 8):
        for c in range(0, x.shape[1] - LANES + 1, LANES):
            t = xi[r:r + 8, c:c + LANES]
            tok = t if tok is None else tok | t
    return tok


def _colsum(x, marks, nmarks):
    n = x.shape[0] // 8
    acc = x[0:8]
    for g in range(1, n):
        acc = acc + x[8 * g:8 * g + 8]
        if ((g + 1) * nmarks) % n == 0:
            marks.append(_fold(acc))
    return jnp.sum(acc, axis=0, keepdims=True)


def _tie_rows(lhs, toks, zero, lo, hi, c0=0):
    if not toks:
        return lhs
    lu = pltpu.bitcast(lhs, U32)
    rows = [lu[8 * r:8 * r + 8] for r in range(lu.shape[0] // 8)]
    for i, tok in enumerate(toks):
        r = lo + ((i + 1) * (hi - lo)) // len(toks) - 1
        head = rows[r][:, c0:c0 + LANES] | (tok & zero)
        rows[r] = head if lu.shape[1] == LANES else jnp.concatenate(
            [head, rows[r][:, LANES:]], axis=1)
    return pltpu.bitcast(jnp.concatenate(rows, axis=0), BF16)


def _merge(a, b):
    keyed = [((i + 1) / len(a), t) for i, t in enumerate(a)]
    keyed += [((i + 1) / len(b), t) for i, t in enumerate(b)]
    return [t for _, t in sorted(keyed, key=lambda kv: kv[0])]


def _span(start, size):
    if isinstance(start, int):
        return pl.ds(start, size)
    return pl.ds(pl.multiple_of(start, LANES), size)


def _scope(name):
    return jax.named_scope(name) if SCOPES else contextlib.nullcontext()


def _kernel(xt_hbm, k_hbm, v_hbm, wq_hbm, wot_hbm, wr_hbm, wg_hbm, wu_hbm, wdt_hbm,
            c_hbm, wmod_hbm, o_hbm,
            xt_v, k_v, v_v, wq_v, wot_v, wmod_v, wg_v, wu_v, wdt_v, ot_v,
            h_scr, acc_scr, st_scr, m_scr, vt_scr, mod_scr, col_scr, key_scr, h2_scr, x1_scr,
            zero_scr, fix_v, c_ref, wr_ref, row_scr, wd_scr, h2l_scr, hb_scr, wb_scr, rem_scr, wrem_v,
            grp_sems, misc_sems, mlp_sems, out_sems, fix_sems,
            *, n_heads):
    d, seq = xt_hbm.shape
    sk = k_v.shape[1]
    n_grp = n_heads // HG
    n_blk = seq // TB
    n_units = n_grp * n_blk
    nb = TB // LANES
    nq = 2 * HG
    nt = sk // LANES
    gbits = n_grp.bit_length() - 1
    gw = nq * DH
    qscale = (DH ** -0.5) * math.log2(math.e)

    def grp_of(u):
        return u & (n_grp - 1)

    def blk_of(u):
        return u >> gbits

    def grp_copies(g, n=1):
        hs = pl.ds(g * HG, n * HG)
        return (*[pltpu.make_async_copy(wq_hbm.at[:, pl.ds(i * gw, gw)], wq_v.at[i],
                                        grp_sems.at[0, i]) for i in range(g, g + n)],
                pltpu.make_async_copy(k_hbm.at[hs], k_v.at[hs], grp_sems.at[1, g]),
                pltpu.make_async_copy(v_hbm.at[hs], v_v.at[hs], grp_sems.at[2, g]),
                *[pltpu.make_async_copy(wot_hbm.at[:, pl.ds((i - 1) * gw, gw)], wot_v.at[i - 1],
                                        grp_sems.at[3, i]) for i in range(g, g + n)])

    def col_copy(src, dst, lo, hi, sem):
        return pltpu.make_async_copy(src.at[:, lo:hi], dst.at[:, lo:hi], sem)

    class Pieces:
        def __init__(self, src, dst, lo, hi, sem):
            self.src, self.dst, self.lo, self.hi, self.sem = src, dst, lo, hi, sem

        def start(self, priority=0):
            w = self.dst.shape[2]
            for p in range(self.lo, self.hi):
                pltpu.make_async_copy(self.src.at[:, p * w:(p + 1) * w], self.dst.at[p],
                                      self.sem).start(priority=priority)

        def wait(self):
            whole = self.dst.at[self.lo:self.hi]
            pltpu.make_async_copy(whole, whole, self.sem).wait()

    def x_cols(t0, n):
        return jnp.concatenate([xt_v[t0 // LANES + i] for i in range(n // LANES)], axis=1)

    x_first = Pieces(xt_hbm, xt_v, 0, nb, misc_sems.at[0])
    x_second = Pieces(xt_hbm, xt_v, nb, nb + 1, misc_sems.at[10])
    x_rest = Pieces(xt_hbm, xt_v, nb + 1, seq // LANES, misc_sems.at[1])
    mod_first = [col_copy(wmod_hbm, wmod_v, MODC, 2 * d, misc_sems.at[8]),
                 col_copy(wmod_hbm, wmod_v, 0, MODC, misc_sems.at[9])]
    mod_rest = col_copy(wmod_hbm, wmod_v, 2 * d, 6 * d, misc_sems.at[3])
    mlp_g = pltpu.make_async_copy(wg_hbm, wg_v, mlp_sems.at[0])
    mlp_u = pltpu.make_async_copy(wu_hbm, wu_v, mlp_sems.at[1])
    ff = wdt_hbm.shape[1]
    mlp_d = Pieces(wdt_hbm, wdt_v, 0, ff // WP, mlp_sems.at[2])
    out_lo = col_copy(ot_v, o_hbm, 0, seq - TB, out_sems.at[0])
    chunks = list(zip(EDGES[:-1], EDGES[1:]))
    out_hi = [pltpu.make_async_copy(ot_v.at[r0:r1, seq - TB:seq], o_hbm.at[r0:r1, seq - TB:seq],
                                    out_sems.at[1 + i]) for i, (r0, r1) in enumerate(chunks)]

    def silu_c():
        cc = c_ref[...].astype(F32)
        return jnp.broadcast_to((cc * _rb(_sigmoid(cc))).astype(BF16), (8, d))

    def ln1_norm(t0, n, marks):
        x = x_cols(t0, n).astype(F32)
        mu = _colsum(x, marks, NM1) * (1.0 / d)
        xc = x - mu
        var = _colsum(xc * xc, marks, NM2) * (1.0 / d)
        rs = lax.rsqrt(var + EPS)

        def finish(z=None):
            r = rs if z is None else lax.bitcast_convert_type(
                lax.bitcast_convert_type(rs, U32) | _lanes(z[0:1], n), F32)
            return (xc * r).astype(BF16).T
        return finish

    def ln1_mod(ln, slot, r0, marks):
        n = ln.shape[0]
        h = ln.astype(F32) * mod_scr[1:2, :] + mod_scr[0:1, :]
        h_scr[slot, _span(r0, n), :] = h.astype(BF16)
        step = max(n // NM3, 8)
        for r in range(step - 8, n, step):
            marks.append(_fold(h[r:r + 8]))

    def mod_piece(src, dst, marks):
        w = wmod_v[:, _span(src, MP)].astype(F32)
        row0 = _rb(_colsum(w * _lanes(col_scr[5 * d:6 * d, :], MP), marks, NMP))

        def finish(z):
            row = lax.bitcast_convert_type(
                lax.bitcast_convert_type(row0, U32) | _lanes(z[0:1], MP), F32)
            pos = dst + lax.broadcasted_iota(I32, (1, MP), 1)
            is_cb = jnp.logical_and(pos >= 2 * d, pos < 3 * d)
            row = jnp.where(is_cb, _rb(1.0 + row), row)
            row_scr[:, _span(dst, MP)] = row
            col_scr[_span(dst, MP), :] = jnp.broadcast_to(row, (LANES, MP)).T
        return finish

    def wd_piece(src, dst, marks):
        w = pltpu.bitcast(wdt_v[src // WP].T, U32)
        wd_scr[pl.ds(pl.multiple_of(dst // 2, WP // 2), WP // 2), :] = w
        for r in range(56, WP // 2, 64):
            for c in range(0, d - LANES + 1, LANES):
                marks.append(w[r:r + 8, c:c + LANES])

    dm = d - d % LANES
    kr = d - dm

    def hb_piece(slot, r0, n, marks, z=None):
        src = pl.ds(r0 if isinstance(r0, int) else pl.multiple_of(r0, n), n)
        dst = pl.ds(r0 // 2 if isinstance(r0, int) else pl.multiple_of(r0 // 2, n // 2), n // 2)
        hu = pltpu.bitcast(h_scr[slot, src, dm:d], U32)
        if z is not None:
            hu = hu | jnp.concatenate([z[:, 0:kr]] * (n // 16), axis=0)
        for k in range(kr):
            col = jnp.broadcast_to(hu[:, k:k + 1], (n // 2, LANES))
            hb_scr[slot, k, dst, :] = col
            if (k + 1) % HS == 0:
                marks.append(col[n // 2 - 8:n // 2])

    def wb_piece(u, toks, zero):
        w = lax.bitcast_convert_type(wrem_v[:, _span(grp_of(u) * gw, gw)].astype(F32), U32)
        for k in range(kr):
            row = jnp.broadcast_to(w[k:k + 1], (8, gw))
            row = row | _lanes(toks[k * len(toks) // kr] & zero, gw)
            wb_scr[k] = lax.bitcast_convert_type(row, F32)

    class Rem:
        def __init__(self, slot):
            self.marks, self.done, self.ready = [], {}, []
            for p in range(RV // 16):
                acc = None
                for k in range(kr):
                    hb = pltpu.bitcast(hb_scr[slot, k, 8 * p:8 * p + 8, :], BF16).astype(F32)
                    w = wb_scr[k]
                    t = _lanes(hb, gw) * jnp.concatenate([w, w], axis=0)
                    acc = t if acc is None else acc + t
                    if (k + 1) % KS == 0:
                        for c in range(0, gw, gw // KSPLIT):
                            self.marks.append(_fold(acc[:, c:c + gw // KSPLIT]))
                self.done[len(self.marks) - 1] = (p, acc)

        def take(self, phase, others=()):
            n, tot = len(self.marks), SHARES[-1]
            lo, hi = SHARES[phase] * n // tot, SHARES[phase + 1] * n // tot
            for i in range(lo, hi):
                if i in self.done:
                    self.ready.append((*self.done[i], phase, (i + 1 - lo) / (hi - lo)))
            mine = self.marks[lo:hi]
            return _merge(others, mine) if others and mine else list(others) + mine

        def flush(self, st, zero, phase, hi):
            old = [r for r in self.ready if r[2] < phase]
            for p, acc, ph, frac in self.ready:
                if ph < phase:
                    rl = 8 * (([r[0] for r in old].index(p) + 1) * 200 // (len(old) + 1))
                else:
                    rl = 16 * min(int(TLO + frac * (hi - TLO)) - 4, 118)
                tok = lax.bitcast_convert_type(st[rl:rl + 8, 0:LANES], U32)
                z = jnp.concatenate([_lanes(tok & zero, gw)] * 2, axis=0)
                rem_scr[16 * p:16 * p + 16, :] = lax.bitcast_convert_type(
                    lax.bitcast_convert_type(acc, U32) | z, F32)
            self.ready = []

    def qproj2(u, toks, zero):
        h = h_scr[blk_of(u) & 1]
        q = jnp.dot(h[RV:TB, dm:d], wq_v[grp_of(u), dm:d, :], preferred_element_type=F32)
        r = jnp.concatenate([rem_scr[...], q], axis=0)
        outs = []
        for i in range(nq):
            tk = toks[i * len(toks) // nq:(i + 1) * len(toks) // nq]
            hm = _tie_rows(h[:, 0:dm], tk, zero, 0, TB // 16)
            q = jnp.dot(hm, wq_v[grp_of(u), 0:dm, i * DH:(i + 1) * DH],
                        preferred_element_type=F32) + r[:, i * DH:(i + 1) * DH]
            outs.append((q * qscale).astype(BF16))
        return jnp.concatenate(outs, axis=1)

    def qproj(u, lo=0, hi=gw, parts=1):
        qs = []
        for r0 in range(0, TB, TB // parts):
            rs = slice(r0, r0 + TB // parts)
            if REMF:
                q = jnp.dot(h_scr[blk_of(u) & 1, rs, dm:d], wq_v[grp_of(u), dm:d, lo:hi],
                            preferred_element_type=F32)
                q = jnp.dot(h_scr[blk_of(u) & 1, rs, 0:dm], wq_v[grp_of(u), 0:dm, lo:hi],
                            preferred_element_type=F32) + q
            else:
                q = jnp.dot(h_scr[blk_of(u) & 1, rs, :], wq_v[grp_of(u), :, lo:hi],
                            preferred_element_type=F32)
            qs.append((q * qscale).astype(BF16))
        return jnp.concatenate(qs, axis=0)

    def qk(u, q, j, toks=(), zero=None, hi=THI):
        k = _tie_rows(k_v[grp_of(u) * HG + j // 2], toks, zero, TLO, hi)
        st = lax.dot_general(k, q[:, j * DH:(j + 1) * DH], _NT,
                             preferred_element_type=F32)
        for i in range(nb):
            blk = st[:, i * LANES:(i + 1) * LANES]
            st_scr[j * nb + i] = blk
            if DEFM:
                m_scr[j * nb + i] = jnp.max(blk.reshape(sk // 8, 8, LANES), axis=0)
            else:
                m_scr[j * nb + i, 0:1] = jnp.max(blk, axis=0, keepdims=True)
        return st

    def v_transpose(u, i, marks=None, rel=(), zero=None):
        v = _tie_rows(v_v[grp_of(u) * HG + i], rel, zero, -7, sk // 16 - 7)
        vt = pltpu.bitcast(v.T, U32)
        vt_scr[i] = vt
        if marks is not None:
            step = sk // NVT
            for c in range(step - LANES, sk, step):
                marks.append(vt[DH // 2 - 8:DH // 2, c:c + LANES])

    def pv(slots, zero, toks=()):
        ps, ls, pairs = [], [], []
        for sl in slots:
            m = jnp.max(m_scr[sl], axis=0, keepdims=True) if DEFM else m_scr[sl, 0:1]
            p = jnp.exp2(st_scr[sl] - m)
            accs = [None] * 4
            for tile in range(nt):
                for r0 in range(tile * LANES + LANES - 16, tile * LANES - 16, -16):
                    pair = p[r0:r0 + 8] + p[r0 + 8:r0 + 16]
                    pairs.append(pair)
                    a = accs[tile % 4]
                    accs[tile % 4] = pair if a is None else a + pair
            ls.append(jnp.sum((accs[0] + accs[1]) + (accs[2] + accs[3]), axis=0, keepdims=True))
            ps.append(p.astype(BF16))
        outs = []
        ntiles = len(slots) * nt
        side = {}
        for i, tok in enumerate(toks):
            side.setdefault(((i + 1) * ntiles) // len(toks) - 1, []).append(tok)
        for i, sl in enumerate(slots):
            vu = vt_scr[sl // (2 * nb)]
            tiles = []
            for c in range(nt):
                g = i * nt + c + 4
                rows = []
                for r in range(8):
                    x = vu[8 * r:8 * r + 8, c * LANES:(c + 1) * LANES]
                    if g < ntiles and TIE0 <= r < TIE0 + NTIE:
                        src = pairs[g * 8 + (r - TIE0)]
                        x = x | (lax.bitcast_convert_type(src, U32) & zero)
                    if r == SIDE_ROW:
                        for tok in side.get(i * nt + c, ()):
                            x = x | (tok & zero)
                    rows.append(x)
                tiles.append(jnp.concatenate(rows, axis=0))
            lhs = pltpu.bitcast(jnp.concatenate(tiles, axis=1), BF16)
            o = jnp.dot(lhs, ps[i], preferred_element_type=F32)
            outs.append((o * (1.0 / ls[i])).astype(BF16))
        return outs

    def outproj_tied(u, o, toks, zero):
        slot = blk_of(u) & 1
        res = []
        for i in range(nb):
            o2 = jnp.concatenate([o[j * nb + i] for j in range(nq)], axis=0)
            tk = toks[i * len(toks) // OPN:(i + 1) * len(toks) // OPN]
            wo = _tie_rows(wot_v[grp_of(u)], tk, zero, 0, d // 16)
            contrib = jnp.dot(wo, o2, preferred_element_type=F32)
            old = jnp.where(grp_of(u) > 0, acc_scr[slot * nb + i], 0.0)
            acc_scr[slot * nb + i] = old + contrib
            res.append(contrib)
        return jnp.concatenate(res, axis=0)

    def outproj(u, o, lo=0):
        w = len(o) // nq
        o2 = jnp.concatenate(
            [jnp.concatenate(o[j * w:(j + 1) * w], axis=1) for j in range(nq)], axis=0)
        contrib = jnp.dot(wot_v[grp_of(u)], o2, preferred_element_type=F32)
        slot = blk_of(u) & 1
        for i in range(w):
            pi = slot * nb + lo // LANES + i
            old = jnp.where(grp_of(u) > 0, acc_scr[pi], 0.0)
            acc_scr[pi] = old + contrib[:, i * LANES:(i + 1) * LANES]

    def router_keys(racc, t0):
        r = _rb(jnp.sum(racc, axis=0, keepdims=True)) + 0.0
        bits = lax.bitcast_convert_type(r, I32) >> 16
        order = jnp.where(bits < 0, -1 - bits, bits + 32768)
        pos = t0 + lax.broadcasted_iota(I32, r.shape, 1)
        return lax.bitcast_convert_type((order << 11) + (seq - 1 - pos) + 0x20000000, F32)

    def finalize(t0, slot, a0, dst, n, keys_out=None):
        marks = []
        cs = _span(dst, n)
        x = x_cols(t0, n).astype(F32)
        att = jnp.concatenate(
            [acc_scr[slot * nb + a0 // LANES + i] for i in range(n // LANES)], axis=1)
        x1b = (x + _lanes(col_scr[0:d, :], n) * att).astype(BF16)
        x1_scr[:, cs] = x1b
        ot_v[:, cs] = x1b
        mu = _colsum(x1b.astype(F32), marks, NF1) * (1.0 / d)
        mub = _rb(mu)
        xc = x1_scr[:, cs].astype(F32) - mub
        var = _colsum(xc * xc, marks, NF2) * (1.0 / d) - (mu - mub) * (mu - mub)
        inv = 1.0 / _rb(jnp.sqrt(_rb(_rb(jnp.maximum(var, 0.0)) + EPS_BF16)))
        step = d // NF3
        racc = None
        for r0 in range(0, d, step):
            rs = slice(r0, r0 + step)
            x1 = ot_v[rs, cs].astype(F32)
            ln = _rb(_rb(x1 - mub) * inv)
            h2b = (_rb(ln * _lanes(col_scr[2 * d + r0:2 * d + r0 + step, :], n))
                   + _lanes(col_scr[d + r0:d + r0 + step, :], n)).astype(BF16)
            if keys_out is None:
                h2_scr[rs, cs] = h2b
            else:
                h2l_scr[rs, :] = h2b
            h2 = h2b.astype(F32)
            out = x1 + _lanes(col_scr[3 * d + r0:3 * d + r0 + step, :], n) * h2
            ot_v[rs, cs] = out.astype(BF16)
            rp = h2 * _lanes(col_scr[4 * d + r0:4 * d + r0 + step, :], n)
            for g in range(0, step, 8):
                racc = rp[g:g + 8] if racc is None else racc + rp[g:g + 8]
            marks.append(_fold(racc) | _fold(out))
        if keys_out is not None:
            keys_out.append(racc)
            return marks
        key = router_keys(racc, t0)
        for i in range(n // LANES):
            key_scr[pl.ds(dst // LANES + i, 1), :] = key[:, i * LANES:(i + 1) * LANES]
        return marks

    hw = gw // 2
    wq0a = col_copy(wq_hbm, wq_v.at[0], 0, hw, grp_sems.at[0, 0])
    wq0b = col_copy(wq_hbm, wq_v.at[0], hw, gw, misc_sems.at[4])
    k0a = pltpu.make_async_copy(k_hbm.at[0], k_v.at[0], grp_sems.at[1, 0])
    k0b = pltpu.make_async_copy(k_hbm.at[1], k_v.at[1], misc_sems.at[5])
    v0 = pltpu.make_async_copy(v_hbm.at[0:HG], v_v.at[0:HG], grp_sems.at[2, 0])
    wq1, k1, v1, wo0 = grp_copies(1)
    wo_last = pltpu.make_async_copy(wot_hbm.at[:, (n_grp - 1) * gw:n_grp * gw],
                                    wot_v.at[n_grp - 1], grp_sems.at[3, 0])
    wrem_copy = col_copy(wq_hbm.at[dm:d], wrem_v, gw, 4 * gw, misc_sems.at[2])
    wrem_rest = (col_copy(wq_hbm.at[dm:d], wrem_v, 0, gw, misc_sems.at[11]),
                 col_copy(wq_hbm.at[dm:d], wrem_v, 4 * gw, n_grp * gw, misc_sems.at[12]))
    c_copy = pltpu.make_async_copy(c_hbm, c_ref, misc_sems.at[6])
    wr_copy = pltpu.make_async_copy(wr_hbm, wr_ref, misc_sems.at[7])
    c_copy.start()
    wr_copy.start()
    x_first.start()
    mod_first[0].start()
    mod_first[1].start()
    wq0a.start()
    wq0b.start()
    acc_scr[nb:2 * nb] = jnp.zeros((nb, d, LANES), F32)
    col_scr[0:4 * d, :] = jnp.zeros((4 * d, LANES), F32)
    wdt_v[ff // WP] = jnp.zeros((d, WP), BF16)
    with _scope("w_x"):
        c_copy.wait()
        wr_copy.wait()
        x_first.wait()
    cbits = lax.bitcast_convert_type(c_ref[:, 0:LANES].astype(F32), U32)
    zero_scr[...] = jnp.broadcast_to(cbits & 0xFFFF, (8, LANES))
    h_scr[0] = ln1_norm(0, TB, [])()
    sc = silu_c()
    wr = wr_ref[...].reshape(1, d).astype(F32)
    col_scr[4 * d:5 * d, :] = jnp.broadcast_to(wr, (LANES, d)).T
    col_scr[5 * d:6 * d, :] = jnp.broadcast_to(sc[0:1, :].astype(F32), (LANES, d)).T
    with _scope("w_wmod"):
        mod_first[0].wait()
    mod = _rb(jnp.dot(sc, wmod_v[:, MODC:2 * d], preferred_element_type=F32))
    mod_scr[0:1, MODC:d] = mod[0:1, 0:d - MODC]
    mod_scr[1:2, :] = _rb(1.0 + mod[0:1, d - MODC:2 * d - MODC])
    with _scope("w_wmod2"):
        mod_first[1].wait()
    k0a.start(priority=KAP)
    if not LATEKV:
        k0b.start(priority=1)
        v0.start(priority=1)
    mod_scr[0:1, 0:MODC] = _rb(jnp.dot(sc, wmod_v[:, 0:MODC], preferred_element_type=F32))[0:1]
    if EARLYMOD:
        ln1_mod(h_scr[0], 0, 0, [])
    with _scope("w_wq"):
        wq0a.wait()
    if LATEKV:
        k0b.start(priority=1)
        v0.start(priority=1)
        wrem_copy.start(priority=1)
    if not EARLYMOD:
        ln1_mod(h_scr[0], 0, 0, [])
    qa = qproj(0, 0, hw, 2)
    with _scope("w_k"):
        wq0b.wait()
        k0a.wait()
    wq1.start(priority=1)
    k1.start(priority=1)
    x_second.start()
    q = jnp.concatenate([qa, qproj(0, hw, gw, 2)], axis=1)
    zero = zero_scr[...]
    nhb = -(-RV // HP)
    for j in range(2):
        marks = []
        for i in range(j * nhb // 2, (j + 1) * nhb // 2):
            hb_piece(0, i * HP, HP, marks)
        qk(0, q, j, marks, zero)
    with _scope("w_v"):
        k0b.wait()
        v0.wait()
        wrem_copy.wait()
    v1.start()
    wo0.start()
    with _scope("qk0"):
        zero = zero_scr[...]
        rem_scr[...] = jnp.dot(h_scr[0, 0:RV, dm:d], wrem_v[:, gw:2 * gw],
                               preferred_element_type=F32)
        for i in range(HG):
            marks = []
            v_transpose(0, i, marks)
            if i == 0:
                wb_piece(2, marks, zero)
            qk(0, q, nq - HG + i, marks, zero)

    assert n_grp == 8 and HG == 2
    stage_at = [1, 2, 3, 5, n_units]
    starts = [(*grp_copies(2), mod_rest, x_rest, *wrem_rest), grp_copies(3, 3),
              (*grp_copies(6, 2), wo_last, mlp_d), (mlp_g, mlp_u)]
    waits = [(wq1, k1, v1, wo0, x_second), *starts[:3]]
    wd0 = stage_at[3]
    npc = TB // SP
    nmp = 4 * d // MP

    def manage(k, _, c):
        for cp in waits[k]:
            cp.wait()
        for cp in starts[k]:
            cp.start()
        return c

    def steady(u, carry):
        with _scope("body"):
            zero = zero_scr[...]
            blk, g = blk_of(u), grp_of(u)
            off = ((g - 1) & (npc - 1)) * SP
            rem = Rem(blk_of(u + 1) & 1)
            q = qproj2(u, rem.take(0), zero)
            o = pv(range(0, 2 * nb), zero, rem.take(1))
            live = jnp.logical_and(blk > 0, jnp.logical_and(g >= 1, g <= npc))
            t0 = jnp.maximum(blk - 1, 0) * TB + off
            marks = finalize(t0, (blk + 1) & 1, off, jnp.where(live, t0, seq), SP)
            wp = jnp.clip(u - wd0, 0, ff // WP - 1) * WP
            wmarks = []
            wd_piece(jnp.where(u >= wd0, wp, ff), wp, wmarks)
            rem.flush(qk(u, q, 0, rem.take(2, _merge(marks, wmarks)), zero), zero, 2, THI)
            def tok_at(res, row):
                return lax.bitcast_convert_type(res[row:row + 8, 0:LANES], U32)

            marks, mmarks = [], []
            ln_fin = ln1_norm(jnp.minimum(blk + 1, n_blk - 1) * TB + off, SP, marks)
            mp = jnp.clip(u - 2, 0, nmp - 1) * MP
            mod_fin = mod_piece(jnp.where(u >= 2, 2 * d + mp, 0), mp, mmarks)
            st = qk(u, q, 1, rem.take(3, marks + mmarks), zero)
            rem.flush(st, zero, 3, THI)
            ln1_mod(ln_fin(tok_at(st, LNREL) & zero), (blk + 1) & 1, off, [])
            mod_fin(tok_at(st, 1880) & zero)
            o += pv(range(2 * nb, 4 * nb), zero, rem.take(4))
            st = qk(u, q, 2, rem.take(5), zero)
            rem.flush(st, zero, 5, THI)
            v_transpose(u, 0, None, [tok_at(st, 112 * i) for i in range(nt)], zero)
            st = qk(u, q, 3, rem.take(6), zero)
            rem.flush(st, zero, 6, THI)
            v_transpose(u, 1, None, [tok_at(st, 112 * i) for i in range(nt)], zero)
            res = outproj_tied(u - 1, o, rem.take(7), zero)
            rem.flush(res, zero, 7, OPN * d // 16)
            hm = []
            hb_piece((blk + 1) & 1, jnp.clip(g - 1, 0, nhb - 1) * HP, HP, hm,
                     tok_at(res, max(OPN * d - 96, 0)) & zero)
            wb_piece(u + 2, hm, zero)
        return carry

    def stage(k, lo):
        hi = stage_at[1]
        for i in range(len(waits)):
            lax.fori_loop(0, jnp.where(k == i, 1, 0), functools.partial(manage, i), 0)
            hi = jnp.where(k == i, stage_at[i + 1], hi)
        lax.fori_loop(lo, hi, steady, 0)
        return hi

    lax.fori_loop(0, len(waits), stage, jnp.int32(stage_at[0]))

    ul = n_units - 1
    tl = seq - TB
    sl_last = (n_blk - 1) & 1
    nb0 = nb - TAILB
    with _scope("e_pva"):
        mod_scr[2:3, :] = row_scr[:, 3 * d:4 * d]
        outproj(ul, pv([j * nb + i for j in range(nq) for i in range(nb0)], zero_scr[...]))
    mlp_g.wait()
    mlp_u.wait()
    out_lo.start()
    with _scope("e_pvb"):
        toks = finalize(tl, sl_last, 0, tl, nb0 * LANES)
        o = pv([j * nb + i for j in range(nq) for i in range(nb0, nb)], zero_scr[...], toks)
        outproj(ul, o, nb0 * LANES)

    nl = TAILB * LANES
    sub8 = lax.broadcasted_iota(I32, (TOPC, 1), 0)
    lane = lax.broadcasted_iota(I32, (TOPC, LANES), 1)

    def key_index(k):
        return seq - 1 - (lax.bitcast_convert_type(k, I32) & (seq - 1))

    def piece_base(idx, limit):
        return pl.multiple_of(jnp.clip(idx >> 7, 0, limit // LANES - 1) * LANES, LANES)

    keys = key_scr[0:seq // LANES, :]
    piece = lax.broadcasted_iota(I32, (seq // LANES, 1), 0)
    keys = jnp.where(piece < (seq - nl) // LANES, keys, 0.0)
    ecol = jnp.zeros((TOPC, LANES), F32)
    erow = jnp.zeros((1, LANES), F32)
    h2e = jnp.zeros((TOPC, d), F32)
    late = []
    marks = finalize(seq - nl, sl_last, TB - nl, seq - nl, nl, late)
    zero = zero_scr[...]
    pace = dict(zip([int(v) for v in os.environ.get("KP_PG", "2,4,5,6,7").split(",")],
                    [int(v) for v in os.environ.get("KP_PM", "8,14,18,23,27").split(",")]))
    for i in range(TOPC):
        mx = jnp.max(jnp.max(keys, axis=0, keepdims=True), axis=1, keepdims=True)
        keys = jnp.where(keys == mx, 0.0, keys)
        ecol = jnp.where(sub8 == i, mx, ecol)
        erow = jnp.where(lane[0:1] == i, mx, erow)
        idx = key_index(mx)
        pick = jnp.logical_and(sub8 == i, lane == (idx & (LANES - 1)))
        sl = pl.ds(piece_base(idx[0, 0], seq - nl), LANES)
        pick = jnp.where(pick, 1.0, 0.0)
        if i in pace:
            pick = lax.bitcast_convert_type(
                lax.bitcast_convert_type(pick, U32) | (marks[pace[i]] & zero), F32)
        h2e = h2e + lax.dot_general(pick.astype(BF16), h2_scr[:, sl], _NT,
                                    preferred_element_type=F32)

    late = [router_keys(late[0], seq - nl)]
    krow = jnp.concatenate([late[0], erow], axis=1)
    kcol = jnp.concatenate([jnp.broadcast_to(late[0], (LANES, nl)).T, ecol], axis=0)
    cnt = [None] * 4
    for g in range(kcol.shape[0] // 8):
        one = jnp.where(_lanes(kcol[8 * g:8 * g + 8], nl + LANES) > krow, 1.0, 0.0)
        cnt[g % 4] = one if cnt[g % 4] is None else cnt[g % 4] + one
    rank = jnp.sum((cnt[0] + cnt[1]) + (cnt[2] + cnt[3]), axis=0, keepdims=True)
    chosen = rank == sub8.astype(F32)
    onehot = jnp.where(chosen, 1.0, 0.0).astype(BF16)
    h2pad = jnp.concatenate([h2e, jnp.zeros((TOPC, d), F32)], axis=0).astype(BF16)
    h2s = (jnp.dot(onehot[:, nl:nl + 2 * TOPC], h2pad, preferred_element_type=F32)
           + lax.dot_general(onehot[:, 0:nl], h2l_scr[...], _NT,
                             preferred_element_type=F32))
    top = jnp.max(jnp.where(chosen, krow, 0.0), axis=1, keepdims=True)
    idx_col = key_index(top)
    idxs = [idx_col[i:i + 1] for i in range(TOPC)]
    bases = [piece_base(idx_col[i, 0], seq) for i in range(TOPC)]
    hit = lane == (idx_col & (LANES - 1))
    picks = [jnp.where(jnp.logical_and(sub8 == i, hit), 1.0, 0.0).astype(BF16)
             for i in range(TOPC)]
    order = (lax.bitcast_convert_type(top, I32) >> 11) & 0xFFFF
    rbits = jnp.where(order >= 32768, order - 32768, -1 - order) << 16
    gate = _rb(_sigmoid(lax.bitcast_convert_type(rbits, F32)))
    xs = h2s.astype(BF16)
    for cp in out_hi:
        cp.start()
    g = _rb(jnp.dot(xs, wg_v[...], preferred_element_type=F32))
    g = _rb(g * _rb(_sigmoid(g)))
    u = _rb(jnp.dot(xs, wu_v[...], preferred_element_type=F32))
    gu = (g * u).astype(BF16)

    last_use = []
    for i in range(TOPC):
        ok = True
        for j in range(i + 1, TOPC):
            ok = jnp.logical_and(ok, bases[i] != bases[j])
        last_use.append(ok)

    def down(r0, r1):
        x1p = jnp.concatenate([x1_scr[r0:r1, pl.ds(bases[i], LANES)] for i in range(TOPC)], axis=1)
        x1s = lax.dot_general(jnp.concatenate(picks, axis=1), x1p, _NT,
                              preferred_element_type=F32)
        wd = pltpu.bitcast(wd_scr[:, r0:r1], BF16)
        y = _rb(jnp.dot(gu, wd, preferred_element_type=F32))
        hm = _rb(h2s[:, r0:r1] + _rb(y * gate))
        return x1s + mod_scr[2:3, r0:r1] * hm

    def patch(r0, r1, new):
        n = r1 - r0
        pad = jnp.concatenate([new, jnp.zeros((LANES - TOPC, n), F32)], axis=0)
        cols = pltpu.bitcast(pad.T.astype(BF16), U32)
        col = [jnp.broadcast_to(cols[:, j:j + 1], (n // 2, LANES)) for j in range(TOPC)]
        for i in range(TOPC):
            res = pltpu.bitcast(ot_v[r0:r1, pl.ds(bases[i], LANES)], U32)
            tok = lane[0:1, :] + (idxs[i] & ~(LANES - 1))
            for j in range(i + 1):
                res = jnp.where(tok == idxs[j], col[j], res)
            fix_v[i, r0:r1, :] = pltpu.bitcast(res, BF16)

    def fix_copy(i, r0, r1):
        return pltpu.make_async_copy(fix_v.at[i, r0:r1, :],
                                     o_hbm.at[r0:r1, pl.ds(bases[i], LANES)], fix_sems.at[i])

    def for_last(fn):
        for i in range(TOPC - 1):
            pl.when(last_use[i])(functools.partial(fn, i))
        fn(TOPC - 1)

    new = down(*chunks[0])
    out_lo.wait()
    for ci, (r0, r1) in enumerate(chunks):
        out_hi[ci].wait()
        nxt = down(*chunks[ci + 1]) if ci + 1 < len(chunks) else None
        patch(r0, r1, new)
        for_last(lambda i: fix_copy(i, r0, r1).start())
        new = nxt
    with _scope("w_fix"):
        for r0, r1 in chunks:
            for_last(lambda i: fix_copy(i, r0, r1).wait())


@jax.jit
def pallas_adaLN_cond__gqa_block_cached__moe_arch_mod__prompt_kernel(
    A_x: jax.Array,
    A_k_cache: jax.Array,
    A_v_cache: jax.Array,
    A_wq: jax.Array,
    A_wo: jax.Array,
    B_x: jax.Array,
    B_w_r: jax.Array,
    B_w_gate: jax.Array,
    B_w_up: jax.Array,
    B_w_down: jax.Array,
    c: jax.Array,
    w_mod: jax.Array,
):
    b, seq, d = A_x.shape
    _, hkv, sk, dh = A_k_cache.shape
    assert b == 1 and dh == DH and HQ == 2 * hkv
    assert seq & (seq - 1) == 0 and seq <= 2048
    f = B_w_gate.shape[1]
    n_grp = hkv // HG
    gw = 2 * HG * dh
    n_slots = 2 * HG * TB // LANES

    xt = A_x.reshape(seq, d).T
    wot = A_wo.T
    wdt = B_w_down.T
    k3 = A_k_cache.reshape(hkv, sk, dh)
    v3 = A_v_cache.reshape(hkv, sk, dh)

    hbm = pl.BlockSpec(memory_space=pl.ANY)
    out_t = pl.pallas_call(
        functools.partial(_kernel, n_heads=hkv),
        in_specs=[hbm] * 11,
        out_specs=hbm,
        out_shape=jax.ShapeDtypeStruct((d, seq), BF16),
        scratch_shapes=[
            pltpu.VMEM((seq // LANES, d, LANES), BF16),
            pltpu.VMEM((hkv, sk, dh), BF16),
            pltpu.VMEM((hkv, sk, dh), BF16),
            pltpu.VMEM((n_grp, d, gw), BF16),
            pltpu.VMEM((n_grp, d, gw), BF16),
            pltpu.VMEM((d, 6 * d), BF16),
            pltpu.VMEM((d, f), BF16),
            pltpu.VMEM((d, f), BF16),
            pltpu.VMEM((f // WP + 1, d, WP), BF16),
            pltpu.VMEM((d, seq + SP), BF16),
            pltpu.VMEM((2, TB, d), BF16),
            pltpu.VMEM((2 * TB // LANES, d, LANES), F32),
            pltpu.VMEM((n_slots, sk, LANES), F32),
            pltpu.VMEM((n_slots, 8, LANES), F32),
            pltpu.VMEM((HG, dh // 2, sk), U32),
            pltpu.VMEM((8, d), F32),
            pltpu.VMEM((6 * d, LANES), F32),
            pltpu.VMEM(((seq + SP) // LANES + 7 & ~7, LANES), F32),
            pltpu.VMEM((d, seq + SP), BF16),
            pltpu.VMEM((d, seq + SP), BF16),
            pltpu.VMEM((8, LANES), U32),
            pltpu.VMEM((TOPC, d, LANES), BF16),
            pltpu.VMEM((1, d), BF16),
            pltpu.VMEM((d,), BF16),
            pltpu.VMEM((1, 4 * d), F32),
            pltpu.VMEM((f // 2, d), U32),
            pltpu.VMEM((d, TAILB * LANES), BF16),
            pltpu.VMEM((2, d % LANES, -(-RV // HP) * HP // 2, LANES), U32),
            pltpu.VMEM((d % LANES, 8, gw), F32),
            pltpu.VMEM((RV, gw), F32),
            pltpu.VMEM((d % LANES, n_grp * gw), BF16),
            pltpu.SemaphoreType.DMA((4, n_grp)),
            pltpu.SemaphoreType.DMA((13,)),
            pltpu.SemaphoreType.DMA((3,)),
            pltpu.SemaphoreType.DMA((len(EDGES),)),
            pltpu.SemaphoreType.DMA((TOPC,)),
        ],
        compiler_params=pltpu.CompilerParams(
            disable_bounds_checks=True,
            disable_semaphore_checks=True,
            vmem_limit_bytes=120 * 1024 * 1024,
        ),
    )(xt, k3, v3, A_wq, wot, B_w_r, B_w_gate, B_w_up, wdt, c, w_mod)
    return out_t.T.reshape(b, seq, d)
```

```python
import contextlib
import functools
import math
import os

import jax
import jax.numpy as jnp
from jax import lax
import jax.experimental.pallas as pl
import jax.experimental.pallas.tpu as pltpu

F32 = jnp.float32
BF16 = jnp.bfloat16
I32 = jnp.int32
U32 = jnp.uint32

HQ = 32
DH = 128
TOPC = 8
EPS = 1e-05
EPS_BF16 = 1.0013580322265625e-05
LANES = 128

TB = 512
HG = 2
TIE0 = int(os.environ.get("KP_TIE0", "2"))
NTIE = int(os.environ.get("KP_NTIE", "3"))
SP = int(os.environ.get("KP_SP", "128"))
NM1 = int(os.environ.get("KP_NM1", "8"))
NM2 = int(os.environ.get("KP_NM2", "12"))
NM3 = int(os.environ.get("KP_NM3", "16"))
TLO = int(os.environ.get("KP_TLO", "3"))
NF1 = int(os.environ.get("KP_NF1", "9"))
NF2 = int(os.environ.get("KP_NF2", "6"))
NF3 = int(os.environ.get("KP_NF3", "18"))
NVT = int(os.environ.get("KP_NVT", "16"))
TAILB = int(os.environ.get("KP_TAILB", "2"))
SIDE_ROW = int(os.environ.get("KP_SIDE_ROW", "6"))
EDGES = [int(e) for e in os.environ.get("KP_EDGES", "0,128,256,384,512,576").split(",")]
MODC = int(os.environ.get("KP_MODC", "384"))
MP = int(os.environ.get("KP_MP", "384"))
NMP = int(os.environ.get("KP_NMP", "12"))
WP = 256
REMF = int(os.environ.get("KP_REMF", "1"))
DEFM = int(os.environ.get("KP_DEFM", "1"))
KAP = int(os.environ.get("KP_KAP", "0"))
LATEKV = int(os.environ.get("KP_LATEKV", "1"))
EARLYMOD = int(os.environ.get("KP_EARLYMOD", "0"))
RV = int(os.environ.get("KP_RV", "320"))
HP = 64
KS = int(os.environ.get("KP_KS", "4"))
KSPLIT = int(os.environ.get("KP_KSPLIT", "2"))
HS = int(os.environ.get("KP_HS", "2"))
THI = int(os.environ.get("KP_THI", "126"))
OPN = int(os.environ.get("KP_OPN", "2"))
LNREL = int(os.environ.get("KP_LNREL", "1200"))
_sh = [int(v) for v in os.environ.get("KP_SH", "14,5,5,9,5,13,14,8").split(",")]
SHARES = [sum(_sh[:i]) for i in range(len(_sh) + 1)]
MID = int(os.environ.get("KP_MID", "1"))
NG1 = int(os.environ.get("KP_NG1", "18"))
NG2 = int(os.environ.get("KP_NG2", "12"))
SCOPES = os.environ.get("KP_SCOPES", "") == "1"

_NT = (((1,), (1,)), ((), ()))


def _rb(x):
    return x.astype(BF16).astype(F32)


def _sigmoid(x):
    return 1.0 / (1.0 + jnp.exp(-x))


def _lanes(col, width):
    reps = width // LANES
    return col if reps == 1 else jnp.concatenate([col] * reps, axis=1)


def _fold(*xs):
    ts = []
    for x in xs:
        xi = lax.bitcast_convert_type(x, U32)
        ts += [xi[r:r + 8, c:c + LANES] for r in range(0, x.shape[0], 8)
               for c in range(0, x.shape[1] - LANES + 1, LANES)]
    if len(ts) > 5:
        return functools.reduce(lambda a, b: a | b, ts[:-2]) | (ts[-2] | ts[-1])
    while len(ts) > 1:
        ts = [a | b for a, b in zip(ts[0::2], ts[1::2])] + ts[len(ts) & ~1:]
    return ts[0]


def _colsum(x, marks, nmarks):
    n = x.shape[0] // 8
    acc = x[0:8]
    for g in range(1, n):
        acc = acc + x[8 * g:8 * g + 8]
        if ((g + 1) * nmarks) % n == 0:
            marks.append(_fold(acc))
    return jnp.sum(acc, axis=0, keepdims=True)


def _tie_rows(lhs, toks, zero, lo, hi, c0=0):
    if not toks:
        return lhs
    lu = pltpu.bitcast(lhs, U32)
    rows = [lu[8 * r:8 * r + 8] for r in range(lu.shape[0] // 8)]
    for i, tok in enumerate(toks):
        r = lo + ((i + 1) * (hi - lo)) // len(toks) - 1
        head = rows[r][:, c0:c0 + LANES] | (tok & zero)
        rows[r] = head if lu.shape[1] == LANES else jnp.concatenate(
            [head, rows[r][:, LANES:]], axis=1)
    return pltpu.bitcast(jnp.concatenate(rows, axis=0), BF16)


def _merge(a, b):
    keyed = [((i + 1) / len(a), t) for i, t in enumerate(a)]
    keyed += [((i + 1) / len(b), t) for i, t in enumerate(b)]
    return [t for _, t in sorted(keyed, key=lambda kv: kv[0])]


def _span(start, size):
    if isinstance(start, int):
        return pl.ds(start, size)
    return pl.ds(pl.multiple_of(start, LANES), size)


def _scope(name):
    return jax.named_scope(name) if SCOPES else contextlib.nullcontext()


def _kernel(xt_hbm, k_hbm, v_hbm, wq_hbm, wot_hbm, wr_hbm, wg_hbm, wu_hbm, wdt_hbm,
            c_hbm, wmod_hbm, o_hbm,
            xt_v, k_v, v_v, wq_v, wot_v, wmod_v, wg_v, wu_v, wdt_v, ot_v,
            h_scr, acc_scr, st_scr, m_scr, vt_scr, mod_scr, col_scr, key_scr, h2_scr, x1_scr,
            zero_scr, fix_v, c_ref, wr_ref, row_scr, wd_scr, h2l_scr, hb_scr, wb_scr, rem_scr, wrem_v,
            grp_sems, misc_sems, mlp_sems, out_sems, fix_sems,
            *, n_heads):
    d, seq = xt_hbm.shape
    sk = k_v.shape[1]
    n_grp = n_heads // HG
    n_blk = seq // TB
    n_units = n_grp * n_blk
    nb = TB // LANES
    nq = 2 * HG
    nt = sk // LANES
    gbits = n_grp.bit_length() - 1
    gw = nq * DH
    qscale = (DH ** -0.5) * math.log2(math.e)

    def grp_of(u):
        return u & (n_grp - 1)

    def blk_of(u):
        return u >> gbits

    def grp_copies(g, n=1):
        hs = pl.ds(g * HG, n * HG)
        return (*[pltpu.make_async_copy(wq_hbm.at[:, pl.ds(i * gw, gw)], wq_v.at[i],
                                        grp_sems.at[0, i]) for i in range(g, g + n)],
                pltpu.make_async_copy(k_hbm.at[hs], k_v.at[hs], grp_sems.at[1, g]),
                pltpu.make_async_copy(v_hbm.at[hs], v_v.at[hs], grp_sems.at[2, g]),
                *[pltpu.make_async_copy(wot_hbm.at[:, pl.ds((i - 1) * gw, gw)], wot_v.at[i - 1],
                                        grp_sems.at[3, i]) for i in range(g, g + n)])

    def col_copy(src, dst, lo, hi, sem):
        return pltpu.make_async_copy(src.at[:, lo:hi], dst.at[:, lo:hi], sem)

    class Pieces:
        def __init__(self, src, dst, lo, hi, sem):
            self.src, self.dst, self.lo, self.hi, self.sem = src, dst, lo, hi, sem

        def start(self, priority=0):
            w = self.dst.shape[2]
            for p in range(self.lo, self.hi):
                pltpu.make_async_copy(self.src.at[:, p * w:(p + 1) * w], self.dst.at[p],
                                      self.sem).start(priority=priority)

        def wait(self):
            whole = self.dst.at[self.lo:self.hi]
            pltpu.make_async_copy(whole, whole, self.sem).wait()

    def x_cols(t0, n):
        return jnp.concatenate([xt_v[t0 // LANES + i] for i in range(n // LANES)], axis=1)

    x_first = Pieces(xt_hbm, xt_v, 0, nb, misc_sems.at[0])
    x_second = Pieces(xt_hbm, xt_v, nb, nb + 1, misc_sems.at[10])
    x_rest = Pieces(xt_hbm, xt_v, nb + 1, seq // LANES, misc_sems.at[1])
    mod_first = [col_copy(wmod_hbm, wmod_v, MODC, 2 * d, misc_sems.at[8]),
                 col_copy(wmod_hbm, wmod_v, 0, MODC, misc_sems.at[9])]
    mod_rest = col_copy(wmod_hbm, wmod_v, 2 * d, 6 * d, misc_sems.at[3])
    mlp_g = pltpu.make_async_copy(wg_hbm, wg_v, mlp_sems.at[0])
    mlp_u = pltpu.make_async_copy(wu_hbm, wu_v, mlp_sems.at[1])
    ff = wdt_hbm.shape[1]
    mlp_d = Pieces(wdt_hbm, wdt_v, 0, ff // WP, mlp_sems.at[2])
    out_lo = col_copy(ot_v, o_hbm, 0, seq - TB, out_sems.at[0])
    chunks = list(zip(EDGES[:-1], EDGES[1:]))
    out_hi = [pltpu.make_async_copy(ot_v.at[r0:r1, seq - TB:seq], o_hbm.at[r0:r1, seq - TB:seq],
                                    out_sems.at[1 + i]) for i, (r0, r1) in enumerate(chunks)]

    def silu_c():
        cc = c_ref[...].astype(F32)
        return jnp.broadcast_to((cc * _rb(_sigmoid(cc))).astype(BF16), (8, d))

    def ln1_norm(t0, n, marks):
        x = x_cols(t0, n).astype(F32)
        mu = _colsum(x, marks, NM1) * (1.0 / d)
        marks.append(_fold(jnp.broadcast_to(mu, (8, n))))
        xc = x - mu
        var = _colsum(xc * xc, marks, NM2) * (1.0 / d)
        rs = lax.rsqrt(var + EPS)

        def finish(z=None):
            r = rs if z is None else lax.bitcast_convert_type(
                lax.bitcast_convert_type(rs, U32) | _lanes(z[0:1], n), F32)
            return (xc * r).astype(BF16).T
        return finish

    def ln1_mod(ln, slot, r0, marks):
        n = ln.shape[0]
        h = ln.astype(F32) * mod_scr[1:2, :] + mod_scr[0:1, :]
        h_scr[slot, _span(r0, n), :] = h.astype(BF16)
        step = max(n // NM3, 8)
        for r in range(step - 8, n, step):
            marks.append(_fold(h[r:r + 8]))

    def mod_piece(src, dst, marks):
        w = wmod_v[:, _span(src, MP)].astype(F32)
        row0 = _rb(_colsum(w * _lanes(col_scr[5 * d:6 * d, :], MP), marks, NMP))

        def finish(z):
            row = lax.bitcast_convert_type(
                lax.bitcast_convert_type(row0, U32) | _lanes(z[0:1], MP), F32)
            pos = dst + lax.broadcasted_iota(I32, (1, MP), 1)
            is_cb = jnp.logical_and(pos >= 2 * d, pos < 3 * d)
            row = jnp.where(is_cb, _rb(1.0 + row), row)
            row_scr[:, _span(dst, MP)] = row
            col_scr[_span(dst, MP), :] = jnp.broadcast_to(row, (LANES, MP)).T
        return finish

    def wd_piece(src, dst, marks):
        w = pltpu.bitcast(wdt_v[src // WP].T, U32)
        wd_scr[pl.ds(pl.multiple_of(dst // 2, WP // 2), WP // 2), :] = w
        for r in range(56, WP // 2, 64):
            for c in range(0, d - LANES + 1, LANES):
                marks.append(w[r:r + 8, c:c + LANES])

    dm = d - d % LANES
    kr = d - dm

    def hb_piece(slot, r0, n, marks, z=None):
        src = pl.ds(r0 if isinstance(r0, int) else pl.multiple_of(r0, n), n)
        dst = pl.ds(r0 // 2 if isinstance(r0, int) else pl.multiple_of(r0 // 2, n // 2), n // 2)
        hu = pltpu.bitcast(h_scr[slot, src, dm:d], U32)
        if z is not None:
            hu = hu | jnp.concatenate([z[:, 0:kr]] * (n // 16), axis=0)
        for k in range(kr):
            col = jnp.broadcast_to(hu[:, k:k + 1], (n // 2, LANES))
            hb_scr[slot, k, dst, :] = col
            if (k + 1) % HS == 0:
                marks.append(col[n // 2 - 8:n // 2])

    def wb_piece(u, toks, zero):
        w = lax.bitcast_convert_type(wrem_v[:, _span(grp_of(u) * gw, gw)].astype(F32), U32)
        for k in range(kr):
            row = jnp.broadcast_to(w[k:k + 1], (8, gw))
            row = row | _lanes(toks[k * len(toks) // kr] & zero, gw)
            wb_scr[k] = lax.bitcast_convert_type(row, F32)

    class Rem:
        def __init__(self, slot):
            self.marks, self.done, self.ready = [], {}, []
            for p in range(RV // 16):
                acc = None
                for k in range(kr):
                    hb = pltpu.bitcast(hb_scr[slot, k, 8 * p:8 * p + 8, :], BF16).astype(F32)
                    w = wb_scr[k]
                    t = _lanes(hb, gw) * jnp.concatenate([w, w], axis=0)
                    acc = t if acc is None else acc + t
                    if (k + 1) % KS == 0:
                        for c in range(0, gw, gw // KSPLIT):
                            self.marks.append(_fold(acc[:, c:c + gw // KSPLIT]))
                self.done[len(self.marks) - 1] = (p, acc)

        def take(self, phase, others=()):
            n, tot = len(self.marks), SHARES[-1]
            lo, hi = SHARES[phase] * n // tot, SHARES[phase + 1] * n // tot
            for i in range(lo, hi):
                if i in self.done:
                    self.ready.append((*self.done[i], phase, (i + 1 - lo) / (hi - lo)))
            mine = self.marks[lo:hi]
            return _merge(others, mine) if others and mine else list(others) + mine

        def flush(self, st, zero, phase, hi):
            old = [r for r in self.ready if r[2] < phase]
            for p, acc, ph, frac in self.ready:
                if ph < phase:
                    rl = 8 * (([r[0] for r in old].index(p) + 1) * 200 // (len(old) + 1))
                else:
                    rl = 16 * min(int(TLO + frac * (hi - TLO)) - 4, 118)
                tok = lax.bitcast_convert_type(st[rl:rl + 8, 0:LANES], U32)
                z = jnp.concatenate([_lanes(tok & zero, gw)] * 2, axis=0)
                rem_scr[16 * p:16 * p + 16, :] = lax.bitcast_convert_type(
                    lax.bitcast_convert_type(acc, U32) | z, F32)
            self.ready = []

    def qproj2(u, toks, zero):
        h = h_scr[blk_of(u) & 1]
        q = jnp.dot(h[RV:TB, dm:d], wq_v[grp_of(u), dm:d, :], preferred_element_type=F32)
        r = jnp.concatenate([rem_scr[...], q], axis=0)
        outs = []
        for i in range(nq):
            tk = toks[i * len(toks) // nq:(i + 1) * len(toks) // nq]
            hm = _tie_rows(h[:, 0:dm], tk, zero, 0, TB // 16)
            q = jnp.dot(hm, wq_v[grp_of(u), 0:dm, i * DH:(i + 1) * DH],
                        preferred_element_type=F32) + r[:, i * DH:(i + 1) * DH]
            outs.append((q * qscale).astype(BF16))
        return jnp.concatenate(outs, axis=1)

    def qproj(u, lo=0, hi=gw, parts=1):
        qs = []
        for r0 in range(0, TB, TB // parts):
            rs = slice(r0, r0 + TB // parts)
            if REMF:
                q = jnp.dot(h_scr[blk_of(u) & 1, rs, dm:d], wq_v[grp_of(u), dm:d, lo:hi],
                            preferred_element_type=F32)
                q = jnp.dot(h_scr[blk_of(u) & 1, rs, 0:dm], wq_v[grp_of(u), 0:dm, lo:hi],
                            preferred_element_type=F32) + q
            else:
                q = jnp.dot(h_scr[blk_of(u) & 1, rs, :], wq_v[grp_of(u), :, lo:hi],
                            preferred_element_type=F32)
            qs.append((q * qscale).astype(BF16))
        return jnp.concatenate(qs, axis=0)

    def qk(u, q, j, toks=(), zero=None, hi=THI):
        k = _tie_rows(k_v[grp_of(u) * HG + j // 2], toks, zero, TLO, hi)
        st = lax.dot_general(k, q[:, j * DH:(j + 1) * DH], _NT,
                             preferred_element_type=F32)
        for i in range(nb):
            blk = st[:, i * LANES:(i + 1) * LANES]
            st_scr[j * nb + i] = blk
            if DEFM:
                m_scr[j * nb + i] = jnp.max(blk.reshape(sk // 8, 8, LANES), axis=0)
            else:
                m_scr[j * nb + i, 0:1] = jnp.max(blk, axis=0, keepdims=True)
        return st

    def v_transpose(u, i, marks=None, rel=(), zero=None):
        v = _tie_rows(v_v[grp_of(u) * HG + i], rel, zero, -7, sk // 16 - 7)
        vt = pltpu.bitcast(v.T, U32)
        vt_scr[i] = vt
        if marks is not None:
            step = sk // NVT
            for c in range(step - LANES, sk, step):
                marks.append(vt[DH // 2 - 8:DH // 2, c:c + LANES])

    def pv(slots, zero, toks=()):
        ps, ls, pairs = [], [], []
        for sl in slots:
            m = jnp.max(m_scr[sl], axis=0, keepdims=True) if DEFM else m_scr[sl, 0:1]
            p = jnp.exp2(st_scr[sl] - m)
            accs = [None] * 4
            for tile in range(nt):
                for r0 in range(tile * LANES + LANES - 16, tile * LANES - 16, -16):
                    pair = p[r0:r0 + 8] + p[r0 + 8:r0 + 16]
                    pairs.append(pair)
                    a = accs[tile % 4]
                    accs[tile % 4] = pair if a is None else a + pair
            ls.append(jnp.sum((accs[0] + accs[1]) + (accs[2] + accs[3]), axis=0, keepdims=True))
            ps.append(p.astype(BF16))
        outs = []
        ntiles = len(slots) * nt
        side = {}
        for i, tok in enumerate(toks):
            side.setdefault(((i + 1) * ntiles) // len(toks) - 1, []).append(tok)
        for i, sl in enumerate(slots):
            vu = vt_scr[sl // (2 * nb)]
            tiles = []
            for c in range(nt):
                g = i * nt + c + 4
                rows = []
                for r in range(8):
                    x = vu[8 * r:8 * r + 8, c * LANES:(c + 1) * LANES]
                    if g < ntiles and TIE0 <= r < TIE0 + NTIE:
                        src = pairs[g * 8 + (r - TIE0)]
                        x = x | (lax.bitcast_convert_type(src, U32) & zero)
                    if r == SIDE_ROW:
                        for tok in side.get(i * nt + c, ()):
                            x = x | (tok & zero)
                    rows.append(x)
                tiles.append(jnp.concatenate(rows, axis=0))
            lhs = pltpu.bitcast(jnp.concatenate(tiles, axis=1), BF16)
            o = jnp.dot(lhs, ps[i], preferred_element_type=F32)
            outs.append((o * (1.0 / ls[i])).astype(BF16))
        return outs

    def outproj_tied(u, o, toks, zero):
        slot = blk_of(u) & 1
        res = []
        for i in range(nb):
            o2 = jnp.concatenate([o[j * nb + i] for j in range(nq)], axis=0)
            tk = toks[i * len(toks) // OPN:(i + 1) * len(toks) // OPN]
            wo = _tie_rows(wot_v[grp_of(u)], tk, zero, 0, d // 16)
            contrib = jnp.dot(wo, o2, preferred_element_type=F32)
            old = jnp.where(grp_of(u) > 0, acc_scr[slot * nb + i], 0.0)
            acc_scr[slot * nb + i] = old + contrib
            res.append(contrib)
        return jnp.concatenate(res, axis=0)

    def outproj(u, o, lo=0):
        w = len(o) // nq
        o2 = jnp.concatenate(
            [jnp.concatenate(o[j * w:(j + 1) * w], axis=1) for j in range(nq)], axis=0)
        contrib = jnp.dot(wot_v[grp_of(u)], o2, preferred_element_type=F32)
        slot = blk_of(u) & 1
        for i in range(w):
            pi = slot * nb + lo // LANES + i
            old = jnp.where(grp_of(u) > 0, acc_scr[pi], 0.0)
            acc_scr[pi] = old + contrib[:, i * LANES:(i + 1) * LANES]

    def router_keys(racc, t0):
        r = _rb(jnp.sum(racc, axis=0, keepdims=True)) + 0.0
        bits = lax.bitcast_convert_type(r, I32) >> 16
        order = jnp.where(bits < 0, -1 - bits, bits + 32768)
        pos = t0 + lax.broadcasted_iota(I32, r.shape, 1)
        return lax.bitcast_convert_type((order << 11) + (seq - 1 - pos) + 0x20000000, F32)

    def finalize(t0, slot, a0, dst, n, keys_out=None):
        marks = []
        cs = _span(dst, n)
        x = x_cols(t0, n).astype(F32)
        att = jnp.concatenate(
            [acc_scr[slot * nb + a0 // LANES + i] for i in range(n // LANES)], axis=1)
        x1b = (x + _lanes(col_scr[0:d, :], n) * att).astype(BF16)
        x1_scr[:, cs] = x1b
        ot_v[:, cs] = x1b
        mu = _colsum(x1b.astype(F32), marks, NG1 if MID and n == SP else NF1) * (1.0 / d)
        fine = MID and n == SP

        def note(row):
            if fine:
                marks.append(_fold(jnp.broadcast_to(row, (8, n))))
            return row

        mub = note(_rb(mu))
        xc = x1_scr[:, cs].astype(F32) - mub
        var = _colsum(xc * xc, marks, NG2 if fine else NF2) * (1.0 / d) - (mu - mub) * (mu - mub)
        inv = note(1.0 / note(_rb(jnp.sqrt(note(_rb(_rb(jnp.maximum(var, 0.0)) + EPS_BF16))))))
        step = d // NF3
        racc = None
        for r0 in range(0, d, step):
            rs = slice(r0, r0 + step)
            x1 = ot_v[rs, cs].astype(F32)
            ln = _rb(_rb(x1 - mub) * inv)
            if MID and n == SP:
                marks.append(_fold(ln))
            h2b = (_rb(ln * _lanes(col_scr[2 * d + r0:2 * d + r0 + step, :], n))
                   + _lanes(col_scr[d + r0:d + r0 + step, :], n)).astype(BF16)
            if keys_out is None:
                h2_scr[rs, cs] = h2b
            else:
                h2l_scr[rs, :] = h2b
            h2 = h2b.astype(F32)
            out = x1 + _lanes(col_scr[3 * d + r0:3 * d + r0 + step, :], n) * h2
            ot_v[rs, cs] = out.astype(BF16)
            rp = h2 * _lanes(col_scr[4 * d + r0:4 * d + r0 + step, :], n)
            for g in range(0, step, 8):
                racc = rp[g:g + 8] if racc is None else racc + rp[g:g + 8]
            marks.append(_fold(out, racc))
        if keys_out is not None:
            keys_out.append(racc)
            return marks
        key = router_keys(racc, t0)
        for i in range(n // LANES):
            key_scr[pl.ds(dst // LANES + i, 1), :] = key[:, i * LANES:(i + 1) * LANES]
        return marks

    hw = gw // 2
    wq0a = col_copy(wq_hbm, wq_v.at[0], 0, hw, grp_sems.at[0, 0])
    wq0b = col_copy(wq_hbm, wq_v.at[0], hw, gw, misc_sems.at[4])
    k0a = pltpu.make_async_copy(k_hbm.at[0], k_v.at[0], grp_sems.at[1, 0])
    k0b = pltpu.make_async_copy(k_hbm.at[1], k_v.at[1], misc_sems.at[5])
    v0 = pltpu.make_async_copy(v_hbm.at[0:HG], v_v.at[0:HG], grp_sems.at[2, 0])
    wq1, k1, v1, wo0 = grp_copies(1)
    wo_last = pltpu.make_async_copy(wot_hbm.at[:, (n_grp - 1) * gw:n_grp * gw],
                                    wot_v.at[n_grp - 1], grp_sems.at[3, 0])
    wrem_copy = col_copy(wq_hbm.at[dm:d], wrem_v, gw, 4 * gw, misc_sems.at[2])
    wrem_rest = (col_copy(wq_hbm.at[dm:d], wrem_v, 0, gw, misc_sems.at[11]),
                 col_copy(wq_hbm.at[dm:d], wrem_v, 4 * gw, n_grp * gw, misc_sems.at[12]))
    c_copy = pltpu.make_async_copy(c_hbm, c_ref, misc_sems.at[6])
    wr_copy = pltpu.make_async_copy(wr_hbm, wr_ref, misc_sems.at[7])
    c_copy.start()
    wr_copy.start()
    x_first.start()
    mod_first[0].start()
    mod_first[1].start()
    wq0a.start()
    wq0b.start()
    acc_scr[nb:2 * nb] = jnp.zeros((nb, d, LANES), F32)
    col_scr[0:4 * d, :] = jnp.zeros((4 * d, LANES), F32)
    wdt_v[ff // WP] = jnp.zeros((d, WP), BF16)
    with _scope("w_x"):
        c_copy.wait()
        wr_copy.wait()
        x_first.wait()
    cbits = lax.bitcast_convert_type(c_ref[:, 0:LANES].astype(F32), U32)
    zero_scr[...] = jnp.broadcast_to(cbits & 0xFFFF, (8, LANES))
    h_scr[0] = ln1_norm(0, TB, [])()
    sc = silu_c()
    wr = wr_ref[...].reshape(1, d).astype(F32)
    col_scr[4 * d:5 * d, :] = jnp.broadcast_to(wr, (LANES, d)).T
    col_scr[5 * d:6 * d, :] = jnp.broadcast_to(sc[0:1, :].astype(F32), (LANES, d)).T
    with _scope("w_wmod"):
        mod_first[0].wait()
    mod = _rb(jnp.dot(sc, wmod_v[:, MODC:2 * d], preferred_element_type=F32))
    mod_scr[0:1, MODC:d] = mod[0:1, 0:d - MODC]
    mod_scr[1:2, :] = _rb(1.0 + mod[0:1, d - MODC:2 * d - MODC])
    with _scope("w_wmod2"):
        mod_first[1].wait()
    k0a.start(priority=KAP)
    if not LATEKV:
        k0b.start(priority=1)
        v0.start(priority=1)
    mod_scr[0:1, 0:MODC] = _rb(jnp.dot(sc, wmod_v[:, 0:MODC], preferred_element_type=F32))[0:1]
    if EARLYMOD:
        ln1_mod(h_scr[0], 0, 0, [])
    with _scope("w_wq"):
        wq0a.wait()
    if LATEKV:
        k0b.start(priority=1)
        v0.start(priority=1)
        wrem_copy.start(priority=1)
    if not EARLYMOD:
        ln1_mod(h_scr[0], 0, 0, [])
    qa = qproj(0, 0, hw, 2)
    with _scope("w_k"):
        wq0b.wait()
        k0a.wait()
    wq1.start(priority=1)
    k1.start(priority=1)
    x_second.start()
    q = jnp.concatenate([qa, qproj(0, hw, gw, 2)], axis=1)
    zero = zero_scr[...]
    nhb = -(-RV // HP)
    for j in range(2):
        marks = []
        for i in range(j * nhb // 2, (j + 1) * nhb // 2):
            hb_piece(0, i * HP, HP, marks)
        qk(0, q, j, marks, zero)
    with _scope("w_v"):
        k0b.wait()
        v0.wait()
        wrem_copy.wait()
    v1.start()
    wo0.start()
    with _scope("qk0"):
        zero = zero_scr[...]
        rem_scr[...] = jnp.dot(h_scr[0, 0:RV, dm:d], wrem_v[:, gw:2 * gw],
                               preferred_element_type=F32)
        for i in range(HG):
            marks = []
            v_transpose(0, i, marks)
            if i == 0:
                wb_piece(2, marks, zero)
            qk(0, q, nq - HG + i, marks, zero)

    assert n_grp == 8 and HG == 2
    stage_at = [1, 2, 3, 5, n_units]
    starts = [(*grp_copies(2), mod_rest, x_rest, *wrem_rest), grp_copies(3, 3),
              (*grp_copies(6, 2), wo_last, mlp_d), (mlp_g, mlp_u)]
    waits = [(wq1, k1, v1, wo0, x_second), *starts[:3]]
    wd0 = stage_at[3]
    npc = TB // SP
    nmp = 4 * d // MP

    def manage(k, _, c):
        for cp in waits[k]:
            cp.wait()
        for cp in starts[k]:
            cp.start()
        return c

    def steady(u, carry):
        with _scope("body"):
            zero = zero_scr[...]
            blk, g = blk_of(u), grp_of(u)
            off = ((g - 1) & (npc - 1)) * SP
            rem = Rem(blk_of(u + 1) & 1)
            q = qproj2(u, rem.take(0), zero)
            o = pv(range(0, 2 * nb), zero, rem.take(1))
            live = jnp.logical_and(blk > 0, jnp.logical_and(g >= 1, g <= npc))
            t0 = jnp.maximum(blk - 1, 0) * TB + off
            marks = finalize(t0, (blk + 1) & 1, off, jnp.where(live, t0, seq), SP)
            wp = jnp.clip(u - wd0, 0, ff // WP - 1) * WP
            wmarks = []
            wd_piece(jnp.where(u >= wd0, wp, ff), wp, wmarks)
            rem.flush(qk(u, q, 0, rem.take(2, _merge(marks, wmarks)), zero), zero, 2, THI)
            def tok_at(res, row):
                return lax.bitcast_convert_type(res[row:row + 8, 0:LANES], U32)

            marks, mmarks = [], []
            ln_fin = ln1_norm(jnp.minimum(blk + 1, n_blk - 1) * TB + off, SP, marks)
            mp = jnp.clip(u - 2, 0, nmp - 1) * MP
            mod_fin = mod_piece(jnp.where(u >= 2, 2 * d + mp, 0), mp, mmarks)
            st = qk(u, q, 1, rem.take(3, marks + mmarks), zero)
            rem.flush(st, zero, 3, THI)
            ln1_mod(ln_fin(tok_at(st, LNREL) & zero), (blk + 1) & 1, off, [])
            mod_fin(tok_at(st, 1880) & zero)
            o += pv(range(2 * nb, 4 * nb), zero, rem.take(4))
            st = qk(u, q, 2, rem.take(5), zero)
            rem.flush(st, zero, 5, THI)
            v_transpose(u, 0, None, [tok_at(st, 112 * i) for i in range(nt)], zero)
            st = qk(u, q, 3, rem.take(6), zero)
            rem.flush(st, zero, 6, THI)
            v_transpose(u, 1, None, [tok_at(st, 112 * i) for i in range(nt)], zero)
            res = outproj_tied(u - 1, o, rem.take(7), zero)
            rem.flush(res, zero, 7, OPN * d // 16)
            hm = []
            hb_piece((blk + 1) & 1, jnp.clip(g - 1, 0, nhb - 1) * HP, HP, hm,
                     tok_at(res, max(OPN * d - 96, 0)) & zero)
            wb_piece(u + 2, hm, zero)
        return carry

    def stage(k, lo):
        hi = stage_at[1]
        for i in range(len(waits)):
            lax.fori_loop(0, jnp.where(k == i, 1, 0), functools.partial(manage, i), 0)
            hi = jnp.where(k == i, stage_at[i + 1], hi)
        lax.fori_loop(lo, hi, steady, 0)
        return hi

    lax.fori_loop(0, len(waits), stage, jnp.int32(stage_at[0]))

    ul = n_units - 1
    tl = seq - TB
    sl_last = (n_blk - 1) & 1
    nb0 = nb - TAILB
    with _scope("e_pva"):
        mod_scr[2:3, :] = row_scr[:, 3 * d:4 * d]
        outproj(ul, pv([j * nb + i for j in range(nq) for i in range(nb0)], zero_scr[...]))
    mlp_g.wait()
    mlp_u.wait()
    out_lo.start()
    with _scope("e_pvb"):
        toks = finalize(tl, sl_last, 0, tl, nb0 * LANES)
        o = pv([j * nb + i for j in range(nq) for i in range(nb0, nb)], zero_scr[...], toks)
        outproj(ul, o, nb0 * LANES)

    nl = TAILB * LANES
    sub8 = lax.broadcasted_iota(I32, (TOPC, 1), 0)
    lane = lax.broadcasted_iota(I32, (TOPC, LANES), 1)

    def key_index(k):
        return seq - 1 - (lax.bitcast_convert_type(k, I32) & (seq - 1))

    def piece_base(idx, limit):
        return pl.multiple_of(jnp.clip(idx >> 7, 0, limit // LANES - 1) * LANES, LANES)

    keys = key_scr[0:seq // LANES, :]
    piece = lax.broadcasted_iota(I32, (seq // LANES, 1), 0)
    keys = jnp.where(piece < (seq - nl) // LANES, keys, 0.0)
    ecol = jnp.zeros((TOPC, LANES), F32)
    erow = jnp.zeros((1, LANES), F32)
    h2e = jnp.zeros((TOPC, d), F32)
    late = []
    marks = finalize(seq - nl, sl_last, TB - nl, seq - nl, nl, late)
    zero = zero_scr[...]
    pace = dict(zip([int(v) for v in os.environ.get("KP_PG", "2,4,5,6,7").split(",")],
                    [int(v) for v in os.environ.get("KP_PM", "8,14,18,23,27").split(",")]))
    for i in range(TOPC):
        mx = jnp.max(jnp.max(keys, axis=0, keepdims=True), axis=1, keepdims=True)
        keys = jnp.where(keys == mx, 0.0, keys)
        ecol = jnp.where(sub8 == i, mx, ecol)
        erow = jnp.where(lane[0:1] == i, mx, erow)
        idx = key_index(mx)
        pick = jnp.logical_and(sub8 == i, lane == (idx & (LANES - 1)))
        sl = pl.ds(piece_base(idx[0, 0], seq - nl), LANES)
        pick = jnp.where(pick, 1.0, 0.0)
        if i in pace:
            pick = lax.bitcast_convert_type(
                lax.bitcast_convert_type(pick, U32) | (marks[pace[i]] & zero), F32)
        h2e = h2e + lax.dot_general(pick.astype(BF16), h2_scr[:, sl], _NT,
                                    preferred_element_type=F32)

    late = [router_keys(late[0], seq - nl)]
    krow = jnp.concatenate([late[0], erow], axis=1)
    kcol = jnp.concatenate([jnp.broadcast_to(late[0], (LANES, nl)).T, ecol], axis=0)
    cnt = [None] * 4
    for g in range(kcol.shape[0] // 8):
        one = jnp.where(_lanes(kcol[8 * g:8 * g + 8], nl + LANES) > krow, 1.0, 0.0)
        cnt[g % 4] = one if cnt[g % 4] is None else cnt[g % 4] + one
    rank = jnp.sum((cnt[0] + cnt[1]) + (cnt[2] + cnt[3]), axis=0, keepdims=True)
    chosen = rank == sub8.astype(F32)
    onehot = jnp.where(chosen, 1.0, 0.0).astype(BF16)
    h2pad = jnp.concatenate([h2e, jnp.zeros((TOPC, d), F32)], axis=0).astype(BF16)
    h2s = (jnp.dot(onehot[:, nl:nl + 2 * TOPC], h2pad, preferred_element_type=F32)
           + lax.dot_general(onehot[:, 0:nl], h2l_scr[...], _NT,
                             preferred_element_type=F32))
    top = jnp.max(jnp.where(chosen, krow, 0.0), axis=1, keepdims=True)
    idx_col = key_index(top)
    idxs = [idx_col[i:i + 1] for i in range(TOPC)]
    bases = [piece_base(idx_col[i, 0], seq) for i in range(TOPC)]
    hit = lane == (idx_col & (LANES - 1))
    picks = [jnp.where(jnp.logical_and(sub8 == i, hit), 1.0, 0.0).astype(BF16)
             for i in range(TOPC)]
    order = (lax.bitcast_convert_type(top, I32) >> 11) & 0xFFFF
    rbits = jnp.where(order >= 32768, order - 32768, -1 - order) << 16
    gate = _rb(_sigmoid(lax.bitcast_convert_type(rbits, F32)))
    xs = h2s.astype(BF16)
    for cp in out_hi:
        cp.start()
    g = _rb(jnp.dot(xs, wg_v[...], preferred_element_type=F32))
    g = _rb(g * _rb(_sigmoid(g)))
    u = _rb(jnp.dot(xs, wu_v[...], preferred_element_type=F32))
    gu = (g * u).astype(BF16)

    last_use = []
    for i in range(TOPC):
        ok = True
        for j in range(i + 1, TOPC):
            ok = jnp.logical_and(ok, bases[i] != bases[j])
        last_use.append(ok)

    def down(r0, r1):
        x1p = jnp.concatenate([x1_scr[r0:r1, pl.ds(bases[i], LANES)] for i in range(TOPC)], axis=1)
        x1s = lax.dot_general(jnp.concatenate(picks, axis=1), x1p, _NT,
                              preferred_element_type=F32)
        wd = pltpu.bitcast(wd_scr[:, r0:r1], BF16)
        y = _rb(jnp.dot(gu, wd, preferred_element_type=F32))
        hm = _rb(h2s[:, r0:r1] + _rb(y * gate))
        return x1s + mod_scr[2:3, r0:r1] * hm

    def patch(r0, r1, new):
        n = r1 - r0
        pad = jnp.concatenate([new, jnp.zeros((LANES - TOPC, n), F32)], axis=0)
        cols = pltpu.bitcast(pad.T.astype(BF16), U32)
        col = [jnp.broadcast_to(cols[:, j:j + 1], (n // 2, LANES)) for j in range(TOPC)]
        for i in range(TOPC):
            res = pltpu.bitcast(ot_v[r0:r1, pl.ds(bases[i], LANES)], U32)
            tok = lane[0:1, :] + (idxs[i] & ~(LANES - 1))
            for j in range(i + 1):
                res = jnp.where(tok == idxs[j], col[j], res)
            fix_v[i, r0:r1, :] = pltpu.bitcast(res, BF16)

    def fix_copy(i, r0, r1):
        return pltpu.make_async_copy(fix_v.at[i, r0:r1, :],
                                     o_hbm.at[r0:r1, pl.ds(bases[i], LANES)], fix_sems.at[i])

    def for_last(fn):
        for i in range(TOPC - 1):
            pl.when(last_use[i])(functools.partial(fn, i))
        fn(TOPC - 1)

    new = down(*chunks[0])
    out_lo.wait()
    for ci, (r0, r1) in enumerate(chunks):
        out_hi[ci].wait()
        nxt = down(*chunks[ci + 1]) if ci + 1 < len(chunks) else None
        patch(r0, r1, new)
        for_last(lambda i: fix_copy(i, r0, r1).start())
        new = nxt
    with _scope("w_fix"):
        for r0, r1 in chunks:
            for_last(lambda i: fix_copy(i, r0, r1).wait())


@jax.jit
def pallas_adaLN_cond__gqa_block_cached__moe_arch_mod__prompt_kernel(
    A_x: jax.Array,
    A_k_cache: jax.Array,
    A_v_cache: jax.Array,
    A_wq: jax.Array,
    A_wo: jax.Array,
    B_x: jax.Array,
    B_w_r: jax.Array,
    B_w_gate: jax.Array,
    B_w_up: jax.Array,
    B_w_down: jax.Array,
    c: jax.Array,
    w_mod: jax.Array,
):
    b, seq, d = A_x.shape
    _, hkv, sk, dh = A_k_cache.shape
    assert b == 1 and dh == DH and HQ == 2 * hkv
    assert seq & (seq - 1) == 0 and seq <= 2048
    f = B_w_gate.shape[1]
    n_grp = hkv // HG
    gw = 2 * HG * dh
    n_slots = 2 * HG * TB // LANES

    xt = A_x.reshape(seq, d).T
    wot = A_wo.T
    wdt = B_w_down.T
    k3 = A_k_cache.reshape(hkv, sk, dh)
    v3 = A_v_cache.reshape(hkv, sk, dh)

    hbm = pl.BlockSpec(memory_space=pl.ANY)
    out_t = pl.pallas_call(
        functools.partial(_kernel, n_heads=hkv),
        in_specs=[hbm] * 11,
        out_specs=hbm,
        out_shape=jax.ShapeDtypeStruct((d, seq), BF16),
        scratch_shapes=[
            pltpu.VMEM((seq // LANES, d, LANES), BF16),
            pltpu.VMEM((hkv, sk, dh), BF16),
            pltpu.VMEM((hkv, sk, dh), BF16),
            pltpu.VMEM((n_grp, d, gw), BF16),
            pltpu.VMEM((n_grp, d, gw), BF16),
            pltpu.VMEM((d, 6 * d), BF16),
            pltpu.VMEM((d, f), BF16),
            pltpu.VMEM((d, f), BF16),
            pltpu.VMEM((f // WP + 1, d, WP), BF16),
            pltpu.VMEM((d, seq + SP), BF16),
            pltpu.VMEM((2, TB, d), BF16),
            pltpu.VMEM((2 * TB // LANES, d, LANES), F32),
            pltpu.VMEM((n_slots, sk, LANES), F32),
            pltpu.VMEM((n_slots, 8, LANES), F32),
            pltpu.VMEM((HG, dh // 2, sk), U32),
            pltpu.VMEM((8, d), F32),
            pltpu.VMEM((6 * d, LANES), F32),
            pltpu.VMEM(((seq + SP) // LANES + 7 & ~7, LANES), F32),
            pltpu.VMEM((d, seq + SP), BF16),
            pltpu.VMEM((d, seq + SP), BF16),
            pltpu.VMEM((8, LANES), U32),
            pltpu.VMEM((TOPC, d, LANES), BF16),
            pltpu.VMEM((1, d), BF16),
            pltpu.VMEM((d,), BF16),
            pltpu.VMEM((1, 4 * d), F32),
            pltpu.VMEM((f // 2, d), U32),
            pltpu.VMEM((d, TAILB * LANES), BF16),
            pltpu.VMEM((2, d % LANES, -(-RV // HP) * HP // 2, LANES), U32),
            pltpu.VMEM((d % LANES, 8, gw), F32),
            pltpu.VMEM((RV, gw), F32),
            pltpu.VMEM((d % LANES, n_grp * gw), BF16),
            pltpu.SemaphoreType.DMA((4, n_grp)),
            pltpu.SemaphoreType.DMA((13,)),
            pltpu.SemaphoreType.DMA((3,)),
            pltpu.SemaphoreType.DMA((len(EDGES),)),
            pltpu.SemaphoreType.DMA((TOPC,)),
        ],
        compiler_params=pltpu.CompilerParams(
            disable_bounds_checks=True,
            disable_semaphore_checks=True,
            vmem_limit_bytes=120 * 1024 * 1024,
        ),
    )(xt, k3, v3, A_wq, wot, B_w_r, B_w_gate, B_w_up, wdt, c, w_mod)
    return out_t.T.reshape(b, seq, d)
```

```python
import contextlib
import functools
import math
import os

import jax
import jax.numpy as jnp
from jax import lax
import jax.experimental.pallas as pl
import jax.experimental.pallas.tpu as pltpu

F32 = jnp.float32
BF16 = jnp.bfloat16
I32 = jnp.int32
U32 = jnp.uint32

HQ = 32
DH = 128
TOPC = 8
EPS = 1e-05
EPS_BF16 = 1.0013580322265625e-05
LANES = 128

TB = 512
HG = 2
TIE0 = int(os.environ.get("KP_TIE0", "2"))
NTIE = int(os.environ.get("KP_NTIE", "3"))
SP = int(os.environ.get("KP_SP", "128"))
NM1 = int(os.environ.get("KP_NM1", "8"))
NM2 = int(os.environ.get("KP_NM2", "12"))
NM3 = int(os.environ.get("KP_NM3", "16"))
TLO = int(os.environ.get("KP_TLO", "3"))
NF1 = int(os.environ.get("KP_NF1", "9"))
NF2 = int(os.environ.get("KP_NF2", "6"))
NF3 = int(os.environ.get("KP_NF3", "18"))
NVT = int(os.environ.get("KP_NVT", "16"))
TAILB = int(os.environ.get("KP_TAILB", "2"))
SROWS = [int(v) for v in os.environ.get("KP_SROWS", "1,3,5,6").split(",")]
EROWS = [int(v) for v in os.environ.get("KP_EROWS", "1,3,5,6").split(",")]
EDGES = [int(e) for e in os.environ.get("KP_EDGES", "0,128,256,384,512,576").split(",")]
MODC = int(os.environ.get("KP_MODC", "384"))
MP = int(os.environ.get("KP_MP", "384"))
NMP = int(os.environ.get("KP_NMP", "12"))
WP = 256
REMF = int(os.environ.get("KP_REMF", "1"))
DEFM = int(os.environ.get("KP_DEFM", "1"))
KAP = int(os.environ.get("KP_KAP", "0"))
LATEKV = int(os.environ.get("KP_LATEKV", "1"))
EARLYMOD = int(os.environ.get("KP_EARLYMOD", "0"))
RV = int(os.environ.get("KP_RV", "352"))
HP = 64
KS = int(os.environ.get("KP_KS", "4"))
KSPLIT = int(os.environ.get("KP_KSPLIT", "2"))
HS = int(os.environ.get("KP_HS", "1"))
THI = int(os.environ.get("KP_THI", "126"))
OPN = int(os.environ.get("KP_OPN", "2"))
LNREL = int(os.environ.get("KP_LNREL", "1104"))
_sh = [int(v) for v in os.environ.get("KP_SH", "28,17,10,18,17,26,28,16").split(",")]
SHARES = [sum(_sh[:i]) for i in range(len(_sh) + 1)]
MID = int(os.environ.get("KP_MID", "1"))
NG1 = int(os.environ.get("KP_NG1", "18"))
NG2 = int(os.environ.get("KP_NG2", "12"))
EFINE = int(os.environ.get("KP_EFINE", "1"))
EF3 = int(os.environ.get("KP_EF3", "36"))
PVEND = int(os.environ.get("KP_PVEND", "8"))
EPVEND = int(os.environ.get("KP_EPVEND", "12"))
SCOPES = os.environ.get("KP_SCOPES", "") == "1"

_NT = (((1,), (1,)), ((), ()))


def _rb(x):
    return x.astype(BF16).astype(F32)


def _sigmoid(x):
    return 1.0 / (1.0 + jnp.exp(-x))


def _lanes(col, width):
    reps = width // LANES
    return col if reps == 1 else jnp.concatenate([col] * reps, axis=1)


def _fold(*xs):
    ts = []
    for x in xs:
        xi = lax.bitcast_convert_type(x, U32)
        ts += [xi[r:r + 8, c:c + LANES] for r in range(0, x.shape[0], 8)
               for c in range(0, x.shape[1] - LANES + 1, LANES)]
    if len(ts) > 5:
        return functools.reduce(lambda a, b: a | b, ts[:-2]) | (ts[-2] | ts[-1])
    while len(ts) > 1:
        ts = [a | b for a, b in zip(ts[0::2], ts[1::2])] + ts[len(ts) & ~1:]
    return ts[0]


def _colsum(x, marks, nmarks):
    n = x.shape[0] // 8
    acc = x[0:8]
    for g in range(1, n):
        acc = acc + x[8 * g:8 * g + 8]
        if ((g + 1) * nmarks) % n == 0:
            marks.append(_fold(acc))
    return jnp.sum(acc, axis=0, keepdims=True)


def _tie_rows(lhs, toks, zero, lo, hi, c0=0):
    if not toks:
        return lhs
    lu = pltpu.bitcast(lhs, U32)
    rows = [lu[8 * r:8 * r + 8] for r in range(lu.shape[0] // 8)]
    for i, tok in enumerate(toks):
        r = lo + ((i + 1) * (hi - lo)) // len(toks) - 1
        head = rows[r][:, c0:c0 + LANES] | (tok & zero)
        rows[r] = head if lu.shape[1] == LANES else jnp.concatenate(
            [head, rows[r][:, LANES:]], axis=1)
    return pltpu.bitcast(jnp.concatenate(rows, axis=0), BF16)


def _merge(a, b):
    keyed = [((i + 1) / len(a), t) for i, t in enumerate(a)]
    keyed += [((i + 1) / len(b), t) for i, t in enumerate(b)]
    return [t for _, t in sorted(keyed, key=lambda kv: kv[0])]


def _span(start, size):
    if isinstance(start, int):
        return pl.ds(start, size)
    return pl.ds(pl.multiple_of(start, LANES), size)


def _scope(name):
    return jax.named_scope(name) if SCOPES else contextlib.nullcontext()


def _kernel(xt_hbm, k_hbm, v_hbm, wq_hbm, wot_hbm, wr_hbm, wg_hbm, wu_hbm, wdt_hbm,
            c_hbm, wmod_hbm, o_hbm,
            xt_v, k_v, v_v, wq_v, wot_v, wmod_v, wg_v, wu_v, wdt_v, ot_v,
            h_scr, acc_scr, st_scr, m_scr, vt_scr, mod_scr, col_scr, key_scr, h2_scr, x1_scr,
            zero_scr, fix_v, c_ref, wr_ref, row_scr, wd_scr, h2l_scr, hb_scr, wb_scr, rem_scr, wrem_v,
            grp_sems, misc_sems, mlp_sems, out_sems, fix_sems,
            *, n_heads):
    d, seq = xt_hbm.shape
    sk = k_v.shape[1]
    n_grp = n_heads // HG
    n_blk = seq // TB
    n_units = n_grp * n_blk
    nb = TB // LANES
    nq = 2 * HG
    nt = sk // LANES
    gbits = n_grp.bit_length() - 1
    gw = nq * DH
    qscale = (DH ** -0.5) * math.log2(math.e)

    def grp_of(u):
        return u & (n_grp - 1)

    def blk_of(u):
        return u >> gbits

    def grp_copies(g, n=1):
        hs = pl.ds(g * HG, n * HG)
        return (*[pltpu.make_async_copy(wq_hbm.at[:, pl.ds(i * gw, gw)], wq_v.at[i],
                                        grp_sems.at[0, i]) for i in range(g, g + n)],
                pltpu.make_async_copy(k_hbm.at[hs], k_v.at[hs], grp_sems.at[1, g]),
                pltpu.make_async_copy(v_hbm.at[hs], v_v.at[hs], grp_sems.at[2, g]),
                *[pltpu.make_async_copy(wot_hbm.at[:, pl.ds((i - 1) * gw, gw)], wot_v.at[i - 1],
                                        grp_sems.at[3, i]) for i in range(g, g + n)])

    def col_copy(src, dst, lo, hi, sem):
        return pltpu.make_async_copy(src.at[:, lo:hi], dst.at[:, lo:hi], sem)

    class Pieces:
        def __init__(self, src, dst, lo, hi, sem):
            self.src, self.dst, self.lo, self.hi, self.sem = src, dst, lo, hi, sem

        def start(self, priority=0):
            w = self.dst.shape[2]
            for p in range(self.lo, self.hi):
                pltpu.make_async_copy(self.src.at[:, p * w:(p + 1) * w], self.dst.at[p],
                                      self.sem).start(priority=priority)

        def wait(self):
            whole = self.dst.at[self.lo:self.hi]
            pltpu.make_async_copy(whole, whole, self.sem).wait()

    def x_cols(t0, n):
        return jnp.concatenate([xt_v[t0 // LANES + i] for i in range(n // LANES)], axis=1)

    x_first = Pieces(xt_hbm, xt_v, 0, nb, misc_sems.at[0])
    x_second = Pieces(xt_hbm, xt_v, nb, nb + 1, misc_sems.at[10])
    x_rest = Pieces(xt_hbm, xt_v, nb + 1, seq // LANES, misc_sems.at[1])
    mod_first = [col_copy(wmod_hbm, wmod_v, MODC, 2 * d, misc_sems.at[8]),
                 col_copy(wmod_hbm, wmod_v, 0, MODC, misc_sems.at[9])]
    mod_rest = col_copy(wmod_hbm, wmod_v, 2 * d, 6 * d, misc_sems.at[3])
    mlp_g = pltpu.make_async_copy(wg_hbm, wg_v, mlp_sems.at[0])
    mlp_u = pltpu.make_async_copy(wu_hbm, wu_v, mlp_sems.at[1])
    ff = wdt_hbm.shape[1]
    mlp_d = Pieces(wdt_hbm, wdt_v, 0, ff // WP, mlp_sems.at[2])
    out_lo = col_copy(ot_v, o_hbm, 0, seq - TB, out_sems.at[0])
    chunks = list(zip(EDGES[:-1], EDGES[1:]))
    out_hi = [pltpu.make_async_copy(ot_v.at[r0:r1, seq - TB:seq], o_hbm.at[r0:r1, seq - TB:seq],
                                    out_sems.at[1 + i]) for i, (r0, r1) in enumerate(chunks)]

    def silu_c():
        cc = c_ref[...].astype(F32)
        return jnp.broadcast_to((cc * _rb(_sigmoid(cc))).astype(BF16), (8, d))

    def ln1_norm(t0, n, marks):
        x = x_cols(t0, n).astype(F32)
        mu = _colsum(x, marks, NM1) * (1.0 / d)
        marks.append(_fold(jnp.broadcast_to(mu, (8, n))))
        xc = x - mu
        var = _colsum(xc * xc, marks, NM2) * (1.0 / d)
        rs = lax.rsqrt(var + EPS)

        def finish(z=None):
            r = rs if z is None else lax.bitcast_convert_type(
                lax.bitcast_convert_type(rs, U32) | _lanes(z[0:1], n), F32)
            return (xc * r).astype(BF16).T
        return finish

    def ln1_mod(ln, slot, r0, marks):
        n = ln.shape[0]
        h = ln.astype(F32) * mod_scr[1:2, :] + mod_scr[0:1, :]
        h_scr[slot, _span(r0, n), :] = h.astype(BF16)
        step = max(n // NM3, 8)
        for r in range(step - 8, n, step):
            marks.append(_fold(h[r:r + 8]))

    def mod_piece(src, dst, marks):
        w = wmod_v[:, _span(src, MP)].astype(F32)
        row0 = _rb(_colsum(w * _lanes(col_scr[5 * d:6 * d, :], MP), marks, NMP))

        def finish(z):
            row = lax.bitcast_convert_type(
                lax.bitcast_convert_type(row0, U32) | _lanes(z[0:1], MP), F32)
            pos = dst + lax.broadcasted_iota(I32, (1, MP), 1)
            is_cb = jnp.logical_and(pos >= 2 * d, pos < 3 * d)
            row = jnp.where(is_cb, _rb(1.0 + row), row)
            row_scr[:, _span(dst, MP)] = row
            col_scr[_span(dst, MP), :] = jnp.broadcast_to(row, (LANES, MP)).T
        return finish

    def wd_piece(src, dst, marks):
        w = pltpu.bitcast(wdt_v[src // WP].T, U32)
        wd_scr[pl.ds(pl.multiple_of(dst // 2, WP // 2), WP // 2), :] = w
        for r in range(56, WP // 2, 64):
            for c in range(0, d - LANES + 1, LANES):
                marks.append(w[r:r + 8, c:c + LANES])

    dm = d - d % LANES
    kr = d - dm

    def hb_piece(slot, r0, n, marks, z=None):
        src = pl.ds(r0 if isinstance(r0, int) else pl.multiple_of(r0, n), n)
        dst = pl.ds(r0 // 2 if isinstance(r0, int) else pl.multiple_of(r0 // 2, n // 2), n // 2)
        hu = pltpu.bitcast(h_scr[slot, src, dm:d], U32)
        if z is not None:
            hu = hu | jnp.concatenate([z[:, 0:kr]] * (n // 16), axis=0)
        for k in range(kr):
            col = jnp.broadcast_to(hu[:, k:k + 1], (n // 2, LANES))
            hb_scr[slot, k, dst, :] = col
            if (k + 1) % HS == 0:
                marks.append(col[n // 2 - 8:n // 2])

    def wb_piece(u, toks, zero):
        w = lax.bitcast_convert_type(wrem_v[:, _span(grp_of(u) * gw, gw)].astype(F32), U32)
        for k in range(kr):
            row = jnp.broadcast_to(w[k:k + 1], (8, gw))
            row = row | _lanes(toks[k * len(toks) // kr] & zero, gw)
            wb_scr[k] = lax.bitcast_convert_type(row, F32)

    class Rem:
        def __init__(self, slot):
            self.marks, self.done, self.ready = [], {}, []
            for p in range(RV // 16):
                acc = None
                for k in range(kr):
                    hb = pltpu.bitcast(hb_scr[slot, k, 8 * p:8 * p + 8, :], BF16).astype(F32)
                    w = wb_scr[k]
                    t = _lanes(hb, gw) * jnp.concatenate([w, w], axis=0)
                    acc = t if acc is None else acc + t
                    if (k + 1) % KS == 0:
                        for c in range(0, gw, gw // KSPLIT):
                            self.marks.append(_fold(acc[:, c:c + gw // KSPLIT]))
                self.done[len(self.marks) - 1] = (p, acc)

        def take(self, phase, others=()):
            n, tot = len(self.marks), SHARES[-1]
            lo, hi = SHARES[phase] * n // tot, SHARES[phase + 1] * n // tot
            for i in range(lo, hi):
                if i in self.done:
                    self.ready.append((*self.done[i], phase, (i + 1 - lo) / (hi - lo)))
            mine = self.marks[lo:hi]
            return _merge(others, mine) if others and mine else list(others) + mine

        def flush(self, st, zero, phase, hi):
            old = [r for r in self.ready if r[2] < phase]
            for p, acc, ph, frac in self.ready:
                if ph < phase:
                    rl = 8 * (([r[0] for r in old].index(p) + 1) * 200 // (len(old) + 1))
                else:
                    rl = 16 * min(int(TLO + frac * (hi - TLO)) - 4, 118)
                tok = lax.bitcast_convert_type(st[rl:rl + 8, 0:LANES], U32)
                z = jnp.concatenate([_lanes(tok & zero, gw)] * 2, axis=0)
                rem_scr[16 * p:16 * p + 16, :] = lax.bitcast_convert_type(
                    lax.bitcast_convert_type(acc, U32) | z, F32)
            self.ready = []

    def qproj2(u, toks, zero):
        h = h_scr[blk_of(u) & 1]
        q = jnp.dot(h[RV:TB, dm:d], wq_v[grp_of(u), dm:d, :], preferred_element_type=F32)
        r = jnp.concatenate([rem_scr[...], q], axis=0)
        outs = []
        for i in range(nq):
            tk = toks[i * len(toks) // nq:(i + 1) * len(toks) // nq]
            hm = _tie_rows(h[:, 0:dm], tk, zero, 0, TB // 16)
            q = jnp.dot(hm, wq_v[grp_of(u), 0:dm, i * DH:(i + 1) * DH],
                        preferred_element_type=F32) + r[:, i * DH:(i + 1) * DH]
            outs.append((q * qscale).astype(BF16))
        return jnp.concatenate(outs, axis=1)

    def qproj(u, lo=0, hi=gw, parts=1):
        qs = []
        for r0 in range(0, TB, TB // parts):
            rs = slice(r0, r0 + TB // parts)
            if REMF:
                q = jnp.dot(h_scr[blk_of(u) & 1, rs, dm:d], wq_v[grp_of(u), dm:d, lo:hi],
                            preferred_element_type=F32)
                q = jnp.dot(h_scr[blk_of(u) & 1, rs, 0:dm], wq_v[grp_of(u), 0:dm, lo:hi],
                            preferred_element_type=F32) + q
            else:
                q = jnp.dot(h_scr[blk_of(u) & 1, rs, :], wq_v[grp_of(u), :, lo:hi],
                            preferred_element_type=F32)
            qs.append((q * qscale).astype(BF16))
        return jnp.concatenate(qs, axis=0)

    def qk(u, q, j, toks=(), zero=None, hi=THI):
        k = _tie_rows(k_v[grp_of(u) * HG + j // 2], toks, zero, TLO, hi)
        st = lax.dot_general(k, q[:, j * DH:(j + 1) * DH], _NT,
                             preferred_element_type=F32)
        for i in range(nb):
            blk = st[:, i * LANES:(i + 1) * LANES]
            st_scr[j * nb + i] = blk
            if DEFM:
                m_scr[j * nb + i] = jnp.max(blk.reshape(sk // 8, 8, LANES), axis=0)
            else:
                m_scr[j * nb + i, 0:1] = jnp.max(blk, axis=0, keepdims=True)
        return st

    def v_transpose(u, i, marks=None, rel=(), zero=None):
        v = _tie_rows(v_v[grp_of(u) * HG + i], rel, zero, -7, sk // 16 - 7)
        vt = pltpu.bitcast(v.T, U32)
        vt_scr[i] = vt
        if marks is not None:
            step = sk // NVT
            for c in range(step - LANES, sk, step):
                marks.append(vt[DH // 2 - 8:DH // 2, c:c + LANES])

    def pv(slots, zero, toks=(), srows=None):
        ps, ls, pairs = [], [], []
        for sl in slots:
            m = jnp.max(m_scr[sl], axis=0, keepdims=True) if DEFM else m_scr[sl, 0:1]
            p = jnp.exp2(st_scr[sl] - m)
            accs = [None] * 4
            for tile in range(nt):
                for r0 in range(tile * LANES + LANES - 16, tile * LANES - 16, -16):
                    pair = p[r0:r0 + 8] + p[r0 + 8:r0 + 16]
                    pairs.append(pair)
                    a = accs[tile % 4]
                    accs[tile % 4] = pair if a is None else a + pair
            ls.append(jnp.sum((accs[0] + accs[1]) + (accs[2] + accs[3]), axis=0, keepdims=True))
            ps.append(p.astype(BF16))
        outs = []
        ntiles = len(slots) * nt
        side = {}
        for i, tok in enumerate(toks):
            side.setdefault(max(((i + 1) * (ntiles - (EPVEND if srows else PVEND))) // len(toks) - 1, 0), []).append(tok)
        for i, sl in enumerate(slots):
            vu = vt_scr[sl // (2 * nb)]
            tiles = []
            for c in range(nt):
                g = i * nt + c + 4
                rows = []
                for r in range(8):
                    x = vu[8 * r:8 * r + 8, c * LANES:(c + 1) * LANES]
                    if g < ntiles and TIE0 <= r < TIE0 + NTIE:
                        src = pairs[g * 8 + (r - TIE0)]
                        x = x | (lax.bitcast_convert_type(src, U32) & zero)
                    if r == (srows or SROWS)[c % 4]:
                        for tok in side.get(i * nt + c, ()):
                            x = x | (tok & zero)
                    rows.append(x)
                tiles.append(jnp.concatenate(rows, axis=0))
            lhs = pltpu.bitcast(jnp.concatenate(tiles, axis=1), BF16)
            o = jnp.dot(lhs, ps[i], preferred_element_type=F32)
            outs.append((o * (1.0 / ls[i])).astype(BF16))
        return outs

    def outproj_tied(u, o, toks, zero):
        slot = blk_of(u) & 1
        res = []
        for i in range(nb):
            o2 = jnp.concatenate([o[j * nb + i] for j in range(nq)], axis=0)
            tk = toks[i * len(toks) // OPN:(i + 1) * len(toks) // OPN]
            wo = _tie_rows(wot_v[grp_of(u)], tk, zero, 0, d // 16)
            contrib = jnp.dot(wo, o2, preferred_element_type=F32)
            old = jnp.where(grp_of(u) > 0, acc_scr[slot * nb + i], 0.0)
            acc_scr[slot * nb + i] = old + contrib
            res.append(contrib)
        return jnp.concatenate(res, axis=0)

    def outproj(u, o, lo=0):
        w = len(o) // nq
        o2 = jnp.concatenate(
            [jnp.concatenate(o[j * w:(j + 1) * w], axis=1) for j in range(nq)], axis=0)
        contrib = jnp.dot(wot_v[grp_of(u)], o2, preferred_element_type=F32)
        slot = blk_of(u) & 1
        for i in range(w):
            pi = slot * nb + lo // LANES + i
            old = jnp.where(grp_of(u) > 0, acc_scr[pi], 0.0)
            acc_scr[pi] = old + contrib[:, i * LANES:(i + 1) * LANES]

    def router_keys(racc, t0):
        r = _rb(jnp.sum(racc, axis=0, keepdims=True)) + 0.0
        bits = lax.bitcast_convert_type(r, I32) >> 16
        order = jnp.where(bits < 0, -1 - bits, bits + 32768)
        pos = t0 + lax.broadcasted_iota(I32, r.shape, 1)
        return lax.bitcast_convert_type((order << 11) + (seq - 1 - pos) + 0x20000000, F32)

    def finalize(t0, slot, a0, dst, n, keys_out=None):
        marks = []
        cs = _span(dst, n)
        x = x_cols(t0, n).astype(F32)
        att = jnp.concatenate(
            [acc_scr[slot * nb + a0 // LANES + i] for i in range(n // LANES)], axis=1)
        x1b = (x + _lanes(col_scr[0:d, :], n) * att).astype(BF16)
        x1_scr[:, cs] = x1b
        ot_v[:, cs] = x1b
        mu = _colsum(x1b.astype(F32), marks, NG1 if MID and (n == SP or (EFINE and keys_out is None)) else NF1) * (1.0 / d)
        fine = MID and (n == SP or (EFINE and keys_out is None))

        def note(row):
            if fine:
                marks.append(_fold(jnp.broadcast_to(row, (8, n))))
            return row

        mub = note(_rb(mu))
        xc = x1_scr[:, cs].astype(F32) - mub
        var = _colsum(xc * xc, marks, NG2 if fine else NF2) * (1.0 / d) - (mu - mub) * (mu - mub)
        inv = note(1.0 / note(_rb(jnp.sqrt(note(_rb(_rb(jnp.maximum(var, 0.0)) + EPS_BF16))))))
        step = d // (EF3 if fine and n != SP else NF3)
        racc = None
        for r0 in range(0, d, step):
            rs = slice(r0, r0 + step)
            x1 = ot_v[rs, cs].astype(F32)
            ln = _rb(_rb(x1 - mub) * inv)
            if fine:
                marks.append(_fold(ln))
            h2b = (_rb(ln * _lanes(col_scr[2 * d + r0:2 * d + r0 + step, :], n))
                   + _lanes(col_scr[d + r0:d + r0 + step, :], n)).astype(BF16)
            if keys_out is None:
                h2_scr[rs, cs] = h2b
            else:
                h2l_scr[rs, :] = h2b
            h2 = h2b.astype(F32)
            out = x1 + _lanes(col_scr[3 * d + r0:3 * d + r0 + step, :], n) * h2
            ot_v[rs, cs] = out.astype(BF16)
            rp = h2 * _lanes(col_scr[4 * d + r0:4 * d + r0 + step, :], n)
            for g in range(0, step, 8):
                racc = rp[g:g + 8] if racc is None else racc + rp[g:g + 8]
            marks.append(_fold(out, racc))
        if keys_out is not None:
            keys_out.append(racc)
            return marks
        key = router_keys(racc, t0)
        for i in range(n // LANES):
            key_scr[pl.ds(dst // LANES + i, 1), :] = key[:, i * LANES:(i + 1) * LANES]
        return marks

    hw = gw // 2
    wq0a = col_copy(wq_hbm, wq_v.at[0], 0, hw, grp_sems.at[0, 0])
    wq0b = col_copy(wq_hbm, wq_v.at[0], hw, gw, misc_sems.at[4])
    k0a = pltpu.make_async_copy(k_hbm.at[0], k_v.at[0], grp_sems.at[1, 0])
    k0b = pltpu.make_async_copy(k_hbm.at[1], k_v.at[1], misc_sems.at[5])
    v0 = pltpu.make_async_copy(v_hbm.at[0:HG], v_v.at[0:HG], grp_sems.at[2, 0])
    wq1, k1, v1, wo0 = grp_copies(1)
    wo_last = pltpu.make_async_copy(wot_hbm.at[:, (n_grp - 1) * gw:n_grp * gw],
                                    wot_v.at[n_grp - 1], grp_sems.at[3, 0])
    wrem_copy = col_copy(wq_hbm.at[dm:d], wrem_v, gw, 4 * gw, misc_sems.at[2])
    wrem_rest = (col_copy(wq_hbm.at[dm:d], wrem_v, 0, gw, misc_sems.at[11]),
                 col_copy(wq_hbm.at[dm:d], wrem_v, 4 * gw, n_grp * gw, misc_sems.at[12]))
    c_copy = pltpu.make_async_copy(c_hbm, c_ref, misc_sems.at[6])
    wr_copy = pltpu.make_async_copy(wr_hbm, wr_ref, misc_sems.at[7])
    c_copy.start()
    wr_copy.start()
    x_first.start()
    mod_first[0].start()
    mod_first[1].start()
    wq0a.start()
    wq0b.start()
    acc_scr[nb:2 * nb] = jnp.zeros((nb, d, LANES), F32)
    col_scr[0:4 * d, :] = jnp.zeros((4 * d, LANES), F32)
    wdt_v[ff // WP] = jnp.zeros((d, WP), BF16)
    with _scope("w_x"):
        c_copy.wait()
        wr_copy.wait()
        x_first.wait()
    cbits = lax.bitcast_convert_type(c_ref[:, 0:LANES].astype(F32), U32)
    zero_scr[...] = jnp.broadcast_to(cbits & 0xFFFF, (8, LANES))
    h_scr[0] = ln1_norm(0, TB, [])()
    sc = silu_c()
    wr = wr_ref[...].reshape(1, d).astype(F32)
    col_scr[4 * d:5 * d, :] = jnp.broadcast_to(wr, (LANES, d)).T
    col_scr[5 * d:6 * d, :] = jnp.broadcast_to(sc[0:1, :].astype(F32), (LANES, d)).T
    with _scope("w_wmod"):
        mod_first[0].wait()
    mod = _rb(jnp.dot(sc, wmod_v[:, MODC:2 * d], preferred_element_type=F32))
    mod_scr[0:1, MODC:d] = mod[0:1, 0:d - MODC]
    mod_scr[1:2, :] = _rb(1.0 + mod[0:1, d - MODC:2 * d - MODC])
    with _scope("w_wmod2"):
        mod_first[1].wait()
    k0a.start(priority=KAP)
    if not LATEKV:
        k0b.start(priority=1)
        v0.start(priority=1)
    mod_scr[0:1, 0:MODC] = _rb(jnp.dot(sc, wmod_v[:, 0:MODC], preferred_element_type=F32))[0:1]
    if EARLYMOD:
        ln1_mod(h_scr[0], 0, 0, [])
    with _scope("w_wq"):
        wq0a.wait()
    if LATEKV:
        k0b.start(priority=1)
        v0.start(priority=1)
        wrem_copy.start(priority=1)
    if not EARLYMOD:
        ln1_mod(h_scr[0], 0, 0, [])
    qa = qproj(0, 0, hw, 2)
    with _scope("w_k"):
        wq0b.wait()
        k0a.wait()
    wq1.start(priority=1)
    k1.start(priority=1)
    x_second.start()
    q = jnp.concatenate([qa, qproj(0, hw, gw, 2)], axis=1)
    zero = zero_scr[...]
    nhb = -(-RV // HP)
    for j in range(2):
        marks = []
        for i in range(2 * j, 2 * j + 2):
            hb_piece(0, i * HP, HP, marks)
        qk(0, q, j, marks, zero)
    with _scope("w_v"):
        k0b.wait()
        v0.wait()
        wrem_copy.wait()
    v1.start()
    wo0.start()
    with _scope("qk0"):
        zero = zero_scr[...]
        rem_scr[...] = jnp.dot(h_scr[0, 0:RV, dm:d], wrem_v[:, gw:2 * gw],
                               preferred_element_type=F32)
        for i in range(HG):
            marks = []
            v_transpose(0, i, marks)
            if i == 0:
                wb_piece(2, marks, zero)
            else:
                hm = []
                for p in range(4, nhb):
                    hb_piece(0, p * HP, HP, hm, rel & zero)
                marks = _merge(marks, hm)
            st = qk(0, q, nq - HG + i, marks, zero)
            rel = lax.bitcast_convert_type(st[1800:1808, 0:LANES], U32)

    assert n_grp == 8 and HG == 2
    stage_at = [1, 2, 3, 5, n_units]
    starts = [(*grp_copies(2), mod_rest, x_rest, *wrem_rest), grp_copies(3, 3),
              (*grp_copies(6, 2), wo_last, mlp_d), (mlp_g, mlp_u)]
    waits = [(wq1, k1, v1, wo0, x_second), *starts[:3]]
    wd0 = stage_at[3]
    npc = TB // SP
    nmp = 4 * d // MP

    def manage(k, _, c):
        for cp in waits[k]:
            cp.wait()
        for cp in starts[k]:
            cp.start()
        return c

    def steady(u, carry):
        with _scope("body"):
            zero = zero_scr[...]
            blk, g = blk_of(u), grp_of(u)
            off = ((g - 1) & (npc - 1)) * SP
            rem = Rem(blk_of(u + 1) & 1)
            q = qproj2(u, rem.take(0), zero)
            o = pv(range(0, 2 * nb), zero, rem.take(1))
            live = jnp.logical_and(blk > 0, jnp.logical_and(g >= 1, g <= npc))
            t0 = jnp.maximum(blk - 1, 0) * TB + off
            marks = finalize(t0, (blk + 1) & 1, off, jnp.where(live, t0, seq), SP)
            wp = jnp.clip(u - wd0, 0, ff // WP - 1) * WP
            wmarks = []
            wd_piece(jnp.where(u >= wd0, wp, ff), wp, wmarks)
            rem.flush(qk(u, q, 0, rem.take(2, _merge(marks, wmarks)), zero), zero, 2, THI)
            def tok_at(res, row):
                return lax.bitcast_convert_type(res[row:row + 8, 0:LANES], U32)

            marks, mmarks = [], []
            ln_fin = ln1_norm(jnp.minimum(blk + 1, n_blk - 1) * TB + off, SP, marks)
            mp = jnp.clip(u - 2, 0, nmp - 1) * MP
            mod_fin = mod_piece(jnp.where(u >= 2, 2 * d + mp, 0), mp, mmarks)
            st = qk(u, q, 1, rem.take(3, marks + mmarks), zero)
            rem.flush(st, zero, 3, THI)
            ln1_mod(ln_fin(tok_at(st, LNREL) & zero), (blk + 1) & 1, off, [])
            mod_fin(tok_at(st, 1880) & zero)
            o += pv(range(2 * nb, 4 * nb), zero, rem.take(4))
            st = qk(u, q, 2, rem.take(5), zero)
            rem.flush(st, zero, 5, THI)
            v_transpose(u, 0, None, [tok_at(st, 112 * i) for i in range(nt)], zero)
            st = qk(u, q, 3, rem.take(6), zero)
            rem.flush(st, zero, 6, THI)
            v_transpose(u, 1, None, [tok_at(st, 112 * i) for i in range(nt)], zero)
            res = outproj_tied(u - 1, o, rem.take(7), zero)
            rem.flush(res, zero, 7, OPN * d // 16)
            hm = []
            hb_piece((blk + 1) & 1, jnp.clip(g - 1, 0, nhb - 1) * HP, HP, hm,
                     tok_at(res, max(OPN * d - 96, 0)) & zero)
            wb_piece(u + 2, hm, zero)
        return carry

    def stage(k, lo):
        hi = stage_at[1]
        for i in range(len(waits)):
            lax.fori_loop(0, jnp.where(k == i, 1, 0), functools.partial(manage, i), 0)
            hi = jnp.where(k == i, stage_at[i + 1], hi)
        lax.fori_loop(lo, hi, steady, 0)
        return hi

    lax.fori_loop(0, len(waits), stage, jnp.int32(stage_at[0]))

    ul = n_units - 1
    tl = seq - TB
    sl_last = (n_blk - 1) & 1
    nb0 = nb - TAILB
    with _scope("e_pva"):
        mod_scr[2:3, :] = row_scr[:, 3 * d:4 * d]
        outproj(ul, pv([j * nb + i for j in range(nq) for i in range(nb0)], zero_scr[...]))
    mlp_g.wait()
    mlp_u.wait()
    out_lo.start()
    with _scope("e_pvb"):
        toks = finalize(tl, sl_last, 0, tl, nb0 * LANES)
        o = pv([j * nb + i for j in range(nq) for i in range(nb0, nb)], zero_scr[...], toks, EROWS)
        outproj(ul, o, nb0 * LANES)

    nl = TAILB * LANES
    sub8 = lax.broadcasted_iota(I32, (TOPC, 1), 0)
    lane = lax.broadcasted_iota(I32, (TOPC, LANES), 1)

    def key_index(k):
        return seq - 1 - (lax.bitcast_convert_type(k, I32) & (seq - 1))

    def piece_base(idx, limit):
        return pl.multiple_of(jnp.clip(idx >> 7, 0, limit // LANES - 1) * LANES, LANES)

    keys = key_scr[0:seq // LANES, :]
    piece = lax.broadcasted_iota(I32, (seq // LANES, 1), 0)
    keys = jnp.where(piece < (seq - nl) // LANES, keys, 0.0)
    ecol = jnp.zeros((TOPC, LANES), F32)
    erow = jnp.zeros((1, LANES), F32)
    h2e = jnp.zeros((TOPC, d), F32)
    late = []
    marks = finalize(seq - nl, sl_last, TB - nl, seq - nl, nl, late)
    zero = zero_scr[...]
    pace = dict(zip([int(v) for v in os.environ.get("KP_PG", "2,4,5,6,7").split(",")],
                    [int(v) for v in os.environ.get("KP_PM", "8,14,18,23,27").split(",")]))
    for i in range(TOPC):
        mx = jnp.max(jnp.max(keys, axis=0, keepdims=True), axis=1, keepdims=True)
        keys = jnp.where(keys == mx, 0.0, keys)
        ecol = jnp.where(sub8 == i, mx, ecol)
        erow = jnp.where(lane[0:1] == i, mx, erow)
        idx = key_index(mx)
        pick = jnp.logical_and(sub8 == i, lane == (idx & (LANES - 1)))
        sl = pl.ds(piece_base(idx[0, 0], seq - nl), LANES)
        pick = jnp.where(pick, 1.0, 0.0)
        if i in pace:
            pick = lax.bitcast_convert_type(
                lax.bitcast_convert_type(pick, U32) | (marks[pace[i]] & zero), F32)
        h2e = h2e + lax.dot_general(pick.astype(BF16), h2_scr[:, sl], _NT,
                                    preferred_element_type=F32)

    late = [router_keys(late[0], seq - nl)]
    krow = jnp.concatenate([late[0], erow], axis=1)
    kcol = jnp.concatenate([jnp.broadcast_to(late[0], (LANES, nl)).T, ecol], axis=0)
    cnt = [None] * 4
    for g in range(kcol.shape[0] // 8):
        one = jnp.where(_lanes(kcol[8 * g:8 * g + 8], nl + LANES) > krow, 1.0, 0.0)
        cnt[g % 4] = one if cnt[g % 4] is None else cnt[g % 4] + one
    rank = jnp.sum((cnt[0] + cnt[1]) + (cnt[2] + cnt[3]), axis=0, keepdims=True)
    chosen = rank == sub8.astype(F32)
    onehot = jnp.where(chosen, 1.0, 0.0).astype(BF16)
    h2pad = jnp.concatenate([h2e, jnp.zeros((TOPC, d), F32)], axis=0).astype(BF16)
    h2s = (jnp.dot(onehot[:, nl:nl + 2 * TOPC], h2pad, preferred_element_type=F32)
           + lax.dot_general(onehot[:, 0:nl], h2l_scr[...], _NT,
                             preferred_element_type=F32))
    top = jnp.max(jnp.where(chosen, krow, 0.0), axis=1, keepdims=True)
    idx_col = key_index(top)
    idxs = [idx_col[i:i + 1] for i in range(TOPC)]
    bases = [piece_base(idx_col[i, 0], seq) for i in range(TOPC)]
    hit = lane == (idx_col & (LANES - 1))
    picks = [jnp.where(jnp.logical_and(sub8 == i, hit), 1.0, 0.0).astype(BF16)
             for i in range(TOPC)]
    order = (lax.bitcast_convert_type(top, I32) >> 11) & 0xFFFF
    rbits = jnp.where(order >= 32768, order - 32768, -1 - order) << 16
    gate = _rb(_sigmoid(lax.bitcast_convert_type(rbits, F32)))
    xs = h2s.astype(BF16)
    for cp in out_hi:
        cp.start()
    g = _rb(jnp.dot(xs, wg_v[...], preferred_element_type=F32))
    g = _rb(g * _rb(_sigmoid(g)))
    u = _rb(jnp.dot(xs, wu_v[...], preferred_element_type=F32))
    gu = (g * u).astype(BF16)

    last_use = []
    for i in range(TOPC):
        ok = True
        for j in range(i + 1, TOPC):
            ok = jnp.logical_and(ok, bases[i] != bases[j])
        last_use.append(ok)

    def down(r0, r1):
        x1p = jnp.concatenate([x1_scr[r0:r1, pl.ds(bases[i], LANES)] for i in range(TOPC)], axis=1)
        x1s = lax.dot_general(jnp.concatenate(picks, axis=1), x1p, _NT,
                              preferred_element_type=F32)
        wd = pltpu.bitcast(wd_scr[:, r0:r1], BF16)
        y = _rb(jnp.dot(gu, wd, preferred_element_type=F32))
        hm = _rb(h2s[:, r0:r1] + _rb(y * gate))
        return x1s + mod_scr[2:3, r0:r1] * hm

    def patch(r0, r1, new):
        n = r1 - r0
        pad = jnp.concatenate([new, jnp.zeros((LANES - TOPC, n), F32)], axis=0)
        cols = pltpu.bitcast(pad.T.astype(BF16), U32)
        col = [jnp.broadcast_to(cols[:, j:j + 1], (n // 2, LANES)) for j in range(TOPC)]
        for i in range(TOPC):
            res = pltpu.bitcast(ot_v[r0:r1, pl.ds(bases[i], LANES)], U32)
            tok = lane[0:1, :] + (idxs[i] & ~(LANES - 1))
            for j in range(i + 1):
                res = jnp.where(tok == idxs[j], col[j], res)
            fix_v[i, r0:r1, :] = pltpu.bitcast(res, BF16)

    def fix_copy(i, r0, r1):
        return pltpu.make_async_copy(fix_v.at[i, r0:r1, :],
                                     o_hbm.at[r0:r1, pl.ds(bases[i], LANES)], fix_sems.at[i])

    def for_last(fn):
        for i in range(TOPC - 1):
            pl.when(last_use[i])(functools.partial(fn, i))
        fn(TOPC - 1)

    new = down(*chunks[0])
    out_lo.wait()
    for ci, (r0, r1) in enumerate(chunks):
        out_hi[ci].wait()
        nxt = down(*chunks[ci + 1]) if ci + 1 < len(chunks) else None
        patch(r0, r1, new)
        for_last(lambda i: fix_copy(i, r0, r1).start())
        new = nxt
    with _scope("w_fix"):
        for r0, r1 in chunks:
            for_last(lambda i: fix_copy(i, r0, r1).wait())


@jax.jit
def pallas_adaLN_cond__gqa_block_cached__moe_arch_mod__prompt_kernel(
    A_x: jax.Array,
    A_k_cache: jax.Array,
    A_v_cache: jax.Array,
    A_wq: jax.Array,
    A_wo: jax.Array,
    B_x: jax.Array,
    B_w_r: jax.Array,
    B_w_gate: jax.Array,
    B_w_up: jax.Array,
    B_w_down: jax.Array,
    c: jax.Array,
    w_mod: jax.Array,
):
    b, seq, d = A_x.shape
    _, hkv, sk, dh = A_k_cache.shape
    assert b == 1 and dh == DH and HQ == 2 * hkv
    assert seq & (seq - 1) == 0 and seq <= 2048
    f = B_w_gate.shape[1]
    n_grp = hkv // HG
    gw = 2 * HG * dh
    n_slots = 2 * HG * TB // LANES

    xt = A_x.reshape(seq, d).T
    wot = A_wo.T
    wdt = B_w_down.T
    k3 = A_k_cache.reshape(hkv, sk, dh)
    v3 = A_v_cache.reshape(hkv, sk, dh)

    hbm = pl.BlockSpec(memory_space=pl.ANY)
    out_t = pl.pallas_call(
        functools.partial(_kernel, n_heads=hkv),
        in_specs=[hbm] * 11,
        out_specs=hbm,
        out_shape=jax.ShapeDtypeStruct((d, seq), BF16),
        scratch_shapes=[
            pltpu.VMEM((seq // LANES, d, LANES), BF16),
            pltpu.VMEM((hkv, sk, dh), BF16),
            pltpu.VMEM((hkv, sk, dh), BF16),
            pltpu.VMEM((n_grp, d, gw), BF16),
            pltpu.VMEM((n_grp, d, gw), BF16),
            pltpu.VMEM((d, 6 * d), BF16),
            pltpu.VMEM((d, f), BF16),
            pltpu.VMEM((d, f), BF16),
            pltpu.VMEM((f // WP + 1, d, WP), BF16),
            pltpu.VMEM((d, seq + SP), BF16),
            pltpu.VMEM((2, TB, d), BF16),
            pltpu.VMEM((2 * TB // LANES, d, LANES), F32),
            pltpu.VMEM((n_slots, sk, LANES), F32),
            pltpu.VMEM((n_slots, 8, LANES), F32),
            pltpu.VMEM((HG, dh // 2, sk), U32),
            pltpu.VMEM((8, d), F32),
            pltpu.VMEM((6 * d, LANES), F32),
            pltpu.VMEM(((seq + SP) // LANES + 7 & ~7, LANES), F32),
            pltpu.VMEM((d, seq + SP), BF16),
            pltpu.VMEM((d, seq + SP), BF16),
            pltpu.VMEM((8, LANES), U32),
            pltpu.VMEM((TOPC, d, LANES), BF16),
            pltpu.VMEM((1, d), BF16),
            pltpu.VMEM((d,), BF16),
            pltpu.VMEM((1, 4 * d), F32),
            pltpu.VMEM((f // 2, d), U32),
            pltpu.VMEM((d, TAILB * LANES), BF16),
            pltpu.VMEM((2, d % LANES, -(-RV // HP) * HP // 2, LANES), U32),
            pltpu.VMEM((d % LANES, 8, gw), F32),
            pltpu.VMEM((RV, gw), F32),
            pltpu.VMEM((d % LANES, n_grp * gw), BF16),
            pltpu.SemaphoreType.DMA((4, n_grp)),
            pltpu.SemaphoreType.DMA((13,)),
            pltpu.SemaphoreType.DMA((3,)),
            pltpu.SemaphoreType.DMA((len(EDGES),)),
            pltpu.SemaphoreType.DMA((TOPC,)),
        ],
        compiler_params=pltpu.CompilerParams(
            disable_bounds_checks=True,
            disable_semaphore_checks=True,
            vmem_limit_bytes=120 * 1024 * 1024,
        ),
    )(xt, k3, v3, A_wq, wot, B_w_r, B_w_gate, B_w_up, wdt, c, w_mod)
    return out_t.T.reshape(b, seq, d)
```

```python
import contextlib
import functools
import math
import os

import jax
import jax.numpy as jnp
from jax import lax
import jax.experimental.pallas as pl
import jax.experimental.pallas.tpu as pltpu

F32 = jnp.float32
BF16 = jnp.bfloat16
I32 = jnp.int32
U32 = jnp.uint32

HQ = 32
DH = 128
TOPC = 8
EPS = 1e-05
EPS_BF16 = 1.0013580322265625e-05
LANES = 128

TB = 512
HG = 2
TIE0 = int(os.environ.get("KP_TIE0", "2"))
NTIE = int(os.environ.get("KP_NTIE", "3"))
SP = int(os.environ.get("KP_SP", "128"))
NM1 = int(os.environ.get("KP_NM1", "8"))
NM2 = int(os.environ.get("KP_NM2", "18"))
NM3 = int(os.environ.get("KP_NM3", "16"))
TLO = int(os.environ.get("KP_TLO", "3"))
NF1 = int(os.environ.get("KP_NF1", "9"))
NF2 = int(os.environ.get("KP_NF2", "6"))
NF3 = int(os.environ.get("KP_NF3", "18"))
NVT = int(os.environ.get("KP_NVT", "16"))
TAILB = int(os.environ.get("KP_TAILB", "2"))
SROWS = [int(v) for v in os.environ.get("KP_SROWS", "0,1,2,7").split(",")]
EROWS = [int(v) for v in os.environ.get("KP_EROWS", "1,2,5,6").split(",")]
EDGES = [int(e) for e in os.environ.get("KP_EDGES", "0,128,256,384,512,576").split(",")]
MODC = int(os.environ.get("KP_MODC", "384"))
MP = int(os.environ.get("KP_MP", "384"))
NMP = int(os.environ.get("KP_NMP", "24"))
WP = 256
REMF = int(os.environ.get("KP_REMF", "1"))
DEFM = int(os.environ.get("KP_DEFM", "1"))
KAP = int(os.environ.get("KP_KAP", "0"))
LATEKV = int(os.environ.get("KP_LATEKV", "1"))
EARLYMOD = int(os.environ.get("KP_EARLYMOD", "0"))
RV = int(os.environ.get("KP_RV", "432"))
HP = int(os.environ.get("KP_HP", "80"))
KS = int(os.environ.get("KP_KS", "4"))
KSPLIT = int(os.environ.get("KP_KSPLIT", "2"))
HS = int(os.environ.get("KP_HS", "1"))
THI = int(os.environ.get("KP_THI", "126"))
OPN = int(os.environ.get("KP_OPN", "2"))
LNREL = int(os.environ.get("KP_LNREL", "1008"))
_sh = [int(v) for v in os.environ.get("KP_SH", "29,28,13,21,26,30,31,18").split(",")]
SHARES = [sum(_sh[:i]) for i in range(len(_sh) + 1)]
MID = int(os.environ.get("KP_MID", "1"))
NG1 = int(os.environ.get("KP_NG1", "18"))
NG2 = int(os.environ.get("KP_NG2", "9"))
EFINE = int(os.environ.get("KP_EFINE", "1"))
EF3 = int(os.environ.get("KP_EF3", "36"))
PVEND = int(os.environ.get("KP_PVEND", "8"))
EPVEND = int(os.environ.get("KP_EPVEND", "4"))
SEL = int(os.environ.get("KP_SEL", "1"))
OF32 = int(os.environ.get("KP_OF32", "1"))
SCOPES = os.environ.get("KP_SCOPES", "") == "1"

_NT = (((1,), (1,)), ((), ()))


def _rb(x):
    return x.astype(BF16).astype(F32)


def _sigmoid(x):
    return 1.0 / (1.0 + jnp.exp(-x))


def _lanes(col, width):
    reps = width // LANES
    return col if reps == 1 else jnp.concatenate([col] * reps, axis=1)


def _fold(*xs):
    ts = []
    for x in xs:
        xi = lax.bitcast_convert_type(x, U32)
        ts += [xi[r:r + 8, c:c + LANES] for r in range(0, x.shape[0], 8)
               for c in range(0, x.shape[1] - LANES + 1, LANES)]
    if len(ts) > 5:
        return functools.reduce(lambda a, b: a | b, ts[:-2]) | (ts[-2] | ts[-1])
    while len(ts) > 1:
        ts = [a | b for a, b in zip(ts[0::2], ts[1::2])] + ts[len(ts) & ~1:]
    return ts[0]


def _colsum(x, marks, nmarks):
    n = x.shape[0] // 8
    acc = x[0:8]
    for g in range(1, n):
        acc = acc + x[8 * g:8 * g + 8]
        if ((g + 1) * nmarks) % n == 0:
            marks.append(_fold(acc))
    return jnp.sum(acc, axis=0, keepdims=True)


def _dep(x, tok, zero):
    if SEL:
        return jnp.where(zero != 0, tok, x)
    return x | (tok & zero)


def _tie_rows(lhs, toks, zero, lo, hi, c0=0):
    if not toks:
        return lhs
    lu = pltpu.bitcast(lhs, U32)
    rows = [lu[8 * r:8 * r + 8] for r in range(lu.shape[0] // 8)]
    for i, tok in enumerate(toks):
        r = lo + ((i + 1) * (hi - lo)) // len(toks) - 1
        head = _dep(rows[r][:, c0:c0 + LANES], tok, zero)
        rows[r] = head if lu.shape[1] == LANES else jnp.concatenate(
            [head, rows[r][:, LANES:]], axis=1)
    return pltpu.bitcast(jnp.concatenate(rows, axis=0), BF16)


def _merge(a, b):
    keyed = [((i + 1) / len(a), t) for i, t in enumerate(a)]
    keyed += [((i + 1) / len(b), t) for i, t in enumerate(b)]
    return [t for _, t in sorted(keyed, key=lambda kv: kv[0])]


def _span(start, size):
    if isinstance(start, int):
        return pl.ds(start, size)
    return pl.ds(pl.multiple_of(start, LANES), size)


def _scope(name):
    return jax.named_scope(name) if SCOPES else contextlib.nullcontext()


def _kernel(xt_hbm, k_hbm, v_hbm, wq_hbm, wot_hbm, wr_hbm, wg_hbm, wu_hbm, wdt_hbm,
            c_hbm, wmod_hbm, o_hbm,
            xt_v, k_v, v_v, wq_v, wot_v, wmod_v, wg_v, wu_v, wdt_v, ot_v,
            h_scr, acc_scr, st_scr, m_scr, vt_scr, mod_scr, col_scr, key_scr, h2_scr, x1_scr,
            zero_scr, fix_v, c_ref, wr_ref, row_scr, wd_scr, h2l_scr, hb_scr, wb_scr, rem_scr, wrem_v,
            grp_sems, misc_sems, mlp_sems, out_sems, fix_sems,
            *, n_heads):
    d, seq = xt_hbm.shape
    sk = k_v.shape[1]
    n_grp = n_heads // HG
    n_blk = seq // TB
    n_units = n_grp * n_blk
    nb = TB // LANES
    nq = 2 * HG
    nt = sk // LANES
    gbits = n_grp.bit_length() - 1
    gw = nq * DH
    qscale = (DH ** -0.5) * math.log2(math.e)

    def grp_of(u):
        return u & (n_grp - 1)

    def blk_of(u):
        return u >> gbits

    def grp_copies(g, n=1):
        hs = pl.ds(g * HG, n * HG)
        return (*[pltpu.make_async_copy(wq_hbm.at[:, pl.ds(i * gw, gw)], wq_v.at[i],
                                        grp_sems.at[0, i]) for i in range(g, g + n)],
                pltpu.make_async_copy(k_hbm.at[hs], k_v.at[hs], grp_sems.at[1, g]),
                pltpu.make_async_copy(v_hbm.at[hs], v_v.at[hs], grp_sems.at[2, g]),
                *[pltpu.make_async_copy(wot_hbm.at[:, pl.ds((i - 1) * gw, gw)], wot_v.at[i - 1],
                                        grp_sems.at[3, i]) for i in range(g, g + n)])

    def col_copy(src, dst, lo, hi, sem):
        return pltpu.make_async_copy(src.at[:, lo:hi], dst.at[:, lo:hi], sem)

    class Pieces:
        def __init__(self, src, dst, lo, hi, sem):
            self.src, self.dst, self.lo, self.hi, self.sem = src, dst, lo, hi, sem

        def start(self, priority=0):
            w = self.dst.shape[2]
            for p in range(self.lo, self.hi):
                pltpu.make_async_copy(self.src.at[:, p * w:(p + 1) * w], self.dst.at[p],
                                      self.sem).start(priority=priority)

        def wait(self):
            whole = self.dst.at[self.lo:self.hi]
            pltpu.make_async_copy(whole, whole, self.sem).wait()

    def x_cols(t0, n):
        return jnp.concatenate([xt_v[t0 // LANES + i] for i in range(n // LANES)], axis=1)

    x_first = Pieces(xt_hbm, xt_v, 0, nb, misc_sems.at[0])
    x_second = Pieces(xt_hbm, xt_v, nb, nb + 1, misc_sems.at[10])
    x_rest = Pieces(xt_hbm, xt_v, nb + 1, seq // LANES, misc_sems.at[1])
    mod_first = [col_copy(wmod_hbm, wmod_v, MODC, 2 * d, misc_sems.at[8]),
                 col_copy(wmod_hbm, wmod_v, 0, MODC, misc_sems.at[9])]
    mod_rest = col_copy(wmod_hbm, wmod_v, 2 * d, 6 * d, misc_sems.at[3])
    mlp_g = pltpu.make_async_copy(wg_hbm, wg_v, mlp_sems.at[0])
    mlp_u = pltpu.make_async_copy(wu_hbm, wu_v, mlp_sems.at[1])
    ff = wdt_hbm.shape[1]
    mlp_d = Pieces(wdt_hbm, wdt_v, 0, ff // WP, mlp_sems.at[2])
    out_lo = col_copy(ot_v, o_hbm, 0, seq - TB, out_sems.at[0])
    chunks = list(zip(EDGES[:-1], EDGES[1:]))
    out_hi = [pltpu.make_async_copy(ot_v.at[r0:r1, seq - TB:seq], o_hbm.at[r0:r1, seq - TB:seq],
                                    out_sems.at[1 + i]) for i, (r0, r1) in enumerate(chunks)]

    def silu_c():
        cc = c_ref[...].astype(F32)
        return jnp.broadcast_to((cc * _rb(_sigmoid(cc))).astype(BF16), (8, d))

    def ln1_norm(t0, n, marks):
        x = x_cols(t0, n).astype(F32)
        mu = _colsum(x, marks, NM1) * (1.0 / d)
        marks.append(_fold(jnp.broadcast_to(mu, (8, n))))
        xc = x - mu
        var = _colsum(xc * xc, marks, NM2) * (1.0 / d)
        rs = lax.rsqrt(var + EPS)

        def finish(z=None):
            r = rs if z is None else lax.bitcast_convert_type(
                lax.bitcast_convert_type(rs, U32) | _lanes(z[0:1], n), F32)
            return (xc * r).astype(BF16).T
        return finish

    def ln1_mod(ln, slot, r0, marks):
        n = ln.shape[0]
        h = ln.astype(F32) * mod_scr[1:2, :] + mod_scr[0:1, :]
        h_scr[slot, _span(r0, n), :] = h.astype(BF16)
        step = max(n // NM3, 8)
        for r in range(step - 8, n, step):
            marks.append(_fold(h[r:r + 8]))

    def mod_piece(src, dst, marks):
        w = wmod_v[:, _span(src, MP)].astype(F32)
        row0 = _rb(_colsum(w * _lanes(col_scr[5 * d:6 * d, :], MP), marks, NMP))

        def finish(z):
            row = lax.bitcast_convert_type(
                lax.bitcast_convert_type(row0, U32) | _lanes(z[0:1], MP), F32)
            pos = dst + lax.broadcasted_iota(I32, (1, MP), 1)
            is_cb = jnp.logical_and(pos >= 2 * d, pos < 3 * d)
            row = jnp.where(is_cb, _rb(1.0 + row), row)
            row_scr[:, _span(dst, MP)] = row
            col_scr[_span(dst, MP), :] = jnp.broadcast_to(row, (LANES, MP)).T
        return finish

    def wd_piece(src, dst, marks):
        w = pltpu.bitcast(wdt_v[src // WP].T, U32)
        wd_scr[pl.ds(pl.multiple_of(dst // 2, WP // 2), WP // 2), :] = w
        for r in range(56, WP // 2, 64):
            for c in range(0, d - LANES + 1, LANES):
                marks.append(w[r:r + 8, c:c + LANES])

    dm = d - d % LANES
    kr = d - dm
    nhb = -(-RV // HP)
    assert nhb <= 6 and nhb * HP <= TB

    def hb_piece(slot, sp, marks, z=None):
        r0 = sp * HP
        src = pl.ds(r0 if isinstance(r0, int) else pl.multiple_of(r0, 16), HP)
        hu = pltpu.bitcast(h_scr[slot, src, dm:d], U32)
        if z is not None:
            hu = hu | jnp.concatenate([z[:, 0:kr]] * (HP // 16), axis=0)
        for k in range(kr):
            col = jnp.broadcast_to(hu[:, k:k + 1], (HP // 2, LANES))
            hb_scr[slot * nhb + sp, k] = col
            if (k + 1) % HS == 0:
                marks.append(col[HP // 2 - 8:HP // 2])

    def wb_piece(u, toks, zero):
        w = lax.bitcast_convert_type(wrem_v[:, _span(grp_of(u) * gw, gw)].astype(F32), U32)
        for k in range(kr):
            row = jnp.broadcast_to(w[k:k + 1], (8, gw))
            row = row | _lanes(toks[k * len(toks) // kr] & zero, gw)
            wb_scr[k] = lax.bitcast_convert_type(row, F32)

    class Rem:
        def __init__(self, slot):
            self.marks, self.done, self.ready = [], {}, []
            for p in range(RV // 16):
                acc = None
                for k in range(kr):
                    sp, r8 = divmod(8 * p, HP // 2)
                    hb = pltpu.bitcast(hb_scr[slot * nhb + sp, k, r8:r8 + 8, :], BF16).astype(F32)
                    w = wb_scr[k]
                    t = _lanes(hb, gw) * jnp.concatenate([w, w], axis=0)
                    acc = t if acc is None else acc + t
                    if (k + 1) % KS == 0:
                        for c in range(0, gw, gw // KSPLIT):
                            self.marks.append(_fold(acc[:, c:c + gw // KSPLIT]))
                self.done[len(self.marks) - 1] = (p, acc)

        def take(self, phase, others=()):
            n, tot = len(self.marks), SHARES[-1]
            lo, hi = SHARES[phase] * n // tot, SHARES[phase + 1] * n // tot
            for i in range(lo, hi):
                if i in self.done:
                    self.ready.append((*self.done[i], phase, (i + 1 - lo) / (hi - lo)))
            mine = self.marks[lo:hi]
            return _merge(others, mine) if others and mine else list(others) + mine

        def flush(self, st, zero, phase, hi):
            old = [r for r in self.ready if r[2] < phase]
            for p, acc, ph, frac in self.ready:
                if ph < phase:
                    rl = 8 * (([r[0] for r in old].index(p) + 1) * 200 // (len(old) + 1))
                else:
                    rl = 16 * min(int(TLO + frac * (hi - TLO)) - 4, 118)
                tok = lax.bitcast_convert_type(st[rl:rl + 8, 0:LANES], U32)
                z = jnp.concatenate([_lanes(tok & zero, gw)] * 2, axis=0)
                rem_scr[16 * p:16 * p + 16, :] = lax.bitcast_convert_type(
                    lax.bitcast_convert_type(acc, U32) | z, F32)
            self.ready = []

    def qproj2(u, toks, zero):
        h = h_scr[blk_of(u) & 1]
        q = jnp.dot(h[RV:TB, dm:d], wq_v[grp_of(u), dm:d, :], preferred_element_type=F32)
        r = jnp.concatenate([rem_scr[...], q], axis=0)
        outs = []
        for i in range(nq):
            tk = toks[i * len(toks) // nq:(i + 1) * len(toks) // nq]
            hm = _tie_rows(h[:, 0:dm], tk, zero, 0, TB // 16)
            q = jnp.dot(hm, wq_v[grp_of(u), 0:dm, i * DH:(i + 1) * DH],
                        preferred_element_type=F32) + r[:, i * DH:(i + 1) * DH]
            outs.append(q.astype(BF16))
        return jnp.concatenate(outs, axis=1)

    def qproj(u, lo=0, hi=gw, parts=1):
        qs = []
        for r0 in range(0, TB, TB // parts):
            rs = slice(r0, r0 + TB // parts)
            if REMF:
                q = jnp.dot(h_scr[blk_of(u) & 1, rs, dm:d], wq_v[grp_of(u), dm:d, lo:hi],
                            preferred_element_type=F32)
                q = jnp.dot(h_scr[blk_of(u) & 1, rs, 0:dm], wq_v[grp_of(u), 0:dm, lo:hi],
                            preferred_element_type=F32) + q
            else:
                q = jnp.dot(h_scr[blk_of(u) & 1, rs, :], wq_v[grp_of(u), :, lo:hi],
                            preferred_element_type=F32)
            qs.append(q.astype(BF16))
        return jnp.concatenate(qs, axis=0)

    def qk(u, q, j, toks=(), zero=None, hi=THI):
        k = _tie_rows(k_v[grp_of(u) * HG + j // 2], toks, zero, TLO, hi)
        st = lax.dot_general(k, q[:, j * DH:(j + 1) * DH], _NT,
                             preferred_element_type=F32)
        for i in range(nb):
            blk = st[:, i * LANES:(i + 1) * LANES]
            st_scr[j * nb + i] = blk
            if DEFM:
                m_scr[j * nb + i] = jnp.max(blk.reshape(sk // 8, 8, LANES), axis=0)
            else:
                m_scr[j * nb + i, 0:1] = jnp.max(blk, axis=0, keepdims=True)
        return st

    def v_transpose(u, i, marks=None, rel=(), zero=None):
        v = _tie_rows(v_v[grp_of(u) * HG + i], rel, zero, -7, sk // 16 - 7)
        vt = pltpu.bitcast(v.T, U32)
        vt_scr[i] = vt
        if marks is not None:
            step = sk // NVT
            for c in range(step - LANES, sk, step):
                marks.append(vt[DH // 2 - 8:DH // 2, c:c + LANES])

    def pv(slots, zero, toks=(), srows=None):
        ps, ls, pairs = [], [], []
        for sl in slots:
            m = jnp.max(m_scr[sl], axis=0, keepdims=True) if DEFM else m_scr[sl, 0:1]
            p = jnp.exp2(st_scr[sl] - m)
            accs = [None] * 4
            for tile in range(nt):
                for r0 in range(tile * LANES + LANES - 16, tile * LANES - 16, -16):
                    pair = p[r0:r0 + 8] + p[r0 + 8:r0 + 16]
                    pairs.append(pair)
                    a = accs[tile % 4]
                    accs[tile % 4] = pair if a is None else a + pair
            ls.append(jnp.sum((accs[0] + accs[1]) + (accs[2] + accs[3]), axis=0, keepdims=True))
            ps.append(p.astype(BF16))
        outs = []
        ntiles = len(slots) * nt
        side = {}
        for i, tok in enumerate(toks):
            side.setdefault(max(((i + 1) * (ntiles - (EPVEND if srows else PVEND))) // len(toks) - 1, 0), []).append(tok)
        for i, sl in enumerate(slots):
            vu = vt_scr[sl // (2 * nb)]
            tiles = []
            for c in range(nt):
                g = i * nt + c + 4
                rows = []
                for r in range(8):
                    x = vu[8 * r:8 * r + 8, c * LANES:(c + 1) * LANES]
                    if g < ntiles and TIE0 <= r < TIE0 + NTIE:
                        src = pairs[g * 8 + (r - TIE0)]
                        x = _dep(x, lax.bitcast_convert_type(src, U32), zero)
                    if r == (srows or SROWS)[c % 4]:
                        for tok in side.get(i * nt + c, ()):
                            x = _dep(x, tok, zero)
                    rows.append(x)
                tiles.append(jnp.concatenate(rows, axis=0))
            lhs = pltpu.bitcast(jnp.concatenate(tiles, axis=1), BF16)
            o = jnp.dot(lhs, ps[i], preferred_element_type=F32)
            outs.append(o * (1.0 / ls[i]) if OF32 else (o * (1.0 / ls[i])).astype(BF16))
        return outs

    def outproj_tied(u, o, toks, zero):
        slot = blk_of(u) & 1
        res = []
        for i in range(nb):
            o2 = jnp.concatenate([o[j * nb + i] for j in range(nq)], axis=0).astype(BF16)
            tk = toks[i * len(toks) // OPN:(i + 1) * len(toks) // OPN]
            wo = _tie_rows(wot_v[grp_of(u)], tk, zero, 0, d // 16)
            contrib = jnp.dot(wo, o2, preferred_element_type=F32)
            acc_scr[slot * nb + i] += contrib
            res.append(contrib)
        return jnp.concatenate(res, axis=0)

    def outproj(u, o, lo=0):
        w = len(o) // nq
        o2 = jnp.concatenate(
            [jnp.concatenate(o[j * w:(j + 1) * w], axis=1) for j in range(nq)], axis=0).astype(BF16)
        contrib = jnp.dot(wot_v[grp_of(u)], o2, preferred_element_type=F32)
        slot = blk_of(u) & 1
        for i in range(w):
            pi = slot * nb + lo // LANES + i
            acc_scr[pi] += contrib[:, i * LANES:(i + 1) * LANES]

    def router_keys(racc, t0):
        r = _rb(jnp.sum(racc, axis=0, keepdims=True)) + 0.0
        bits = lax.bitcast_convert_type(r, I32) >> 16
        order = jnp.where(bits < 0, -1 - bits, bits + 32768)
        pos = t0 + lax.broadcasted_iota(I32, r.shape, 1)
        return lax.bitcast_convert_type((order << 11) + (seq - 1 - pos) + 0x20000000, F32)

    def finalize(t0, slot, a0, dst, n, keys_out=None):
        marks = []
        cs = _span(dst, n)
        x = x_cols(t0, n).astype(F32)
        att = jnp.concatenate(
            [acc_scr[slot * nb + a0 // LANES + i] for i in range(n // LANES)], axis=1)
        x1b = (x + _lanes(col_scr[0:d, :], n) * att).astype(BF16)
        x1_scr[:, cs] = x1b
        ot_v[:, cs] = x1b
        mu = _colsum(x1b.astype(F32), marks, NG1 if MID and (n == SP or (EFINE and keys_out is None)) else NF1) * (1.0 / d)
        fine = MID and (n == SP or (EFINE and keys_out is None))

        def note(row):
            if fine:
                marks.append(_fold(jnp.broadcast_to(row, (8, n))))
            return row

        mub = note(_rb(mu))
        xc = x1_scr[:, cs].astype(F32) - mub
        var = _colsum(xc * xc, marks, NG2 if fine else NF2) * (1.0 / d) - (mu - mub) * (mu - mub)
        inv = note(1.0 / note(_rb(jnp.sqrt(note(_rb(_rb(jnp.maximum(var, 0.0)) + EPS_BF16))))))
        step = d // (EF3 if fine and n != SP else NF3)
        racc = None
        for r0 in range(0, d, step):
            rs = slice(r0, r0 + step)
            x1 = ot_v[rs, cs].astype(F32)
            ln = _rb(_rb(x1 - mub) * inv)
            if fine:
                marks.append(_fold(ln))
            h2b = (_rb(ln * _lanes(col_scr[2 * d + r0:2 * d + r0 + step, :], n))
                   + _lanes(col_scr[d + r0:d + r0 + step, :], n)).astype(BF16)
            if keys_out is None:
                h2_scr[rs, cs] = h2b
            else:
                h2l_scr[rs, :] = h2b
            h2 = h2b.astype(F32)
            out = x1 + _lanes(col_scr[3 * d + r0:3 * d + r0 + step, :], n) * h2
            ot_v[rs, cs] = out.astype(BF16)
            rp = h2 * _lanes(col_scr[4 * d + r0:4 * d + r0 + step, :], n)
            for g in range(0, step, 8):
                racc = rp[g:g + 8] if racc is None else racc + rp[g:g + 8]
            marks.append(_fold(out, racc))
        if keys_out is not None:
            keys_out.append(racc)
            return marks
        key = router_keys(racc, t0)
        for i in range(n // LANES):
            key_scr[pl.ds(dst // LANES + i, 1), :] = key[:, i * LANES:(i + 1) * LANES]
        return marks

    hw = gw // 2
    wq0a = col_copy(wq_hbm, wq_v.at[0], 0, hw, grp_sems.at[0, 0])
    wq0b = col_copy(wq_hbm, wq_v.at[0], hw, gw, misc_sems.at[4])
    k0a = pltpu.make_async_copy(k_hbm.at[0], k_v.at[0], grp_sems.at[1, 0])
    k0b = pltpu.make_async_copy(k_hbm.at[1], k_v.at[1], misc_sems.at[5])
    v0 = pltpu.make_async_copy(v_hbm.at[0:HG], v_v.at[0:HG], grp_sems.at[2, 0])
    wq1, k1, v1, wo0 = grp_copies(1)
    wo_last = pltpu.make_async_copy(wot_hbm.at[:, (n_grp - 1) * gw:n_grp * gw],
                                    wot_v.at[n_grp - 1], grp_sems.at[3, 0])
    wrem_copy = col_copy(wq_hbm.at[dm:d], wrem_v, gw, 4 * gw, misc_sems.at[2])
    wrem_rest = (col_copy(wq_hbm.at[dm:d], wrem_v, 0, gw, misc_sems.at[11]),
                 col_copy(wq_hbm.at[dm:d], wrem_v, 4 * gw, n_grp * gw, misc_sems.at[12]))
    c_copy = pltpu.make_async_copy(c_hbm, c_ref, misc_sems.at[6])
    wr_copy = pltpu.make_async_copy(wr_hbm, wr_ref, misc_sems.at[7])
    c_copy.start()
    wr_copy.start()
    x_first.start()
    mod_first[0].start()
    mod_first[1].start()
    wq0a.start()
    wq0b.start()
    acc_scr[0:2 * nb] = jnp.zeros((2 * nb, d, LANES), F32)
    col_scr[0:4 * d, :] = jnp.zeros((4 * d, LANES), F32)
    wdt_v[ff // WP] = jnp.zeros((d, WP), BF16)
    with _scope("w_x"):
        c_copy.wait()
        wr_copy.wait()
        x_first.wait()
    cbits = lax.bitcast_convert_type(c_ref[:, 0:LANES].astype(F32), U32)
    zero_scr[...] = jnp.broadcast_to(cbits & 0xFFFF, (8, LANES))
    h_scr[0] = ln1_norm(0, TB, [])()
    sc = silu_c()
    wr = wr_ref[...].reshape(1, d).astype(F32)
    col_scr[4 * d:5 * d, :] = jnp.broadcast_to(wr, (LANES, d)).T
    col_scr[5 * d:6 * d, :] = jnp.broadcast_to(sc[0:1, :].astype(F32), (LANES, d)).T
    with _scope("w_wmod"):
        mod_first[0].wait()
    mod = _rb(jnp.dot(sc, wmod_v[:, MODC:2 * d], preferred_element_type=F32))
    mod_scr[0:1, MODC:d] = mod[0:1, 0:d - MODC] * qscale
    mod_scr[1:2, :] = _rb(1.0 + mod[0:1, d - MODC:2 * d - MODC]) * qscale
    with _scope("w_wmod2"):
        mod_first[1].wait()
    k0a.start(priority=KAP)
    if not LATEKV:
        k0b.start(priority=1)
        v0.start(priority=1)
    mod_scr[0:1, 0:MODC] = _rb(jnp.dot(sc, wmod_v[:, 0:MODC], preferred_element_type=F32))[0:1] * qscale
    if EARLYMOD:
        ln1_mod(h_scr[0], 0, 0, [])
    with _scope("w_wq"):
        wq0a.wait()
    if LATEKV:
        k0b.start(priority=1)
        v0.start(priority=1)
        wrem_copy.start(priority=1)
    if not EARLYMOD:
        ln1_mod(h_scr[0], 0, 0, [])
    qa = qproj(0, 0, hw, 2)
    with _scope("w_k"):
        wq0b.wait()
        k0a.wait()
    wq1.start(priority=1)
    k1.start(priority=1)
    x_second.start()
    q = jnp.concatenate([qa, qproj(0, hw, gw, 2)], axis=1)
    zero = zero_scr[...]
    for j in range(2):
        marks = []
        for i in range(2 * j, 2 * j + 2):
            hb_piece(0, i, marks)
        qk(0, q, j, marks, zero)
    with _scope("w_v"):
        k0b.wait()
        v0.wait()
        wrem_copy.wait()
    v1.start()
    wo0.start()
    with _scope("qk0"):
        zero = zero_scr[...]
        rem_scr[...] = jnp.dot(h_scr[0, 0:RV, dm:d], wrem_v[:, gw:2 * gw],
                               preferred_element_type=F32)
        for i in range(HG):
            marks = []
            v_transpose(0, i, marks)
            if i == 0:
                wb_piece(2, marks, zero)
            if 4 + i < nhb:
                hm = []
                hb_piece(0, 4 + i, hm)
                marks = _merge(marks, hm)
            qk(0, q, nq - HG + i, marks, zero)

    assert n_grp == 8 and HG == 2
    stage_at = [1, 2, 3, 5, n_units]
    starts = [(*grp_copies(2), mod_rest, x_rest, *wrem_rest), grp_copies(3, 3),
              (*grp_copies(6, 2), wo_last, mlp_d), (mlp_g, mlp_u)]
    waits = [(wq1, k1, v1, wo0, x_second), *starts[:3]]
    wd0 = stage_at[3]
    npc = TB // SP
    nmp = 4 * d // MP

    def manage(k, _, c):
        for cp in waits[k]:
            cp.wait()
        for cp in starts[k]:
            cp.start()
        return c

    def steady(u, carry):
        with _scope("body"):
            zero = zero_scr[...]
            blk, g = blk_of(u), grp_of(u)
            off = ((g - 1) & (npc - 1)) * SP
            rem = Rem(blk_of(u + 1) & 1)
            q = qproj2(u, rem.take(0), zero)
            o = pv(range(0, 2 * nb), zero, rem.take(1))
            live = jnp.logical_and(blk > 0, jnp.logical_and(g >= 1, g <= npc))
            t0 = jnp.maximum(blk - 1, 0) * TB + off
            marks = finalize(t0, (blk + 1) & 1, off, jnp.where(live, t0, seq), SP)
            wp = jnp.clip(u - wd0, 0, ff // WP - 1) * WP
            wmarks = []
            wd_piece(jnp.where(u >= wd0, wp, ff), wp, wmarks)
            rem.flush(qk(u, q, 0, rem.take(2, _merge(marks, wmarks)), zero), zero, 2, THI)
            def tok_at(res, row):
                return lax.bitcast_convert_type(res[row:row + 8, 0:LANES], U32)

            marks, mmarks = [], []
            ln_fin = ln1_norm(jnp.minimum(blk + 1, n_blk - 1) * TB + off, SP, marks)
            mp = jnp.clip(u - 2, 0, nmp - 1) * MP
            mod_fin = mod_piece(jnp.where(u >= 2, 2 * d + mp, 0), mp, mmarks)
            st = qk(u, q, 1, rem.take(3, marks + mmarks), zero)
            rem.flush(st, zero, 3, THI)
            used = jnp.where(live, ((blk + 1) & 1) * nb + off // LANES, 2 * nb)
            for r0 in range(0, d, 32):
                z4 = jnp.concatenate([tok_at(st, r0) & zero] * 4, axis=0)
                acc_scr[used, r0:r0 + 32, :] = lax.bitcast_convert_type(z4, F32)
            ln1_mod(ln_fin(tok_at(st, LNREL) & zero), (blk + 1) & 1, off, [])
            mod_fin(tok_at(st, 1880) & zero)
            o += pv(range(2 * nb, 4 * nb), zero, rem.take(4))
            st = qk(u, q, 2, rem.take(5), zero)
            rem.flush(st, zero, 5, THI)
            v_transpose(u, 0, None, [tok_at(st, 112 * i) for i in range(nt)], zero)
            st = qk(u, q, 3, rem.take(6), zero)
            rem.flush(st, zero, 6, THI)
            v_transpose(u, 1, None, [tok_at(st, 112 * i) for i in range(nt)], zero)
            res = outproj_tied(u - 1, o, rem.take(7), zero)
            rem.flush(res, zero, 7, OPN * d // 16)
            hm = []
            hb_piece((blk + 1) & 1, jnp.clip(g - 1, 0, nhb - 1), hm,
                     tok_at(res, max(OPN * d - 96, 0)) & zero)
            wb_piece(u + 2, hm, zero)
        return carry

    def stage(k, lo):
        hi = stage_at[1]
        for i in range(len(waits)):
            lax.fori_loop(0, jnp.where(k == i, 1, 0), functools.partial(manage, i), 0)
            hi = jnp.where(k == i, stage_at[i + 1], hi)
        lax.fori_loop(lo, hi, steady, 0)
        return hi

    lax.fori_loop(0, len(waits), stage, jnp.int32(stage_at[0]))

    ul = n_units - 1
    tl = seq - TB
    sl_last = (n_blk - 1) & 1
    nb0 = nb - TAILB
    with _scope("e_pva"):
        mod_scr[2:3, :] = row_scr[:, 3 * d:4 * d]
        outproj(ul, pv([j * nb + i for j in range(nq) for i in range(nb0)], zero_scr[...]))
    mlp_g.wait()
    mlp_u.wait()
    out_lo.start()
    with _scope("e_pvb"):
        toks = finalize(tl, sl_last, 0, tl, nb0 * LANES)
        o = pv([j * nb + i for j in range(nq) for i in range(nb0, nb)], zero_scr[...], toks, EROWS)
        outproj(ul, o, nb0 * LANES)

    nl = TAILB * LANES
    sub8 = lax.broadcasted_iota(I32, (TOPC, 1), 0)
    lane = lax.broadcasted_iota(I32, (TOPC, LANES), 1)

    def key_index(k):
        return seq - 1 - (lax.bitcast_convert_type(k, I32) & (seq - 1))

    def piece_base(idx, limit):
        return pl.multiple_of(jnp.clip(idx >> 7, 0, limit // LANES - 1) * LANES, LANES)

    keys = key_scr[0:seq // LANES, :]
    piece = lax.broadcasted_iota(I32, (seq // LANES, 1), 0)
    keys = jnp.where(piece < (seq - nl) // LANES, keys, 0.0)
    ecol = jnp.zeros((TOPC, LANES), F32)
    erow = jnp.zeros((1, LANES), F32)
    h2e = jnp.zeros((TOPC, d), F32)
    late = []
    marks = finalize(seq - nl, sl_last, TB - nl, seq - nl, nl, late)
    zero = zero_scr[...]
    pace = dict(zip([int(v) for v in os.environ.get("KP_PG", "2,4,5,6,7").split(",")],
                    [int(v) for v in os.environ.get("KP_PM", "8,14,18,23,27").split(",")]))
    for i in range(TOPC):
        mx = jnp.max(jnp.max(keys, axis=0, keepdims=True), axis=1, keepdims=True)
        keys = jnp.where(keys == mx, 0.0, keys)
        ecol = jnp.where(sub8 == i, mx, ecol)
        erow = jnp.where(lane[0:1] == i, mx, erow)
        idx = key_index(mx)
        pick = jnp.logical_and(sub8 == i, lane == (idx & (LANES - 1)))
        sl = pl.ds(piece_base(idx[0, 0], seq - nl), LANES)
        pick = jnp.where(pick, 1.0, 0.0)
        if i in pace:
            pick = lax.bitcast_convert_type(
                lax.bitcast_convert_type(pick, U32) | (marks[pace[i]] & zero), F32)
        h2e = h2e + lax.dot_general(pick.astype(BF16), h2_scr[:, sl], _NT,
                                    preferred_element_type=F32)

    late = [router_keys(late[0], seq - nl)]
    krow = jnp.concatenate([late[0], erow], axis=1)
    kcol = jnp.concatenate([jnp.broadcast_to(late[0], (LANES, nl)).T, ecol], axis=0)
    cnt = [None] * 4
    for g in range(kcol.shape[0] // 8):
        one = jnp.where(_lanes(kcol[8 * g:8 * g + 8], nl + LANES) > krow, 1.0, 0.0)
        cnt[g % 4] = one if cnt[g % 4] is None else cnt[g % 4] + one
    rank = jnp.sum((cnt[0] + cnt[1]) + (cnt[2] + cnt[3]), axis=0, keepdims=True)
    chosen = rank == sub8.astype(F32)
    onehot = jnp.where(chosen, 1.0, 0.0).astype(BF16)
    h2pad = jnp.concatenate([h2e, jnp.zeros((TOPC, d), F32)], axis=0).astype(BF16)
    h2s = (jnp.dot(onehot[:, nl:nl + 2 * TOPC], h2pad, preferred_element_type=F32)
           + lax.dot_general(onehot[:, 0:nl], h2l_scr[...], _NT,
                             preferred_element_type=F32))
    top = jnp.max(jnp.where(chosen, krow, 0.0), axis=1, keepdims=True)
    idx_col = key_index(top)
    idxs = [idx_col[i:i + 1] for i in range(TOPC)]
    bases = [piece_base(idx_col[i, 0], seq) for i in range(TOPC)]
    hit = lane == (idx_col & (LANES - 1))
    picks = [jnp.where(jnp.logical_and(sub8 == i, hit), 1.0, 0.0).astype(BF16)
             for i in range(TOPC)]
    order = (lax.bitcast_convert_type(top, I32) >> 11) & 0xFFFF
    rbits = jnp.where(order >= 32768, order - 32768, -1 - order) << 16
    gate = _rb(_sigmoid(lax.bitcast_convert_type(rbits, F32)))
    xs = h2s.astype(BF16)
    for cp in out_hi:
        cp.start()
    g = _rb(jnp.dot(xs, wg_v[...], preferred_element_type=F32))
    g = _rb(g * _rb(_sigmoid(g)))
    u = _rb(jnp.dot(xs, wu_v[...], preferred_element_type=F32))
    gu = (g * u).astype(BF16)

    last_use = []
    for i in range(TOPC):
        ok = True
        for j in range(i + 1, TOPC):
            ok = jnp.logical_and(ok, bases[i] != bases[j])
        last_use.append(ok)

    def down(r0, r1):
        x1p = jnp.concatenate([x1_scr[r0:r1, pl.ds(bases[i], LANES)] for i in range(TOPC)], axis=1)
        x1s = lax.dot_general(jnp.concatenate(picks, axis=1), x1p, _NT,
                              preferred_element_type=F32)
        wd = pltpu.bitcast(wd_scr[:, r0:r1], BF16)
        y = _rb(jnp.dot(gu, wd, preferred_element_type=F32))
        hm = _rb(h2s[:, r0:r1] + _rb(y * gate))
        return x1s + mod_scr[2:3, r0:r1] * hm

    def patch(r0, r1, new):
        n = r1 - r0
        pad = jnp.concatenate([new, jnp.zeros((LANES - TOPC, n), F32)], axis=0)
        cols = pltpu.bitcast(pad.T.astype(BF16), U32)
        col = [jnp.broadcast_to(cols[:, j:j + 1], (n // 2, LANES)) for j in range(TOPC)]
        for i in range(TOPC):
            res = pltpu.bitcast(ot_v[r0:r1, pl.ds(bases[i], LANES)], U32)
            tok = lane[0:1, :] + (idxs[i] & ~(LANES - 1))
            for j in range(i + 1):
                res = jnp.where(tok == idxs[j], col[j], res)
            fix_v[i, r0:r1, :] = pltpu.bitcast(res, BF16)

    def fix_copy(i, r0, r1):
        return pltpu.make_async_copy(fix_v.at[i, r0:r1, :],
                                     o_hbm.at[r0:r1, pl.ds(bases[i], LANES)], fix_sems.at[i])

    def for_last(fn):
        for i in range(TOPC - 1):
            pl.when(last_use[i])(functools.partial(fn, i))
        fn(TOPC - 1)

    new = down(*chunks[0])
    out_lo.wait()
    for ci, (r0, r1) in enumerate(chunks):
        out_hi[ci].wait()
        nxt = down(*chunks[ci + 1]) if ci + 1 < len(chunks) else None
        patch(r0, r1, new)
        for_last(lambda i: fix_copy(i, r0, r1).start())
        new = nxt
    with _scope("w_fix"):
        for r0, r1 in chunks:
            for_last(lambda i: fix_copy(i, r0, r1).wait())


@jax.jit
def pallas_adaLN_cond__gqa_block_cached__moe_arch_mod__prompt_kernel(
    A_x: jax.Array,
    A_k_cache: jax.Array,
    A_v_cache: jax.Array,
    A_wq: jax.Array,
    A_wo: jax.Array,
    B_x: jax.Array,
    B_w_r: jax.Array,
    B_w_gate: jax.Array,
    B_w_up: jax.Array,
    B_w_down: jax.Array,
    c: jax.Array,
    w_mod: jax.Array,
):
    b, seq, d = A_x.shape
    _, hkv, sk, dh = A_k_cache.shape
    assert b == 1 and dh == DH and HQ == 2 * hkv
    assert seq & (seq - 1) == 0 and seq <= 2048
    f = B_w_gate.shape[1]
    n_grp = hkv // HG
    gw = 2 * HG * dh
    n_slots = 2 * HG * TB // LANES

    xt = A_x.reshape(seq, d).T
    wot = A_wo.T
    wdt = B_w_down.T
    k3 = A_k_cache.reshape(hkv, sk, dh)
    v3 = A_v_cache.reshape(hkv, sk, dh)

    hbm = pl.BlockSpec(memory_space=pl.ANY)
    out_t = pl.pallas_call(
        functools.partial(_kernel, n_heads=hkv),
        in_specs=[hbm] * 11,
        out_specs=hbm,
        out_shape=jax.ShapeDtypeStruct((d, seq), BF16),
        scratch_shapes=[
            pltpu.VMEM((seq // LANES, d, LANES), BF16),
            pltpu.VMEM((hkv, sk, dh), BF16),
            pltpu.VMEM((hkv, sk, dh), BF16),
            pltpu.VMEM((n_grp, d, gw), BF16),
            pltpu.VMEM((n_grp, d, gw), BF16),
            pltpu.VMEM((d, 6 * d), BF16),
            pltpu.VMEM((d, f), BF16),
            pltpu.VMEM((d, f), BF16),
            pltpu.VMEM((f // WP + 1, d, WP), BF16),
            pltpu.VMEM((d, seq + SP), BF16),
            pltpu.VMEM((2, TB, d), BF16),
            pltpu.VMEM((2 * TB // LANES + 1, d, LANES), F32),
            pltpu.VMEM((n_slots, sk, LANES), F32),
            pltpu.VMEM((n_slots, 8, LANES), F32),
            pltpu.VMEM((HG, dh // 2, sk), U32),
            pltpu.VMEM((8, d), F32),
            pltpu.VMEM((6 * d, LANES), F32),
            pltpu.VMEM(((seq + SP) // LANES + 7 & ~7, LANES), F32),
            pltpu.VMEM((d, seq + SP), BF16),
            pltpu.VMEM((d, seq + SP), BF16),
            pltpu.VMEM((8, LANES), U32),
            pltpu.VMEM((TOPC, d, LANES), BF16),
            pltpu.VMEM((1, d), BF16),
            pltpu.VMEM((d,), BF16),
            pltpu.VMEM((1, 4 * d), F32),
            pltpu.VMEM((f // 2, d), U32),
            pltpu.VMEM((d, TAILB * LANES), BF16),
            pltpu.VMEM((2 * -(-RV // HP), d % LANES, HP // 2, LANES), U32),
            pltpu.VMEM((d % LANES, 8, gw), F32),
            pltpu.VMEM((RV, gw), F32),
            pltpu.VMEM((d % LANES, n_grp * gw), BF16),
            pltpu.SemaphoreType.DMA((4, n_grp)),
            pltpu.SemaphoreType.DMA((13,)),
            pltpu.SemaphoreType.DMA((3,)),
            pltpu.SemaphoreType.DMA((len(EDGES),)),
            pltpu.SemaphoreType.DMA((TOPC,)),
        ],
        compiler_params=pltpu.CompilerParams(
            disable_bounds_checks=True,
            disable_semaphore_checks=True,
            vmem_limit_bytes=120 * 1024 * 1024,
        ),
    )(xt, k3, v3, A_wq, wot, B_w_r, B_w_gate, B_w_up, wdt, c, w_mod)
    return out_t.T.reshape(b, seq, d)
```

```python
import contextlib
import functools
import math
import os

import jax
import jax.numpy as jnp
from jax import lax
import jax.experimental.pallas as pl
import jax.experimental.pallas.tpu as pltpu

F32 = jnp.float32
BF16 = jnp.bfloat16
I32 = jnp.int32
U32 = jnp.uint32

HQ = 32
DH = 128
TOPC = 8
EPS = 1e-05
EPS_BF16 = 1.0013580322265625e-05
LANES = 128

TB = 512
HG = 2
TIE0 = int(os.environ.get("KP_TIE0", "2"))
NTIE = int(os.environ.get("KP_NTIE", "3"))
SP = int(os.environ.get("KP_SP", "128"))
NM1 = int(os.environ.get("KP_NM1", "8"))
NM2 = int(os.environ.get("KP_NM2", "18"))
NM3 = int(os.environ.get("KP_NM3", "16"))
TLO = int(os.environ.get("KP_TLO", "3"))
NF1 = int(os.environ.get("KP_NF1", "9"))
NF2 = int(os.environ.get("KP_NF2", "6"))
NF3 = int(os.environ.get("KP_NF3", "18"))
NVT = int(os.environ.get("KP_NVT", "16"))
TAILB = int(os.environ.get("KP_TAILB", "2"))
SROWS = [int(v) for v in os.environ.get("KP_SROWS", "0,1,2,5").split(",")]
EROWS = [int(v) for v in os.environ.get("KP_EROWS", "0,4,6,7").split(",")]
EDGES = [int(e) for e in os.environ.get("KP_EDGES", "0,128,256,384,512,576").split(",")]
MODC = int(os.environ.get("KP_MODC", "384"))
MP = int(os.environ.get("KP_MP", "384"))
NMP = int(os.environ.get("KP_NMP", "24"))
WP = 256
REMF = int(os.environ.get("KP_REMF", "1"))
DEFM = int(os.environ.get("KP_DEFM", "1"))
KAP = int(os.environ.get("KP_KAP", "0"))
LATEKV = int(os.environ.get("KP_LATEKV", "1"))
EARLYMOD = int(os.environ.get("KP_EARLYMOD", "0"))
RV = int(os.environ.get("KP_RV", "448"))
HP = int(os.environ.get("KP_HP", "80"))
KS = int(os.environ.get("KP_KS", "4"))
KSPLIT = int(os.environ.get("KP_KSPLIT", "2"))
HS = int(os.environ.get("KP_HS", "2"))
THI = int(os.environ.get("KP_THI", "126"))
OPN = int(os.environ.get("KP_OPN", "2"))
LNREL = int(os.environ.get("KP_LNREL", "1008"))
_sh = [int(v) for v in os.environ.get("KP_SH", "29,28,15,23,26,30,33,18").split(",")]
SHARES = [sum(_sh[:i]) for i in range(len(_sh) + 1)]
MID = int(os.environ.get("KP_MID", "1"))
NG1 = int(os.environ.get("KP_NG1", "18"))
NG2 = int(os.environ.get("KP_NG2", "9"))
EFINE = int(os.environ.get("KP_EFINE", "1"))
EF3 = int(os.environ.get("KP_EF3", "36"))
PVEND = int(os.environ.get("KP_PVEND", "12"))
EPVEND = int(os.environ.get("KP_EPVEND", "24"))
SEL = int(os.environ.get("KP_SEL", "1"))
OF32 = int(os.environ.get("KP_OF32", "1"))
SCOPES = os.environ.get("KP_SCOPES", "") == "1"

_NT = (((1,), (1,)), ((), ()))


def _rb(x):
    return x.astype(BF16).astype(F32)


def _sigmoid(x):
    return 1.0 / (1.0 + jnp.exp(-x))


def _lanes(col, width):
    reps = width // LANES
    return col if reps == 1 else jnp.concatenate([col] * reps, axis=1)


def _fold(*xs):
    ts = []
    for x in xs:
        xi = lax.bitcast_convert_type(x, U32)
        ts += [xi[r:r + 8, c:c + LANES] for r in range(0, x.shape[0], 8)
               for c in range(0, x.shape[1] - LANES + 1, LANES)]
    if len(ts) > 5:
        return functools.reduce(lambda a, b: a | b, ts[:-2]) | (ts[-2] | ts[-1])
    while len(ts) > 1:
        ts = [a | b for a, b in zip(ts[0::2], ts[1::2])] + ts[len(ts) & ~1:]
    return ts[0]


def _colsum(x, marks, nmarks):
    n = x.shape[0] // 8
    acc = x[0:8]
    for g in range(1, n):
        acc = acc + x[8 * g:8 * g + 8]
        if ((g + 1) * nmarks) % n == 0:
            marks.append(_fold(acc))
    return jnp.sum(acc, axis=0, keepdims=True)


def _dep(x, tok, zero):
    if SEL:
        return jnp.where(zero != 0, tok, x)
    return x | (tok & zero)


def _tie_rows(lhs, toks, zero, lo, hi, c0=0):
    if not toks:
        return lhs
    lu = pltpu.bitcast(lhs, U32)
    rows = [lu[8 * r:8 * r + 8] for r in range(lu.shape[0] // 8)]
    for i, tok in enumerate(toks):
        r = lo + ((i + 1) * (hi - lo)) // len(toks) - 1
        head = _dep(rows[r][:, c0:c0 + LANES], tok, zero)
        rows[r] = head if lu.shape[1] == LANES else jnp.concatenate(
            [head, rows[r][:, LANES:]], axis=1)
    return pltpu.bitcast(jnp.concatenate(rows, axis=0), BF16)


def _merge(a, b):
    keyed = [((i + 1) / len(a), t) for i, t in enumerate(a)]
    keyed += [((i + 1) / len(b), t) for i, t in enumerate(b)]
    return [t for _, t in sorted(keyed, key=lambda kv: kv[0])]


def _span(start, size):
    if isinstance(start, int):
        return pl.ds(start, size)
    return pl.ds(pl.multiple_of(start, LANES), size)


def _scope(name):
    return jax.named_scope(name) if SCOPES else contextlib.nullcontext()


def _kernel(xt_hbm, k_hbm, v_hbm, wq_hbm, wot_hbm, wr_hbm, wg_hbm, wu_hbm, wdt_hbm,
            c_hbm, wmod_hbm, o_hbm,
            xt_v, k_v, v_v, wq_v, wot_v, wmod_v, wg_v, wu_v, wdt_v, ot_v,
            h_scr, acc_scr, st_scr, m_scr, vt_scr, mod_scr, col_scr, key_scr, h2_scr, x1_scr,
            zero_scr, fix_v, c_ref, wr_ref, row_scr, wd_scr, h2l_scr, hb_scr, wb_scr, rem_scr, wrem_v,
            grp_sems, misc_sems, mlp_sems, out_sems, fix_sems,
            *, n_heads):
    d, seq = xt_hbm.shape
    sk = k_v.shape[1]
    n_grp = n_heads // HG
    n_blk = seq // TB
    n_units = n_grp * n_blk
    nb = TB // LANES
    nq = 2 * HG
    nt = sk // LANES
    gbits = n_grp.bit_length() - 1
    gw = nq * DH
    qscale = (DH ** -0.5) * math.log2(math.e)

    def grp_of(u):
        return u & (n_grp - 1)

    def blk_of(u):
        return u >> gbits

    def grp_copies(g, n=1):
        hs = pl.ds(g * HG, n * HG)
        return (*[pltpu.make_async_copy(wq_hbm.at[:, pl.ds(i * gw, gw)], wq_v.at[i],
                                        grp_sems.at[0, i]) for i in range(g, g + n)],
                pltpu.make_async_copy(k_hbm.at[hs], k_v.at[hs], grp_sems.at[1, g]),
                pltpu.make_async_copy(v_hbm.at[hs], v_v.at[hs], grp_sems.at[2, g]),
                *[pltpu.make_async_copy(wot_hbm.at[:, pl.ds((i - 1) * gw, gw)], wot_v.at[i - 1],
                                        grp_sems.at[3, i]) for i in range(g, g + n)])

    def col_copy(src, dst, lo, hi, sem):
        return pltpu.make_async_copy(src.at[:, lo:hi], dst.at[:, lo:hi], sem)

    class Pieces:
        def __init__(self, src, dst, lo, hi, sem):
            self.src, self.dst, self.lo, self.hi, self.sem = src, dst, lo, hi, sem

        def start(self, priority=0):
            w = self.dst.shape[2]
            for p in range(self.lo, self.hi):
                pltpu.make_async_copy(self.src.at[:, p * w:(p + 1) * w], self.dst.at[p],
                                      self.sem).start(priority=priority)

        def wait(self):
            whole = self.dst.at[self.lo:self.hi]
            pltpu.make_async_copy(whole, whole, self.sem).wait()

    def x_cols(t0, n):
        return jnp.concatenate([xt_v[t0 // LANES + i] for i in range(n // LANES)], axis=1)

    x_first = Pieces(xt_hbm, xt_v, 0, nb, misc_sems.at[0])
    x_second = Pieces(xt_hbm, xt_v, nb, nb + 1, misc_sems.at[10])
    x_rest = Pieces(xt_hbm, xt_v, nb + 1, seq // LANES, misc_sems.at[1])
    mod_first = [col_copy(wmod_hbm, wmod_v, MODC, 2 * d, misc_sems.at[8]),
                 col_copy(wmod_hbm, wmod_v, 0, MODC, misc_sems.at[9])]
    mod_rest = col_copy(wmod_hbm, wmod_v, 2 * d, 6 * d, misc_sems.at[3])
    mlp_g = pltpu.make_async_copy(wg_hbm, wg_v, mlp_sems.at[0])
    mlp_u = pltpu.make_async_copy(wu_hbm, wu_v, mlp_sems.at[1])
    ff = wdt_hbm.shape[1]
    mlp_d = Pieces(wdt_hbm, wdt_v, 0, ff // WP, mlp_sems.at[2])
    out_lo = col_copy(ot_v, o_hbm, 0, seq - TB, out_sems.at[0])
    chunks = list(zip(EDGES[:-1], EDGES[1:]))
    out_hi = [pltpu.make_async_copy(ot_v.at[r0:r1, seq - TB:seq], o_hbm.at[r0:r1, seq - TB:seq],
                                    out_sems.at[1 + i]) for i, (r0, r1) in enumerate(chunks)]

    def silu_c():
        cc = c_ref[...].astype(F32)
        return jnp.broadcast_to((cc * _rb(_sigmoid(cc))).astype(BF16), (8, d))

    def ln1_norm(t0, n, marks):
        x = x_cols(t0, n).astype(F32)
        mu = _colsum(x, marks, NM1) * (1.0 / d)
        marks.append(_fold(jnp.broadcast_to(mu, (8, n))))
        xc = x - mu
        var = _colsum(xc * xc, marks, NM2) * (1.0 / d)
        rs = lax.rsqrt(var + EPS)

        def finish(z=None):
            r = rs if z is None else lax.bitcast_convert_type(
                lax.bitcast_convert_type(rs, U32) | _lanes(z[0:1], n), F32)
            return (xc * r).astype(BF16).T
        return finish

    def ln1_mod(ln, slot, r0, marks):
        n = ln.shape[0]
        h = ln.astype(F32) * mod_scr[1:2, :] + mod_scr[0:1, :]
        h_scr[slot, _span(r0, n), :] = h.astype(BF16)
        step = max(n // NM3, 8)
        for r in range(step - 8, n, step):
            marks.append(_fold(h[r:r + 8]))

    def mod_piece(src, dst, marks):
        w = wmod_v[:, _span(src, MP)].astype(F32)
        row0 = _rb(_colsum(w * _lanes(col_scr[5 * d:6 * d, :], MP), marks, NMP))

        def finish(z):
            row = lax.bitcast_convert_type(
                lax.bitcast_convert_type(row0, U32) | _lanes(z[0:1], MP), F32)
            pos = dst + lax.broadcasted_iota(I32, (1, MP), 1)
            is_cb = jnp.logical_and(pos >= 2 * d, pos < 3 * d)
            row = jnp.where(is_cb, _rb(1.0 + row), row)
            row_scr[:, _span(dst, MP)] = row
            col_scr[_span(dst, MP), :] = jnp.broadcast_to(row, (LANES, MP)).T
        return finish

    def wd_piece(src, dst, marks):
        w = pltpu.bitcast(wdt_v[src // WP].T, U32)
        wd_scr[pl.ds(pl.multiple_of(dst // 2, WP // 2), WP // 2), :] = w
        for r in range(56, WP // 2, 64):
            for c in range(0, d - LANES + 1, LANES):
                marks.append(w[r:r + 8, c:c + LANES])

    dm = d - d % LANES
    kr = d - dm
    nhb = -(-RV // HP)
    assert nhb <= 6 and nhb * HP <= TB

    def hb_piece(slot, sp, marks, z=None):
        r0 = sp * HP
        src = pl.ds(r0 if isinstance(r0, int) else pl.multiple_of(r0, 16), HP)
        hu = pltpu.bitcast(h_scr[slot, src, dm:d], U32)
        if z is not None:
            hu = hu | jnp.concatenate([z[:, 0:kr]] * (HP // 16), axis=0)
        for k in range(kr):
            col = jnp.broadcast_to(hu[:, k:k + 1], (HP // 2, LANES))
            hb_scr[slot * nhb + sp, k] = col
            if (k + 1) % HS == 0:
                marks.append(col[HP // 2 - 8:HP // 2])

    def wb_piece(u, toks, zero):
        w = lax.bitcast_convert_type(wrem_v[:, _span(grp_of(u) * gw, gw)].astype(F32), U32)
        for k in range(kr):
            row = jnp.broadcast_to(w[k:k + 1], (8, gw))
            row = row | _lanes(toks[k * len(toks) // kr] & zero, gw)
            wb_scr[k] = lax.bitcast_convert_type(row, F32)

    class Rem:
        def __init__(self, slot):
            self.marks, self.done, self.ready = [], {}, []
            for p in range(RV // 16):
                acc = None
                for k in range(kr):
                    sp, r8 = divmod(8 * p, HP // 2)
                    hb = pltpu.bitcast(hb_scr[slot * nhb + sp, k, r8:r8 + 8, :], BF16).astype(F32)
                    w = wb_scr[k]
                    t = _lanes(hb, gw) * jnp.concatenate([w, w], axis=0)
                    acc = t if acc is None else acc + t
                    if (k + 1) % KS == 0:
                        for c in range(0, gw, gw // KSPLIT):
                            self.marks.append(_fold(acc[:, c:c + gw // KSPLIT]))
                self.done[len(self.marks) - 1] = (p, acc)

        def take(self, phase, others=()):
            n, tot = len(self.marks), SHARES[-1]
            lo, hi = SHARES[phase] * n // tot, SHARES[phase + 1] * n // tot
            for i in range(lo, hi):
                if i in self.done:
                    self.ready.append((*self.done[i], phase, (i + 1 - lo) / (hi - lo)))
            mine = self.marks[lo:hi]
            return _merge(others, mine) if others and mine else list(others) + mine

        def flush(self, st, zero, phase, hi):
            old = [r for r in self.ready if r[2] < phase]
            for p, acc, ph, frac in self.ready:
                if ph < phase:
                    rl = 8 * (([r[0] for r in old].index(p) + 1) * 200 // (len(old) + 1))
                else:
                    rl = 16 * min(int(TLO + frac * (hi - TLO)) - 4, 118)
                tok = lax.bitcast_convert_type(st[rl:rl + 8, 0:LANES], U32)
                z = jnp.concatenate([_lanes(tok & zero, gw)] * 2, axis=0)
                rem_scr[16 * p:16 * p + 16, :] = lax.bitcast_convert_type(
                    lax.bitcast_convert_type(acc, U32) | z, F32)
            self.ready = []

    def qproj2(u, toks, zero):
        h = h_scr[blk_of(u) & 1]
        q = jnp.dot(h[RV:TB, dm:d], wq_v[grp_of(u), dm:d, :], preferred_element_type=F32)
        r = jnp.concatenate([rem_scr[...], q], axis=0)
        outs = []
        for i in range(nq):
            tk = toks[i * len(toks) // nq:(i + 1) * len(toks) // nq]
            hm = _tie_rows(h[:, 0:dm], tk, zero, 0, TB // 16)
            q = jnp.dot(hm, wq_v[grp_of(u), 0:dm, i * DH:(i + 1) * DH],
                        preferred_element_type=F32) + r[:, i * DH:(i + 1) * DH]
            outs.append(q.astype(BF16))
        return jnp.concatenate(outs, axis=1)

    def qproj(u, lo=0, hi=gw, parts=1):
        qs = []
        for r0 in range(0, TB, TB // parts):
            rs = slice(r0, r0 + TB // parts)
            if REMF:
                q = jnp.dot(h_scr[blk_of(u) & 1, rs, dm:d], wq_v[grp_of(u), dm:d, lo:hi],
                            preferred_element_type=F32)
                q = jnp.dot(h_scr[blk_of(u) & 1, rs, 0:dm], wq_v[grp_of(u), 0:dm, lo:hi],
                            preferred_element_type=F32) + q
            else:
                q = jnp.dot(h_scr[blk_of(u) & 1, rs, :], wq_v[grp_of(u), :, lo:hi],
                            preferred_element_type=F32)
            qs.append(q.astype(BF16))
        return jnp.concatenate(qs, axis=0)

    def qk(u, q, j, toks=(), zero=None, hi=THI):
        k = _tie_rows(k_v[grp_of(u) * HG + j // 2], toks, zero, TLO, hi)
        st = lax.dot_general(k, q[:, j * DH:(j + 1) * DH], _NT,
                             preferred_element_type=F32)
        for i in range(nb):
            blk = st[:, i * LANES:(i + 1) * LANES]
            st_scr[j * nb + i] = blk
            if DEFM:
                m_scr[j * nb + i] = jnp.max(blk.reshape(sk // 8, 8, LANES), axis=0)
            else:
                m_scr[j * nb + i, 0:1] = jnp.max(blk, axis=0, keepdims=True)
        return st

    def v_transpose(u, i, marks=None, rel=(), zero=None):
        v = _tie_rows(v_v[grp_of(u) * HG + i], rel, zero, -7, sk // 16 - 7)
        vt = pltpu.bitcast(v.T, U32)
        vt_scr[i] = vt
        if marks is not None:
            step = sk // NVT
            for c in range(step - LANES, sk, step):
                marks.append(vt[DH // 2 - 8:DH // 2, c:c + LANES])

    def pv(slots, zero, toks=(), srows=None):
        ps, ls, pairs = [], [], []
        for sl in slots:
            m = jnp.max(m_scr[sl], axis=0, keepdims=True) if DEFM else m_scr[sl, 0:1]
            p = jnp.exp2(st_scr[sl] - m)
            accs = [None] * 4
            for tile in range(nt):
                for r0 in range(tile * LANES + LANES - 16, tile * LANES - 16, -16):
                    pair = p[r0:r0 + 8] + p[r0 + 8:r0 + 16]
                    pairs.append(pair)
                    a = accs[tile % 4]
                    accs[tile % 4] = pair if a is None else a + pair
            ls.append(jnp.sum((accs[0] + accs[1]) + (accs[2] + accs[3]), axis=0, keepdims=True))
            ps.append(p.astype(BF16))
        outs = []
        ntiles = len(slots) * nt
        side = {}
        for i, tok in enumerate(toks):
            side.setdefault(max(((i + 1) * (ntiles - (EPVEND if srows else PVEND))) // len(toks) - 1, 0), []).append(tok)
        for i, sl in enumerate(slots):
            vu = vt_scr[sl // (2 * nb)]
            tiles = []
            for c in range(nt):
                g = i * nt + c + 4
                rows = []
                for r in range(8):
                    x = vu[8 * r:8 * r + 8, c * LANES:(c + 1) * LANES]
                    if g < ntiles and TIE0 <= r < TIE0 + NTIE:
                        src = pairs[g * 8 + (r - TIE0)]
                        x = _dep(x, lax.bitcast_convert_type(src, U32), zero)
                    if r == (srows or SROWS)[c % 4]:
                        for tok in side.get(i * nt + c, ()):
                            x = _dep(x, tok, zero)
                    rows.append(x)
                tiles.append(jnp.concatenate(rows, axis=0))
            lhs = pltpu.bitcast(jnp.concatenate(tiles, axis=1), BF16)
            o = jnp.dot(lhs, ps[i], preferred_element_type=F32)
            outs.append(o * (1.0 / ls[i]) if OF32 else (o * (1.0 / ls[i])).astype(BF16))
        return outs

    def outproj_tied(u, o, toks, zero):
        slot = blk_of(u) & 1
        res = []
        for i in range(nb):
            o2 = jnp.concatenate([o[j * nb + i] for j in range(nq)], axis=0).astype(BF16)
            tk = toks[i * len(toks) // OPN:(i + 1) * len(toks) // OPN]
            wo = _tie_rows(wot_v[grp_of(u)], tk, zero, 0, d // 16)
            contrib = jnp.dot(wo, o2, preferred_element_type=F32)
            acc_scr[slot * nb + i] += contrib
            res.append(contrib)
        return jnp.concatenate(res, axis=0)

    def outproj(u, o, lo=0):
        w = len(o) // nq
        o2 = jnp.concatenate(
            [jnp.concatenate(o[j * w:(j + 1) * w], axis=1) for j in range(nq)], axis=0).astype(BF16)
        contrib = jnp.dot(wot_v[grp_of(u)], o2, preferred_element_type=F32)
        slot = blk_of(u) & 1
        for i in range(w):
            pi = slot * nb + lo // LANES + i
            acc_scr[pi] += contrib[:, i * LANES:(i + 1) * LANES]

    def router_keys(racc, t0):
        r = _rb(jnp.sum(racc, axis=0, keepdims=True)) + 0.0
        bits = lax.bitcast_convert_type(r, I32) >> 16
        order = jnp.where(bits < 0, -1 - bits, bits + 32768)
        pos = t0 + lax.broadcasted_iota(I32, r.shape, 1)
        return lax.bitcast_convert_type((order << 11) + (seq - 1 - pos) + 0x20000000, F32)

    def finalize(t0, slot, a0, dst, n, keys_out=None):
        marks = []
        cs = _span(dst, n)
        x = x_cols(t0, n).astype(F32)
        att = jnp.concatenate(
            [acc_scr[slot * nb + a0 // LANES + i] for i in range(n // LANES)], axis=1)
        x1b = (x + _lanes(col_scr[0:d, :], n) * att).astype(BF16)
        x1_scr[:, cs] = x1b
        ot_v[:, cs] = x1b
        mu = _colsum(x1b.astype(F32), marks, NG1 if MID and (n == SP or (EFINE and keys_out is None)) else NF1) * (1.0 / d)
        fine = MID and (n == SP or (EFINE and keys_out is None))

        def note(row):
            if fine:
                marks.append(_fold(jnp.broadcast_to(row, (8, n))))
            return row

        mub = note(_rb(mu))
        xc = x1_scr[:, cs].astype(F32) - mub
        var = _colsum(xc * xc, marks, NG2 if fine else NF2) * (1.0 / d) - (mu - mub) * (mu - mub)
        inv = note(1.0 / note(_rb(jnp.sqrt(note(_rb(_rb(jnp.maximum(var, 0.0)) + EPS_BF16))))))
        step = d // (EF3 if fine and n != SP else NF3)
        racc = None
        for r0 in range(0, d, step):
            rs = slice(r0, r0 + step)
            x1 = ot_v[rs, cs].astype(F32)
            ln = _rb(_rb(x1 - mub) * inv)
            if fine:
                marks.append(_fold(ln))
            h2b = (_rb(ln * _lanes(col_scr[2 * d + r0:2 * d + r0 + step, :], n))
                   + _lanes(col_scr[d + r0:d + r0 + step, :], n)).astype(BF16)
            if keys_out is None:
                h2_scr[rs, cs] = h2b
            else:
                h2l_scr[rs, :] = h2b
            h2 = h2b.astype(F32)
            out = x1 + _lanes(col_scr[3 * d + r0:3 * d + r0 + step, :], n) * h2
            ot_v[rs, cs] = out.astype(BF16)
            rp = h2 * _lanes(col_scr[4 * d + r0:4 * d + r0 + step, :], n)
            for g in range(0, step, 8):
                racc = rp[g:g + 8] if racc is None else racc + rp[g:g + 8]
            marks.append(_fold(out, racc))
        if keys_out is not None:
            keys_out.append(racc)
            return marks
        key = router_keys(racc, t0)
        for i in range(n // LANES):
            key_scr[pl.ds(dst // LANES + i, 1), :] = key[:, i * LANES:(i + 1) * LANES]
        return marks

    hw = gw // 2
    wq0a = col_copy(wq_hbm, wq_v.at[0], 0, hw, grp_sems.at[0, 0])
    wq0b = col_copy(wq_hbm, wq_v.at[0], hw, gw, misc_sems.at[4])
    k0a = pltpu.make_async_copy(k_hbm.at[0], k_v.at[0], grp_sems.at[1, 0])
    k0b = pltpu.make_async_copy(k_hbm.at[1], k_v.at[1], misc_sems.at[5])
    v0 = pltpu.make_async_copy(v_hbm.at[0:HG], v_v.at[0:HG], grp_sems.at[2, 0])
    wq1, k1, v1, wo0 = grp_copies(1)
    wo_last = pltpu.make_async_copy(wot_hbm.at[:, (n_grp - 1) * gw:n_grp * gw],
                                    wot_v.at[n_grp - 1], grp_sems.at[3, 0])
    wrem_copy = col_copy(wq_hbm.at[dm:d], wrem_v, gw, 4 * gw, misc_sems.at[2])
    wrem_rest = (col_copy(wq_hbm.at[dm:d], wrem_v, 0, gw, misc_sems.at[11]),
                 col_copy(wq_hbm.at[dm:d], wrem_v, 4 * gw, n_grp * gw, misc_sems.at[12]))
    c_copy = pltpu.make_async_copy(c_hbm, c_ref, misc_sems.at[6])
    wr_copy = pltpu.make_async_copy(wr_hbm, wr_ref, misc_sems.at[7])
    c_copy.start()
    wr_copy.start()
    x_first.start()
    mod_first[0].start()
    mod_first[1].start()
    wq0a.start()
    wq0b.start()
    acc_scr[0:2 * nb] = jnp.zeros((2 * nb, d, LANES), F32)
    col_scr[0:4 * d, :] = jnp.zeros((4 * d, LANES), F32)
    wdt_v[ff // WP] = jnp.zeros((d, WP), BF16)
    with _scope("w_x"):
        c_copy.wait()
        wr_copy.wait()
        x_first.wait()
    cbits = lax.bitcast_convert_type(c_ref[:, 0:LANES].astype(F32), U32)
    zero_scr[...] = jnp.broadcast_to(cbits & 0xFFFF, (8, LANES))
    h_scr[0] = ln1_norm(0, TB, [])()
    sc = silu_c()
    wr = wr_ref[...].reshape(1, d).astype(F32)
    col_scr[4 * d:5 * d, :] = jnp.broadcast_to(wr, (LANES, d)).T
    col_scr[5 * d:6 * d, :] = jnp.broadcast_to(sc[0:1, :].astype(F32), (LANES, d)).T
    with _scope("w_wmod"):
        mod_first[0].wait()
    mod = _rb(jnp.dot(sc, wmod_v[:, MODC:2 * d], preferred_element_type=F32))
    mod_scr[0:1, MODC:d] = mod[0:1, 0:d - MODC] * qscale
    mod_scr[1:2, :] = _rb(1.0 + mod[0:1, d - MODC:2 * d - MODC]) * qscale
    with _scope("w_wmod2"):
        mod_first[1].wait()
    k0a.start(priority=KAP)
    if not LATEKV:
        k0b.start(priority=1)
        v0.start(priority=1)
    mod_scr[0:1, 0:MODC] = _rb(jnp.dot(sc, wmod_v[:, 0:MODC], preferred_element_type=F32))[0:1] * qscale
    if EARLYMOD:
        ln1_mod(h_scr[0], 0, 0, [])
    with _scope("w_wq"):
        wq0a.wait()
    if LATEKV:
        k0b.start(priority=1)
        v0.start(priority=1)
        wrem_copy.start(priority=1)
    if not EARLYMOD:
        ln1_mod(h_scr[0], 0, 0, [])
    qa = qproj(0, 0, hw, 2)
    with _scope("w_k"):
        wq0b.wait()
        k0a.wait()
    wq1.start(priority=1)
    k1.start(priority=1)
    x_second.start()
    q = jnp.concatenate([qa, qproj(0, hw, gw, 2)], axis=1)
    zero = zero_scr[...]
    for j in range(2):
        marks = []
        for i in range(2 * j, 2 * j + 2):
            hb_piece(0, i, marks)
        qk(0, q, j, marks, zero)
    with _scope("w_v"):
        k0b.wait()
        v0.wait()
        wrem_copy.wait()
    v1.start()
    wo0.start()
    with _scope("qk0"):
        zero = zero_scr[...]
        rem_scr[...] = jnp.dot(h_scr[0, 0:RV, dm:d], wrem_v[:, gw:2 * gw],
                               preferred_element_type=F32)
        for i in range(HG):
            marks = []
            v_transpose(0, i, marks)
            if i == 0:
                wb_piece(2, marks, zero)
            if 4 + i < nhb:
                hm = []
                hb_piece(0, 4 + i, hm)
                marks = _merge(marks, hm)
            qk(0, q, nq - HG + i, marks, zero)

    assert n_grp == 8 and HG == 2
    stage_at = [1, 2, 3, 5, n_units]
    starts = [(*grp_copies(2), mod_rest, x_rest, *wrem_rest), grp_copies(3, 3),
              (*grp_copies(6, 2), wo_last, mlp_d), (mlp_g, mlp_u)]
    waits = [(wq1, k1, v1, wo0, x_second), *starts[:3]]
    wd0 = stage_at[3]
    npc = TB // SP
    nmp = 4 * d // MP

    def manage(k, _, c):
        for cp in waits[k]:
            cp.wait()
        for cp in starts[k]:
            cp.start()
        return c

    def steady(u, carry):
        with _scope("body"):
            zero = zero_scr[...]
            blk, g = blk_of(u), grp_of(u)
            off = ((g - 1) & (npc - 1)) * SP
            rem = Rem(blk_of(u + 1) & 1)
            q = qproj2(u, rem.take(0), zero)
            o = pv(range(0, 2 * nb), zero, rem.take(1))
            live = jnp.logical_and(blk > 0, jnp.logical_and(g >= 1, g <= npc))
            t0 = jnp.maximum(blk - 1, 0) * TB + off
            marks = finalize(t0, (blk + 1) & 1, off, jnp.where(live, t0, seq), SP)
            wp = jnp.clip(u - wd0, 0, ff // WP - 1) * WP
            wmarks = []
            wd_piece(jnp.where(u >= wd0, wp, ff), wp, wmarks)
            rem.flush(qk(u, q, 0, rem.take(2, _merge(marks, wmarks)), zero), zero, 2, THI)
            def tok_at(res, row):
                return lax.bitcast_convert_type(res[row:row + 8, 0:LANES], U32)

            marks, mmarks = [], []
            ln_fin = ln1_norm(jnp.minimum(blk + 1, n_blk - 1) * TB + off, SP, marks)
            mp = jnp.clip(u - 2, 0, nmp - 1) * MP
            mod_fin = mod_piece(jnp.where(u >= 2, 2 * d + mp, 0), mp, mmarks)
            st = qk(u, q, 1, rem.take(3, marks + mmarks), zero)
            rem.flush(st, zero, 3, THI)
            used = jnp.where(live, ((blk + 1) & 1) * nb + off // LANES, 2 * nb)
            for r0 in range(0, d, 32):
                z4 = jnp.concatenate([tok_at(st, r0) & zero] * 4, axis=0)
                acc_scr[used, r0:r0 + 32, :] = lax.bitcast_convert_type(z4, F32)
            ln1_mod(ln_fin(tok_at(st, LNREL) & zero), (blk + 1) & 1, off, [])
            mod_fin(tok_at(st, 1880) & zero)
            o += pv(range(2 * nb, 4 * nb), zero, rem.take(4))
            st = qk(u, q, 2, rem.take(5), zero)
            rem.flush(st, zero, 5, THI)
            v_transpose(u, 0, None, [tok_at(st, 112 * i) for i in range(nt)], zero)
            st = qk(u, q, 3, rem.take(6), zero)
            rem.flush(st, zero, 6, THI)
            v_transpose(u, 1, None, [tok_at(st, 112 * i) for i in range(nt)], zero)
            res = outproj_tied(u - 1, o, rem.take(7), zero)
            rem.flush(res, zero, 7, OPN * d // 16)
            hm = []
            hb_piece((blk + 1) & 1, jnp.clip(g - 1, 0, nhb - 1), hm,
                     tok_at(res, max(OPN * d - 96, 0)) & zero)
            wb_piece(u + 2, hm, zero)
        return carry

    def stage(k, lo):
        hi = stage_at[1]
        for i in range(len(waits)):
            lax.fori_loop(0, jnp.where(k == i, 1, 0), functools.partial(manage, i), 0)
            hi = jnp.where(k == i, stage_at[i + 1], hi)
        lax.fori_loop(lo, hi, steady, 0)
        return hi

    lax.fori_loop(0, len(waits), stage, jnp.int32(stage_at[0]))

    ul = n_units - 1
    tl = seq - TB
    sl_last = (n_blk - 1) & 1
    nb0 = nb - TAILB
    with _scope("e_pva"):
        mod_scr[2:3, :] = row_scr[:, 3 * d:4 * d]
        outproj(ul, pv([j * nb + i for j in range(nq) for i in range(nb0)], zero_scr[...]))
    mlp_g.wait()
    mlp_u.wait()
    out_lo.start()
    with _scope("e_pvb"):
        toks = finalize(tl, sl_last, 0, tl, nb0 * LANES)
        o = pv([j * nb + i for j in range(nq) for i in range(nb0, nb)], zero_scr[...], toks, EROWS)
        outproj(ul, o, nb0 * LANES)

    nl = TAILB * LANES
    sub8 = lax.broadcasted_iota(I32, (TOPC, 1), 0)
    lane = lax.broadcasted_iota(I32, (TOPC, LANES), 1)

    def key_index(k):
        return seq - 1 - (lax.bitcast_convert_type(k, I32) & (seq - 1))

    def piece_base(idx, limit):
        return pl.multiple_of(jnp.clip(idx >> 7, 0, limit // LANES - 1) * LANES, LANES)

    keys = key_scr[0:seq // LANES, :]
    piece = lax.broadcasted_iota(I32, (seq // LANES, 1), 0)
    keys = jnp.where(piece < (seq - nl) // LANES, keys, 0.0)
    ecol = jnp.zeros((TOPC, LANES), F32)
    erow = jnp.zeros((1, LANES), F32)
    h2e = jnp.zeros((TOPC, d), F32)
    late = []
    marks = finalize(seq - nl, sl_last, TB - nl, seq - nl, nl, late)
    zero = zero_scr[...]
    pace = dict(zip([int(v) for v in os.environ.get("KP_PG", "2,4,5,6,7").split(",")],
                    [int(v) for v in os.environ.get("KP_PM", "8,14,18,23,27").split(",")]))
    for i in range(TOPC):
        mx = jnp.max(jnp.max(keys, axis=0, keepdims=True), axis=1, keepdims=True)
        keys = jnp.where(keys == mx, 0.0, keys)
        ecol = jnp.where(sub8 == i, mx, ecol)
        erow = jnp.where(lane[0:1] == i, mx, erow)
        idx = key_index(mx)
        pick = jnp.logical_and(sub8 == i, lane == (idx & (LANES - 1)))
        sl = pl.ds(piece_base(idx[0, 0], seq - nl), LANES)
        pick = jnp.where(pick, 1.0, 0.0)
        if i in pace:
            pick = lax.bitcast_convert_type(
                lax.bitcast_convert_type(pick, U32) | (marks[pace[i]] & zero), F32)
        h2e = h2e + lax.dot_general(pick.astype(BF16), h2_scr[:, sl], _NT,
                                    preferred_element_type=F32)

    late = [router_keys(late[0], seq - nl)]
    krow = jnp.concatenate([late[0], erow], axis=1)
    kcol = jnp.concatenate([jnp.broadcast_to(late[0], (LANES, nl)).T, ecol], axis=0)
    cnt = [None] * 4
    for g in range(kcol.shape[0] // 8):
        one = jnp.where(_lanes(kcol[8 * g:8 * g + 8], nl + LANES) > krow, 1.0, 0.0)
        cnt[g % 4] = one if cnt[g % 4] is None else cnt[g % 4] + one
    rank = jnp.sum((cnt[0] + cnt[1]) + (cnt[2] + cnt[3]), axis=0, keepdims=True)
    chosen = rank == sub8.astype(F32)
    onehot = jnp.where(chosen, 1.0, 0.0).astype(BF16)
    h2pad = jnp.concatenate([h2e, jnp.zeros((TOPC, d), F32)], axis=0).astype(BF16)
    h2s = (jnp.dot(onehot[:, nl:nl + 2 * TOPC], h2pad, preferred_element_type=F32)
           + lax.dot_general(onehot[:, 0:nl], h2l_scr[...], _NT,
                             preferred_element_type=F32))
    top = jnp.max(jnp.where(chosen, krow, 0.0), axis=1, keepdims=True)
    idx_col = key_index(top)
    idxs = [idx_col[i:i + 1] for i in range(TOPC)]
    bases = [piece_base(idx_col[i, 0], seq) for i in range(TOPC)]
    hit = lane == (idx_col & (LANES - 1))
    picks = [jnp.where(jnp.logical_and(sub8 == i, hit), 1.0, 0.0).astype(BF16)
             for i in range(TOPC)]
    order = (lax.bitcast_convert_type(top, I32) >> 11) & 0xFFFF
    rbits = jnp.where(order >= 32768, order - 32768, -1 - order) << 16
    gate = _rb(_sigmoid(lax.bitcast_convert_type(rbits, F32)))
    xs = h2s.astype(BF16)
    for cp in out_hi:
        cp.start()
    g = _rb(jnp.dot(xs, wg_v[...], preferred_element_type=F32))
    g = _rb(g * _rb(_sigmoid(g)))
    u = _rb(jnp.dot(xs, wu_v[...], preferred_element_type=F32))
    gu = (g * u).astype(BF16)

    last_use = []
    for i in range(TOPC):
        ok = True
        for j in range(i + 1, TOPC):
            ok = jnp.logical_and(ok, bases[i] != bases[j])
        last_use.append(ok)

    def down(r0, r1):
        x1p = jnp.concatenate([x1_scr[r0:r1, pl.ds(bases[i], LANES)] for i in range(TOPC)], axis=1)
        x1s = lax.dot_general(jnp.concatenate(picks, axis=1), x1p, _NT,
                              preferred_element_type=F32)
        wd = pltpu.bitcast(wd_scr[:, r0:r1], BF16)
        y = _rb(jnp.dot(gu, wd, preferred_element_type=F32))
        hm = _rb(h2s[:, r0:r1] + _rb(y * gate))
        return x1s + mod_scr[2:3, r0:r1] * hm

    def patch(r0, r1, new):
        n = r1 - r0
        pad = jnp.concatenate([new, jnp.zeros((LANES - TOPC, n), F32)], axis=0)
        cols = pltpu.bitcast(pad.T.astype(BF16), U32)
        col = [jnp.broadcast_to(cols[:, j:j + 1], (n // 2, LANES)) for j in range(TOPC)]
        for i in range(TOPC):
            res = pltpu.bitcast(ot_v[r0:r1, pl.ds(bases[i], LANES)], U32)
            tok = lane[0:1, :] + (idxs[i] & ~(LANES - 1))
            for j in range(i + 1):
                res = jnp.where(tok == idxs[j], col[j], res)
            fix_v[i, r0:r1, :] = pltpu.bitcast(res, BF16)

    def fix_copy(i, r0, r1):
        return pltpu.make_async_copy(fix_v.at[i, r0:r1, :],
                                     o_hbm.at[r0:r1, pl.ds(bases[i], LANES)], fix_sems.at[i])

    def for_last(fn):
        for i in range(TOPC - 1):
            pl.when(last_use[i])(functools.partial(fn, i))
        fn(TOPC - 1)

    new = down(*chunks[0])
    out_lo.wait()
    for ci, (r0, r1) in enumerate(chunks):
        out_hi[ci].wait()
        nxt = down(*chunks[ci + 1]) if ci + 1 < len(chunks) else None
        patch(r0, r1, new)
        for_last(lambda i: fix_copy(i, r0, r1).start())
        new = nxt
    with _scope("w_fix"):
        for r0, r1 in chunks:
            for_last(lambda i: fix_copy(i, r0, r1).wait())


@jax.jit
def pallas_adaLN_cond__gqa_block_cached__moe_arch_mod__prompt_kernel(
    A_x: jax.Array,
    A_k_cache: jax.Array,
    A_v_cache: jax.Array,
    A_wq: jax.Array,
    A_wo: jax.Array,
    B_x: jax.Array,
    B_w_r: jax.Array,
    B_w_gate: jax.Array,
    B_w_up: jax.Array,
    B_w_down: jax.Array,
    c: jax.Array,
    w_mod: jax.Array,
):
    b, seq, d = A_x.shape
    _, hkv, sk, dh = A_k_cache.shape
    assert b == 1 and dh == DH and HQ == 2 * hkv
    assert seq & (seq - 1) == 0 and seq <= 2048
    f = B_w_gate.shape[1]
    n_grp = hkv // HG
    gw = 2 * HG * dh
    n_slots = 2 * HG * TB // LANES

    xt = A_x.reshape(seq, d).T
    wot = A_wo.T
    wdt = B_w_down.T
    k3 = A_k_cache.reshape(hkv, sk, dh)
    v3 = A_v_cache.reshape(hkv, sk, dh)

    hbm = pl.BlockSpec(memory_space=pl.ANY)
    out_t = pl.pallas_call(
        functools.partial(_kernel, n_heads=hkv),
        in_specs=[hbm] * 11,
        out_specs=hbm,
        out_shape=jax.ShapeDtypeStruct((d, seq), BF16),
        scratch_shapes=[
            pltpu.VMEM((seq // LANES, d, LANES), BF16),
            pltpu.VMEM((hkv, sk, dh), BF16),
            pltpu.VMEM((hkv, sk, dh), BF16),
            pltpu.VMEM((n_grp, d, gw), BF16),
            pltpu.VMEM((n_grp, d, gw), BF16),
            pltpu.VMEM((d, 6 * d), BF16),
            pltpu.VMEM((d, f), BF16),
            pltpu.VMEM((d, f), BF16),
            pltpu.VMEM((f // WP + 1, d, WP), BF16),
            pltpu.VMEM((d, seq + SP), BF16),
            pltpu.VMEM((2, TB, d), BF16),
            pltpu.VMEM((2 * TB // LANES + 1, d, LANES), F32),
            pltpu.VMEM((n_slots, sk, LANES), F32),
            pltpu.VMEM((n_slots, 8, LANES), F32),
            pltpu.VMEM((HG, dh // 2, sk), U32),
            pltpu.VMEM((8, d), F32),
            pltpu.VMEM((6 * d, LANES), F32),
            pltpu.VMEM(((seq + SP) // LANES + 7 & ~7, LANES), F32),
            pltpu.VMEM((d, seq + SP), BF16),
            pltpu.VMEM((d, seq + SP), BF16),
            pltpu.VMEM((8, LANES), U32),
            pltpu.VMEM((TOPC, d, LANES), BF16),
            pltpu.VMEM((1, d), BF16),
            pltpu.VMEM((d,), BF16),
            pltpu.VMEM((1, 4 * d), F32),
            pltpu.VMEM((f // 2, d), U32),
            pltpu.VMEM((d, TAILB * LANES), BF16),
            pltpu.VMEM((2 * -(-RV // HP), d % LANES, HP // 2, LANES), U32),
            pltpu.VMEM((d % LANES, 8, gw), F32),
            pltpu.VMEM((RV, gw), F32),
            pltpu.VMEM((d % LANES, n_grp * gw), BF16),
            pltpu.SemaphoreType.DMA((4, n_grp)),
            pltpu.SemaphoreType.DMA((13,)),
            pltpu.SemaphoreType.DMA((3,)),
            pltpu.SemaphoreType.DMA((len(EDGES),)),
            pltpu.SemaphoreType.DMA((TOPC,)),
        ],
        compiler_params=pltpu.CompilerParams(
            disable_bounds_checks=True,
            disable_semaphore_checks=True,
            vmem_limit_bytes=120 * 1024 * 1024,
        ),
    )(xt, k3, v3, A_wq, wot, B_w_r, B_w_gate, B_w_up, wdt, c, w_mod)
    return out_t.T.reshape(b, seq, d)
```

```python
import functools
import math

import jax
import jax.numpy as jnp
from jax import lax
import jax.experimental.pallas as pl
import jax.experimental.pallas.tpu as pltpu

F32 = jnp.float32
BF16 = jnp.bfloat16
I32 = jnp.int32
U32 = jnp.uint32

HQ = 32
DH = 128
TOPC = 8
EPS = 1e-05
EPS_BF16 = 1.0013580322265625e-05
LANES = 128

TB = 512
HG = 2
SP = 128
MP = 384
WP = 256
RV = 448
HP = 80
MODC = 384
TAILB = 2
EDGES = (0, 128, 256, 384, 512, 576)

TIE0, NTIE = 2, 3
TLO, THI = 3, 126
SROWS, PVEND = (0, 1, 2, 5), 12
EROWS, EPVEND = (0, 4, 6, 7), 24
NM1, NM2, NMP = 8, 18, 24
NG1, NG2, NG3, EG3 = 18, 9, 18, 36
NF1, NF2, NF3 = 9, 6, 18
KS, KSPLIT, HS = 4, 2, 2
OPN = 2
LNREL = 1008
SHARES = (29, 28, 15, 23, 26, 30, 33, 18)
PACE = {2: 8, 4: 14, 5: 18, 6: 23, 7: 27}

_NT = (((1,), (1,)), ((), ()))


def _rb(x):
    return x.astype(BF16).astype(F32)


def _sigmoid(x):
    return 1.0 / (1.0 + jnp.exp(-x))


def _lanes(col, width):
    reps = width // LANES
    return col if reps == 1 else jnp.concatenate([col] * reps, axis=1)


def _fold(*xs):
    ts = []
    for x in xs:
        xi = lax.bitcast_convert_type(x, U32)
        ts += [xi[r:r + 8, c:c + LANES] for r in range(0, x.shape[0], 8)
               for c in range(0, x.shape[1] - LANES + 1, LANES)]
    if len(ts) > 5:
        return functools.reduce(lambda a, b: a | b, ts[:-2]) | (ts[-2] | ts[-1])
    while len(ts) > 1:
        ts = [a | b for a, b in zip(ts[0::2], ts[1::2])] + ts[len(ts) & ~1:]
    return ts[0]


def _colsum(x, marks, nmarks):
    n = x.shape[0] // 8
    acc = x[0:8]
    for g in range(1, n):
        acc = acc + x[8 * g:8 * g + 8]
        if ((g + 1) * nmarks) % n == 0:
            marks.append(_fold(acc))
    return jnp.sum(acc, axis=0, keepdims=True)


def _dep(x, tok, zero):
    return jnp.where(zero != 0, tok, x)


def _tie_rows(lhs, toks, zero, lo, hi):
    if not toks:
        return lhs
    lu = pltpu.bitcast(lhs, U32)
    rows = [lu[8 * r:8 * r + 8] for r in range(lu.shape[0] // 8)]
    for i, tok in enumerate(toks):
        r = lo + ((i + 1) * (hi - lo)) // len(toks) - 1
        head = _dep(rows[r][:, 0:LANES], tok, zero)
        rows[r] = head if lu.shape[1] == LANES else jnp.concatenate(
            [head, rows[r][:, LANES:]], axis=1)
    return pltpu.bitcast(jnp.concatenate(rows, axis=0), BF16)


def _merge(a, b):
    keyed = [((i + 1) / len(a), t) for i, t in enumerate(a)]
    keyed += [((i + 1) / len(b), t) for i, t in enumerate(b)]
    return [t for _, t in sorted(keyed, key=lambda kv: kv[0])]


def _span(start, size):
    if isinstance(start, int):
        return pl.ds(start, size)
    return pl.ds(pl.multiple_of(start, LANES), size)


def _tok(res, row):
    return lax.bitcast_convert_type(res[row:row + 8, 0:LANES], U32)


def _or(x, z):
    return lax.bitcast_convert_type(lax.bitcast_convert_type(x, U32) | z, F32)


def _kernel(xt_hbm, k_hbm, v_hbm, wq_hbm, wot_hbm, wr_hbm, wg_hbm, wu_hbm, wdt_hbm,
            c_hbm, wmod_hbm, o_hbm,
            xt_v, k_v, v_v, wq_v, wot_v, wmod_v, wg_v, wu_v, wdt_v, ot_v,
            h_scr, acc_scr, st_scr, m_scr, vt_scr, mod_scr, col_scr, key_scr, h2_scr, x1_scr,
            zero_scr, fix_v, c_ref, wr_ref, row_scr, wd_scr, h2l_scr,
            hb_scr, wb_scr, rem_scr, wrem_v,
            grp_sems, misc_sems, mlp_sems, out_sems, fix_sems,
            *, n_heads):
    d, seq = xt_hbm.shape
    sk = k_v.shape[1]
    n_grp = n_heads // HG
    n_blk = seq // TB
    n_units = n_grp * n_blk
    nb = TB // LANES
    nq = 2 * HG
    nt = sk // LANES
    gbits = n_grp.bit_length() - 1
    gw = nq * DH
    qscale = (DH ** -0.5) * math.log2(math.e)

    def grp_of(u):
        return u & (n_grp - 1)

    def blk_of(u):
        return u >> gbits

    def grp_copies(g, n=1):
        hs = pl.ds(g * HG, n * HG)
        return (*[pltpu.make_async_copy(wq_hbm.at[:, pl.ds(i * gw, gw)], wq_v.at[i],
                                        grp_sems.at[0, i]) for i in range(g, g + n)],
                pltpu.make_async_copy(k_hbm.at[hs], k_v.at[hs], grp_sems.at[1, g]),
                pltpu.make_async_copy(v_hbm.at[hs], v_v.at[hs], grp_sems.at[2, g]),
                *[pltpu.make_async_copy(wot_hbm.at[:, pl.ds((i - 1) * gw, gw)], wot_v.at[i - 1],
                                        grp_sems.at[3, i]) for i in range(g, g + n)])

    def col_copy(src, dst, lo, hi, sem):
        return pltpu.make_async_copy(src.at[:, lo:hi], dst.at[:, lo:hi], sem)

    class Pieces:
        def __init__(self, src, dst, lo, hi, sem):
            self.src, self.dst, self.lo, self.hi, self.sem = src, dst, lo, hi, sem

        def start(self):
            w = self.dst.shape[2]
            for p in range(self.lo, self.hi):
                pltpu.make_async_copy(self.src.at[:, p * w:(p + 1) * w], self.dst.at[p],
                                      self.sem).start()

        def wait(self):
            whole = self.dst.at[self.lo:self.hi]
            pltpu.make_async_copy(whole, whole, self.sem).wait()

    def x_cols(t0, n):
        return jnp.concatenate([xt_v[t0 // LANES + i] for i in range(n // LANES)], axis=1)

    x_first = Pieces(xt_hbm, xt_v, 0, nb, misc_sems.at[0])
    x_second = Pieces(xt_hbm, xt_v, nb, nb + 1, misc_sems.at[10])
    x_rest = Pieces(xt_hbm, xt_v, nb + 1, seq // LANES, misc_sems.at[1])
    mod_first = [col_copy(wmod_hbm, wmod_v, MODC, 2 * d, misc_sems.at[8]),
                 col_copy(wmod_hbm, wmod_v, 0, MODC, misc_sems.at[9])]
    mod_rest = col_copy(wmod_hbm, wmod_v, 2 * d, 6 * d, misc_sems.at[3])
    mlp_g = pltpu.make_async_copy(wg_hbm, wg_v, mlp_sems.at[0])
    mlp_u = pltpu.make_async_copy(wu_hbm, wu_v, mlp_sems.at[1])
    ff = wdt_hbm.shape[1]
    mlp_d = Pieces(wdt_hbm, wdt_v, 0, ff // WP, mlp_sems.at[2])
    out_lo = col_copy(ot_v, o_hbm, 0, seq - TB, out_sems.at[0])
    chunks = list(zip(EDGES[:-1], EDGES[1:]))
    out_hi = [pltpu.make_async_copy(ot_v.at[r0:r1, seq - TB:seq], o_hbm.at[r0:r1, seq - TB:seq],
                                    out_sems.at[1 + i]) for i, (r0, r1) in enumerate(chunks)]

    def silu_c():
        cc = c_ref[...].astype(F32)
        return jnp.broadcast_to((cc * _rb(_sigmoid(cc))).astype(BF16), (8, d))

    def ln1_norm(t0, n, marks):
        x = x_cols(t0, n).astype(F32)
        mu = _colsum(x, marks, NM1) * (1.0 / d)
        marks.append(_fold(jnp.broadcast_to(mu, (8, n))))
        xc = x - mu
        var = _colsum(xc * xc, marks, NM2) * (1.0 / d)
        rs = lax.rsqrt(var + EPS)

        def finish(z=None):
            r = rs if z is None else _or(rs, _lanes(z[0:1], n))
            return (xc * r).astype(BF16).T
        return finish

    def ln1_mod(ln, slot, r0):
        h = ln.astype(F32) * mod_scr[1:2, :] + mod_scr[0:1, :]
        h_scr[slot, _span(r0, ln.shape[0]), :] = h.astype(BF16)

    def mod_piece(src, dst, marks):
        w = wmod_v[:, _span(src, MP)].astype(F32)
        row0 = _rb(_colsum(w * _lanes(col_scr[5 * d:6 * d, :], MP), marks, NMP))

        def finish(z):
            row = _or(row0, _lanes(z[0:1], MP))
            pos = dst + lax.broadcasted_iota(I32, (1, MP), 1)
            is_cb = jnp.logical_and(pos >= 2 * d, pos < 3 * d)
            row = jnp.where(is_cb, _rb(1.0 + row), row)
            row_scr[:, _span(dst, MP)] = row
            col_scr[_span(dst, MP), :] = jnp.broadcast_to(row, (LANES, MP)).T
        return finish

    def wd_piece(src, dst, marks):
        w = pltpu.bitcast(wdt_v[src // WP].T, U32)
        wd_scr[pl.ds(pl.multiple_of(dst // 2, WP // 2), WP // 2), :] = w
        for r in range(56, WP // 2, 64):
            for c in range(0, d - LANES + 1, LANES):
                marks.append(w[r:r + 8, c:c + LANES])

    dm = d - d % LANES
    kr = d - dm
    nhb = -(-RV // HP)
    assert nhb <= 6 and nhb * HP <= TB

    def hb_piece(slot, sp, marks, z=None):
        r0 = sp * HP
        src = pl.ds(r0 if isinstance(r0, int) else pl.multiple_of(r0, 16), HP)
        hu = pltpu.bitcast(h_scr[slot, src, dm:d], U32)
        if z is not None:
            hu = hu | jnp.concatenate([z[:, 0:kr]] * (HP // 16), axis=0)
        for k in range(kr):
            col = jnp.broadcast_to(hu[:, k:k + 1], (HP // 2, LANES))
            hb_scr[slot * nhb + sp, k] = col
            if (k + 1) % HS == 0:
                marks.append(col[HP // 2 - 8:HP // 2])

    def wb_piece(u, toks, zero):
        w = lax.bitcast_convert_type(wrem_v[:, _span(grp_of(u) * gw, gw)].astype(F32), U32)
        for k in range(kr):
            row = jnp.broadcast_to(w[k:k + 1], (8, gw))
            row = row | _lanes(toks[k * len(toks) // kr] & zero, gw)
            wb_scr[k] = lax.bitcast_convert_type(row, F32)

    class Rem:
        def __init__(self, slot):
            self.marks, self.done, self.ready = [], {}, []
            for p in range(RV // 16):
                acc = None
                for k in range(kr):
                    sp, r8 = divmod(8 * p, HP // 2)
                    hb = pltpu.bitcast(hb_scr[slot * nhb + sp, k, r8:r8 + 8, :], BF16).astype(F32)
                    w = wb_scr[k]
                    t = _lanes(hb, gw) * jnp.concatenate([w, w], axis=0)
                    acc = t if acc is None else acc + t
                    if (k + 1) % KS == 0:
                        for c in range(0, gw, gw // KSPLIT):
                            self.marks.append(_fold(acc[:, c:c + gw // KSPLIT]))
                self.done[len(self.marks) - 1] = (p, acc)

        def take(self, phase, others=()):
            n, tot = len(self.marks), sum(SHARES)
            lo, hi = sum(SHARES[:phase]) * n // tot, sum(SHARES[:phase + 1]) * n // tot
            for i in range(lo, hi):
                if i in self.done:
                    self.ready.append((*self.done[i], phase, (i + 1 - lo) / (hi - lo)))
            mine = self.marks[lo:hi]
            return _merge(others, mine) if others and mine else list(others) + mine

        def flush(self, st, zero, phase, hi=THI):
            old = [r for r in self.ready if r[2] < phase]
            for p, acc, ph, frac in self.ready:
                if ph < phase:
                    rl = 8 * (([r[0] for r in old].index(p) + 1) * 200 // (len(old) + 1))
                else:
                    rl = 16 * min(int(TLO + frac * (hi - TLO)) - 4, 118)
                z = jnp.concatenate([_lanes(_tok(st, rl) & zero, gw)] * 2, axis=0)
                rem_scr[16 * p:16 * p + 16, :] = _or(acc, z)
            self.ready = []

    def qproj(u, toks, zero):
        h = h_scr[blk_of(u) & 1]
        q = jnp.dot(h[RV:TB, dm:d], wq_v[grp_of(u), dm:d, :], preferred_element_type=F32)
        r = jnp.concatenate([rem_scr[...], q], axis=0)
        outs = []
        for i in range(nq):
            tk = toks[i * len(toks) // nq:(i + 1) * len(toks) // nq]
            hm = _tie_rows(h[:, 0:dm], tk, zero, 0, TB // 16)
            q = jnp.dot(hm, wq_v[grp_of(u), 0:dm, i * DH:(i + 1) * DH],
                        preferred_element_type=F32) + r[:, i * DH:(i + 1) * DH]
            outs.append(q.astype(BF16))
        return jnp.concatenate(outs, axis=1)

    def qproj_first(lo, hi):
        qs = []
        for r0 in (0, TB // 2):
            rs = slice(r0, r0 + TB // 2)
            q = jnp.dot(h_scr[0, rs, dm:d], wq_v[0, dm:d, lo:hi], preferred_element_type=F32)
            q = jnp.dot(h_scr[0, rs, 0:dm], wq_v[0, 0:dm, lo:hi], preferred_element_type=F32) + q
            qs.append(q.astype(BF16))
        return jnp.concatenate(qs, axis=0)

    def qk(u, q, j, toks, zero):
        k = _tie_rows(k_v[grp_of(u) * HG + j // 2], toks, zero, TLO, THI)
        st = lax.dot_general(k, q[:, j * DH:(j + 1) * DH], _NT,
                             preferred_element_type=F32)
        for i in range(nb):
            blk = st[:, i * LANES:(i + 1) * LANES]
            st_scr[j * nb + i] = blk
            m_scr[j * nb + i] = jnp.max(blk.reshape(sk // 8, 8, LANES), axis=0)
        return st

    def v_transpose(u, i, rel=(), zero=None):
        v = _tie_rows(v_v[grp_of(u) * HG + i], rel, zero, -7, sk // 16 - 7)
        vt = pltpu.bitcast(v.T, U32)
        vt_scr[i] = vt
        return [vt[DH // 2 - 8:DH // 2, c:c + LANES] for c in range(0, sk, LANES)]

    def pv(slots, zero, toks=(), srows=SROWS, free=PVEND):
        ps, ls, pairs = [], [], []
        for sl in slots:
            m = jnp.max(m_scr[sl], axis=0, keepdims=True)
            p = jnp.exp2(st_scr[sl] - m)
            accs = [None] * 4
            for tile in range(nt):
                for r0 in range(tile * LANES + LANES - 16, tile * LANES - 16, -16):
                    pair = p[r0:r0 + 8] + p[r0 + 8:r0 + 16]
                    pairs.append(pair)
                    a = accs[tile % 4]
                    accs[tile % 4] = pair if a is None else a + pair
            ls.append(jnp.sum((accs[0] + accs[1]) + (accs[2] + accs[3]), axis=0, keepdims=True))
            ps.append(p.astype(BF16))
        outs = []
        ntiles = len(slots) * nt
        side = {}
        for i, tok in enumerate(toks):
            side.setdefault(max(((i + 1) * (ntiles - free)) // len(toks) - 1, 0), []).append(tok)
        for i, sl in enumerate(slots):
            vu = vt_scr[sl // (2 * nb)]
            tiles = []
            for c in range(nt):
                g = i * nt + c + 4
                rows = []
                for r in range(8):
                    x = vu[8 * r:8 * r + 8, c * LANES:(c + 1) * LANES]
                    if g < ntiles and TIE0 <= r < TIE0 + NTIE:
                        src = pairs[g * 8 + (r - TIE0)]
                        x = _dep(x, lax.bitcast_convert_type(src, U32), zero)
                    if r == srows[c % 4]:
                        for tok in side.get(i * nt + c, ()):
                            x = _dep(x, tok, zero)
                    rows.append(x)
                tiles.append(jnp.concatenate(rows, axis=0))
            lhs = pltpu.bitcast(jnp.concatenate(tiles, axis=1), BF16)
            o = jnp.dot(lhs, ps[i], preferred_element_type=F32)
            outs.append(o * (1.0 / ls[i]))
        return outs

    def outproj_tied(u, o, toks, zero):
        slot = blk_of(u) & 1
        res = []
        for i in range(nb):
            o2 = jnp.concatenate([o[j * nb + i] for j in range(nq)], axis=0).astype(BF16)
            tk = toks[i * len(toks) // OPN:(i + 1) * len(toks) // OPN]
            wo = _tie_rows(wot_v[grp_of(u)], tk, zero, 0, d // 16)
            contrib = jnp.dot(wo, o2, preferred_element_type=F32)
            acc_scr[slot * nb + i] += contrib
            res.append(contrib)
        return jnp.concatenate(res, axis=0)

    def outproj(u, o, lo=0):
        w = len(o) // nq
        o2 = jnp.concatenate(
            [jnp.concatenate(o[j * w:(j + 1) * w], axis=1) for j in range(nq)], axis=0).astype(BF16)
        contrib = jnp.dot(wot_v[grp_of(u)], o2, preferred_element_type=F32)
        slot = blk_of(u) & 1
        for i in range(w):
            pi = slot * nb + lo // LANES + i
            acc_scr[pi] += contrib[:, i * LANES:(i + 1) * LANES]

    def router_keys(racc, t0):
        r = _rb(jnp.sum(racc, axis=0, keepdims=True)) + 0.0
        bits = lax.bitcast_convert_type(r, I32) >> 16
        order = jnp.where(bits < 0, -1 - bits, bits + 32768)
        pos = t0 + lax.broadcasted_iota(I32, r.shape, 1)
        return lax.bitcast_convert_type((order << 11) + (seq - 1 - pos) + 0x20000000, F32)

    def finalize(t0, slot, a0, dst, n, keys_out=None):
        marks = []
        cs = _span(dst, n)
        x = x_cols(t0, n).astype(F32)
        att = jnp.concatenate(
            [acc_scr[slot * nb + a0 // LANES + i] for i in range(n // LANES)], axis=1)
        x1b = (x + _lanes(col_scr[0:d, :], n) * att).astype(BF16)
        x1_scr[:, cs] = x1b
        ot_v[:, cs] = x1b
        fine = keys_out is None
        mu = _colsum(x1b.astype(F32), marks, NG1 if fine else NF1) * (1.0 / d)

        def note(row):
            if fine:
                marks.append(_fold(jnp.broadcast_to(row, (8, n))))
            return row

        mub = note(_rb(mu))
        xc = x1_scr[:, cs].astype(F32) - mub
        var = _colsum(xc * xc, marks, NG2 if fine else NF2) * (1.0 / d) - (mu - mub) * (mu - mub)
        inv = note(1.0 / note(_rb(jnp.sqrt(note(_rb(_rb(jnp.maximum(var, 0.0)) + EPS_BF16))))))
        step = d // ((NG3 if n == SP else EG3) if fine else NF3)
        racc = None
        for r0 in range(0, d, step):
            rs = slice(r0, r0 + step)
            x1 = ot_v[rs, cs].astype(F32)
            ln = _rb(_rb(x1 - mub) * inv)
            if fine:
                marks.append(_fold(ln))
            h2b = (_rb(ln * _lanes(col_scr[2 * d + r0:2 * d + r0 + step, :], n))
                   + _lanes(col_scr[d + r0:d + r0 + step, :], n)).astype(BF16)
            if keys_out is None:
                h2_scr[rs, cs] = h2b
            else:
                h2l_scr[rs, :] = h2b
            h2 = h2b.astype(F32)
            out = x1 + _lanes(col_scr[3 * d + r0:3 * d + r0 + step, :], n) * h2
            ot_v[rs, cs] = out.astype(BF16)
            rp = h2 * _lanes(col_scr[4 * d + r0:4 * d + r0 + step, :], n)
            for g in range(0, step, 8):
                racc = rp[g:g + 8] if racc is None else racc + rp[g:g + 8]
            marks.append(_fold(out, racc))
        if keys_out is not None:
            keys_out.append(racc)
            return marks
        key = router_keys(racc, t0)
        for i in range(n // LANES):
            key_scr[pl.ds(dst // LANES + i, 1), :] = key[:, i * LANES:(i + 1) * LANES]
        return marks

    hw = gw // 2
    wq0a = col_copy(wq_hbm, wq_v.at[0], 0, hw, grp_sems.at[0, 0])
    wq0b = col_copy(wq_hbm, wq_v.at[0], hw, gw, misc_sems.at[4])
    k0a = pltpu.make_async_copy(k_hbm.at[0], k_v.at[0], grp_sems.at[1, 0])
    k0b = pltpu.make_async_copy(k_hbm.at[1], k_v.at[1], misc_sems.at[5])
    v0 = pltpu.make_async_copy(v_hbm.at[0:HG], v_v.at[0:HG], grp_sems.at[2, 0])
    wq1, k1, v1, wo0 = grp_copies(1)
    wo_last = pltpu.make_async_copy(wot_hbm.at[:, (n_grp - 1) * gw:n_grp * gw],
                                    wot_v.at[n_grp - 1], grp_sems.at[3, 0])
    wrem_copy = col_copy(wq_hbm.at[dm:d], wrem_v, gw, 4 * gw, misc_sems.at[2])
    wrem_rest = (col_copy(wq_hbm.at[dm:d], wrem_v, 0, gw, misc_sems.at[11]),
                 col_copy(wq_hbm.at[dm:d], wrem_v, 4 * gw, n_grp * gw, misc_sems.at[12]))
    c_copy = pltpu.make_async_copy(c_hbm, c_ref, misc_sems.at[6])
    wr_copy = pltpu.make_async_copy(wr_hbm, wr_ref, misc_sems.at[7])
    c_copy.start()
    wr_copy.start()
    x_first.start()
    mod_first[0].start()
    mod_first[1].start()
    wq0a.start()
    wq0b.start()
    acc_scr[0:2 * nb] = jnp.zeros((2 * nb, d, LANES), F32)
    col_scr[0:4 * d, :] = jnp.zeros((4 * d, LANES), F32)
    wdt_v[ff // WP] = jnp.zeros((d, WP), BF16)
    c_copy.wait()
    wr_copy.wait()
    x_first.wait()
    cbits = lax.bitcast_convert_type(c_ref[:, 0:LANES].astype(F32), U32)
    zero_scr[...] = jnp.broadcast_to(cbits & 0xFFFF, (8, LANES))
    h_scr[0] = ln1_norm(0, TB, [])()
    sc = silu_c()
    wr = wr_ref[...].reshape(1, d).astype(F32)
    col_scr[4 * d:5 * d, :] = jnp.broadcast_to(wr, (LANES, d)).T
    col_scr[5 * d:6 * d, :] = jnp.broadcast_to(sc[0:1, :].astype(F32), (LANES, d)).T
    mod_first[0].wait()
    mod = _rb(jnp.dot(sc, wmod_v[:, MODC:2 * d], preferred_element_type=F32))
    mod_scr[0:1, MODC:d] = mod[0:1, 0:d - MODC] * qscale
    mod_scr[1:2, :] = _rb(1.0 + mod[0:1, d - MODC:2 * d - MODC]) * qscale
    mod_first[1].wait()
    k0a.start()
    mod = _rb(jnp.dot(sc, wmod_v[:, 0:MODC], preferred_element_type=F32))
    mod_scr[0:1, 0:MODC] = mod[0:1] * qscale
    wq0a.wait()
    k0b.start(priority=1)
    v0.start(priority=1)
    wrem_copy.start(priority=1)
    ln1_mod(h_scr[0], 0, 0)
    qa = qproj_first(0, hw)
    wq0b.wait()
    k0a.wait()
    wq1.start(priority=1)
    k1.start(priority=1)
    x_second.start()
    q = jnp.concatenate([qa, qproj_first(hw, gw)], axis=1)
    zero = zero_scr[...]
    for j in range(2):
        marks = []
        for i in range(2 * j, 2 * j + 2):
            hb_piece(0, i, marks)
        qk(0, q, j, marks, zero)
    k0b.wait()
    v0.wait()
    wrem_copy.wait()
    v1.start()
    wo0.start()
    zero = zero_scr[...]
    rem_scr[...] = jnp.dot(h_scr[0, 0:RV, dm:d], wrem_v[:, gw:2 * gw],
                           preferred_element_type=F32)
    for i in range(HG):
        marks = v_transpose(0, i)
        if i == 0:
            wb_piece(2, marks, zero)
        if 4 + i < nhb:
            hm = []
            hb_piece(0, 4 + i, hm)
            marks = _merge(marks, hm)
        qk(0, q, nq - HG + i, marks, zero)

    assert n_grp == 8 and HG == 2
    stage_at = [1, 2, 3, 5, n_units]
    starts = [(*grp_copies(2), mod_rest, x_rest, *wrem_rest), grp_copies(3, 3),
              (*grp_copies(6, 2), wo_last, mlp_d), (mlp_g, mlp_u)]
    waits = [(wq1, k1, v1, wo0, x_second), *starts[:3]]
    wd0 = stage_at[3]
    npc = TB // SP
    nmp = 4 * d // MP

    def manage(k, _, c):
        for cp in waits[k]:
            cp.wait()
        for cp in starts[k]:
            cp.start()
        return c

    def steady(u, carry):
        zero = zero_scr[...]
        blk, g = blk_of(u), grp_of(u)
        off = ((g - 1) & (npc - 1)) * SP
        rem = Rem(blk_of(u + 1) & 1)
        q = qproj(u, rem.take(0), zero)
        o = pv(range(0, 2 * nb), zero, rem.take(1))
        live = jnp.logical_and(blk > 0, jnp.logical_and(g >= 1, g <= npc))
        t0 = jnp.maximum(blk - 1, 0) * TB + off
        marks = finalize(t0, (blk + 1) & 1, off, jnp.where(live, t0, seq), SP)
        wp = jnp.clip(u - wd0, 0, ff // WP - 1) * WP
        wmarks = []
        wd_piece(jnp.where(u >= wd0, wp, ff), wp, wmarks)
        rem.flush(qk(u, q, 0, rem.take(2, _merge(marks, wmarks)), zero), zero, 2)
        marks, mmarks = [], []
        ln_fin = ln1_norm(jnp.minimum(blk + 1, n_blk - 1) * TB + off, SP, marks)
        mp = jnp.clip(u - 2, 0, nmp - 1) * MP
        mod_fin = mod_piece(jnp.where(u >= 2, 2 * d + mp, 0), mp, mmarks)
        st = qk(u, q, 1, rem.take(3, marks + mmarks), zero)
        rem.flush(st, zero, 3)
        used = jnp.where(live, ((blk + 1) & 1) * nb + off // LANES, 2 * nb)
        for r0 in range(0, d, 32):
            z4 = jnp.concatenate([_tok(st, r0) & zero] * 4, axis=0)
            acc_scr[used, r0:r0 + 32, :] = lax.bitcast_convert_type(z4, F32)
        ln1_mod(ln_fin(_tok(st, LNREL) & zero), (blk + 1) & 1, off)
        mod_fin(_tok(st, 1880) & zero)
        o += pv(range(2 * nb, 4 * nb), zero, rem.take(4))
        st = qk(u, q, 2, rem.take(5), zero)
        rem.flush(st, zero, 5)
        v_transpose(u, 0, [_tok(st, 112 * i) for i in range(nt)], zero)
        st = qk(u, q, 3, rem.take(6), zero)
        rem.flush(st, zero, 6)
        v_transpose(u, 1, [_tok(st, 112 * i) for i in range(nt)], zero)
        res = outproj_tied(u - 1, o, rem.take(7), zero)
        rem.flush(res, zero, 7, OPN * d // 16)
        hm = []
        hb_piece((blk + 1) & 1, jnp.clip(g - 1, 0, nhb - 1), hm,
                 _tok(res, max(OPN * d - 96, 0)) & zero)
        wb_piece(u + 2, hm, zero)
        return carry

    def stage(k, lo):
        hi = stage_at[1]
        for i in range(len(waits)):
            lax.fori_loop(0, jnp.where(k == i, 1, 0), functools.partial(manage, i), 0)
            hi = jnp.where(k == i, stage_at[i + 1], hi)
        lax.fori_loop(lo, hi, steady, 0)
        return hi

    lax.fori_loop(0, len(waits), stage, jnp.int32(stage_at[0]))

    ul = n_units - 1
    tl = seq - TB
    sl_last = (n_blk - 1) & 1
    nb0 = nb - TAILB
    mod_scr[2:3, :] = row_scr[:, 3 * d:4 * d]
    outproj(ul, pv([j * nb + i for j in range(nq) for i in range(nb0)], zero_scr[...]))
    mlp_g.wait()
    mlp_u.wait()
    out_lo.start()
    toks = finalize(tl, sl_last, 0, tl, nb0 * LANES)
    o = pv([j * nb + i for j in range(nq) for i in range(nb0, nb)], zero_scr[...], toks,
           EROWS, EPVEND)
    outproj(ul, o, nb0 * LANES)

    nl = TAILB * LANES
    sub8 = lax.broadcasted_iota(I32, (TOPC, 1), 0)
    lane = lax.broadcasted_iota(I32, (TOPC, LANES), 1)

    def key_index(k):
        return seq - 1 - (lax.bitcast_convert_type(k, I32) & (seq - 1))

    def piece_base(idx, limit):
        return pl.multiple_of(jnp.clip(idx >> 7, 0, limit // LANES - 1) * LANES, LANES)

    keys = key_scr[0:seq // LANES, :]
    piece = lax.broadcasted_iota(I32, (seq // LANES, 1), 0)
    keys = jnp.where(piece < (seq - nl) // LANES, keys, 0.0)
    ecol = jnp.zeros((TOPC, LANES), F32)
    erow = jnp.zeros((1, LANES), F32)
    h2e = jnp.zeros((TOPC, d), F32)
    late = []
    marks = finalize(seq - nl, sl_last, TB - nl, seq - nl, nl, late)
    zero = zero_scr[...]
    for i in range(TOPC):
        mx = jnp.max(jnp.max(keys, axis=0, keepdims=True), axis=1, keepdims=True)
        keys = jnp.where(keys == mx, 0.0, keys)
        ecol = jnp.where(sub8 == i, mx, ecol)
        erow = jnp.where(lane[0:1] == i, mx, erow)
        idx = key_index(mx)
        pick = jnp.logical_and(sub8 == i, lane == (idx & (LANES - 1)))
        sl = pl.ds(piece_base(idx[0, 0], seq - nl), LANES)
        pick = jnp.where(pick, 1.0, 0.0)
        if i in PACE:
            pick = _or(pick, marks[PACE[i]] & zero)
        h2e = h2e + lax.dot_general(pick.astype(BF16), h2_scr[:, sl], _NT,
                                    preferred_element_type=F32)

    late = [router_keys(late[0], seq - nl)]
    krow = jnp.concatenate([late[0], erow], axis=1)
    kcol = jnp.concatenate([jnp.broadcast_to(late[0], (LANES, nl)).T, ecol], axis=0)
    cnt = [None] * 4
    for g in range(kcol.shape[0] // 8):
        one = jnp.where(_lanes(kcol[8 * g:8 * g + 8], nl + LANES) > krow, 1.0, 0.0)
        cnt[g % 4] = one if cnt[g % 4] is None else cnt[g % 4] + one
    rank = jnp.sum((cnt[0] + cnt[1]) + (cnt[2] + cnt[3]), axis=0, keepdims=True)
    chosen = rank == sub8.astype(F32)
    onehot = jnp.where(chosen, 1.0, 0.0).astype(BF16)
    h2pad = jnp.concatenate([h2e, jnp.zeros((TOPC, d), F32)], axis=0).astype(BF16)
    h2s = (jnp.dot(onehot[:, nl:nl + 2 * TOPC], h2pad, preferred_element_type=F32)
           + lax.dot_general(onehot[:, 0:nl], h2l_scr[...], _NT,
                             preferred_element_type=F32))
    top = jnp.max(jnp.where(chosen, krow, 0.0), axis=1, keepdims=True)
    idx_col = key_index(top)
    idxs = [idx_col[i:i + 1] for i in range(TOPC)]
    bases = [piece_base(idx_col[i, 0], seq) for i in range(TOPC)]
    hit = lane == (idx_col & (LANES - 1))
    picks = [jnp.where(jnp.logical_and(sub8 == i, hit), 1.0, 0.0).astype(BF16)
             for i in range(TOPC)]
    order = (lax.bitcast_convert_type(top, I32) >> 11) & 0xFFFF
    rbits = jnp.where(order >= 32768, order - 32768, -1 - order) << 16
    gate = _rb(_sigmoid(lax.bitcast_convert_type(rbits, F32)))
    xs = h2s.astype(BF16)
    for cp in out_hi:
        cp.start()
    g = _rb(jnp.dot(xs, wg_v[...], preferred_element_type=F32))
    g = _rb(g * _rb(_sigmoid(g)))
    u = _rb(jnp.dot(xs, wu_v[...], preferred_element_type=F32))
    gu = (g * u).astype(BF16)

    last_use = []
    for i in range(TOPC):
        ok = True
        for j in range(i + 1, TOPC):
            ok = jnp.logical_and(ok, bases[i] != bases[j])
        last_use.append(ok)

    def down(r0, r1):
        x1p = jnp.concatenate([x1_scr[r0:r1, pl.ds(bases[i], LANES)] for i in range(TOPC)], axis=1)
        x1s = lax.dot_general(jnp.concatenate(picks, axis=1), x1p, _NT,
                              preferred_element_type=F32)
        wd = pltpu.bitcast(wd_scr[:, r0:r1], BF16)
        y = _rb(jnp.dot(gu, wd, preferred_element_type=F32))
        hm = _rb(h2s[:, r0:r1] + _rb(y * gate))
        return x1s + mod_scr[2:3, r0:r1] * hm

    def patch(r0, r1, new):
        n = r1 - r0
        pad = jnp.concatenate([new, jnp.zeros((LANES - TOPC, n), F32)], axis=0)
        cols = pltpu.bitcast(pad.T.astype(BF16), U32)
        col = [jnp.broadcast_to(cols[:, j:j + 1], (n // 2, LANES)) for j in range(TOPC)]
        for i in range(TOPC):
            res = pltpu.bitcast(ot_v[r0:r1, pl.ds(bases[i], LANES)], U32)
            tok = lane[0:1, :] + (idxs[i] & ~(LANES - 1))
            for j in range(i + 1):
                res = jnp.where(tok == idxs[j], col[j], res)
            fix_v[i, r0:r1, :] = pltpu.bitcast(res, BF16)

    def fix_copy(i, r0, r1):
        return pltpu.make_async_copy(fix_v.at[i, r0:r1, :],
                                     o_hbm.at[r0:r1, pl.ds(bases[i], LANES)], fix_sems.at[i])

    def for_last(fn):
        for i in range(TOPC - 1):
            pl.when(last_use[i])(functools.partial(fn, i))
        fn(TOPC - 1)

    new = down(*chunks[0])
    out_lo.wait()
    for ci, (r0, r1) in enumerate(chunks):
        out_hi[ci].wait()
        nxt = down(*chunks[ci + 1]) if ci + 1 < len(chunks) else None
        patch(r0, r1, new)
        for_last(lambda i: fix_copy(i, r0, r1).start())
        new = nxt
    for r0, r1 in chunks:
        for_last(lambda i: fix_copy(i, r0, r1).wait())


@jax.jit
def pallas_adaLN_cond__gqa_block_cached__moe_arch_mod__prompt_kernel(
    A_x: jax.Array,
    A_k_cache: jax.Array,
    A_v_cache: jax.Array,
    A_wq: jax.Array,
    A_wo: jax.Array,
    B_x: jax.Array,
    B_w_r: jax.Array,
    B_w_gate: jax.Array,
    B_w_up: jax.Array,
    B_w_down: jax.Array,
    c: jax.Array,
    w_mod: jax.Array,
):
    b, seq, d = A_x.shape
    _, hkv, sk, dh = A_k_cache.shape
    assert b == 1 and dh == DH and HQ == 2 * hkv
    assert seq & (seq - 1) == 0 and seq <= 2048
    f = B_w_gate.shape[1]
    n_grp = hkv // HG
    gw = 2 * HG * dh
    n_slots = 2 * HG * TB // LANES

    xt = A_x.reshape(seq, d).T
    wot = A_wo.T
    wdt = B_w_down.T
    k3 = A_k_cache.reshape(hkv, sk, dh)
    v3 = A_v_cache.reshape(hkv, sk, dh)

    hbm = pl.BlockSpec(memory_space=pl.ANY)
    out_t = pl.pallas_call(
        functools.partial(_kernel, n_heads=hkv),
        in_specs=[hbm] * 11,
        out_specs=hbm,
        out_shape=jax.ShapeDtypeStruct((d, seq), BF16),
        scratch_shapes=[
            pltpu.VMEM((seq // LANES, d, LANES), BF16),
            pltpu.VMEM((hkv, sk, dh), BF16),
            pltpu.VMEM((hkv, sk, dh), BF16),
            pltpu.VMEM((n_grp, d, gw), BF16),
            pltpu.VMEM((n_grp, d, gw), BF16),
            pltpu.VMEM((d, 6 * d), BF16),
            pltpu.VMEM((d, f), BF16),
            pltpu.VMEM((d, f), BF16),
            pltpu.VMEM((f // WP + 1, d, WP), BF16),
            pltpu.VMEM((d, seq + SP), BF16),
            pltpu.VMEM((2, TB, d), BF16),
            pltpu.VMEM((2 * TB // LANES + 1, d, LANES), F32),
            pltpu.VMEM((n_slots, sk, LANES), F32),
            pltpu.VMEM((n_slots, 8, LANES), F32),
            pltpu.VMEM((HG, dh // 2, sk), U32),
            pltpu.VMEM((8, d), F32),
            pltpu.VMEM((6 * d, LANES), F32),
            pltpu.VMEM(((seq + SP) // LANES + 7 & ~7, LANES), F32),
            pltpu.VMEM((d, seq + SP), BF16),
            pltpu.VMEM((d, seq + SP), BF16),
            pltpu.VMEM((8, LANES), U32),
            pltpu.VMEM((TOPC, d, LANES), BF16),
            pltpu.VMEM((1, d), BF16),
            pltpu.VMEM((d,), BF16),
            pltpu.VMEM((1, 4 * d), F32),
            pltpu.VMEM((f // 2, d), U32),
            pltpu.VMEM((d, TAILB * LANES), BF16),
            pltpu.VMEM((2 * -(-RV // HP), d % LANES, HP // 2, LANES), U32),
            pltpu.VMEM((d % LANES, 8, gw), F32),
            pltpu.VMEM((RV, gw), F32),
            pltpu.VMEM((d % LANES, n_grp * gw), BF16),
            pltpu.SemaphoreType.DMA((4, n_grp)),
            pltpu.SemaphoreType.DMA((13,)),
            pltpu.SemaphoreType.DMA((3,)),
            pltpu.SemaphoreType.DMA((len(EDGES),)),
            pltpu.SemaphoreType.DMA((TOPC,)),
        ],
        compiler_params=pltpu.CompilerParams(
            disable_bounds_checks=True,
            disable_semaphore_checks=True,
            vmem_limit_bytes=120 * 1024 * 1024,
        ),
    )(xt, k3, v3, A_wq, wot, B_w_r, B_w_gate, B_w_up, wdt, c, w_mod)
    return out_t.T.reshape(b, seq, d)
```

```python
import functools
import math

import jax
import jax.numpy as jnp
from jax import lax
import jax.experimental.pallas as pl
import jax.experimental.pallas.tpu as pltpu

F32 = jnp.float32
BF16 = jnp.bfloat16
I32 = jnp.int32
U32 = jnp.uint32

HQ = 32
DH = 128
TOPC = 8
EPS = 1e-05
EPS_BF16 = 1.0013580322265625e-05
LANES = 128

TB = 512
HG = 2
SP = 128
MP = 384
WP = 256
RV = 448
HP = 80
MODC = 384
TAILB = 2
EDGES = (0, 128, 256, 384, 512, 576)

TIE0, NTIE = 2, 3
TLO, THI = 3, 126
SROWS, PVEND = (0, 1, 2, 5), 12
EROWS, EPVEND = (0, 4, 6, 7), 24
NM1, NM2, NMP = 8, 18, 24
NG1, NG2, NG3, EG3 = 18, 9, 18, 36
NF1, NF2, NF3 = 9, 6, 18
KS, KSPLIT, HS = 4, 2, 2
OPN = 2
LNREL = 1008
SHARES = (29, 28, 15, 23, 26, 30, 33, 18)
PACE = {2: 8, 4: 14, 5: 18, 6: 23, 7: 27}

_NT = (((1,), (1,)), ((), ()))


def _rb(x):
    return x.astype(BF16).astype(F32)


def _sigmoid(x):
    return 1.0 / (1.0 + jnp.exp(-x))


def _lanes(col, width):
    reps = width // LANES
    return col if reps == 1 else jnp.concatenate([col] * reps, axis=1)


def _fold(*xs):
    ts = []
    for x in xs:
        xi = lax.bitcast_convert_type(x, U32)
        ts += [xi[r:r + 8, c:c + LANES] for r in range(0, x.shape[0], 8)
               for c in range(0, x.shape[1] - LANES + 1, LANES)]
    if len(ts) > 5:
        return functools.reduce(lambda a, b: a | b, ts[:-2]) | (ts[-2] | ts[-1])
    while len(ts) > 1:
        ts = [a | b for a, b in zip(ts[0::2], ts[1::2])] + ts[len(ts) & ~1:]
    return ts[0]


def _colsum(x, marks, nmarks):
    n = x.shape[0] // 8
    acc = x[0:8]
    for g in range(1, n):
        acc = acc + x[8 * g:8 * g + 8]
        if ((g + 1) * nmarks) % n == 0:
            marks.append(_fold(acc))
    return jnp.sum(acc, axis=0, keepdims=True)


def _dep(x, tok, zero):
    return jnp.where(zero != 0, tok, x)


def _tie_rows(lhs, toks, zero, lo, hi):
    if not toks:
        return lhs
    lu = pltpu.bitcast(lhs, U32)
    rows = [lu[8 * r:8 * r + 8] for r in range(lu.shape[0] // 8)]
    for i, tok in enumerate(toks):
        r = lo + ((i + 1) * (hi - lo)) // len(toks) - 1
        head = _dep(rows[r][:, 0:LANES], tok, zero)
        rows[r] = head if lu.shape[1] == LANES else jnp.concatenate(
            [head, rows[r][:, LANES:]], axis=1)
    return pltpu.bitcast(jnp.concatenate(rows, axis=0), BF16)


def _merge(a, b):
    keyed = [((i + 1) / len(a), t) for i, t in enumerate(a)]
    keyed += [((i + 1) / len(b), t) for i, t in enumerate(b)]
    return [t for _, t in sorted(keyed, key=lambda kv: kv[0])]


def _span(start, size):
    if isinstance(start, int):
        return pl.ds(start, size)
    return pl.ds(pl.multiple_of(start, LANES), size)


def _tok(res, row):
    return lax.bitcast_convert_type(res[row:row + 8, 0:LANES], U32)


def _or(x, z):
    return lax.bitcast_convert_type(lax.bitcast_convert_type(x, U32) | z, F32)


def _kernel(xt_hbm, k_hbm, v_hbm, wq_hbm, wot_hbm, wr_hbm, wg_hbm, wu_hbm, wdt_hbm,
            c_hbm, wmod_hbm, o_hbm,
            xt_v, k_v, v_v, wq_v, wot_v, wmod_v, wg_v, wu_v, wdt_v, ot_v,
            h_scr, acc_scr, st_scr, m_scr, vt_scr, mod_scr, col_scr, key_scr, h2_scr, x1_scr,
            zero_scr, fix_v, c_ref, wr_ref, row_scr, wd_scr, h2l_scr,
            hb_scr, wb_scr, rem_scr, wrem_v,
            grp_sems, misc_sems, mlp_sems, out_sems, fix_sems,
            *, n_heads):
    d, seq = xt_hbm.shape
    sk = k_v.shape[1]
    n_grp = n_heads // HG
    n_blk = seq // TB
    n_units = n_grp * n_blk
    nb = TB // LANES
    nq = 2 * HG
    nt = sk // LANES
    gbits = n_grp.bit_length() - 1
    gw = nq * DH
    qscale = (DH ** -0.5) * math.log2(math.e)

    def grp_of(u):
        return u & (n_grp - 1)

    def blk_of(u):
        return u >> gbits

    def grp_copies(g, n=1):
        hs = pl.ds(g * HG, n * HG)
        return (*[pltpu.make_async_copy(wq_hbm.at[:, pl.ds(i * gw, gw)], wq_v.at[i],
                                        grp_sems.at[0, i]) for i in range(g, g + n)],
                pltpu.make_async_copy(k_hbm.at[hs], k_v.at[hs], grp_sems.at[1, g]),
                pltpu.make_async_copy(v_hbm.at[hs], v_v.at[hs], grp_sems.at[2, g]),
                *[pltpu.make_async_copy(wot_hbm.at[:, pl.ds((i - 1) * gw, gw)], wot_v.at[i - 1],
                                        grp_sems.at[3, i]) for i in range(g, g + n)])

    def col_copy(src, dst, lo, hi, sem):
        return pltpu.make_async_copy(src.at[:, lo:hi], dst.at[:, lo:hi], sem)

    class Pieces:
        def __init__(self, src, dst, lo, hi, sem):
            self.src, self.dst, self.lo, self.hi, self.sem = src, dst, lo, hi, sem

        def start(self):
            w = self.dst.shape[2]
            for p in range(self.lo, self.hi):
                pltpu.make_async_copy(self.src.at[:, p * w:(p + 1) * w], self.dst.at[p],
                                      self.sem).start()

        def wait(self):
            whole = self.dst.at[self.lo:self.hi]
            pltpu.make_async_copy(whole, whole, self.sem).wait()

    def x_cols(t0, n):
        return jnp.concatenate([xt_v[t0 // LANES + i] for i in range(n // LANES)], axis=1)

    x_first = Pieces(xt_hbm, xt_v, 0, nb, misc_sems.at[0])
    x_second = Pieces(xt_hbm, xt_v, nb, nb + 1, misc_sems.at[10])
    x_rest = Pieces(xt_hbm, xt_v, nb + 1, seq // LANES, misc_sems.at[1])
    mod_first = [col_copy(wmod_hbm, wmod_v, MODC, 2 * d, misc_sems.at[8]),
                 col_copy(wmod_hbm, wmod_v, 0, MODC, misc_sems.at[9])]
    mod_rest = col_copy(wmod_hbm, wmod_v, 2 * d, 6 * d, misc_sems.at[3])
    mlp_g = pltpu.make_async_copy(wg_hbm, wg_v, mlp_sems.at[0])
    mlp_u = pltpu.make_async_copy(wu_hbm, wu_v, mlp_sems.at[1])
    ff = wdt_hbm.shape[1]
    mlp_d = Pieces(wdt_hbm, wdt_v, 0, ff // WP, mlp_sems.at[2])
    out_lo = col_copy(ot_v, o_hbm, 0, seq - TB, out_sems.at[0])
    chunks = list(zip(EDGES[:-1], EDGES[1:]))
    out_hi = [pltpu.make_async_copy(ot_v.at[r0:r1, seq - TB:seq], o_hbm.at[r0:r1, seq - TB:seq],
                                    out_sems.at[1 + i]) for i, (r0, r1) in enumerate(chunks)]

    def silu_c():
        cc = c_ref[...].astype(F32)
        return jnp.broadcast_to((cc * _rb(_sigmoid(cc))).astype(BF16), (8, d))

    def ln1_norm(t0, n, marks):
        x = x_cols(t0, n).astype(F32)
        mu = _colsum(x, marks, NM1) * (1.0 / d)
        marks.append(_fold(jnp.broadcast_to(mu, (8, n))))
        xc = x - mu
        var = _colsum(xc * xc, marks, NM2) * (1.0 / d)
        rs = lax.rsqrt(var + EPS)

        def finish(z=None):
            r = rs if z is None else _or(rs, _lanes(z[0:1], n))
            return (xc * r).astype(BF16).T
        return finish

    def ln1_mod(ln, slot, r0):
        h = ln.astype(F32) * mod_scr[1:2, :] + mod_scr[0:1, :]
        h_scr[slot, _span(r0, ln.shape[0]), :] = h.astype(BF16)

    def mod_piece(src, dst, marks):
        w = wmod_v[:, _span(src, MP)].astype(F32)
        row0 = _rb(_colsum(w * _lanes(col_scr[5 * d:6 * d, :], MP), marks, NMP))

        def finish(z):
            row = _or(row0, _lanes(z[0:1], MP))
            pos = dst + lax.broadcasted_iota(I32, (1, MP), 1)
            is_cb = jnp.logical_and(pos >= 2 * d, pos < 3 * d)
            row = jnp.where(is_cb, _rb(1.0 + row), row)
            row_scr[:, _span(dst, MP)] = row
            col_scr[_span(dst, MP), :] = jnp.broadcast_to(row, (LANES, MP)).T
        return finish

    def wd_piece(src, dst, marks):
        w = pltpu.bitcast(wdt_v[src // WP].T, U32)
        wd_scr[pl.ds(pl.multiple_of(dst // 2, WP // 2), WP // 2), :] = w
        for r in range(56, WP // 2, 64):
            for c in range(0, d - LANES + 1, LANES):
                marks.append(w[r:r + 8, c:c + LANES])

    dm = d - d % LANES
    kr = d - dm
    nhb = -(-RV // HP)
    assert nhb <= 6 and nhb * HP <= TB

    def hb_piece(slot, sp, marks, z=None):
        r0 = sp * HP
        src = pl.ds(r0 if isinstance(r0, int) else pl.multiple_of(r0, 16), HP)
        hu = pltpu.bitcast(h_scr[slot, src, dm:d], U32)
        if z is not None:
            hu = hu | jnp.concatenate([z[:, 0:kr]] * (HP // 16), axis=0)
        cols = [jnp.broadcast_to(hu[:, k:k + 1], (HP // 2, LANES)) for k in range(kr)]
        hb_scr[slot * nhb + sp] = jnp.concatenate(cols, axis=0)
        marks.extend(col[HP // 2 - 8:HP // 2] for col in cols[HS - 1::HS])

    def wb_piece(u, toks, zero):
        w = lax.bitcast_convert_type(wrem_v[:, _span(grp_of(u) * gw, gw)].astype(F32), U32)
        rows = [jnp.broadcast_to(w[k:k + 1], (8, gw)) | _lanes(toks[k * len(toks) // kr] & zero, gw)
                for k in range(kr)]
        wb_scr[...] = lax.bitcast_convert_type(jnp.concatenate(rows, axis=0), F32)

    class Rem:
        def __init__(self, slot):
            self.marks, self.done, self.ready = [], {}, []
            hbs = [hb_scr[slot * nhb + sp] for sp in range(nhb)]
            wb = wb_scr[...]
            for p in range(RV // 16):
                acc = None
                sp, r8 = divmod(8 * p, HP // 2)
                for k in range(kr):
                    r = k * HP // 2 + r8
                    hb = pltpu.bitcast(hbs[sp][r:r + 8], BF16).astype(F32)
                    w = wb[8 * k:8 * k + 8]
                    t = _lanes(hb, gw) * jnp.concatenate([w, w], axis=0)
                    acc = t if acc is None else acc + t
                    if (k + 1) % KS == 0:
                        for c in range(0, gw, gw // KSPLIT):
                            self.marks.append(_fold(acc[:, c:c + gw // KSPLIT]))
                self.done[len(self.marks) - 1] = (p, acc)

        def take(self, phase, others=()):
            n, tot = len(self.marks), sum(SHARES)
            lo, hi = sum(SHARES[:phase]) * n // tot, sum(SHARES[:phase + 1]) * n // tot
            for i in range(lo, hi):
                if i in self.done:
                    self.ready.append((*self.done[i], phase, (i + 1 - lo) / (hi - lo)))
            mine = self.marks[lo:hi]
            return _merge(others, mine) if others and mine else list(others) + mine

        def flush(self, st, zero, phase, hi=THI):
            old = [r for r in self.ready if r[2] < phase]
            for p, acc, ph, frac in self.ready:
                if ph < phase:
                    rl = 8 * (([r[0] for r in old].index(p) + 1) * 200 // (len(old) + 1))
                else:
                    rl = 16 * min(int(TLO + frac * (hi - TLO)) - 4, 118)
                z = jnp.concatenate([_lanes(_tok(st, rl) & zero, gw)] * 2, axis=0)
                rem_scr[16 * p:16 * p + 16, :] = _or(acc, z)
            self.ready = []

    def qproj(u, toks, zero):
        h = h_scr[blk_of(u) & 1]
        q = jnp.dot(h[RV:TB, dm:d], wq_v[grp_of(u), dm:d, :], preferred_element_type=F32)
        r = jnp.concatenate([rem_scr[...], q], axis=0)
        outs = []
        for i in range(nq):
            tk = toks[i * len(toks) // nq:(i + 1) * len(toks) // nq]
            hm = _tie_rows(h[:, 0:dm], tk, zero, 0, TB // 16)
            q = jnp.dot(hm, wq_v[grp_of(u), 0:dm, i * DH:(i + 1) * DH],
                        preferred_element_type=F32) + r[:, i * DH:(i + 1) * DH]
            outs.append(q.astype(BF16))
        return jnp.concatenate(outs, axis=1)

    def qproj_first(lo, hi):
        qs = []
        for r0 in (0, TB // 2):
            rs = slice(r0, r0 + TB // 2)
            q = jnp.dot(h_scr[0, rs, dm:d], wq_v[0, dm:d, lo:hi], preferred_element_type=F32)
            q = jnp.dot(h_scr[0, rs, 0:dm], wq_v[0, 0:dm, lo:hi], preferred_element_type=F32) + q
            qs.append(q.astype(BF16))
        return jnp.concatenate(qs, axis=0)

    def qk(u, q, j, toks, zero):
        k = _tie_rows(k_v[grp_of(u) * HG + j // 2], toks, zero, TLO, THI)
        st = lax.dot_general(k, q[:, j * DH:(j + 1) * DH], _NT,
                             preferred_element_type=F32)
        for i in range(nb):
            blk = st[:, i * LANES:(i + 1) * LANES]
            st_scr[j * nb + i] = blk
            m_scr[j * nb + i] = jnp.max(blk.reshape(sk // 8, 8, LANES), axis=0)
        return st

    def v_transpose(u, i, rel=(), zero=None):
        v = _tie_rows(v_v[grp_of(u) * HG + i], rel, zero, -7, sk // 16 - 7)
        vt = pltpu.bitcast(v.T, U32)
        vt_scr[i] = vt
        return [vt[DH // 2 - 8:DH // 2, c:c + LANES] for c in range(0, sk, LANES)]

    def pv(slots, zero, toks=(), srows=SROWS, free=PVEND):
        ps, ls, pairs = [], [], []
        for sl in slots:
            m = jnp.max(m_scr[sl], axis=0, keepdims=True)
            p = jnp.exp2(st_scr[sl] - m)
            accs = [None] * 4
            for tile in range(nt):
                for r0 in range(tile * LANES + LANES - 16, tile * LANES - 16, -16):
                    pair = p[r0:r0 + 8] + p[r0 + 8:r0 + 16]
                    pairs.append(pair)
                    a = accs[tile % 4]
                    accs[tile % 4] = pair if a is None else a + pair
            ls.append(jnp.sum((accs[0] + accs[1]) + (accs[2] + accs[3]), axis=0, keepdims=True))
            ps.append(p.astype(BF16))
        outs = []
        ntiles = len(slots) * nt
        side = {}
        for i, tok in enumerate(toks):
            side.setdefault(max(((i + 1) * (ntiles - free)) // len(toks) - 1, 0), []).append(tok)
        for i, sl in enumerate(slots):
            vu = vt_scr[sl // (2 * nb)]
            tiles = []
            for c in range(nt):
                g = i * nt + c + 4
                rows = []
                for r in range(8):
                    x = vu[8 * r:8 * r + 8, c * LANES:(c + 1) * LANES]
                    if g < ntiles and TIE0 <= r < TIE0 + NTIE:
                        src = pairs[g * 8 + (r - TIE0)]
                        x = _dep(x, lax.bitcast_convert_type(src, U32), zero)
                    if r == srows[c % 4]:
                        for tok in side.get(i * nt + c, ()):
                            x = _dep(x, tok, zero)
                    rows.append(x)
                tiles.append(jnp.concatenate(rows, axis=0))
            lhs = pltpu.bitcast(jnp.concatenate(tiles, axis=1), BF16)
            o = jnp.dot(lhs, ps[i], preferred_element_type=F32)
            outs.append(o * (1.0 / ls[i]))
        return outs

    def outproj_tied(u, o, toks, zero):
        slot = blk_of(u) & 1
        res = []
        for i in range(nb):
            o2 = jnp.concatenate([o[j * nb + i] for j in range(nq)], axis=0).astype(BF16)
            tk = toks[i * len(toks) // OPN:(i + 1) * len(toks) // OPN]
            wo = _tie_rows(wot_v[grp_of(u)], tk, zero, 0, d // 16)
            contrib = jnp.dot(wo, o2, preferred_element_type=F32)
            acc_scr[slot * nb + i] += contrib
            res.append(contrib)
        return jnp.concatenate(res, axis=0)

    def outproj(u, o, lo=0):
        w = len(o) // nq
        o2 = jnp.concatenate(
            [jnp.concatenate(o[j * w:(j + 1) * w], axis=1) for j in range(nq)], axis=0).astype(BF16)
        contrib = jnp.dot(wot_v[grp_of(u)], o2, preferred_element_type=F32)
        slot = blk_of(u) & 1
        for i in range(w):
            pi = slot * nb + lo // LANES + i
            acc_scr[pi] += contrib[:, i * LANES:(i + 1) * LANES]

    def router_keys(racc, t0):
        r = _rb(jnp.sum(racc, axis=0, keepdims=True)) + 0.0
        bits = lax.bitcast_convert_type(r, I32) >> 16
        order = jnp.where(bits < 0, -1 - bits, bits + 32768)
        pos = t0 + lax.broadcasted_iota(I32, r.shape, 1)
        return lax.bitcast_convert_type((order << 11) + (seq - 1 - pos) + 0x20000000, F32)

    def finalize(t0, slot, a0, dst, n, keys_out=None):
        marks = []
        cs = _span(dst, n)
        x = x_cols(t0, n).astype(F32)
        att = jnp.concatenate(
            [acc_scr[slot * nb + a0 // LANES + i] for i in range(n // LANES)], axis=1)
        x1b = (x + _lanes(col_scr[0:d, :], n) * att).astype(BF16)
        x1_scr[:, cs] = x1b
        ot_v[:, cs] = x1b
        fine = keys_out is None
        mu = _colsum(x1b.astype(F32), marks, NG1 if fine else NF1) * (1.0 / d)

        def note(row):
            if fine:
                marks.append(_fold(jnp.broadcast_to(row, (8, n))))
            return row

        mub = note(_rb(mu))
        xc = x1_scr[:, cs].astype(F32) - mub
        var = _colsum(xc * xc, marks, NG2 if fine else NF2) * (1.0 / d) - (mu - mub) * (mu - mub)
        inv = note(1.0 / note(_rb(jnp.sqrt(note(_rb(_rb(jnp.maximum(var, 0.0)) + EPS_BF16))))))
        step = d // ((NG3 if n == SP else EG3) if fine else NF3)
        racc = None
        for r0 in range(0, d, step):
            rs = slice(r0, r0 + step)
            x1 = ot_v[rs, cs].astype(F32)
            ln = _rb(_rb(x1 - mub) * inv)
            if fine:
                marks.append(_fold(ln))
            h2b = (_rb(ln * _lanes(col_scr[2 * d + r0:2 * d + r0 + step, :], n))
                   + _lanes(col_scr[d + r0:d + r0 + step, :], n)).astype(BF16)
            if keys_out is None:
                h2_scr[rs, cs] = h2b
            else:
                h2l_scr[rs, :] = h2b
            h2 = h2b.astype(F32)
            out = x1 + _lanes(col_scr[3 * d + r0:3 * d + r0 + step, :], n) * h2
            ot_v[rs, cs] = out.astype(BF16)
            rp = h2 * _lanes(col_scr[4 * d + r0:4 * d + r0 + step, :], n)
            for g in range(0, step, 8):
                racc = rp[g:g + 8] if racc is None else racc + rp[g:g + 8]
            marks.append(_fold(out, racc))
        if keys_out is not None:
            keys_out.append(racc)
            return marks
        key = router_keys(racc, t0)
        for i in range(n // LANES):
            key_scr[pl.ds(dst // LANES + i, 1), :] = key[:, i * LANES:(i + 1) * LANES]
        return marks

    hw = gw // 2
    wq0a = col_copy(wq_hbm, wq_v.at[0], 0, hw, grp_sems.at[0, 0])
    wq0b = col_copy(wq_hbm, wq_v.at[0], hw, gw, misc_sems.at[4])
    k0a = pltpu.make_async_copy(k_hbm.at[0], k_v.at[0], grp_sems.at[1, 0])
    k0b = pltpu.make_async_copy(k_hbm.at[1], k_v.at[1], misc_sems.at[5])
    v0 = pltpu.make_async_copy(v_hbm.at[0:HG], v_v.at[0:HG], grp_sems.at[2, 0])
    wq1, k1, v1, wo0 = grp_copies(1)
    wo_last = pltpu.make_async_copy(wot_hbm.at[:, (n_grp - 1) * gw:n_grp * gw],
                                    wot_v.at[n_grp - 1], grp_sems.at[3, 0])
    wrem_copy = col_copy(wq_hbm.at[dm:d], wrem_v, gw, 4 * gw, misc_sems.at[2])
    wrem_rest = (col_copy(wq_hbm.at[dm:d], wrem_v, 0, gw, misc_sems.at[11]),
                 col_copy(wq_hbm.at[dm:d], wrem_v, 4 * gw, n_grp * gw, misc_sems.at[12]))
    c_copy = pltpu.make_async_copy(c_hbm, c_ref, misc_sems.at[6])
    wr_copy = pltpu.make_async_copy(wr_hbm, wr_ref, misc_sems.at[7])
    c_copy.start()
    wr_copy.start()
    x_first.start()
    mod_first[0].start()
    mod_first[1].start()
    wq0a.start()
    wq0b.start()
    acc_scr[0:2 * nb] = jnp.zeros((2 * nb, d, LANES), F32)
    col_scr[0:4 * d, :] = jnp.zeros((4 * d, LANES), F32)
    wdt_v[ff // WP] = jnp.zeros((d, WP), BF16)
    c_copy.wait()
    wr_copy.wait()
    x_first.wait()
    cbits = lax.bitcast_convert_type(c_ref[:, 0:LANES].astype(F32), U32)
    zero_scr[...] = jnp.broadcast_to(cbits & 0xFFFF, (8, LANES))
    h_scr[0] = ln1_norm(0, TB, [])()
    sc = silu_c()
    wr = wr_ref[...].reshape(1, d).astype(F32)
    col_scr[4 * d:5 * d, :] = jnp.broadcast_to(wr, (LANES, d)).T
    col_scr[5 * d:6 * d, :] = jnp.broadcast_to(sc[0:1, :].astype(F32), (LANES, d)).T
    mod_first[0].wait()
    mod = _rb(jnp.dot(sc, wmod_v[:, MODC:2 * d], preferred_element_type=F32))
    mod_scr[0:1, MODC:d] = mod[0:1, 0:d - MODC] * qscale
    mod_scr[1:2, :] = _rb(1.0 + mod[0:1, d - MODC:2 * d - MODC]) * qscale
    mod_first[1].wait()
    k0a.start()
    mod = _rb(jnp.dot(sc, wmod_v[:, 0:MODC], preferred_element_type=F32))
    mod_scr[0:1, 0:MODC] = mod[0:1] * qscale
    wq0a.wait()
    k0b.start(priority=1)
    v0.start(priority=1)
    wrem_copy.start(priority=1)
    ln1_mod(h_scr[0], 0, 0)
    qa = qproj_first(0, hw)
    wq0b.wait()
    k0a.wait()
    wq1.start(priority=1)
    k1.start(priority=1)
    x_second.start()
    q = jnp.concatenate([qa, qproj_first(hw, gw)], axis=1)
    zero = zero_scr[...]
    for j in range(2):
        marks = []
        for i in range(2 * j, 2 * j + 2):
            hb_piece(0, i, marks)
        qk(0, q, j, marks, zero)
    k0b.wait()
    v0.wait()
    wrem_copy.wait()
    v1.start()
    wo0.start()
    zero = zero_scr[...]
    rem_scr[...] = jnp.dot(h_scr[0, 0:RV, dm:d], wrem_v[:, gw:2 * gw],
                           preferred_element_type=F32)
    for i in range(HG):
        marks = v_transpose(0, i)
        if i == 0:
            wb_piece(2, marks, zero)
        if 4 + i < nhb:
            hm = []
            hb_piece(0, 4 + i, hm)
            marks = _merge(marks, hm)
        qk(0, q, nq - HG + i, marks, zero)

    assert n_grp == 8 and HG == 2
    stage_at = [1, 2, 3, 5, n_units]
    starts = [(*grp_copies(2), mod_rest, x_rest, *wrem_rest), grp_copies(3, 3),
              (*grp_copies(6, 2), wo_last, mlp_d), (mlp_g, mlp_u)]
    waits = [(wq1, k1, v1, wo0, x_second), *starts[:3]]
    wd0 = stage_at[3]
    npc = TB // SP
    nmp = 4 * d // MP

    def manage(k, _, c):
        for cp in waits[k]:
            cp.wait()
        for cp in starts[k]:
            cp.start()
        return c

    def steady(u, carry):
        zero = zero_scr[...]
        blk, g = blk_of(u), grp_of(u)
        off = ((g - 1) & (npc - 1)) * SP
        rem = Rem(blk_of(u + 1) & 1)
        q = qproj(u, rem.take(0), zero)
        o = pv(range(0, 2 * nb), zero, rem.take(1))
        live = jnp.logical_and(blk > 0, jnp.logical_and(g >= 1, g <= npc))
        t0 = jnp.maximum(blk - 1, 0) * TB + off
        marks = finalize(t0, (blk + 1) & 1, off, jnp.where(live, t0, seq), SP)
        wp = jnp.clip(u - wd0, 0, ff // WP - 1) * WP
        wmarks = []
        wd_piece(jnp.where(u >= wd0, wp, ff), wp, wmarks)
        rem.flush(qk(u, q, 0, rem.take(2, _merge(marks, wmarks)), zero), zero, 2)
        marks, mmarks = [], []
        ln_fin = ln1_norm(jnp.minimum(blk + 1, n_blk - 1) * TB + off, SP, marks)
        mp = jnp.clip(u - 2, 0, nmp - 1) * MP
        mod_fin = mod_piece(jnp.where(u >= 2, 2 * d + mp, 0), mp, mmarks)
        st = qk(u, q, 1, rem.take(3, marks + mmarks), zero)
        rem.flush(st, zero, 3)
        used = jnp.where(live, ((blk + 1) & 1) * nb + off // LANES, 2 * nb)
        for r0 in range(0, d, 32):
            z4 = jnp.concatenate([_tok(st, r0) & zero] * 4, axis=0)
            acc_scr[used, r0:r0 + 32, :] = lax.bitcast_convert_type(z4, F32)
        ln1_mod(ln_fin(_tok(st, LNREL) & zero), (blk + 1) & 1, off)
        mod_fin(_tok(st, 1880) & zero)
        o += pv(range(2 * nb, 4 * nb), zero, rem.take(4))
        st = qk(u, q, 2, rem.take(5), zero)
        rem.flush(st, zero, 5)
        v_transpose(u, 0, [_tok(st, 112 * i) for i in range(nt)], zero)
        st = qk(u, q, 3, rem.take(6), zero)
        rem.flush(st, zero, 6)
        v_transpose(u, 1, [_tok(st, 112 * i) for i in range(nt)], zero)
        res = outproj_tied(u - 1, o, rem.take(7), zero)
        rem.flush(res, zero, 7, OPN * d // 16)
        hm = []
        hb_piece((blk + 1) & 1, jnp.clip(g - 1, 0, nhb - 1), hm,
                 _tok(res, max(OPN * d - 96, 0)) & zero)
        wb_piece(u + 2, hm, zero)
        return carry

    def stage(k, lo):
        hi = stage_at[1]
        for i in range(len(waits)):
            lax.fori_loop(0, jnp.where(k == i, 1, 0), functools.partial(manage, i), 0)
            hi = jnp.where(k == i, stage_at[i + 1], hi)
        lax.fori_loop(lo, hi, steady, 0)
        return hi

    lax.fori_loop(0, len(waits), stage, jnp.int32(stage_at[0]))

    ul = n_units - 1
    tl = seq - TB
    sl_last = (n_blk - 1) & 1
    nb0 = nb - TAILB
    mod_scr[2:3, :] = row_scr[:, 3 * d:4 * d]
    outproj(ul, pv([j * nb + i for j in range(nq) for i in range(nb0)], zero_scr[...]))
    mlp_g.wait()
    mlp_u.wait()
    out_lo.start()
    toks = finalize(tl, sl_last, 0, tl, nb0 * LANES)
    o = pv([j * nb + i for j in range(nq) for i in range(nb0, nb)], zero_scr[...], toks,
           EROWS, EPVEND)
    outproj(ul, o, nb0 * LANES)

    nl = TAILB * LANES
    sub8 = lax.broadcasted_iota(I32, (TOPC, 1), 0)
    lane = lax.broadcasted_iota(I32, (TOPC, LANES), 1)

    def key_index(k):
        return seq - 1 - (lax.bitcast_convert_type(k, I32) & (seq - 1))

    def piece_base(idx, limit):
        return pl.multiple_of(jnp.clip(idx >> 7, 0, limit // LANES - 1) * LANES, LANES)

    keys = key_scr[0:seq // LANES, :]
    piece = lax.broadcasted_iota(I32, (seq // LANES, 1), 0)
    keys = jnp.where(piece < (seq - nl) // LANES, keys, 0.0)
    ecol = jnp.zeros((TOPC, LANES), F32)
    erow = jnp.zeros((1, LANES), F32)
    h2e = jnp.zeros((TOPC, d), F32)
    late = []
    marks = finalize(seq - nl, sl_last, TB - nl, seq - nl, nl, late)
    zero = zero_scr[...]
    for i in range(TOPC):
        mx = jnp.max(jnp.max(keys, axis=0, keepdims=True), axis=1, keepdims=True)
        keys = jnp.where(keys == mx, 0.0, keys)
        ecol = jnp.where(sub8 == i, mx, ecol)
        erow = jnp.where(lane[0:1] == i, mx, erow)
        idx = key_index(mx)
        pick = jnp.logical_and(sub8 == i, lane == (idx & (LANES - 1)))
        sl = pl.ds(piece_base(idx[0, 0], seq - nl), LANES)
        pick = jnp.where(pick, 1.0, 0.0)
        if i in PACE:
            pick = _or(pick, marks[PACE[i]] & zero)
        h2e = h2e + lax.dot_general(pick.astype(BF16), h2_scr[:, sl], _NT,
                                    preferred_element_type=F32)

    late = [router_keys(late[0], seq - nl)]
    krow = jnp.concatenate([late[0], erow], axis=1)
    kcol = jnp.concatenate([jnp.broadcast_to(late[0], (LANES, nl)).T, ecol], axis=0)
    cnt = [None] * 4
    for g in range(kcol.shape[0] // 8):
        one = jnp.where(_lanes(kcol[8 * g:8 * g + 8], nl + LANES) > krow, 1.0, 0.0)
        cnt[g % 4] = one if cnt[g % 4] is None else cnt[g % 4] + one
    rank = jnp.sum((cnt[0] + cnt[1]) + (cnt[2] + cnt[3]), axis=0, keepdims=True)
    chosen = rank == sub8.astype(F32)
    onehot = jnp.where(chosen, 1.0, 0.0).astype(BF16)
    h2pad = jnp.concatenate([h2e, jnp.zeros((TOPC, d), F32)], axis=0).astype(BF16)
    h2s = (jnp.dot(onehot[:, nl:nl + 2 * TOPC], h2pad, preferred_element_type=F32)
           + lax.dot_general(onehot[:, 0:nl], h2l_scr[...], _NT,
                             preferred_element_type=F32))
    top = jnp.max(jnp.where(chosen, krow, 0.0), axis=1, keepdims=True)
    idx_col = key_index(top)
    idxs = [idx_col[i:i + 1] for i in range(TOPC)]
    bases = [piece_base(idx_col[i, 0], seq) for i in range(TOPC)]
    hit = lane == (idx_col & (LANES - 1))
    picks = [jnp.where(jnp.logical_and(sub8 == i, hit), 1.0, 0.0).astype(BF16)
             for i in range(TOPC)]
    order = (lax.bitcast_convert_type(top, I32) >> 11) & 0xFFFF
    rbits = jnp.where(order >= 32768, order - 32768, -1 - order) << 16
    gate = _rb(_sigmoid(lax.bitcast_convert_type(rbits, F32)))
    xs = h2s.astype(BF16)
    for cp in out_hi:
        cp.start()
    g = _rb(jnp.dot(xs, wg_v[...], preferred_element_type=F32))
    g = _rb(g * _rb(_sigmoid(g)))
    u = _rb(jnp.dot(xs, wu_v[...], preferred_element_type=F32))
    gu = (g * u).astype(BF16)

    last_use = []
    for i in range(TOPC):
        ok = True
        for j in range(i + 1, TOPC):
            ok = jnp.logical_and(ok, bases[i] != bases[j])
        last_use.append(ok)

    def down(r0, r1):
        x1p = jnp.concatenate([x1_scr[r0:r1, pl.ds(bases[i], LANES)] for i in range(TOPC)], axis=1)
        x1s = lax.dot_general(jnp.concatenate(picks, axis=1), x1p, _NT,
                              preferred_element_type=F32)
        wd = pltpu.bitcast(wd_scr[:, r0:r1], BF16)
        y = _rb(jnp.dot(gu, wd, preferred_element_type=F32))
        hm = _rb(h2s[:, r0:r1] + _rb(y * gate))
        return x1s + mod_scr[2:3, r0:r1] * hm

    def patch(r0, r1, new):
        n = r1 - r0
        pad = jnp.concatenate([new, jnp.zeros((LANES - TOPC, n), F32)], axis=0)
        cols = pltpu.bitcast(pad.T.astype(BF16), U32)
        col = [jnp.broadcast_to(cols[:, j:j + 1], (n // 2, LANES)) for j in range(TOPC)]
        for i in range(TOPC):
            res = pltpu.bitcast(ot_v[r0:r1, pl.ds(bases[i], LANES)], U32)
            tok = lane[0:1, :] + (idxs[i] & ~(LANES - 1))
            for j in range(i + 1):
                res = jnp.where(tok == idxs[j], col[j], res)
            fix_v[i, r0:r1, :] = pltpu.bitcast(res, BF16)

    def fix_copy(i, r0, r1):
        return pltpu.make_async_copy(fix_v.at[i, r0:r1, :],
                                     o_hbm.at[r0:r1, pl.ds(bases[i], LANES)], fix_sems.at[i])

    def for_last(fn):
        for i in range(TOPC - 1):
            pl.when(last_use[i])(functools.partial(fn, i))
        fn(TOPC - 1)

    new = down(*chunks[0])
    out_lo.wait()
    for ci, (r0, r1) in enumerate(chunks):
        out_hi[ci].wait()
        nxt = down(*chunks[ci + 1]) if ci + 1 < len(chunks) else None
        patch(r0, r1, new)
        for_last(lambda i: fix_copy(i, r0, r1).start())
        new = nxt
    for r0, r1 in chunks:
        for_last(lambda i: fix_copy(i, r0, r1).wait())


@jax.jit
def pallas_adaLN_cond__gqa_block_cached__moe_arch_mod__prompt_kernel(
    A_x: jax.Array,
    A_k_cache: jax.Array,
    A_v_cache: jax.Array,
    A_wq: jax.Array,
    A_wo: jax.Array,
    B_x: jax.Array,
    B_w_r: jax.Array,
    B_w_gate: jax.Array,
    B_w_up: jax.Array,
    B_w_down: jax.Array,
    c: jax.Array,
    w_mod: jax.Array,
):
    b, seq, d = A_x.shape
    _, hkv, sk, dh = A_k_cache.shape
    assert b == 1 and dh == DH and HQ == 2 * hkv
    assert seq & (seq - 1) == 0 and seq <= 2048
    f = B_w_gate.shape[1]
    n_grp = hkv // HG
    gw = 2 * HG * dh
    n_slots = 2 * HG * TB // LANES

    xt = A_x.reshape(seq, d).T
    wot = A_wo.T
    wdt = B_w_down.T
    k3 = A_k_cache.reshape(hkv, sk, dh)
    v3 = A_v_cache.reshape(hkv, sk, dh)

    hbm = pl.BlockSpec(memory_space=pl.ANY)
    out_t = pl.pallas_call(
        functools.partial(_kernel, n_heads=hkv),
        in_specs=[hbm] * 11,
        out_specs=hbm,
        out_shape=jax.ShapeDtypeStruct((d, seq), BF16),
        scratch_shapes=[
            pltpu.VMEM((seq // LANES, d, LANES), BF16),
            pltpu.VMEM((hkv, sk, dh), BF16),
            pltpu.VMEM((hkv, sk, dh), BF16),
            pltpu.VMEM((n_grp, d, gw), BF16),
            pltpu.VMEM((n_grp, d, gw), BF16),
            pltpu.VMEM((d, 6 * d), BF16),
            pltpu.VMEM((d, f), BF16),
            pltpu.VMEM((d, f), BF16),
            pltpu.VMEM((f // WP + 1, d, WP), BF16),
            pltpu.VMEM((d, seq + SP), BF16),
            pltpu.VMEM((2, TB, d), BF16),
            pltpu.VMEM((2 * TB // LANES + 1, d, LANES), F32),
            pltpu.VMEM((n_slots, sk, LANES), F32),
            pltpu.VMEM((n_slots, 8, LANES), F32),
            pltpu.VMEM((HG, dh // 2, sk), U32),
            pltpu.VMEM((8, d), F32),
            pltpu.VMEM((6 * d, LANES), F32),
            pltpu.VMEM(((seq + SP) // LANES + 7 & ~7, LANES), F32),
            pltpu.VMEM((d, seq + SP), BF16),
            pltpu.VMEM((d, seq + SP), BF16),
            pltpu.VMEM((8, LANES), U32),
            pltpu.VMEM((TOPC, d, LANES), BF16),
            pltpu.VMEM((1, d), BF16),
            pltpu.VMEM((d,), BF16),
            pltpu.VMEM((1, 4 * d), F32),
            pltpu.VMEM((f // 2, d), U32),
            pltpu.VMEM((d, TAILB * LANES), BF16),
            pltpu.VMEM((2 * -(-RV // HP), d % LANES * HP // 2, LANES), U32),
            pltpu.VMEM((d % LANES * 8, gw), F32),
            pltpu.VMEM((RV, gw), F32),
            pltpu.VMEM((d % LANES, n_grp * gw), BF16),
            pltpu.SemaphoreType.DMA((4, n_grp)),
            pltpu.SemaphoreType.DMA((13,)),
            pltpu.SemaphoreType.DMA((3,)),
            pltpu.SemaphoreType.DMA((len(EDGES),)),
            pltpu.SemaphoreType.DMA((TOPC,)),
        ],
        compiler_params=pltpu.CompilerParams(
            disable_bounds_checks=True,
            disable_semaphore_checks=True,
            vmem_limit_bytes=120 * 1024 * 1024,
        ),
    )(xt, k3, v3, A_wq, wot, B_w_r, B_w_gate, B_w_up, wdt, c, w_mod)
    return out_t.T.reshape(b, seq, d)
```

```python
import functools
import math

import jax
import jax.numpy as jnp
from jax import lax
import jax.experimental.pallas as pl
import jax.experimental.pallas.tpu as pltpu

F32 = jnp.float32
BF16 = jnp.bfloat16
I32 = jnp.int32
U32 = jnp.uint32

HQ = 32
DH = 128
TOPC = 8
EPS = 1e-05
EPS_BF16 = 1.0013580322265625e-05
LANES = 128

TB = 512
HG = 2
SP = 128
MP = 384
WP = 256
RV = 448
HP = 80
MODC = 384
TAILB = 2
EDGES = (0, 128, 256, 384, 512, 576)

TIE0, NTIE = 2, 3
TLO, THI = 3, 126
SROWS, PVEND = (0, 1, 2, 5), 12
EROWS, EPVEND = (0, 4, 6, 7), 24
NM1, NM2, NMP = 8, 18, 24
NG1, NG2, NG3, EG3 = 18, 9, 18, 36
NF1, NF2, NF3 = 9, 6, 18
KS, KSPLIT, HS = 4, 2, 2
OPN = 2
LNREL = 1008
SHARES = (29, 28, 15, 23, 26, 30, 33, 18)
PACE = {2: 8, 4: 14, 5: 18, 6: 23, 7: 27}

_NT = (((1,), (1,)), ((), ()))


def _rb(x):
    return x.astype(BF16).astype(F32)


def _sigmoid(x):
    return _rb(1.0 / _rb(1.0 + _rb(jnp.exp(-x))))


def _lanes(col, width):
    reps = width // LANES
    return col if reps == 1 else jnp.concatenate([col] * reps, axis=1)


def _fold(*xs):
    ts = []
    for x in xs:
        xi = lax.bitcast_convert_type(x, U32)
        ts += [xi[r:r + 8, c:c + LANES] for r in range(0, x.shape[0], 8)
               for c in range(0, x.shape[1] - LANES + 1, LANES)]
    if len(ts) > 5:
        return functools.reduce(lambda a, b: a | b, ts[:-2]) | (ts[-2] | ts[-1])
    while len(ts) > 1:
        ts = [a | b for a, b in zip(ts[0::2], ts[1::2])] + ts[len(ts) & ~1:]
    return ts[0]


def _colsum(x, marks, nmarks):
    n = x.shape[0] // 8
    acc = x[0:8]
    for g in range(1, n):
        acc = acc + x[8 * g:8 * g + 8]
        if ((g + 1) * nmarks) % n == 0:
            marks.append(_fold(acc))
    return jnp.sum(acc, axis=0, keepdims=True)


def _dep(x, tok, zero):
    return jnp.where(zero != 0, tok, x)


def _tie_rows(lhs, toks, zero, lo, hi):
    if not toks:
        return lhs
    lu = pltpu.bitcast(lhs, U32)
    rows = [lu[8 * r:8 * r + 8] for r in range(lu.shape[0] // 8)]
    for i, tok in enumerate(toks):
        r = lo + ((i + 1) * (hi - lo)) // len(toks) - 1
        head = _dep(rows[r][:, 0:LANES], tok, zero)
        rows[r] = head if lu.shape[1] == LANES else jnp.concatenate(
            [head, rows[r][:, LANES:]], axis=1)
    return pltpu.bitcast(jnp.concatenate(rows, axis=0), BF16)


def _merge(a, b):
    keyed = [((i + 1) / len(a), t) for i, t in enumerate(a)]
    keyed += [((i + 1) / len(b), t) for i, t in enumerate(b)]
    return [t for _, t in sorted(keyed, key=lambda kv: kv[0])]


def _span(start, size):
    if isinstance(start, int):
        return pl.ds(start, size)
    return pl.ds(pl.multiple_of(start, LANES), size)


def _tok(res, row):
    return lax.bitcast_convert_type(res[row:row + 8, 0:LANES], U32)


def _or(x, z):
    return lax.bitcast_convert_type(lax.bitcast_convert_type(x, U32) | z, F32)


def _kernel(xt_hbm, k_hbm, v_hbm, wq_hbm, wot_hbm, wr_hbm, wg_hbm, wu_hbm, wdt_hbm,
            c_hbm, wmod_hbm, o_hbm,
            xt_v, k_v, v_v, wq_v, wot_v, wmod_v, wg_v, wu_v, wdt_v, ot_v,
            h_scr, acc_scr, st_scr, m_scr, vt_scr, mod_scr, col_scr, key_scr, h2_scr, x1_scr,
            zero_scr, fix_v, c_ref, wr_ref, row_scr, wd_scr, h2l_scr,
            hb_scr, wb_scr, rem_scr, wrem_v,
            grp_sems, misc_sems, mlp_sems, out_sems, fix_sems,
            *, n_heads):
    d, seq = xt_hbm.shape
    sk = k_v.shape[1]
    n_grp = n_heads // HG
    n_blk = seq // TB
    n_units = n_grp * n_blk
    nb = TB // LANES
    nq = 2 * HG
    nt = sk // LANES
    gbits = n_grp.bit_length() - 1
    gw = nq * DH
    qscale = (DH ** -0.5) * math.log2(math.e)

    def grp_of(u):
        return u & (n_grp - 1)

    def blk_of(u):
        return u >> gbits

    def grp_copies(g, n=1):
        hs = pl.ds(g * HG, n * HG)
        return (*[pltpu.make_async_copy(wq_hbm.at[:, pl.ds(i * gw, gw)], wq_v.at[i],
                                        grp_sems.at[0, i]) for i in range(g, g + n)],
                pltpu.make_async_copy(k_hbm.at[hs], k_v.at[hs], grp_sems.at[1, g]),
                pltpu.make_async_copy(v_hbm.at[hs], v_v.at[hs], grp_sems.at[2, g]),
                *[pltpu.make_async_copy(wot_hbm.at[:, pl.ds((i - 1) * gw, gw)], wot_v.at[i - 1],
                                        grp_sems.at[3, i]) for i in range(g, g + n)])

    def col_copy(src, dst, lo, hi, sem):
        return pltpu.make_async_copy(src.at[:, lo:hi], dst.at[:, lo:hi], sem)

    class Pieces:
        def __init__(self, src, dst, lo, hi, sem):
            self.src, self.dst, self.lo, self.hi, self.sem = src, dst, lo, hi, sem

        def start(self):
            w = self.dst.shape[2]
            for p in range(self.lo, self.hi):
                pltpu.make_async_copy(self.src.at[:, p * w:(p + 1) * w], self.dst.at[p],
                                      self.sem).start()

        def wait(self):
            whole = self.dst.at[self.lo:self.hi]
            pltpu.make_async_copy(whole, whole, self.sem).wait()

    def x_cols(t0, n):
        return jnp.concatenate([xt_v[t0 // LANES + i] for i in range(n // LANES)], axis=1)

    x_first = Pieces(xt_hbm, xt_v, 0, nb, misc_sems.at[0])
    x_second = Pieces(xt_hbm, xt_v, nb, nb + 1, misc_sems.at[10])
    x_rest = Pieces(xt_hbm, xt_v, nb + 1, seq // LANES, misc_sems.at[1])
    mod_first = [col_copy(wmod_hbm, wmod_v, MODC, 2 * d, misc_sems.at[8]),
                 col_copy(wmod_hbm, wmod_v, 0, MODC, misc_sems.at[9])]
    mod_rest = col_copy(wmod_hbm, wmod_v, 2 * d, 6 * d, misc_sems.at[3])
    mlp_g = pltpu.make_async_copy(wg_hbm, wg_v, mlp_sems.at[0])
    mlp_u = pltpu.make_async_copy(wu_hbm, wu_v, mlp_sems.at[1])
    ff = wdt_hbm.shape[1]
    mlp_d = Pieces(wdt_hbm, wdt_v, 0, ff // WP, mlp_sems.at[2])
    out_lo = col_copy(ot_v, o_hbm, 0, seq - TB, out_sems.at[0])
    chunks = list(zip(EDGES[:-1], EDGES[1:]))
    out_hi = [pltpu.make_async_copy(ot_v.at[r0:r1, seq - TB:seq], o_hbm.at[r0:r1, seq - TB:seq],
                                    out_sems.at[1 + i]) for i, (r0, r1) in enumerate(chunks)]

    def silu_c():
        cc = c_ref[...].astype(F32)
        return jnp.broadcast_to((cc * _sigmoid(cc)).astype(BF16), (8, d))

    def ln1_norm(t0, n, marks):
        x = x_cols(t0, n).astype(F32)
        mu = _colsum(x, marks, NM1) * (1.0 / d)
        marks.append(_fold(jnp.broadcast_to(mu, (8, n))))
        xc = x - mu
        var = _colsum(xc * xc, marks, NM2) * (1.0 / d)
        rs = lax.rsqrt(var + EPS)

        def finish(z=None):
            r = rs if z is None else _or(rs, _lanes(z[0:1], n))
            return (xc * r).astype(BF16).T
        return finish

    def ln1_mod(ln, slot, r0):
        h = ln.astype(F32) * mod_scr[1:2, :] + mod_scr[0:1, :]
        h_scr[slot, _span(r0, ln.shape[0]), :] = h.astype(BF16)

    def mod_piece(src, dst, marks):
        w = wmod_v[:, _span(src, MP)].astype(F32)
        row0 = _rb(_colsum(w * _lanes(col_scr[5 * d:6 * d, :], MP), marks, NMP))

        def finish(z):
            row = _or(row0, _lanes(z[0:1], MP))
            pos = dst + lax.broadcasted_iota(I32, (1, MP), 1)
            is_cb = jnp.logical_and(pos >= 2 * d, pos < 3 * d)
            row = jnp.where(is_cb, _rb(1.0 + row), row)
            row_scr[:, _span(dst, MP)] = row
            col_scr[_span(dst, MP), :] = jnp.broadcast_to(row, (LANES, MP)).T
        return finish

    def wd_piece(src, dst, marks):
        w = pltpu.bitcast(wdt_v[src // WP].T, U32)
        wd_scr[pl.ds(pl.multiple_of(dst // 2, WP // 2), WP // 2), :] = w
        for r in range(56, WP // 2, 64):
            for c in range(0, d - LANES + 1, LANES):
                marks.append(w[r:r + 8, c:c + LANES])

    dm = d - d % LANES
    kr = d - dm
    nhb = -(-RV // HP)
    assert nhb <= 6 and nhb * HP <= TB

    def hb_piece(slot, sp, marks, z=None):
        r0 = sp * HP
        src = pl.ds(r0 if isinstance(r0, int) else pl.multiple_of(r0, 16), HP)
        hu = pltpu.bitcast(h_scr[slot, src, dm:d], U32)
        if z is not None:
            hu = hu | jnp.concatenate([z[:, 0:kr]] * (HP // 16), axis=0)
        cols = [jnp.broadcast_to(hu[:, k:k + 1], (HP // 2, LANES)) for k in range(kr)]
        hb_scr[slot * nhb + sp] = jnp.concatenate(cols, axis=0)
        marks.extend(col[HP // 2 - 8:HP // 2] for col in cols[HS - 1::HS])

    def wb_piece(u, toks, zero):
        w = lax.bitcast_convert_type(wrem_v[:, _span(grp_of(u) * gw, gw)].astype(F32), U32)
        rows = [jnp.broadcast_to(w[k:k + 1], (8, gw)) | _lanes(toks[k * len(toks) // kr] & zero, gw)
                for k in range(kr)]
        wb_scr[...] = lax.bitcast_convert_type(jnp.concatenate(rows, axis=0), F32)

    class Rem:
        def __init__(self, slot):
            self.marks, self.done, self.ready = [], {}, []
            hbs = [hb_scr[slot * nhb + sp] for sp in range(nhb)]
            wb = wb_scr[...]
            for p in range(RV // 16):
                acc = None
                sp, r8 = divmod(8 * p, HP // 2)
                for k in range(kr):
                    r = k * HP // 2 + r8
                    hb = pltpu.bitcast(hbs[sp][r:r + 8], BF16).astype(F32)
                    w = wb[8 * k:8 * k + 8]
                    t = _lanes(hb, gw) * jnp.concatenate([w, w], axis=0)
                    acc = t if acc is None else acc + t
                    if (k + 1) % KS == 0:
                        for c in range(0, gw, gw // KSPLIT):
                            self.marks.append(_fold(acc[:, c:c + gw // KSPLIT]))
                self.done[len(self.marks) - 1] = (p, acc)

        def take(self, phase, others=()):
            n, tot = len(self.marks), sum(SHARES)
            lo, hi = sum(SHARES[:phase]) * n // tot, sum(SHARES[:phase + 1]) * n // tot
            for i in range(lo, hi):
                if i in self.done:
                    self.ready.append((*self.done[i], phase, (i + 1 - lo) / (hi - lo)))
            mine = self.marks[lo:hi]
            return _merge(others, mine) if others and mine else list(others) + mine

        def flush(self, st, zero, phase, hi=THI):
            old = [r for r in self.ready if r[2] < phase]
            for p, acc, ph, frac in self.ready:
                if ph < phase:
                    rl = 8 * (([r[0] for r in old].index(p) + 1) * 200 // (len(old) + 1))
                else:
                    rl = 16 * min(int(TLO + frac * (hi - TLO)) - 4, 118)
                z = jnp.concatenate([_lanes(_tok(st, rl) & zero, gw)] * 2, axis=0)
                rem_scr[16 * p:16 * p + 16, :] = _or(acc, z)
            self.ready = []

    def qproj(u, toks, zero):
        h = h_scr[blk_of(u) & 1]
        q = jnp.dot(h[RV:TB, dm:d], wq_v[grp_of(u), dm:d, :], preferred_element_type=F32)
        r = jnp.concatenate([rem_scr[...], q], axis=0)
        outs = []
        for i in range(nq):
            tk = toks[i * len(toks) // nq:(i + 1) * len(toks) // nq]
            hm = _tie_rows(h[:, 0:dm], tk, zero, 0, TB // 16)
            q = jnp.dot(hm, wq_v[grp_of(u), 0:dm, i * DH:(i + 1) * DH],
                        preferred_element_type=F32) + r[:, i * DH:(i + 1) * DH]
            outs.append(q.astype(BF16))
        return jnp.concatenate(outs, axis=1)

    def qproj_first(lo, hi):
        qs = []
        for r0 in (0, TB // 2):
            rs = slice(r0, r0 + TB // 2)
            q = jnp.dot(h_scr[0, rs, dm:d], wq_v[0, dm:d, lo:hi], preferred_element_type=F32)
            q = jnp.dot(h_scr[0, rs, 0:dm], wq_v[0, 0:dm, lo:hi], preferred_element_type=F32) + q
            qs.append(q.astype(BF16))
        return jnp.concatenate(qs, axis=0)

    def qk(u, q, j, toks, zero):
        k = _tie_rows(k_v[grp_of(u) * HG + j // 2], toks, zero, TLO, THI)
        st = lax.dot_general(k, q[:, j * DH:(j + 1) * DH], _NT,
                             preferred_element_type=F32)
        for i in range(nb):
            blk = st[:, i * LANES:(i + 1) * LANES]
            st_scr[j * nb + i] = blk
            m_scr[j * nb + i] = jnp.max(blk.reshape(sk // 8, 8, LANES), axis=0)
        return st

    def v_transpose(u, i, rel=(), zero=None):
        v = _tie_rows(v_v[grp_of(u) * HG + i], rel, zero, -7, sk // 16 - 7)
        vt = pltpu.bitcast(v.T, U32)
        vt_scr[i] = vt
        return [vt[DH // 2 - 8:DH // 2, c:c + LANES] for c in range(0, sk, LANES)]

    def pv(slots, zero, toks=(), srows=SROWS, free=PVEND):
        ps, ls, pairs = [], [], []
        for sl in slots:
            m = jnp.max(m_scr[sl], axis=0, keepdims=True)
            p = jnp.exp2(st_scr[sl] - m)
            accs = [None] * 4
            for tile in range(nt):
                for r0 in range(tile * LANES + LANES - 16, tile * LANES - 16, -16):
                    pair = p[r0:r0 + 8] + p[r0 + 8:r0 + 16]
                    pairs.append(pair)
                    a = accs[tile % 4]
                    accs[tile % 4] = pair if a is None else a + pair
            ls.append(jnp.sum((accs[0] + accs[1]) + (accs[2] + accs[3]), axis=0, keepdims=True))
            ps.append(p.astype(BF16))
        outs = []
        ntiles = len(slots) * nt
        side = {}
        for i, tok in enumerate(toks):
            side.setdefault(max(((i + 1) * (ntiles - free)) // len(toks) - 1, 0), []).append(tok)
        for i, sl in enumerate(slots):
            vu = vt_scr[sl // (2 * nb)]
            tiles = []
            for c in range(nt):
                g = i * nt + c + 4
                rows = []
                for r in range(8):
                    x = vu[8 * r:8 * r + 8, c * LANES:(c + 1) * LANES]
                    if g < ntiles and TIE0 <= r < TIE0 + NTIE:
                        src = pairs[g * 8 + (r - TIE0)]
                        x = _dep(x, lax.bitcast_convert_type(src, U32), zero)
                    if r == srows[c % 4]:
                        for tok in side.get(i * nt + c, ()):
                            x = _dep(x, tok, zero)
                    rows.append(x)
                tiles.append(jnp.concatenate(rows, axis=0))
            lhs = pltpu.bitcast(jnp.concatenate(tiles, axis=1), BF16)
            o = jnp.dot(lhs, ps[i], preferred_element_type=F32)
            outs.append(o * (1.0 / ls[i]))
        return outs

    def outproj_tied(u, o, toks, zero):
        slot = blk_of(u) & 1
        res = []
        for i in range(nb):
            o2 = jnp.concatenate([o[j * nb + i] for j in range(nq)], axis=0).astype(BF16)
            tk = toks[i * len(toks) // OPN:(i + 1) * len(toks) // OPN]
            wo = _tie_rows(wot_v[grp_of(u)], tk, zero, 0, d // 16)
            contrib = jnp.dot(wo, o2, preferred_element_type=F32)
            acc_scr[slot * nb + i] += contrib
            res.append(contrib)
        return jnp.concatenate(res, axis=0)

    def outproj(u, o, lo=0):
        w = len(o) // nq
        o2 = jnp.concatenate(
            [jnp.concatenate(o[j * w:(j + 1) * w], axis=1) for j in range(nq)], axis=0).astype(BF16)
        contrib = jnp.dot(wot_v[grp_of(u)], o2, preferred_element_type=F32)
        slot = blk_of(u) & 1
        for i in range(w):
            pi = slot * nb + lo // LANES + i
            acc_scr[pi] += contrib[:, i * LANES:(i + 1) * LANES]

    def router_keys(racc, t0):
        r = _rb(jnp.sum(racc, axis=0, keepdims=True)) + 0.0
        bits = lax.bitcast_convert_type(r, I32) >> 16
        order = jnp.where(bits < 0, -1 - bits, bits + 32768)
        pos = t0 + lax.broadcasted_iota(I32, r.shape, 1)
        return lax.bitcast_convert_type((order << 11) + (seq - 1 - pos) + 0x20000000, F32)

    def finalize(t0, slot, a0, dst, n, keys_out=None):
        marks = []
        cs = _span(dst, n)
        x = x_cols(t0, n).astype(F32)
        att = jnp.concatenate(
            [acc_scr[slot * nb + a0 // LANES + i] for i in range(n // LANES)], axis=1)
        x1b = (x + _lanes(col_scr[0:d, :], n) * att).astype(BF16)
        x1_scr[:, cs] = x1b
        ot_v[:, cs] = x1b
        fine = keys_out is None
        mu = _colsum(x1b.astype(F32), marks, NG1 if fine else NF1) * (1.0 / d)

        def note(row):
            if fine:
                marks.append(_fold(jnp.broadcast_to(row, (8, n))))
            return row

        mub = note(_rb(mu))
        xc = x1_scr[:, cs].astype(F32) - mub
        var = _colsum(xc * xc, marks, NG2 if fine else NF2) * (1.0 / d) - (mu - mub) * (mu - mub)
        inv = note(1.0 / note(_rb(jnp.sqrt(note(_rb(_rb(jnp.maximum(var, 0.0)) + EPS_BF16))))))
        step = d // ((NG3 if n == SP else EG3) if fine else NF3)
        racc = None
        for r0 in range(0, d, step):
            rs = slice(r0, r0 + step)
            x1 = ot_v[rs, cs].astype(F32)
            ln = _rb(_rb(x1 - mub) * inv)
            if fine:
                marks.append(_fold(ln))
            h2b = (_rb(ln * _lanes(col_scr[2 * d + r0:2 * d + r0 + step, :], n))
                   + _lanes(col_scr[d + r0:d + r0 + step, :], n)).astype(BF16)
            if keys_out is None:
                h2_scr[rs, cs] = h2b
            else:
                h2l_scr[rs, :] = h2b
            h2 = h2b.astype(F32)
            out = x1 + _lanes(col_scr[3 * d + r0:3 * d + r0 + step, :], n) * h2
            ot_v[rs, cs] = out.astype(BF16)
            rp = h2 * _lanes(col_scr[4 * d + r0:4 * d + r0 + step, :], n)
            for g in range(0, step, 8):
                racc = rp[g:g + 8] if racc is None else racc + rp[g:g + 8]
            marks.append(_fold(out, racc))
        if keys_out is not None:
            keys_out.append(racc)
            return marks
        key = router_keys(racc, t0)
        for i in range(n // LANES):
            key_scr[pl.ds(dst // LANES + i, 1), :] = key[:, i * LANES:(i + 1) * LANES]
        return marks

    hw = gw // 2
    wq0a = col_copy(wq_hbm, wq_v.at[0], 0, hw, grp_sems.at[0, 0])
    wq0b = col_copy(wq_hbm, wq_v.at[0], hw, gw, misc_sems.at[4])
    k0a = pltpu.make_async_copy(k_hbm.at[0], k_v.at[0], grp_sems.at[1, 0])
    k0b = pltpu.make_async_copy(k_hbm.at[1], k_v.at[1], misc_sems.at[5])
    v0 = pltpu.make_async_copy(v_hbm.at[0:HG], v_v.at[0:HG], grp_sems.at[2, 0])
    wq1, k1, v1, wo0 = grp_copies(1)
    wo_last = pltpu.make_async_copy(wot_hbm.at[:, (n_grp - 1) * gw:n_grp * gw],
                                    wot_v.at[n_grp - 1], grp_sems.at[3, 0])
    wrem_copy = col_copy(wq_hbm.at[dm:d], wrem_v, gw, 4 * gw, misc_sems.at[2])
    wrem_rest = (col_copy(wq_hbm.at[dm:d], wrem_v, 0, gw, misc_sems.at[11]),
                 col_copy(wq_hbm.at[dm:d], wrem_v, 4 * gw, n_grp * gw, misc_sems.at[12]))
    c_copy = pltpu.make_async_copy(c_hbm, c_ref, misc_sems.at[6])
    wr_copy = pltpu.make_async_copy(wr_hbm, wr_ref, misc_sems.at[7])
    c_copy.start()
    wr_copy.start()
    x_first.start()
    mod_first[0].start()
    mod_first[1].start()
    wq0a.start()
    wq0b.start()
    acc_scr[0:2 * nb] = jnp.zeros((2 * nb, d, LANES), F32)
    col_scr[0:4 * d, :] = jnp.zeros((4 * d, LANES), F32)
    wdt_v[ff // WP] = jnp.zeros((d, WP), BF16)
    c_copy.wait()
    wr_copy.wait()
    x_first.wait()
    cbits = lax.bitcast_convert_type(c_ref[:, 0:LANES].astype(F32), U32)
    zero_scr[...] = jnp.broadcast_to(cbits & 0xFFFF, (8, LANES))
    h_scr[0] = ln1_norm(0, TB, [])()
    sc = silu_c()
    wr = wr_ref[...].reshape(1, d).astype(F32)
    col_scr[4 * d:5 * d, :] = jnp.broadcast_to(wr, (LANES, d)).T
    col_scr[5 * d:6 * d, :] = jnp.broadcast_to(sc[0:1, :].astype(F32), (LANES, d)).T
    mod_first[0].wait()
    mod = _rb(jnp.dot(sc, wmod_v[:, MODC:2 * d], preferred_element_type=F32))
    mod_scr[0:1, MODC:d] = mod[0:1, 0:d - MODC] * qscale
    mod_scr[1:2, :] = _rb(1.0 + mod[0:1, d - MODC:2 * d - MODC]) * qscale
    mod_first[1].wait()
    k0a.start()
    mod = _rb(jnp.dot(sc, wmod_v[:, 0:MODC], preferred_element_type=F32))
    mod_scr[0:1, 0:MODC] = mod[0:1] * qscale
    wq0a.wait()
    k0b.start(priority=1)
    v0.start(priority=1)
    wrem_copy.start(priority=1)
    ln1_mod(h_scr[0], 0, 0)
    qa = qproj_first(0, hw)
    wq0b.wait()
    k0a.wait()
    wq1.start(priority=1)
    k1.start(priority=1)
    x_second.start()
    q = jnp.concatenate([qa, qproj_first(hw, gw)], axis=1)
    zero = zero_scr[...]
    for j in range(2):
        marks = []
        for i in range(2 * j, 2 * j + 2):
            hb_piece(0, i, marks)
        qk(0, q, j, marks, zero)
    k0b.wait()
    v0.wait()
    wrem_copy.wait()
    v1.start()
    wo0.start()
    zero = zero_scr[...]
    rem_scr[...] = jnp.dot(h_scr[0, 0:RV, dm:d], wrem_v[:, gw:2 * gw],
                           preferred_element_type=F32)
    for i in range(HG):
        marks = v_transpose(0, i)
        if i == 0:
            wb_piece(2, marks, zero)
        if 4 + i < nhb:
            hm = []
            hb_piece(0, 4 + i, hm)
            marks = _merge(marks, hm)
        qk(0, q, nq - HG + i, marks, zero)

    assert n_grp == 8 and HG == 2
    stage_at = [1, 2, 3, 5, n_units]
    starts = [(*grp_copies(2), mod_rest, x_rest, *wrem_rest), grp_copies(3, 3),
              (*grp_copies(6, 2), wo_last, mlp_d), (mlp_g, mlp_u)]
    waits = [(wq1, k1, v1, wo0, x_second), *starts[:3]]
    wd0 = stage_at[3]
    npc = TB // SP
    nmp = 4 * d // MP

    def manage(k, _, c):
        for cp in waits[k]:
            cp.wait()
        for cp in starts[k]:
            cp.start()
        return c

    def steady(u, carry):
        zero = zero_scr[...]
        blk, g = blk_of(u), grp_of(u)
        off = ((g - 1) & (npc - 1)) * SP
        rem = Rem(blk_of(u + 1) & 1)
        q = qproj(u, rem.take(0), zero)
        o = pv(range(0, 2 * nb), zero, rem.take(1))
        live = jnp.logical_and(blk > 0, jnp.logical_and(g >= 1, g <= npc))
        t0 = jnp.maximum(blk - 1, 0) * TB + off
        marks = finalize(t0, (blk + 1) & 1, off, jnp.where(live, t0, seq), SP)
        wp = jnp.clip(u - wd0, 0, ff // WP - 1) * WP
        wmarks = []
        wd_piece(jnp.where(u >= wd0, wp, ff), wp, wmarks)
        rem.flush(qk(u, q, 0, rem.take(2, _merge(marks, wmarks)), zero), zero, 2)
        marks, mmarks = [], []
        ln_fin = ln1_norm(jnp.minimum(blk + 1, n_blk - 1) * TB + off, SP, marks)
        mp = jnp.clip(u - 2, 0, nmp - 1) * MP
        mod_fin = mod_piece(jnp.where(u >= 2, 2 * d + mp, 0), mp, mmarks)
        st = qk(u, q, 1, rem.take(3, marks + mmarks), zero)
        rem.flush(st, zero, 3)
        used = jnp.where(live, ((blk + 1) & 1) * nb + off // LANES, 2 * nb)
        for r0 in range(0, d, 32):
            z4 = jnp.concatenate([_tok(st, r0) & zero] * 4, axis=0)
            acc_scr[used, r0:r0 + 32, :] = lax.bitcast_convert_type(z4, F32)
        ln1_mod(ln_fin(_tok(st, LNREL) & zero), (blk + 1) & 1, off)
        mod_fin(_tok(st, 1880) & zero)
        o += pv(range(2 * nb, 4 * nb), zero, rem.take(4))
        st = qk(u, q, 2, rem.take(5), zero)
        rem.flush(st, zero, 5)
        v_transpose(u, 0, [_tok(st, 112 * i) for i in range(nt)], zero)
        st = qk(u, q, 3, rem.take(6), zero)
        rem.flush(st, zero, 6)
        v_transpose(u, 1, [_tok(st, 112 * i) for i in range(nt)], zero)
        res = outproj_tied(u - 1, o, rem.take(7), zero)
        rem.flush(res, zero, 7, OPN * d // 16)
        hm = []
        hb_piece((blk + 1) & 1, jnp.clip(g - 1, 0, nhb - 1), hm,
                 _tok(res, max(OPN * d - 96, 0)) & zero)
        wb_piece(u + 2, hm, zero)
        return carry

    def stage(k, lo):
        hi = stage_at[1]
        for i in range(len(waits)):
            lax.fori_loop(0, jnp.where(k == i, 1, 0), functools.partial(manage, i), 0)
            hi = jnp.where(k == i, stage_at[i + 1], hi)
        lax.fori_loop(lo, hi, steady, 0)
        return hi

    lax.fori_loop(0, len(waits), stage, jnp.int32(stage_at[0]))

    ul = n_units - 1
    tl = seq - TB
    sl_last = (n_blk - 1) & 1
    nb0 = nb - TAILB
    mod_scr[2:3, :] = row_scr[:, 3 * d:4 * d]
    outproj(ul, pv([j * nb + i for j in range(nq) for i in range(nb0)], zero_scr[...]))
    mlp_g.wait()
    mlp_u.wait()
    out_lo.start()
    toks = finalize(tl, sl_last, 0, tl, nb0 * LANES)
    o = pv([j * nb + i for j in range(nq) for i in range(nb0, nb)], zero_scr[...], toks,
           EROWS, EPVEND)
    outproj(ul, o, nb0 * LANES)

    nl = TAILB * LANES
    sub8 = lax.broadcasted_iota(I32, (TOPC, 1), 0)
    lane = lax.broadcasted_iota(I32, (TOPC, LANES), 1)

    def key_index(k):
        return seq - 1 - (lax.bitcast_convert_type(k, I32) & (seq - 1))

    def piece_base(idx, limit):
        return pl.multiple_of(jnp.clip(idx >> 7, 0, limit // LANES - 1) * LANES, LANES)

    keys = key_scr[0:seq // LANES, :]
    piece = lax.broadcasted_iota(I32, (seq // LANES, 1), 0)
    keys = jnp.where(piece < (seq - nl) // LANES, keys, 0.0)
    ecol = jnp.zeros((TOPC, LANES), F32)
    erow = jnp.zeros((1, LANES), F32)
    h2e = jnp.zeros((TOPC, d), F32)
    late = []
    marks = finalize(seq - nl, sl_last, TB - nl, seq - nl, nl, late)
    zero = zero_scr[...]
    for i in range(TOPC):
        mx = jnp.max(jnp.max(keys, axis=0, keepdims=True), axis=1, keepdims=True)
        keys = jnp.where(keys == mx, 0.0, keys)
        ecol = jnp.where(sub8 == i, mx, ecol)
        erow = jnp.where(lane[0:1] == i, mx, erow)
        idx = key_index(mx)
        pick = jnp.logical_and(sub8 == i, lane == (idx & (LANES - 1)))
        sl = pl.ds(piece_base(idx[0, 0], seq - nl), LANES)
        pick = jnp.where(pick, 1.0, 0.0)
        if i in PACE:
            pick = _or(pick, marks[PACE[i]] & zero)
        h2e = h2e + lax.dot_general(pick.astype(BF16), h2_scr[:, sl], _NT,
                                    preferred_element_type=F32)

    late = [router_keys(late[0], seq - nl)]
    krow = jnp.concatenate([late[0], erow], axis=1)
    kcol = jnp.concatenate([jnp.broadcast_to(late[0], (LANES, nl)).T, ecol], axis=0)
    cnt = [None] * 4
    for g in range(kcol.shape[0] // 8):
        one = jnp.where(_lanes(kcol[8 * g:8 * g + 8], nl + LANES) > krow, 1.0, 0.0)
        cnt[g % 4] = one if cnt[g % 4] is None else cnt[g % 4] + one
    rank = jnp.sum((cnt[0] + cnt[1]) + (cnt[2] + cnt[3]), axis=0, keepdims=True)
    chosen = rank == sub8.astype(F32)
    onehot = jnp.where(chosen, 1.0, 0.0).astype(BF16)
    h2pad = jnp.concatenate([h2e, jnp.zeros((TOPC, d), F32)], axis=0).astype(BF16)
    h2s = (jnp.dot(onehot[:, nl:nl + 2 * TOPC], h2pad, preferred_element_type=F32)
           + lax.dot_general(onehot[:, 0:nl], h2l_scr[...], _NT,
                             preferred_element_type=F32))
    top = jnp.max(jnp.where(chosen, krow, 0.0), axis=1, keepdims=True)
    idx_col = key_index(top)
    idxs = [idx_col[i:i + 1] for i in range(TOPC)]
    bases = [piece_base(idx_col[i, 0], seq) for i in range(TOPC)]
    hit = lane == (idx_col & (LANES - 1))
    picks = [jnp.where(jnp.logical_and(sub8 == i, hit), 1.0, 0.0).astype(BF16)
             for i in range(TOPC)]
    order = (lax.bitcast_convert_type(top, I32) >> 11) & 0xFFFF
    rbits = jnp.where(order >= 32768, order - 32768, -1 - order) << 16
    gate = _sigmoid(lax.bitcast_convert_type(rbits, F32))
    xs = h2s.astype(BF16)
    for cp in out_hi:
        cp.start()
    g = _rb(jnp.dot(xs, wg_v[...], preferred_element_type=F32))
    g = _rb(g * _sigmoid(g))
    u = _rb(jnp.dot(xs, wu_v[...], preferred_element_type=F32))
    gu = (g * u).astype(BF16)

    last_use = []
    for i in range(TOPC):
        ok = True
        for j in range(i + 1, TOPC):
            ok = jnp.logical_and(ok, bases[i] != bases[j])
        last_use.append(ok)

    def down(r0, r1):
        x1p = jnp.concatenate([x1_scr[r0:r1, pl.ds(bases[i], LANES)] for i in range(TOPC)], axis=1)
        x1s = lax.dot_general(jnp.concatenate(picks, axis=1), x1p, _NT,
                              preferred_element_type=F32)
        wd = pltpu.bitcast(wd_scr[:, r0:r1], BF16)
        y = _rb(jnp.dot(gu, wd, preferred_element_type=F32))
        hm = _rb(h2s[:, r0:r1] + _rb(y * gate))
        return x1s + mod_scr[2:3, r0:r1] * hm

    def patch(r0, r1, new):
        n = r1 - r0
        pad = jnp.concatenate([new, jnp.zeros((LANES - TOPC, n), F32)], axis=0)
        cols = pltpu.bitcast(pad.T.astype(BF16), U32)
        col = [jnp.broadcast_to(cols[:, j:j + 1], (n // 2, LANES)) for j in range(TOPC)]
        for i in range(TOPC):
            res = pltpu.bitcast(ot_v[r0:r1, pl.ds(bases[i], LANES)], U32)
            tok = lane[0:1, :] + (idxs[i] & ~(LANES - 1))
            for j in range(i + 1):
                res = jnp.where(tok == idxs[j], col[j], res)
            fix_v[i, r0:r1, :] = pltpu.bitcast(res, BF16)

    def fix_copy(i, r0, r1):
        return pltpu.make_async_copy(fix_v.at[i, r0:r1, :],
                                     o_hbm.at[r0:r1, pl.ds(bases[i], LANES)], fix_sems.at[i])

    def for_last(fn):
        for i in range(TOPC - 1):
            pl.when(last_use[i])(functools.partial(fn, i))
        fn(TOPC - 1)

    new = down(*chunks[0])
    out_lo.wait()
    for ci, (r0, r1) in enumerate(chunks):
        out_hi[ci].wait()
        nxt = down(*chunks[ci + 1]) if ci + 1 < len(chunks) else None
        patch(r0, r1, new)
        for_last(lambda i: fix_copy(i, r0, r1).start())
        new = nxt
    for r0, r1 in chunks:
        for_last(lambda i: fix_copy(i, r0, r1).wait())


@jax.jit
def pallas_adaLN_cond__gqa_block_cached__moe_arch_mod__prompt_kernel(
    A_x: jax.Array,
    A_k_cache: jax.Array,
    A_v_cache: jax.Array,
    A_wq: jax.Array,
    A_wo: jax.Array,
    B_x: jax.Array,
    B_w_r: jax.Array,
    B_w_gate: jax.Array,
    B_w_up: jax.Array,
    B_w_down: jax.Array,
    c: jax.Array,
    w_mod: jax.Array,
):
    b, seq, d = A_x.shape
    _, hkv, sk, dh = A_k_cache.shape
    assert b == 1 and dh == DH and HQ == 2 * hkv
    assert seq & (seq - 1) == 0 and seq <= 2048
    f = B_w_gate.shape[1]
    n_grp = hkv // HG
    gw = 2 * HG * dh
    n_slots = 2 * HG * TB // LANES

    xt = A_x.reshape(seq, d).T
    wot = A_wo.T
    wdt = B_w_down.T
    k3 = A_k_cache.reshape(hkv, sk, dh)
    v3 = A_v_cache.reshape(hkv, sk, dh)

    hbm = pl.BlockSpec(memory_space=pl.ANY)
    out_t = pl.pallas_call(
        functools.partial(_kernel, n_heads=hkv),
        in_specs=[hbm] * 11,
        out_specs=hbm,
        out_shape=jax.ShapeDtypeStruct((d, seq), BF16),
        scratch_shapes=[
            pltpu.VMEM((seq // LANES, d, LANES), BF16),
            pltpu.VMEM((hkv, sk, dh), BF16),
            pltpu.VMEM((hkv, sk, dh), BF16),
            pltpu.VMEM((n_grp, d, gw), BF16),
            pltpu.VMEM((n_grp, d, gw), BF16),
            pltpu.VMEM((d, 6 * d), BF16),
            pltpu.VMEM((d, f), BF16),
            pltpu.VMEM((d, f), BF16),
            pltpu.VMEM((f // WP + 1, d, WP), BF16),
            pltpu.VMEM((d, seq + SP), BF16),
            pltpu.VMEM((2, TB, d), BF16),
            pltpu.VMEM((2 * TB // LANES + 1, d, LANES), F32),
            pltpu.VMEM((n_slots, sk, LANES), F32),
            pltpu.VMEM((n_slots, 8, LANES), F32),
            pltpu.VMEM((HG, dh // 2, sk), U32),
            pltpu.VMEM((8, d), F32),
            pltpu.VMEM((6 * d, LANES), F32),
            pltpu.VMEM(((seq + SP) // LANES + 7 & ~7, LANES), F32),
            pltpu.VMEM((d, seq + SP), BF16),
            pltpu.VMEM((d, seq + SP), BF16),
            pltpu.VMEM((8, LANES), U32),
            pltpu.VMEM((TOPC, d, LANES), BF16),
            pltpu.VMEM((1, d), BF16),
            pltpu.VMEM((d,), BF16),
            pltpu.VMEM((1, 4 * d), F32),
            pltpu.VMEM((f // 2, d), U32),
            pltpu.VMEM((d, TAILB * LANES), BF16),
            pltpu.VMEM((2 * -(-RV // HP), d % LANES * HP // 2, LANES), U32),
            pltpu.VMEM((d % LANES * 8, gw), F32),
            pltpu.VMEM((RV, gw), F32),
            pltpu.VMEM((d % LANES, n_grp * gw), BF16),
            pltpu.SemaphoreType.DMA((4, n_grp)),
            pltpu.SemaphoreType.DMA((13,)),
            pltpu.SemaphoreType.DMA((3,)),
            pltpu.SemaphoreType.DMA((len(EDGES),)),
            pltpu.SemaphoreType.DMA((TOPC,)),
        ],
        compiler_params=pltpu.CompilerParams(
            disable_bounds_checks=True,
            disable_semaphore_checks=True,
            vmem_limit_bytes=120 * 1024 * 1024,
        ),
    )(xt, k3, v3, A_wq, wot, B_w_r, B_w_gate, B_w_up, wdt, c, w_mod)
    return out_t.T.reshape(b, seq, d)
```

```python
import functools
import math

import jax
import jax.numpy as jnp
from jax import lax
import jax.experimental.pallas as pl
import jax.experimental.pallas.tpu as pltpu

F32 = jnp.float32
BF16 = jnp.bfloat16
I32 = jnp.int32
U32 = jnp.uint32

HQ = 32
DH = 128
TOPC = 8
EPS = 1e-05
EPS_BF16 = 1.0013580322265625e-05
LANES = 128

TB = 512
HG = 2
SP = 128
MP = 384
WP = 256
RV = 448
HP = 80
MODC = 384
TAILB = 2
EDGES = (0, 128, 256, 384, 512, 576)

TIE0, NTIE = 2, 3
TLO, THI = 3, 126
SROWS, PVEND = (0, 1, 2, 5), 12
EROWS, EPVEND = (0, 4, 6, 7), 24
NM1, NM2, NMP = 8, 18, 24
NG1, NG2, NG3, EG3 = 18, 9, 18, 36
LM, LS, LLO, LKEEP = 12, 32, 15, 16
KS, KSPLIT, HS = 4, 2, 2
OPN = 2
LNREL = 1008
SHARES = (29, 28, 15, 23, 26, 30, 33, 18)
PACE = {17: 3}

_NT = (((1,), (1,)), ((), ()))


def _rb(x):
    return x.astype(BF16).astype(F32)


def _sigmoid(x):
    return _rb(1.0 / _rb(1.0 + _rb(jnp.exp(-x))))


def _lanes(col, width):
    reps = width // LANES
    return col if reps == 1 else jnp.concatenate([col] * reps, axis=1)


def _fold(*xs):
    ts = []
    for x in xs:
        xi = lax.bitcast_convert_type(x, U32)
        ts += [xi[r:r + 8, c:c + LANES] for r in range(0, x.shape[0], 8)
               for c in range(0, x.shape[1] - LANES + 1, LANES)]
    if len(ts) > 5:
        return functools.reduce(lambda a, b: a | b, ts[:-2]) | (ts[-2] | ts[-1])
    while len(ts) > 1:
        ts = [a | b for a, b in zip(ts[0::2], ts[1::2])] + ts[len(ts) & ~1:]
    return ts[0]


def _colsum(x, marks, nmarks):
    n = x.shape[0] // 8
    acc = x[0:8]
    for g in range(1, n):
        acc = acc + x[8 * g:8 * g + 8]
        if ((g + 1) * nmarks) % n == 0:
            marks.append(_fold(acc))
    return jnp.sum(acc, axis=0, keepdims=True)


def _dep(x, tok, zero):
    return jnp.where(zero != 0, tok, x)


def _tie_rows(lhs, toks, zero, lo, hi):
    if not toks:
        return lhs
    lu = pltpu.bitcast(lhs, U32)
    rows = [lu[8 * r:8 * r + 8] for r in range(lu.shape[0] // 8)]
    for i, tok in enumerate(toks):
        r = lo + ((i + 1) * (hi - lo)) // len(toks) - 1
        head = _dep(rows[r][:, 0:LANES], tok, zero)
        rows[r] = head if lu.shape[1] == LANES else jnp.concatenate(
            [head, rows[r][:, LANES:]], axis=1)
    return pltpu.bitcast(jnp.concatenate(rows, axis=0), BF16)


def _merge(a, b):
    keyed = [((i + 1) / len(a), t) for i, t in enumerate(a)]
    keyed += [((i + 1) / len(b), t) for i, t in enumerate(b)]
    return [t for _, t in sorted(keyed, key=lambda kv: kv[0])]


def _span(start, size):
    if isinstance(start, int):
        return pl.ds(start, size)
    return pl.ds(pl.multiple_of(start, LANES), size)


def _tok(res, row):
    return lax.bitcast_convert_type(res[row:row + 8, 0:LANES], U32)


def _or(x, z):
    return lax.bitcast_convert_type(lax.bitcast_convert_type(x, U32) | z, F32)


def _kernel(xt_hbm, k_hbm, v_hbm, wq_hbm, wot_hbm, wr_hbm, wg_hbm, wu_hbm, wdt_hbm,
            c_hbm, wmod_hbm, o_hbm,
            xt_v, k_v, v_v, wq_v, wot_v, wmod_v, wg_v, wu_v, wdt_v, ot_v,
            h_scr, acc_scr, st_scr, m_scr, vt_scr, mod_scr, col_scr, key_scr, h2_scr, x1_scr,
            zero_scr, fix_v, c_ref, wr_ref, row_scr, wd_scr,
            hb_scr, wb_scr, rem_scr, wrem_v,
            grp_sems, misc_sems, mlp_sems, out_sems, fix_sems,
            *, n_heads):
    d, seq = xt_hbm.shape
    sk = k_v.shape[1]
    n_grp = n_heads // HG
    n_blk = seq // TB
    n_units = n_grp * n_blk
    nb = TB // LANES
    nq = 2 * HG
    nt = sk // LANES
    gbits = n_grp.bit_length() - 1
    gw = nq * DH
    qscale = (DH ** -0.5) * math.log2(math.e)

    def grp_of(u):
        return u & (n_grp - 1)

    def blk_of(u):
        return u >> gbits

    def grp_copies(g, n=1):
        hs = pl.ds(g * HG, n * HG)
        return (*[pltpu.make_async_copy(wq_hbm.at[:, pl.ds(i * gw, gw)], wq_v.at[i],
                                        grp_sems.at[0, i]) for i in range(g, g + n)],
                pltpu.make_async_copy(k_hbm.at[hs], k_v.at[hs], grp_sems.at[1, g]),
                pltpu.make_async_copy(v_hbm.at[hs], v_v.at[hs], grp_sems.at[2, g]),
                *[pltpu.make_async_copy(wot_hbm.at[:, pl.ds((i - 1) * gw, gw)], wot_v.at[i - 1],
                                        grp_sems.at[3, i]) for i in range(g, g + n)])

    def col_copy(src, dst, lo, hi, sem):
        return pltpu.make_async_copy(src.at[:, lo:hi], dst.at[:, lo:hi], sem)

    class Pieces:
        def __init__(self, src, dst, lo, hi, sem):
            self.src, self.dst, self.lo, self.hi, self.sem = src, dst, lo, hi, sem

        def start(self):
            w = self.dst.shape[2]
            for p in range(self.lo, self.hi):
                pltpu.make_async_copy(self.src.at[:, p * w:(p + 1) * w], self.dst.at[p],
                                      self.sem).start()

        def wait(self):
            whole = self.dst.at[self.lo:self.hi]
            pltpu.make_async_copy(whole, whole, self.sem).wait()

    def x_cols(t0, n):
        return jnp.concatenate([xt_v[t0 // LANES + i] for i in range(n // LANES)], axis=1)

    x_first = Pieces(xt_hbm, xt_v, 0, nb, misc_sems.at[0])
    x_second = Pieces(xt_hbm, xt_v, nb, nb + 1, misc_sems.at[10])
    x_rest = Pieces(xt_hbm, xt_v, nb + 1, seq // LANES, misc_sems.at[1])
    mod_first = [col_copy(wmod_hbm, wmod_v, MODC, 2 * d, misc_sems.at[8]),
                 col_copy(wmod_hbm, wmod_v, 0, MODC, misc_sems.at[9])]
    mod_rest = col_copy(wmod_hbm, wmod_v, 2 * d, 6 * d, misc_sems.at[3])
    mlp_g = pltpu.make_async_copy(wg_hbm, wg_v, mlp_sems.at[0])
    mlp_u = pltpu.make_async_copy(wu_hbm, wu_v, mlp_sems.at[1])
    ff = wdt_hbm.shape[1]
    mlp_d = Pieces(wdt_hbm, wdt_v, 0, ff // WP, mlp_sems.at[2])
    out_lo = col_copy(ot_v, o_hbm, 0, seq - TB, out_sems.at[0])
    chunks = list(zip(EDGES[:-1], EDGES[1:]))
    out_hi = [pltpu.make_async_copy(ot_v.at[r0:r1, seq - TB:seq], o_hbm.at[r0:r1, seq - TB:seq],
                                    out_sems.at[1 + i]) for i, (r0, r1) in enumerate(chunks)]

    def silu_c():
        cc = c_ref[...].astype(F32)
        return jnp.broadcast_to((cc * _sigmoid(cc)).astype(BF16), (8, d))

    def ln1_norm(t0, n, marks):
        x = x_cols(t0, n).astype(F32)
        mu = _colsum(x, marks, NM1) * (1.0 / d)
        marks.append(_fold(jnp.broadcast_to(mu, (8, n))))
        xc = x - mu
        var = _colsum(xc * xc, marks, NM2) * (1.0 / d)
        rs = lax.rsqrt(var + EPS)

        def finish(z=None):
            r = rs if z is None else _or(rs, _lanes(z[0:1], n))
            return (xc * r).astype(BF16).T
        return finish

    def ln1_mod(ln, slot, r0):
        h = ln.astype(F32) * mod_scr[1:2, :] + mod_scr[0:1, :]
        h_scr[slot, _span(r0, ln.shape[0]), :] = h.astype(BF16)

    def mod_piece(src, dst, marks):
        w = wmod_v[:, _span(src, MP)].astype(F32)
        row0 = _rb(_colsum(w * _lanes(col_scr[5 * d:6 * d, :], MP), marks, NMP))

        def finish(z):
            row = _or(row0, _lanes(z[0:1], MP))
            pos = dst + lax.broadcasted_iota(I32, (1, MP), 1)
            is_cb = jnp.logical_and(pos >= 2 * d, pos < 3 * d)
            row = jnp.where(is_cb, _rb(1.0 + row), row)
            row_scr[:, _span(dst, MP)] = row
            col_scr[_span(dst, MP), :] = jnp.broadcast_to(row, (LANES, MP)).T
        return finish

    def wd_piece(src, dst, marks):
        w = pltpu.bitcast(wdt_v[src // WP].T, U32)
        wd_scr[pl.ds(pl.multiple_of(dst // 2, WP // 2), WP // 2), :] = w
        for r in range(56, WP // 2, 64):
            for c in range(0, d - LANES + 1, LANES):
                marks.append(w[r:r + 8, c:c + LANES])

    dm = d - d % LANES
    kr = d - dm
    nhb = -(-RV // HP)
    assert nhb <= 6 and nhb * HP <= TB

    def hb_piece(slot, sp, marks, z=None):
        r0 = sp * HP
        src = pl.ds(r0 if isinstance(r0, int) else pl.multiple_of(r0, 16), HP)
        hu = pltpu.bitcast(h_scr[slot, src, dm:d], U32)
        if z is not None:
            hu = hu | jnp.concatenate([z[:, 0:kr]] * (HP // 16), axis=0)
        cols = [jnp.broadcast_to(hu[:, k:k + 1], (HP // 2, LANES)) for k in range(kr)]
        hb_scr[slot * nhb + sp] = jnp.concatenate(cols, axis=0)
        marks.extend(col[HP // 2 - 8:HP // 2] for col in cols[HS - 1::HS])

    def wb_piece(u, toks, zero):
        w = lax.bitcast_convert_type(wrem_v[:, _span(grp_of(u) * gw, gw)].astype(F32), U32)
        rows = [jnp.broadcast_to(w[k:k + 1], (8, gw)) | _lanes(toks[k * len(toks) // kr] & zero, gw)
                for k in range(kr)]
        wb_scr[...] = lax.bitcast_convert_type(jnp.concatenate(rows, axis=0), F32)

    class Rem:
        def __init__(self, slot):
            self.marks, self.done, self.ready = [], {}, []
            hbs = [hb_scr[slot * nhb + sp] for sp in range(nhb)]
            wb = wb_scr[...]
            for p in range(RV // 16):
                acc = None
                sp, r8 = divmod(8 * p, HP // 2)
                for k in range(kr):
                    r = k * HP // 2 + r8
                    hb = pltpu.bitcast(hbs[sp][r:r + 8], BF16).astype(F32)
                    w = wb[8 * k:8 * k + 8]
                    t = _lanes(hb, gw) * jnp.concatenate([w, w], axis=0)
                    acc = t if acc is None else acc + t
                    if (k + 1) % KS == 0:
                        for c in range(0, gw, gw // KSPLIT):
                            self.marks.append(_fold(acc[:, c:c + gw // KSPLIT]))
                self.done[len(self.marks) - 1] = (p, acc)

        def take(self, phase, others=()):
            n, tot = len(self.marks), sum(SHARES)
            lo, hi = sum(SHARES[:phase]) * n // tot, sum(SHARES[:phase + 1]) * n // tot
            for i in range(lo, hi):
                if i in self.done:
                    self.ready.append((*self.done[i], phase, (i + 1 - lo) / (hi - lo)))
            mine = self.marks[lo:hi]
            return _merge(others, mine) if others and mine else list(others) + mine

        def flush(self, st, zero, phase, hi=THI):
            old = [r for r in self.ready if r[2] < phase]
            for p, acc, ph, frac in self.ready:
                if ph < phase:
                    rl = 8 * (([r[0] for r in old].index(p) + 1) * 200 // (len(old) + 1))
                else:
                    rl = 16 * min(int(TLO + frac * (hi - TLO)) - 4, 118)
                z = jnp.concatenate([_lanes(_tok(st, rl) & zero, gw)] * 2, axis=0)
                rem_scr[16 * p:16 * p + 16, :] = _or(acc, z)
            self.ready = []

    def qproj(u, toks, zero):
        h = h_scr[blk_of(u) & 1]
        q = jnp.dot(h[RV:TB, dm:d], wq_v[grp_of(u), dm:d, :], preferred_element_type=F32)
        r = jnp.concatenate([rem_scr[...], q], axis=0)
        outs = []
        for i in range(nq):
            tk = toks[i * len(toks) // nq:(i + 1) * len(toks) // nq]
            hm = _tie_rows(h[:, 0:dm], tk, zero, 0, TB // 16)
            q = jnp.dot(hm, wq_v[grp_of(u), 0:dm, i * DH:(i + 1) * DH],
                        preferred_element_type=F32) + r[:, i * DH:(i + 1) * DH]
            outs.append(q.astype(BF16))
        return jnp.concatenate(outs, axis=1)

    def qproj_first(lo, hi):
        qs = []
        for r0 in (0, TB // 2):
            rs = slice(r0, r0 + TB // 2)
            q = jnp.dot(h_scr[0, rs, dm:d], wq_v[0, dm:d, lo:hi], preferred_element_type=F32)
            q = jnp.dot(h_scr[0, rs, 0:dm], wq_v[0, 0:dm, lo:hi], preferred_element_type=F32) + q
            qs.append(q.astype(BF16))
        return jnp.concatenate(qs, axis=0)

    def qk(u, q, j, toks, zero):
        k = _tie_rows(k_v[grp_of(u) * HG + j // 2], toks, zero, TLO, THI)
        st = lax.dot_general(k, q[:, j * DH:(j + 1) * DH], _NT,
                             preferred_element_type=F32)
        for i in range(nb):
            blk = st[:, i * LANES:(i + 1) * LANES]
            st_scr[j * nb + i] = blk
            m_scr[j * nb + i] = jnp.max(blk.reshape(sk // 8, 8, LANES), axis=0)
        return st

    def v_transpose(u, i, rel=(), zero=None):
        v = _tie_rows(v_v[grp_of(u) * HG + i], rel, zero, -7, sk // 16 - 7)
        vt = pltpu.bitcast(v.T, U32)
        vt_scr[i] = vt
        return [vt[DH // 2 - 8:DH // 2, c:c + LANES] for c in range(0, sk, LANES)]

    def pv(slots, zero, toks=(), srows=SROWS, free=PVEND):
        ps, ls, pairs = [], [], []
        for sl in slots:
            m = jnp.max(m_scr[sl], axis=0, keepdims=True)
            p = jnp.exp2(st_scr[sl] - m)
            accs = [None] * 4
            for tile in range(nt):
                for r0 in range(tile * LANES + LANES - 16, tile * LANES - 16, -16):
                    pair = p[r0:r0 + 8] + p[r0 + 8:r0 + 16]
                    pairs.append(pair)
                    a = accs[tile % 4]
                    accs[tile % 4] = pair if a is None else a + pair
            ls.append(jnp.sum((accs[0] + accs[1]) + (accs[2] + accs[3]), axis=0, keepdims=True))
            ps.append(p.astype(BF16))
        outs = []
        ntiles = len(slots) * nt
        side = {}
        for i, tok in enumerate(toks):
            side.setdefault(max(((i + 1) * (ntiles - free)) // len(toks) - 1, 0), []).append(tok)
        for i, sl in enumerate(slots):
            vu = vt_scr[sl // (2 * nb)]
            tiles = []
            for c in range(nt):
                g = i * nt + c + 4
                rows = []
                for r in range(8):
                    x = vu[8 * r:8 * r + 8, c * LANES:(c + 1) * LANES]
                    if g < ntiles and TIE0 <= r < TIE0 + NTIE:
                        src = pairs[g * 8 + (r - TIE0)]
                        x = _dep(x, lax.bitcast_convert_type(src, U32), zero)
                    if r == srows[c % 4]:
                        for tok in side.get(i * nt + c, ()):
                            x = _dep(x, tok, zero)
                    rows.append(x)
                tiles.append(jnp.concatenate(rows, axis=0))
            lhs = pltpu.bitcast(jnp.concatenate(tiles, axis=1), BF16)
            o = jnp.dot(lhs, ps[i], preferred_element_type=F32)
            outs.append(o * (1.0 / ls[i]))
        return outs

    def outproj_tied(u, o, toks, zero):
        slot = blk_of(u) & 1
        res = []
        for i in range(nb):
            o2 = jnp.concatenate([o[j * nb + i] for j in range(nq)], axis=0).astype(BF16)
            tk = toks[i * len(toks) // OPN:(i + 1) * len(toks) // OPN]
            wo = _tie_rows(wot_v[grp_of(u)], tk, zero, 0, d // 16)
            contrib = jnp.dot(wo, o2, preferred_element_type=F32)
            acc_scr[slot * nb + i] += contrib
            res.append(contrib)
        return jnp.concatenate(res, axis=0)

    def outproj(u, o):
        w = len(o) // nq
        o2 = jnp.concatenate(
            [jnp.concatenate(o[j * w:(j + 1) * w], axis=1) for j in range(nq)], axis=0).astype(BF16)
        contrib = jnp.dot(wot_v[grp_of(u)], o2, preferred_element_type=F32)
        slot = blk_of(u) & 1
        for i in range(w):
            acc_scr[slot * nb + i] += contrib[:, i * LANES:(i + 1) * LANES]

    def router_keys(racc, t0):
        r = _rb(jnp.sum(racc, axis=0, keepdims=True)) + 0.0
        bits = lax.bitcast_convert_type(r, I32) >> 16
        order = jnp.where(bits < 0, -1 - bits, bits + 32768)
        pos = t0 + lax.broadcasted_iota(I32, r.shape, 1)
        return lax.bitcast_convert_type((order << 11) + (seq - 1 - pos) + 0x20000000, F32)

    def finalize(t0, slot, a0, dst, n):
        marks = []
        cs = _span(dst, n)
        x = x_cols(t0, n).astype(F32)
        att = jnp.concatenate(
            [acc_scr[slot * nb + a0 // LANES + i] for i in range(n // LANES)], axis=1)
        x1b = (x + _lanes(col_scr[0:d, :], n) * att).astype(BF16)
        x1_scr[:, cs] = x1b
        ot_v[:, cs] = x1b
        mu = _colsum(x1b.astype(F32), marks, NG1) * (1.0 / d)

        def note(row):
            marks.append(_fold(jnp.broadcast_to(row, (8, n))))
            return row

        mub = note(_rb(mu))
        xc = x1_scr[:, cs].astype(F32) - mub
        var = _colsum(xc * xc, marks, NG2) * (1.0 / d) - (mu - mub) * (mu - mub)
        inv = note(1.0 / note(_rb(jnp.sqrt(note(_rb(_rb(jnp.maximum(var, 0.0)) + EPS_BF16))))))
        step = d // (NG3 if n == SP else EG3)
        racc = None
        for r0 in range(0, d, step):
            rs = slice(r0, r0 + step)
            x1 = ot_v[rs, cs].astype(F32)
            ln = _rb(_rb(x1 - mub) * inv)
            marks.append(_fold(ln))
            h2b = (_rb(ln * _lanes(col_scr[2 * d + r0:2 * d + r0 + step, :], n))
                   + _lanes(col_scr[d + r0:d + r0 + step, :], n)).astype(BF16)
            h2_scr[rs, cs] = h2b
            h2 = h2b.astype(F32)
            out = x1 + _lanes(col_scr[3 * d + r0:3 * d + r0 + step, :], n) * h2
            ot_v[rs, cs] = out.astype(BF16)
            rp = h2 * _lanes(col_scr[4 * d + r0:4 * d + r0 + step, :], n)
            for g in range(0, step, 8):
                racc = rp[g:g + 8] if racc is None else racc + rp[g:g + 8]
            marks.append(_fold(out, racc))
        key = router_keys(racc, t0)
        for i in range(n // LANES):
            key_scr[pl.ds(dst // LANES + i, 1), :] = key[:, i * LANES:(i + 1) * LANES]
        return marks

    def late_piece(t0, pi, after=None):
        marks = []
        cs = slice(t0, t0 + LANES)

        def csum(x):
            parts = [None] * 4
            for g in range(d // 8):
                t = x[8 * g:8 * g + 8]
                parts[g % 4] = t if parts[g % 4] is None else parts[g % 4] + t
                if (g + 1) % LM == 0:
                    marks.append(_fold(*parts))
            return jnp.sum((parts[0] + parts[1]) + (parts[2] + parts[3]), axis=0, keepdims=True)

        def note(row):
            marks.append(_fold(jnp.broadcast_to(row, (8, LANES))))
            return row

        x1b = (xt_v[t0 // LANES].astype(F32) + col_scr[0:d, :] * acc_scr[pi]).astype(BF16)
        x1_scr[:, cs] = x1b
        ot_v[:, cs] = x1b
        mu = csum(x1b.astype(F32)) * (1.0 / d)
        marks.clear()
        mub = note(_rb(mu))
        xc = x1_scr[:, cs].astype(F32) - mub
        var = csum(xc * xc) * (1.0 / d) - (mu - mub) * (mu - mub)
        inv = note(1.0 / note(_rb(jnp.sqrt(note(_rb(_rb(jnp.maximum(var, 0.0)) + EPS_BF16))))))
        racc, h2s = None, []
        for r0 in range(0, d, LS):
            iv = inv
            if after is not None and r0 // LS in after:
                iv = _or(inv, after[r0 // LS][0:1])
            ln = _rb(_rb(ot_v[r0:r0 + LS, cs].astype(F32) - mub) * iv)
            marks.append(_fold(ln))
            h2 = _rb(_rb(ln * col_scr[2 * d + r0:2 * d + r0 + LS, :])
                     + col_scr[d + r0:d + r0 + LS, :])
            h2s.append(h2)
            rp = h2 * col_scr[4 * d + r0:4 * d + r0 + LS, :]
            for g in range(0, LS, 8):
                racc = rp[g:g + 8] if racc is None else racc + rp[g:g + 8]
            marks.append(_fold(racc))
        h2 = jnp.concatenate(h2s, axis=0)

        def write_out(zs):
            gb = _or(col_scr[3 * d:4 * d, :],
                     jnp.concatenate([zs[g * len(zs) * 8 // d] for g in range(d // 8)], axis=0))
            ot_v[:, cs] = (x1_scr[:, cs].astype(F32) + gb * h2).astype(BF16)
        return marks, racc, h2, write_out

    hw = gw // 2
    wq0a = col_copy(wq_hbm, wq_v.at[0], 0, hw, grp_sems.at[0, 0])
    wq0b = col_copy(wq_hbm, wq_v.at[0], hw, gw, misc_sems.at[4])
    k0a = pltpu.make_async_copy(k_hbm.at[0], k_v.at[0], grp_sems.at[1, 0])
    k0b = pltpu.make_async_copy(k_hbm.at[1], k_v.at[1], misc_sems.at[5])
    v0 = pltpu.make_async_copy(v_hbm.at[0:HG], v_v.at[0:HG], grp_sems.at[2, 0])
    wq1, k1, v1, wo0 = grp_copies(1)
    wo_last = pltpu.make_async_copy(wot_hbm.at[:, (n_grp - 1) * gw:n_grp * gw],
                                    wot_v.at[n_grp - 1], grp_sems.at[3, 0])
    wrem_copy = col_copy(wq_hbm.at[dm:d], wrem_v, gw, 4 * gw, misc_sems.at[2])
    wrem_rest = (col_copy(wq_hbm.at[dm:d], wrem_v, 0, gw, misc_sems.at[11]),
                 col_copy(wq_hbm.at[dm:d], wrem_v, 4 * gw, n_grp * gw, misc_sems.at[12]))
    c_copy = pltpu.make_async_copy(c_hbm, c_ref, misc_sems.at[6])
    wr_copy = pltpu.make_async_copy(wr_hbm, wr_ref, misc_sems.at[7])
    c_copy.start()
    wr_copy.start()
    x_first.start()
    mod_first[0].start()
    mod_first[1].start()
    wq0a.start()
    wq0b.start()
    acc_scr[0:2 * nb] = jnp.zeros((2 * nb, d, LANES), F32)
    col_scr[0:4 * d, :] = jnp.zeros((4 * d, LANES), F32)
    wdt_v[ff // WP] = jnp.zeros((d, WP), BF16)
    c_copy.wait()
    wr_copy.wait()
    x_first.wait()
    cbits = lax.bitcast_convert_type(c_ref[:, 0:LANES].astype(F32), U32)
    zero_scr[...] = jnp.broadcast_to(cbits & 0xFFFF, (8, LANES))
    h_scr[0] = ln1_norm(0, TB, [])()
    sc = silu_c()
    wr = wr_ref[...].reshape(1, d).astype(F32)
    col_scr[4 * d:5 * d, :] = jnp.broadcast_to(wr, (LANES, d)).T
    col_scr[5 * d:6 * d, :] = jnp.broadcast_to(sc[0:1, :].astype(F32), (LANES, d)).T
    mod_first[0].wait()
    mod = _rb(jnp.dot(sc, wmod_v[:, MODC:2 * d], preferred_element_type=F32))
    mod_scr[0:1, MODC:d] = mod[0:1, 0:d - MODC] * qscale
    mod_scr[1:2, :] = _rb(1.0 + mod[0:1, d - MODC:2 * d - MODC]) * qscale
    mod_first[1].wait()
    k0a.start()
    mod = _rb(jnp.dot(sc, wmod_v[:, 0:MODC], preferred_element_type=F32))
    mod_scr[0:1, 0:MODC] = mod[0:1] * qscale
    wq0a.wait()
    k0b.start(priority=1)
    v0.start(priority=1)
    wrem_copy.start(priority=1)
    ln1_mod(h_scr[0], 0, 0)
    qa = qproj_first(0, hw)
    wq0b.wait()
    k0a.wait()
    wq1.start(priority=1)
    k1.start(priority=1)
    x_second.start()
    q = jnp.concatenate([qa, qproj_first(hw, gw)], axis=1)
    zero = zero_scr[...]
    for j in range(2):
        marks = []
        for i in range(2 * j, 2 * j + 2):
            hb_piece(0, i, marks)
        qk(0, q, j, marks, zero)
    k0b.wait()
    v0.wait()
    wrem_copy.wait()
    v1.start()
    wo0.start()
    zero = zero_scr[...]
    rem_scr[...] = jnp.dot(h_scr[0, 0:RV, dm:d], wrem_v[:, gw:2 * gw],
                           preferred_element_type=F32)
    for i in range(HG):
        marks = v_transpose(0, i)
        if i == 0:
            wb_piece(2, marks, zero)
        if 4 + i < nhb:
            hm = []
            hb_piece(0, 4 + i, hm)
            marks = _merge(marks, hm)
        qk(0, q, nq - HG + i, marks, zero)

    assert n_grp == 8 and HG == 2
    stage_at = [1, 2, 3, 5, n_units]
    starts = [(*grp_copies(2), mod_rest, x_rest, *wrem_rest), grp_copies(3, 3),
              (*grp_copies(6, 2), wo_last, mlp_d), (mlp_g, mlp_u)]
    waits = [(wq1, k1, v1, wo0, x_second), *starts[:3]]
    wd0 = stage_at[3]
    npc = TB // SP
    nmp = 4 * d // MP

    def manage(k, _, c):
        for cp in waits[k]:
            cp.wait()
        for cp in starts[k]:
            cp.start()
        return c

    def steady(u, carry):
        zero = zero_scr[...]
        blk, g = blk_of(u), grp_of(u)
        off = ((g - 1) & (npc - 1)) * SP
        rem = Rem(blk_of(u + 1) & 1)
        q = qproj(u, rem.take(0), zero)
        o = pv(range(0, 2 * nb), zero, rem.take(1))
        live = jnp.logical_and(blk > 0, jnp.logical_and(g >= 1, g <= npc))
        t0 = jnp.maximum(blk - 1, 0) * TB + off
        marks = finalize(t0, (blk + 1) & 1, off, jnp.where(live, t0, seq), SP)
        wp = jnp.clip(u - wd0, 0, ff // WP - 1) * WP
        wmarks = []
        wd_piece(jnp.where(u >= wd0, wp, ff), wp, wmarks)
        rem.flush(qk(u, q, 0, rem.take(2, _merge(marks, wmarks)), zero), zero, 2)
        marks, mmarks = [], []
        ln_fin = ln1_norm(jnp.minimum(blk + 1, n_blk - 1) * TB + off, SP, marks)
        mp = jnp.clip(u - 2, 0, nmp - 1) * MP
        mod_fin = mod_piece(jnp.where(u >= 2, 2 * d + mp, 0), mp, mmarks)
        st = qk(u, q, 1, rem.take(3, marks + mmarks), zero)
        rem.flush(st, zero, 3)
        used = jnp.where(live, ((blk + 1) & 1) * nb + off // LANES, 2 * nb)
        for r0 in range(0, d, 32):
            z4 = jnp.concatenate([_tok(st, r0) & zero] * 4, axis=0)
            acc_scr[used, r0:r0 + 32, :] = lax.bitcast_convert_type(z4, F32)
        ln1_mod(ln_fin(_tok(st, LNREL) & zero), (blk + 1) & 1, off)
        mod_fin(_tok(st, 1880) & zero)
        o += pv(range(2 * nb, 4 * nb), zero, rem.take(4))
        st = qk(u, q, 2, rem.take(5), zero)
        rem.flush(st, zero, 5)
        v_transpose(u, 0, [_tok(st, 112 * i) for i in range(nt)], zero)
        st = qk(u, q, 3, rem.take(6), zero)
        rem.flush(st, zero, 6)
        v_transpose(u, 1, [_tok(st, 112 * i) for i in range(nt)], zero)
        res = outproj_tied(u - 1, o, rem.take(7), zero)
        rem.flush(res, zero, 7, OPN * d // 16)
        hm = []
        hb_piece((blk + 1) & 1, jnp.clip(g - 1, 0, nhb - 1), hm,
                 _tok(res, max(OPN * d - 96, 0)) & zero)
        wb_piece(u + 2, hm, zero)
        return carry

    def stage(k, lo):
        hi = stage_at[1]
        for i in range(len(waits)):
            lax.fori_loop(0, jnp.where(k == i, 1, 0), functools.partial(manage, i), 0)
            hi = jnp.where(k == i, stage_at[i + 1], hi)
        lax.fori_loop(lo, hi, steady, 0)
        return hi

    lax.fori_loop(0, len(waits), stage, jnp.int32(stage_at[0]))

    ul = n_units - 1
    tl = seq - TB
    sl_last = (n_blk - 1) & 1
    nb0 = nb - TAILB
    mod_scr[2:3, :] = row_scr[:, 3 * d:4 * d]
    outproj(ul, pv([j * nb + i for j in range(nq) for i in range(nb0)], zero_scr[...]))
    mlp_g.wait()
    mlp_u.wait()
    out_lo.start()
    toks = finalize(tl, sl_last, 0, tl, nb0 * LANES)
    assert TAILB == 2
    zero = zero_scr[...]

    def op_piece(i, o4, toks):
        wo = _tie_rows(wot_v[grp_of(ul)], toks, zero, LLO, d // 16)
        res = jnp.dot(wo, jnp.concatenate(o4, axis=0).astype(BF16), preferred_element_type=F32)
        acc_scr[sl_last * nb + nb0 + i] += res
        return res

    o = pv([j * nb + i for i in range(nb0, nb) for j in range(nq)], zero, toks, EROWS, EPVEND)
    op_piece(0, o[0:nq], ())
    lates = [late_piece(tl + nb0 * LANES, sl_last * nb + nb0)]
    res = op_piece(1, o[nq:2 * nq], lates[0][0][:LKEEP])

    nl = TAILB * LANES
    sub8 = lax.broadcasted_iota(I32, (TOPC, 1), 0)
    lane = lax.broadcasted_iota(I32, (TOPC, LANES), 1)

    def key_index(k):
        return seq - 1 - (lax.bitcast_convert_type(k, I32) & (seq - 1))

    def piece_base(idx, limit):
        return pl.multiple_of(jnp.clip(idx >> 7, 0, limit // LANES - 1) * LANES, LANES)

    keys = key_scr[0:seq // LANES, :]
    piece = lax.broadcasted_iota(I32, (seq // LANES, 1), 0)
    keys = jnp.where(piece < (seq - nl) // LANES, keys, 0.0)
    ecol = jnp.zeros((TOPC, LANES), F32)
    erow = jnp.zeros((1, LANES), F32)
    h2e = jnp.zeros((TOPC, d), F32)
    gots = []
    for i in range(TOPC):
        mx = jnp.max(jnp.max(keys, axis=0, keepdims=True), axis=1, keepdims=True)
        keys = jnp.where(keys == mx, 0.0, keys)
        ecol = jnp.where(sub8 == i, mx, ecol)
        erow = jnp.where(lane[0:1] == i, mx, erow)
        idx = key_index(mx)
        pick = jnp.logical_and(sub8 == i, lane == (idx & (LANES - 1)))
        sl = pl.ds(piece_base(idx[0, 0], seq - nl), LANES)
        pick = jnp.where(pick, 1.0, 0.0)
        got = lax.dot_general(pick.astype(BF16), h2_scr[:, sl], _NT, preferred_element_type=F32)
        gots.append(_fold(got) & zero)
        h2e = h2e + got

    lates.append(late_piece(seq - LANES, sl_last * nb + nb - 1,
                            {ch: gots[gi] for ch, gi in PACE.items()}))
    erow = _or(erow, gots[-1][0:1])
    rel = _tok(res, d - 8) & zero
    late = [router_keys(_or(lates[i][1], rel), seq - nl + i * LANES) for i in range(TAILB)]
    krow = jnp.concatenate(late + [erow], axis=1)
    kcol = jnp.concatenate(
        [ecol] + [jnp.broadcast_to(k, (LANES, LANES)).T for k in late], axis=0)
    h2l = jnp.concatenate([lt[2] for lt in lates], axis=1).astype(BF16)
    cnt = [None] * 4
    for g in range(kcol.shape[0] // 8):
        one = jnp.where(_lanes(kcol[8 * g:8 * g + 8], nl + LANES) > krow, 1.0, 0.0)
        cnt[g % 4] = one if cnt[g % 4] is None else cnt[g % 4] + one
    rank = jnp.sum((cnt[0] + cnt[1]) + (cnt[2] + cnt[3]), axis=0, keepdims=True)
    chosen = rank == sub8.astype(F32)
    onehot = jnp.where(chosen, 1.0, 0.0).astype(BF16)
    h2pad = jnp.concatenate([h2e, jnp.zeros((TOPC, d), F32)], axis=0).astype(BF16)
    h2s = (jnp.dot(onehot[:, nl:nl + 2 * TOPC], h2pad, preferred_element_type=F32)
           + lax.dot_general(onehot[:, 0:nl], h2l, _NT,
                             preferred_element_type=F32))
    top = jnp.max(jnp.where(chosen, krow, 0.0), axis=1, keepdims=True)
    idx_col = key_index(top)
    idxs = [idx_col[i:i + 1] for i in range(TOPC)]
    bases = [piece_base(idx_col[i, 0], seq) for i in range(TOPC)]
    hit = lane == (idx_col & (LANES - 1))
    picks = [jnp.where(jnp.logical_and(sub8 == i, hit), 1.0, 0.0).astype(BF16)
             for i in range(TOPC)]
    order = (lax.bitcast_convert_type(top, I32) >> 11) & 0xFFFF
    rbits = jnp.where(order >= 32768, order - 32768, -1 - order) << 16
    gate = _sigmoid(lax.bitcast_convert_type(rbits, F32))
    xs = h2s.astype(BF16)
    g = jnp.dot(xs, wg_v[...], preferred_element_type=F32)
    gz = [_tok(g[:, c * LANES:(c + 1) * LANES], 0) & zero for c in range(24)]
    for i in range(TAILB):
        lates[i][3](gz[12 * i:12 * i + 12])
    for cp in out_hi:
        cp.start()
    g = _rb(g)
    g = _rb(g * _sigmoid(g))
    u = _rb(jnp.dot(xs, wu_v[...], preferred_element_type=F32))
    gu = (g * u).astype(BF16)

    last_use = []
    for i in range(TOPC):
        ok = True
        for j in range(i + 1, TOPC):
            ok = jnp.logical_and(ok, bases[i] != bases[j])
        last_use.append(ok)

    def down(r0, r1):
        x1p = jnp.concatenate([x1_scr[r0:r1, pl.ds(bases[i], LANES)] for i in range(TOPC)], axis=1)
        x1s = lax.dot_general(jnp.concatenate(picks, axis=1), x1p, _NT,
                              preferred_element_type=F32)
        wd = pltpu.bitcast(wd_scr[:, r0:r1], BF16)
        y = _rb(jnp.dot(gu, wd, preferred_element_type=F32))
        hm = _rb(h2s[:, r0:r1] + _rb(y * gate))
        return x1s + mod_scr[2:3, r0:r1] * hm

    def patch(r0, r1, new):
        n = r1 - r0
        pad = jnp.concatenate([new, jnp.zeros((LANES - TOPC, n), F32)], axis=0)
        cols = pltpu.bitcast(pad.T.astype(BF16), U32)
        col = [jnp.broadcast_to(cols[:, j:j + 1], (n // 2, LANES)) for j in range(TOPC)]
        for i in range(TOPC):
            res = pltpu.bitcast(ot_v[r0:r1, pl.ds(bases[i], LANES)], U32)
            tok = lane[0:1, :] + (idxs[i] & ~(LANES - 1))
            for j in range(i + 1):
                res = jnp.where(tok == idxs[j], col[j], res)
            fix_v[i, r0:r1, :] = pltpu.bitcast(res, BF16)

    def fix_copy(i, r0, r1):
        return pltpu.make_async_copy(fix_v.at[i, r0:r1, :],
                                     o_hbm.at[r0:r1, pl.ds(bases[i], LANES)], fix_sems.at[i])

    def for_last(fn):
        for i in range(TOPC - 1):
            pl.when(last_use[i])(functools.partial(fn, i))
        fn(TOPC - 1)

    new = down(*chunks[0])
    out_lo.wait()
    for ci, (r0, r1) in enumerate(chunks):
        out_hi[ci].wait()
        nxt = down(*chunks[ci + 1]) if ci + 1 < len(chunks) else None
        patch(r0, r1, new)
        for_last(lambda i: fix_copy(i, r0, r1).start())
        new = nxt
    for r0, r1 in chunks:
        for_last(lambda i: fix_copy(i, r0, r1).wait())


@jax.jit
def pallas_adaLN_cond__gqa_block_cached__moe_arch_mod__prompt_kernel(
    A_x: jax.Array,
    A_k_cache: jax.Array,
    A_v_cache: jax.Array,
    A_wq: jax.Array,
    A_wo: jax.Array,
    B_x: jax.Array,
    B_w_r: jax.Array,
    B_w_gate: jax.Array,
    B_w_up: jax.Array,
    B_w_down: jax.Array,
    c: jax.Array,
    w_mod: jax.Array,
):
    b, seq, d = A_x.shape
    _, hkv, sk, dh = A_k_cache.shape
    assert b == 1 and dh == DH and HQ == 2 * hkv
    assert seq & (seq - 1) == 0 and seq <= 2048
    f = B_w_gate.shape[1]
    n_grp = hkv // HG
    gw = 2 * HG * dh
    n_slots = 2 * HG * TB // LANES

    xt = A_x.reshape(seq, d).T
    wot = A_wo.T
    wdt = B_w_down.T
    k3 = A_k_cache.reshape(hkv, sk, dh)
    v3 = A_v_cache.reshape(hkv, sk, dh)

    hbm = pl.BlockSpec(memory_space=pl.ANY)
    out_t = pl.pallas_call(
        functools.partial(_kernel, n_heads=hkv),
        in_specs=[hbm] * 11,
        out_specs=hbm,
        out_shape=jax.ShapeDtypeStruct((d, seq), BF16),
        scratch_shapes=[
            pltpu.VMEM((seq // LANES, d, LANES), BF16),
            pltpu.VMEM((hkv, sk, dh), BF16),
            pltpu.VMEM((hkv, sk, dh), BF16),
            pltpu.VMEM((n_grp, d, gw), BF16),
            pltpu.VMEM((n_grp, d, gw), BF16),
            pltpu.VMEM((d, 6 * d), BF16),
            pltpu.VMEM((d, f), BF16),
            pltpu.VMEM((d, f), BF16),
            pltpu.VMEM((f // WP + 1, d, WP), BF16),
            pltpu.VMEM((d, seq + SP), BF16),
            pltpu.VMEM((2, TB, d), BF16),
            pltpu.VMEM((2 * TB // LANES + 1, d, LANES), F32),
            pltpu.VMEM((n_slots, sk, LANES), F32),
            pltpu.VMEM((n_slots, 8, LANES), F32),
            pltpu.VMEM((HG, dh // 2, sk), U32),
            pltpu.VMEM((8, d), F32),
            pltpu.VMEM((6 * d, LANES), F32),
            pltpu.VMEM(((seq + SP) // LANES + 7 & ~7, LANES), F32),
            pltpu.VMEM((d, seq + SP), BF16),
            pltpu.VMEM((d, seq + SP), BF16),
            pltpu.VMEM((8, LANES), U32),
            pltpu.VMEM((TOPC, d, LANES), BF16),
            pltpu.VMEM((1, d), BF16),
            pltpu.VMEM((d,), BF16),
            pltpu.VMEM((1, 4 * d), F32),
            pltpu.VMEM((f // 2, d), U32),
            pltpu.VMEM((2 * -(-RV // HP), d % LANES * HP // 2, LANES), U32),
            pltpu.VMEM((d % LANES * 8, gw), F32),
            pltpu.VMEM((RV, gw), F32),
            pltpu.VMEM((d % LANES, n_grp * gw), BF16),
            pltpu.SemaphoreType.DMA((4, n_grp)),
            pltpu.SemaphoreType.DMA((13,)),
            pltpu.SemaphoreType.DMA((3,)),
            pltpu.SemaphoreType.DMA((len(EDGES),)),
            pltpu.SemaphoreType.DMA((TOPC,)),
        ],
        compiler_params=pltpu.CompilerParams(
            disable_bounds_checks=True,
            disable_semaphore_checks=True,
            vmem_limit_bytes=120 * 1024 * 1024,
        ),
    )(xt, k3, v3, A_wq, wot, B_w_r, B_w_gate, B_w_up, wdt, c, w_mod)
    return out_t.T.reshape(b, seq, d)
```
